```python
import jax
import jax.numpy as jnp

def _softmax(x, axis=-1):
    return jax.nn.softmax(x, axis=axis)
def _gelu(x):
    return jax.nn.gelu(x, approximate=True)
def _silu(x):
    return jax.nn.silu(x)
def _sigmoid(x):
    return jax.nn.sigmoid(x)
def _layernorm(x, axis=-1, eps=1e-5):
    m = jnp.mean(x, axis=axis, keepdims=True)
    v = jnp.var(x, axis=axis, keepdims=True)
    return (x - m) / jnp.sqrt(v + eps)
def _scatter_add(tgt, idx, src, axis=0):
    return tgt.at[idx].add(src)
def _segment_sum(src, seg, n):
    return jax.ops.segment_sum(src, seg, n)
class _Rng:
    def __init__(self, key):
        self._k = key
    def _next(self):
        self._k, sub = jax.random.split(self._k)
        return sub
    def normal(self, shape):
        return jax.random.normal(self._next(), shape, dtype=jnp.bfloat16)
    def randint(self, lo, hi, shape):
        return jax.random.randint(self._next(), shape, lo, hi, dtype=jnp.int32)
    def uniform(self, shape, lo=0.0, hi=1.0):
        return jax.random.uniform(self._next(), shape, jnp.bfloat16, lo, hi)
    def permutation(self, n):
        return jax.random.permutation(self._next(), n)


kernel_name = 'interleave_layers__ssm_conv_h3__mixer_s_mlp__prompt'

def setup_inputs():
    _rng = _Rng(jax.random.key(int.from_bytes(__import__("os").urandom(4), "little")))
    _w = (lambda a: (lambda t: t.astype(jnp.bfloat16) if jnp.issubdtype(t.dtype, jnp.floating) else t)(jnp.asarray(a)))
    def _A_setup():
        B, S, D = 1, 2048, 1024
        ks = 4
        return {
            "q": _w((lambda *s: _rng.normal(s) * 0.05)(B, S, D)),
            "k": _w((lambda *s: _rng.normal(s) * 0.05)(B, S, D)),
            "v": _w((lambda *s: _rng.normal(s) * 0.05)(B, S, D)),
            "shift_k": _w((lambda *s: _rng.normal(s) * 0.05)(D, ks) * 0.5),
            "ssm_k": _w((lambda *s: _rng.normal(s) * 0.05)(D, S) * (1.0 / S ** 0.5)),
            "ssm_D": _w((lambda *s: _rng.normal(s) * 0.05)(D)),
        }
    _A_in = _A_setup()

    def _B_setup():
        B, S, D, F = 1, 2048, 1024, 3584
        return {
            "x":  _w((lambda *s: _rng.normal(s) * 0.05)(B, S, D)),
            "w1": _w((lambda *s: _rng.normal(s) * 0.05)(D, D) * (D ** -0.5)),
            "w2": _w((lambda *s: _rng.normal(s) * 0.05)(D, D) * (D ** -0.5)),
            "w3": _w((lambda *s: _rng.normal(s) * 0.05)(D, F) * (D ** -0.5)),
            "w4": _w((lambda *s: _rng.normal(s) * 0.05)(F, D) * (F ** -0.5)),
        }
    _B_in = _B_setup()

    return {
        "A_q": _A_in["q"],
        "A_k": _A_in["k"],
        "A_v": _A_in["v"],
        "A_shift_k": _A_in["shift_k"],
        "A_ssm_k": _A_in["ssm_k"],
        "A_ssm_D": _A_in["ssm_D"],
        "B_x": _B_in["x"],
        "B_w1": _B_in["w1"],
        "B_w2": _B_in["w2"],
        "B_w3": _B_in["w3"],
        "B_w4": _B_in["w4"],
    }

def reference(A_q, A_k, A_v, A_shift_k, A_ssm_k, A_ssm_D, B_x, B_w1, B_w2, B_w3, B_w4):
    def _A_ref(q, k, v, shift_k, ssm_k, ssm_D):
        B, S, D = q.shape
        ks = shift_k.shape[-1]
        k_pad = jnp.pad(k, ((0, 0), (ks - 1, 0), (0, 0)))
        k_shift = jnp.zeros_like(k)
        for t in range(ks):
            k_shift = k_shift + k_pad[:, t:t + S, :] * shift_k[:, ks - 1 - t][None, None, :]
        kv = k_shift * v
        L = 2 * S
        kv_pad = jnp.pad(kv, ((0, 0), (0, S), (0, 0)))
        kf_pad = jnp.pad(ssm_k, ((0, 0), (0, S)))
        kv_f = (lambda x, axes=(-2,-1): jnp.fft.rfft2(x.astype(jnp.float32), axes=axes))(kv_pad[:, None, :, :], axes=(1, 2))
        kf_f = (lambda x, axes=(-2,-1): jnp.fft.rfft2(x.astype(jnp.float32), axes=axes))(kf_pad[:, None, :], axes=(1, 2))
        kf_f = (lambda x, *d: x.transpose(*d))(kf_f, 1, 2, 0)
        y_f = kv_f * kf_f[None, :, :, :]
        y = (lambda x, s, axes=(-2,-1): jnp.fft.irfft2(x, s=s, axes=axes).astype(jnp.bfloat16))(y_f, (1, L), axes=(1, 2))[:, 0, :S, :]
        y = y + kv * ssm_D[None, None, :]
        return q * y

    def _B_ref(x, w1, w2, w3, w4):
        B, S, D = x.shape
        h = _gelu(_layernorm(x, axis=-1) @ w1)
        c = D // 4
        g0 = jnp.pad(h[:, :, 0*c:1*c], ((0, 0), (1, 0), (0, 0)))[:, :S, :]
        g1 = jnp.pad(h[:, :, 1*c:2*c], ((0, 0), (0, 1), (0, 0)))[:, 1:, :]
        g2 = jnp.pad(h[:, :, 2*c:3*c], ((0, 0), (2, 0), (0, 0)))[:, :S, :]
        g3 = jnp.pad(h[:, :, 3*c:   ], ((0, 0), (0, 2), (0, 0)))[:, 2:, :]
        hs = jnp.concatenate([g0, g1, g2, g3], axis=-1) @ w2
        x1 = x + hs
        h2 = _gelu(_layernorm(x1, axis=-1) @ w3) @ w4
        return x1 + h2

    x = A_q
    x = x + _A_ref(_layernorm(x, axis=-1), A_k, A_v, A_shift_k, A_ssm_k, A_ssm_D)
    x = x + _B_ref(_layernorm(x, axis=-1), B_w1, B_w2, B_w3, B_w4)
    x = x + _A_ref(_layernorm(x, axis=-1), A_k, A_v, A_shift_k, A_ssm_k, A_ssm_D)
    x = x + _B_ref(_layernorm(x, axis=-1), B_w1, B_w2, B_w3, B_w4)
    return x
```

```python
import math

import jax
import jax.numpy as jnp
from jax import lax
import jax.experimental.pallas as pl
import jax.experimental.pallas.tpu as pltpu


f32, bf16, u32, i32 = jnp.float32, jnp.bfloat16, jnp.uint32, jnp.int32

S, D, FF = 2048, 1024, 3584
TM = 256
NB = S // TM
G = 2 * NB
CB = 128
NA = S // CB
NO = 4
TF = 512
NC = FF // TF
R = 16
NS = TM // R
LG = D // 128
EPS = 1e-5
CS = CB + 8
BS = 3 * CS
H0 = NA * BS + 16
C0 = math.sqrt(2.0 / math.pi)
C1 = C0 * 0.044715


def _ln(x):
    m = jnp.mean(x, axis=-1, keepdims=True)
    xc = x - m
    v = jnp.mean(xc * xc, axis=-1, keepdims=True)
    return xc * lax.rsqrt(v + EPS)


def _gelu(x):
    hx = 0.5 * x
    return hx + hx * jnp.tanh(x * (C0 + C1 * (x * x)))


def _mm(a, b):
    return jnp.dot(a, b, preferred_element_type=f32)


def _tok(vals):
    t = None
    for v in vals:
        b = pltpu.bitcast(v, u32)
        for i in range(b.shape[0] // 8):
            for j in range(b.shape[1] // 128):
                p = b[i * 8:(i + 1) * 8, j * 128:(j + 1) * 128]
                t = p if t is None else t | p
    return t


def _pin(x, vals, zero):
    if not vals:
        return x
    top = pltpu.bitcast(pltpu.bitcast(x[0:16, 0:128], u32) | (_tok(vals) & zero), bf16)
    row0 = jnp.concatenate([top, x[0:16, 128:]], axis=1)
    return jnp.concatenate([row0, x[16:]], axis=0)


def _pin_at(x, pins, zero):
    if not pins:
        return x
    out, last = [], 0
    for k in sorted({k for k, _ in pins}):
        if k * 16 > last:
            out.append(x[last:k * 16])
        blk = x[k * 16:(k + 1) * 16]
        for (kk, n), vals in pins.items():
            if kk != k:
                continue
            top = pltpu.bitcast(pltpu.bitcast(blk[:, n * 128:(n + 1) * 128], u32) | (_tok(vals) & zero), bf16)
            parts = ([blk[:, :n * 128]] if n > 0 else []) + [top] + (
                [blk[:, (n + 1) * 128:]] if (n + 1) * 128 < blk.shape[1] else [])
            blk = jnp.concatenate(parts, axis=1) if len(parts) > 1 else top
        out.append(blk)
        last = (k + 1) * 16
    if last < x.shape[0]:
        out.append(x[last:])
    return jnp.concatenate(out, axis=0) if len(out) > 1 else out[0]


def _spread(items, n):
    return [items[(i * len(items)) // n:((i + 1) * len(items)) // n] for i in range(n)]


def _kernel(q_hbm, k_hbm, v_hbm, sk_hbm, hk_hbm, dd_hbm, w1_hbm, w2_hbm, w3_hbm, w4_hbm,
            o_hbm,
            w1b, w2b, w3b, w4b, kbuf, vbuf, hkb, qbuf, skb, ddb,
            Fm, Gm, skf, kf, ZA, ZB, YA, YB, ybuf, xbuf, ubuf, hbuf, z3buf,
            zsm, sem):
    obuf = vbuf

    def cp_k(c):
        return pltpu.make_async_copy(k_hbm.at[0, :, pl.ds(c * 128, 128)],
                                     kbuf.at[pl.ds(16, S), pl.ds(c * 128, 128)], sem.at[3 * c])

    def cp_v(c):
        return pltpu.make_async_copy(v_hbm.at[0, :, pl.ds(c * 128, 128)],
                                     vbuf.at[:, pl.ds(c * 128, 128)], sem.at[3 * c + 1])

    def cp_h(c):
        return pltpu.make_async_copy(hk_hbm.at[pl.ds(c * 128, 128), :],
                                     hkb.at[pl.ds(c * 128, 128), :], sem.at[3 * c + 2])

    def cp_o(j):
        return pltpu.make_async_copy(obuf.at[pl.ds(j * TM, TM), :],
                                     o_hbm.at[0, pl.ds(j * TM, TM), :], sem.at[3 * LG + 7 + j])

    cp_sk = pltpu.make_async_copy(sk_hbm, skb, sem.at[3 * LG])
    cp_dd = pltpu.make_async_copy(dd_hbm, ddb, sem.at[3 * LG + 1])
    cp_q = pltpu.make_async_copy(q_hbm.at[0], qbuf, sem.at[3 * LG + 2])
    cp_w1 = pltpu.make_async_copy(w1_hbm, w1b, sem.at[3 * LG + 3])
    cp_w2 = pltpu.make_async_copy(w2_hbm, w2b, sem.at[3 * LG + 4])
    cp_w3 = pltpu.make_async_copy(w3_hbm, w3b, sem.at[3 * LG + 5])
    cp_w4 = pltpu.make_async_copy(w4_hbm, w4b, sem.at[3 * LG + 6])

    def wait_grp(c):
        cp_k(c).wait()
        cp_v(c).wait()
        cp_h(c).wait()

    cp_sk.start()
    cp_dd.start()
    for c in range(LG):
        cp_k(c).start()
        cp_v(c).start()
        cp_h(c).start()
    for cp in (cp_q, cp_w1, cp_w2, cp_w3, cp_w4):
        cp.start()

    zsm[0] = 0
    kbuf[0:16, :] = jnp.zeros((16, D), bf16)
    hbuf[0:8, :] = jnp.zeros((8, D), f32)
    hbuf[S + 8:S + 16, :] = jnp.zeros((8, D), f32)

    ri = lax.broadcasted_iota(i32, (CB, CB), 0)
    ci = lax.broadcasted_iota(i32, (CB, CB), 1)

    def _freq(i):
        return jnp.where(i < CB // 2, 2 * i, 2 * i - (CB - 1))

    ang = (((2 * _freq(ri) + 1) * ci) & (4 * CB - 1)).astype(f32) * (math.pi / (2 * CB))
    fc, fs = jnp.cos(ang), -jnp.sin(ang)
    sg = jnp.where(ri < CB // 2, 1.0, -1.0)
    for par, (pc, ps) in enumerate(((fc, fs), (fc * sg, fs * sg))):
        pc, ps = pltpu.bitcast(pc.astype(bf16), u32), pltpu.bitcast(ps.astype(bf16), u32)
        for g in range(CB // 16):
            Fm[par, 16 * g:16 * g + 8, :] = pc[8 * g:8 * g + 8]
            Fm[par, 16 * g + 8:16 * g + 16, :] = ps[8 * g:8 * g + 8]
    rg = lax.broadcasted_iota(i32, (CB, 2 * CB), 0)
    cg = lax.broadcasted_iota(i32, (CB, 2 * CB), 1)
    pos = cg >> 1
    ang = (((2 * _freq(pos) + 1) * rg) & (4 * CB - 1)).astype(f32) * (math.pi / (2 * CB))
    gm = jnp.where((cg & 1) == 0, jnp.cos(ang), -jnp.sin(ang)) * (1.0 / CB)
    Gm[0] = pltpu.bitcast(gm.astype(bf16), u32)
    Gm[1] = pltpu.bitcast(jnp.where(pos < CB // 2, gm, -gm).astype(bf16), u32)

    cp_sk.wait()
    cp_dd.wait()
    sk32 = skb[...].astype(f32)
    for t in range(4):
        skf[t] = jnp.broadcast_to(sk32[t:t + 1, :], (8, D))
    skf[4] = jnp.broadcast_to(ddb[...].astype(f32).reshape(1, D), (8, D))

    def zero_vec():
        return jnp.full((8, 128), zsm[0], i32).astype(u32)

    def bmul(x, row8):
        n = x.shape[0] // 8
        return (x.reshape(n, 8, 128) * row8[None]).reshape(x.shape)

    def dsl(start, size, align):
        return pl.ds(start if isinstance(start, int) else pl.multiple_of(start, align), size)

    def unil(z):
        return (jnp.concatenate([z[32 * g:32 * g + 16] for g in range(CB // 16)], axis=0),
                jnp.concatenate([z[32 * g + 16:32 * g + 32] for g in range(CB // 16)], axis=0))

    def fwdh1(c, i, o, pins=None):
        Z = (ZA if c % 2 == 0 else ZB).at[dsl(H0 + i * 2 * BS, 2 * BS, 8), :]
        ls = slice(c * 128, (c + 1) * 128)
        a = 2 * i + o
        hh = lax.dot_general(_pin_at(pltpu.bitcast(Fm[o], bf16), pins, zero_vec()), hkb[ls, dsl(a * CB, CB, CB)], (((1,), (1,)), ((), ())),
                             preferred_element_type=f32)
        cc, dd = unil(hh)
        b = o * BS
        Z[b:b + CB, :] = cc
        Z[b + CS:b + CS + CB, :] = dd - cc
        Z[b + 2 * CS:b + 2 * CS + CB, :] = cc + dd
        return cc + dd

    def fwdx1(c, i, o, pins=None):
        Z = (ZA if c % 2 == 0 else ZB).at[dsl(i * 2 * BS, 2 * BS, 8), :]
        ls = slice(c * 128, (c + 1) * 128)
        if o == 0:
            kf[...] = kbuf[dsl(i * 2 * CB, 2 * CB + 16, 16), ls].astype(f32)
        a = 2 * i + o
        b0 = 16 + o * CB
        ks = bmul(kf[b0:b0 + CB, :], skf[0, :, ls])
        for t in range(1, 4):
            ks = ks + bmul(kf[b0 - t:b0 - t + CB, :], skf[t, :, ls])
        kv = (ks * vbuf[dsl(a * CB, CB, CB), ls].astype(f32)).astype(bf16)
        xh = _mm(_pin_at(pltpu.bitcast(Fm[o], bf16), pins, zero_vec()), kv)
        xr, xm = unil(xh)
        b = o * BS
        Z[b:b + CB, :] = xr
        Z[b + CS:b + CS + CB, :] = xm
        Z[b + 2 * CS:b + 2 * CS + CB, :] = xr + xm
        return xr + xm

    def add_skip(c):
        Z = ZA if c % 2 == 0 else ZB
        d8 = skf[4, :, c * 128:(c + 1) * 128][None]
        for k, sgn in ((0, 1), (1, -1), (2, 1)):
            b = H0 + k * CS
            z = Z[b:b + CB, :].reshape(CB // 8, 8, 128)
            Z[b:b + CB, :] = (z + d8 if sgn > 0 else z - d8).reshape(CB, 128)

    def fwd2(c, i):
        for o in range(2):
            fwdh1(c, i, o)
        for o in range(2):
            fwdx1(c, i, o)

    def mac_gen(c, i):
        Z, Y = (ZA, YA) if c % 2 == 0 else (ZB, YB)
        Z = Z.at[dsl(i * 16, 2 * H0 - CB + 16, 16), :]
        X, H = 0, H0
        prev = [None, None]
        for a0 in range(0, NA, NO):
            for h in range(2):
                def ld(ref, a):
                    b = ref + a * BS + h * 8
                    return tuple(Z[b + k * CS:b + k * CS + 8, :] for k in range(3))
                K = [None] * NO
                hw = {}
                for ap in range(a0 + NO):
                    xa, xb, xs = ld(X, ap)
                    for o in range(NO):
                        dl = a0 + o - ap
                        if dl < 0:
                            continue
                        if dl not in hw:
                            hw[dl] = ld(H, dl)
                        hc, he, hf = hw[dl]
                        t = (hc * xs, xa * he, xb * hf)
                        K[o] = t if K[o] is None else tuple(u + w for u, w in zip(K[o], t))
                        inj = yield K[o][2]
                        if inj is not None:
                            K[o] = (K[o][0], K[o][1], K[o][2] + inj)
                for o in range(NO):
                    re, im = K[o][0] - K[o][2], K[o][0] + K[o][1]
                    out = (re, im) if prev[h] is None else (re - prev[h][1], im + prev[h][0])
                    prev[h] = (re, im)
                    Y[a0 + o, dsl(i * 16 + h * 8, 8, 8), :] = pltpu.pack_elementwise(
                        list(out), packed_dtype=bf16).astype(u32)

    def inv1(c, i, o, pins=None):
        Y = YA if c % 2 == 0 else YB
        a = 2 * i + o
        y = _mm(_pin_at(pltpu.bitcast(Gm[o], bf16), pins, zero_vec()), pltpu.bitcast(Y[a], bf16))
        yv = ybuf.at[dsl(a * (CB // 2), CB // 2, CB // 2), :]
        for g in range(CB // 16):
            yv[8 * g:8 * g + 8, c * 128:(c + 1) * 128] = pltpu.pack_elementwise(
                [y[16 * g:16 * g + 8], y[16 * g + 8:16 * g + 16]], packed_dtype=bf16).astype(u32)

    def inv2(c, i):
        inv1(c, i, 0)
        inv1(c, i, 1)

    def xinit(c, i):
        n = (48, 48, 64)[c]
        r = dsl(3 * TM + 8 * (0, 48, 96)[c] + i * n, n, 16)
        xbuf[r, :] = qbuf[r, :].astype(f32)

    def conv():
        wait_grp(0)
        for i in range(NA // 2):
            fwd2(0, i)
        for c in range(LG):
            if c + 1 < LG:
                wait_grp(c + 1)
            if c == 5:
                cp_q.wait()
            add_skip(c)

            def it(i, carry, c=c):
                gen = mac_gen(c, i)
                P0, DP, NP_, R0, DR, G0 = (int(x) for x in '12,8,16,155,10,4'.split(','))
                rec = [next(gen)]
                while len(rec) <= P0 + (NP_ - 1) * DP:
                    rec.append(gen.send(None))
                pins = {k: {} for k in ('i0', 'i1', 'h0', 'h1', 'x0', 'x1')}
                names = 'h0,x0,h1,x1'.split(',')
                for n in range(NP_):
                    r = ((n + 1) * 16) // NP_ - 1
                    pins[names[n % len(names)]][(r, 0)] = [rec[P0 + n * DP]]
                res = []
                if c > 0:
                    inv1(c - 1, i, 0, pins['i0'])
                    inv1(c - 1, i, 1, pins['i1'])
                if c + 1 < LG:
                    res = [fwdh1(c + 1, i, 0, pins['h0']), fwdh1(c + 1, i, 1, pins['h1']),
                           fwdx1(c + 1, i, 0, pins['x0']), fwdx1(c + 1, i, 1, pins['x1'])]
                inj = {}
                if res:
                    zero = zero_vec()
                    for g in range(G0, CB // 16):
                        tk = _tok([z[16 * g + 8:16 * g + 16] for z in res]) & zero
                        inj[R0 + (g - G0) * DR] = pltpu.bitcast(tk, f32)
                n = len(rec)
                try:
                    while True:
                        gen.send(inj.get(n))
                        n += 1
                except StopIteration:
                    pass
                if c >= 5:
                    xinit(c - 5, i)
                return carry
            lax.fori_loop(0, NA // 2, it, 0)
        for i in range(NA // 2):
            inv2(LG - 1, i)

    conv()

    def rows(j):
        return j * TM if isinstance(j, int) else pl.multiple_of(j * TM, TM)

    def s0_strip(j, s, from_q=False):
        r = rows(j)
        sl = slice(s * R, (s + 1) * R)
        xv = xbuf.at[pl.ds(r, TM), :]
        uv = ubuf.at[pl.ds(r, TM), :]
        x = qbuf[r + s * R:r + (s + 1) * R, :].astype(f32) if from_q else xv[sl, :]
        r2 = j * (TM // 2) if isinstance(j, int) else pl.multiple_of(j * (TM // 2), TM // 2)
        yw = ybuf.at[pl.ds(r2, TM // 2), :][s * 8:(s + 1) * 8, :]
        y = jnp.concatenate([pltpu.unpack_elementwise(yw, index=k, packed_dtype=bf16, unpacked_dtype=f32)
                             for k in range(2)], axis=0)
        x1 = x + _ln(x) * y
        u = _ln(x1)
        xv[sl, :] = x1 + u
        uv[sl, :] = u
        return _ln(u).astype(bf16)

    def m1(j, z1, pins=None):
        r = rows(j)
        if pins is None:
            hbuf[pl.ds(r + 8, TM), :] = _gelu(_mm(z1, w1b[...]))
        else:
            n = len(pins)
            w = D // n
            zero = zero_vec()
            for i in range(n):
                hbuf[pl.ds(r + 8, TM), i * w:(i + 1) * w] = _gelu(
                    _mm(_pin(z1, pins[i], zero), w1b[:, i * w:(i + 1) * w]))

    def m2_dot(j, pins=None):
        r = rows(j)
        c = D // 4
        hv = hbuf.at[pl.ds(r, TM + 16), :]
        hs_in = jnp.concatenate([
            hv[8 - 1:8 - 1 + TM, 0 * c:1 * c], hv[8 + 1:8 + 1 + TM, 1 * c:2 * c],
            hv[8 - 2:8 - 2 + TM, 2 * c:3 * c], hv[8 + 2:8 + 2 + TM, 3 * c:4 * c]],
            axis=-1).astype(bf16)
        if pins is None:
            return _mm(hs_in, w2b[...])
        n = len(pins)
        w = D // n
        zero = zero_vec()
        return jnp.concatenate(
            [_mm(_pin(hs_in, pins[i], zero), w2b[:, i * w:(i + 1) * w]) for i in range(n)], axis=1)

    def ln3(j, hs):
        r = rows(j)
        xv = xbuf.at[pl.ds(r, TM), :]
        uv = ubuf.at[pl.ds(r, TM), :]
        for s in range(NS):
            sl = slice(s * R, (s + 1) * R)
            x1p = uv[sl, :] + hs[sl, :]
            xv[sl, :] += hs[sl, :]
            z3buf[sl, :] = _ln(x1p).astype(bf16)

    def m34(j, pins=None, to_x=True, to_o=True):
        r = rows(j)
        z3 = z3buf[...]
        zero = zero_vec()
        pins = pins or [[] for _ in range(2 * NC)]
        acc = None
        for c in range(NC):
            a = _gelu(_mm(_pin(z3, pins[2 * c], zero), w3b[:, c * TF:(c + 1) * TF])).astype(bf16)
            p = _mm(_pin(a, pins[2 * c + 1], zero), w4b[c * TF:(c + 1) * TF, :])
            acc = p if acc is None else acc + p
        xn = xbuf[pl.ds(r, TM), :] + acc
        if to_x:
            xbuf[pl.ds(r, TM), :] = xn
        if to_o:
            obuf[pl.ds(r, TM), :] = xn.astype(bf16)

    def cat(zs):
        return jnp.concatenate(zs, axis=0)

    def prologue():
        cp_w1.wait()
        cp_w2.wait()
        z0 = [s0_strip(0, s, True) for s in range(NS)]
        z1 = [s0_strip(1, s, True) for s in range(NS)]
        m1(0, cat(z0), [[]] + _spread(z1, 8)[:7])
        z2 = [s0_strip(2, s, True) for s in range(NS)]
        m1(1, cat(z1), [[]] + _spread(z2, 8)[:7])
        hs = m2_dot(0)
        m1(2, cat(z2))
        ln3(0, hs)

    prologue()
    cp_w3.wait()
    cp_w4.wait()

    def body(g, carry):
        j = lax.rem(g + 3, NB)
        zs = [s0_strip(j, s) for s in range(NS)]
        jg = lax.rem(g, NB)
        m34(jg, [[]] + _spread(zs, 2 * NC - 1))
        j1 = lax.rem(g + 1, NB)
        hs = m2_dot(j1)
        m1(j, cat(zs))
        ln3(j1, hs)

        @pl.when(g >= NB)
        def _():
            cp_o(jg).start()
        return carry

    lax.fori_loop(0, G - 3, body, 0)

    def body3(j, carry):
        m34(j, to_x=False)
        ln3(j + 1, m2_dot(j + 1))
        cp_o(j).start()
        return carry

    lax.fori_loop(NB - 3, NB - 1, body3, 0)
    m34(NB - 1, to_x=False)
    cp_o(NB - 1).start()
    for j in range(NB):
        cp_o(j).wait()


@jax.jit
def pallas_interleave_layers__ssm_conv_h3__mixer_s_mlp__prompt_kernel(
    A_q, A_k, A_v, A_shift_k, A_ssm_k, A_ssm_D, B_x, B_w1, B_w2, B_w3, B_w4,
):
    del B_x
    vm = pltpu.VMEM
    scratch = [
        vm((D, D), bf16), vm((D, D), bf16), vm((D, FF), bf16), vm((FF, D), bf16),
        vm((S + 16, D), bf16), vm((S, D), bf16), vm((D, S), bf16), vm((S, D), bf16),
        vm((4, D), bf16), vm((D,), bf16),
        vm((2, CB, CB), u32), vm((2, CB // 2, 2 * CB), u32),
        vm((5, 8, D), f32),
        vm((2 * CB + 16, 128), f32),
        vm((2 * H0, 128), f32), vm((2 * H0, 128), f32),
        vm((NA, CB, 128), u32), vm((NA, CB, 128), u32),
        vm((S // 2, D), u32), vm((S, D), f32), vm((S, D), f32),
        vm((S + 16, D), f32), vm((TM, D), bf16),
        pltpu.SMEM((1,), i32),
        pltpu.SemaphoreType.DMA((3 * LG + 7 + NB,)),
    ]
    return pl.pallas_call(
        _kernel,
        out_shape=jax.ShapeDtypeStruct(A_q.shape, bf16),
        in_specs=[pl.BlockSpec(memory_space=pl.ANY)] * 10,
        out_specs=pl.BlockSpec(memory_space=pl.ANY),
        scratch_shapes=scratch,
        compiler_params=pltpu.CompilerParams(vmem_limit_bytes=100 * 1024 * 1024),
    )(A_q, A_k, A_v, A_shift_k.T, A_ssm_k, A_ssm_D, B_w1, B_w2, B_w3, B_w4)
```

```python
import math

import jax
import jax.numpy as jnp
from jax import lax
import jax.experimental.pallas as pl
import jax.experimental.pallas.tpu as pltpu


f32, bf16, u32, i32 = jnp.float32, jnp.bfloat16, jnp.uint32, jnp.int32

S, D, FF = 2048, 1024, 3584
TM = 256
NB = S // TM
G = 2 * NB
CB = 128
NA = S // CB
NO = 4
TF = 512
NC = FF // TF
R = 16
NS = TM // R
LG = D // 128
KR = int('1')
EPS = 1e-5
CS = CB + 8
BS = 3 * CS
H0 = NA * BS + 16
C0 = math.sqrt(2.0 / math.pi)
C1 = C0 * 0.044715


def _ln(x):
    m = jnp.mean(x, axis=-1, keepdims=True)
    xc = x - m
    v = jnp.mean(xc * xc, axis=-1, keepdims=True)
    return xc * lax.rsqrt(v + EPS)


def _ln_t(x):
    m = jnp.mean(x, axis=-1, keepdims=True)
    xc = x - m
    v = jnp.mean(xc * xc, axis=-1, keepdims=True)
    r = lax.rsqrt(v + EPS)
    n = x.shape[0]
    return xc * r, [[jnp.broadcast_to(m, (n, 128))], [jnp.broadcast_to(r, (n, 128))]]


def _gelu(x):
    hx = 0.5 * x
    return hx + hx * jnp.tanh(x * (C0 + C1 * (x * x)))


def _mm(a, b):
    return jnp.dot(a, b, preferred_element_type=f32)


def _tok(vals):
    t = None
    for v in vals:
        b = pltpu.bitcast(v, u32)
        for i in range(b.shape[0] // 8):
            for j in range(b.shape[1] // 128):
                p = b[i * 8:(i + 1) * 8, j * 128:(j + 1) * 128]
                t = p if t is None else t | p
    return t


def _pin(x, vals, zero):
    if not vals:
        return x
    top = pltpu.bitcast(pltpu.bitcast(x[0:16, 0:128], u32) | (_tok(vals) & zero), bf16)
    row0 = jnp.concatenate([top, x[0:16, 128:]], axis=1)
    return jnp.concatenate([row0, x[16:]], axis=0)


def _pin_at(x, pins, zero):
    if not pins:
        return x
    out, last = [], 0
    for k in sorted({k for k, _ in pins}):
        if k * 16 > last:
            out.append(x[last:k * 16])
        blk = x[k * 16:(k + 1) * 16]
        for (kk, n), vals in pins.items():
            if kk != k:
                continue
            top = pltpu.bitcast(pltpu.bitcast(blk[:, n * 128:(n + 1) * 128], u32) | (_tok(vals) & zero), bf16)
            parts = ([blk[:, :n * 128]] if n > 0 else []) + [top] + (
                [blk[:, (n + 1) * 128:]] if (n + 1) * 128 < blk.shape[1] else [])
            blk = jnp.concatenate(parts, axis=1) if len(parts) > 1 else top
        out.append(blk)
        last = (k + 1) * 16
    if last < x.shape[0]:
        out.append(x[last:])
    return jnp.concatenate(out, axis=0) if len(out) > 1 else out[0]


def _spread(items, n):
    return [items[(i * len(items)) // n:((i + 1) * len(items)) // n] for i in range(n)]


def _kernel(q_hbm, k_hbm, v_hbm, sk_hbm, hk_hbm, dd_hbm, w1_hbm, w2_hbm, w3_hbm, w4_hbm,
            o_hbm,
            w1b, w2b, w3b, w4b, kbuf, vbuf, hkb, qbuf, skb, ddb,
            Fm, Gm, skf, kf, ZA, ZB, YA, YB, ybuf, xbuf, ubuf, hbuf, z3buf, z1buf,
            zsm, sem):
    obuf = vbuf

    def cp_kvh(c, r0, nr, si):
        ch = pl.ds(c * 128, 128)
        return (
            pltpu.make_async_copy(k_hbm.at[0, pl.ds(r0, nr), ch], kbuf.at[pl.ds(16 + r0, nr), ch], sem.at[si]),
            pltpu.make_async_copy(v_hbm.at[0, pl.ds(r0, nr), ch], vbuf.at[pl.ds(r0, nr), ch], sem.at[si + 1]),
            pltpu.make_async_copy(hk_hbm.at[ch, pl.ds(r0, nr)], hkb.at[ch, pl.ds(r0, nr)], sem.at[si + 2]))

    N1 = NA // 2 // int('2')

    def cp_g0(i):
        return cp_kvh(0, i * 2 * TM, 2 * TM, 3 * i)

    def cp_g1(n):
        return cp_kvh(1, n * (S // N1), S // N1, 3 * (4 + n))

    def cp_grp(c):
        return cp_kvh(c, 0, S, 3 * (6 + c))

    SB = 3 * (6 + LG)

    def cp_q(j0, nb, si):
        return pltpu.make_async_copy(q_hbm.at[0, pl.ds(j0 * TM, nb * TM), :],
                                     qbuf.at[pl.ds(j0 * TM, nb * TM), :], sem.at[si])

    def cp_o(j):
        return pltpu.make_async_copy(obuf.at[pl.ds(j * TM, TM), :],
                                     o_hbm.at[0, pl.ds(j * TM, TM), :], sem.at[SB + 11 + j])

    cp_sk = pltpu.make_async_copy(sk_hbm, skb, sem.at[SB])
    cp_dd = pltpu.make_async_copy(dd_hbm, ddb, sem.at[SB + 1])
    cp_q0 = cp_q(0, 3, SB + 2)

    def cp_qb(j):
        return cp_q(j, 1, SB + 11 + NB + j - 3)

    cp_w1 = pltpu.make_async_copy(w1_hbm, w1b, sem.at[SB + 3])
    cp_w2 = pltpu.make_async_copy(w2_hbm, w2b, sem.at[SB + 4])
    FA = KR * TF
    cp_w34a = (
        pltpu.make_async_copy(w3_hbm.at[:, pl.ds(0, FA)], w3b.at[:, pl.ds(0, FA)], sem.at[SB + 5]),
        pltpu.make_async_copy(w4_hbm.at[pl.ds(0, FA), :], w4b.at[pl.ds(0, FA), :], sem.at[SB + 6]))
    cp_w34b = (
        pltpu.make_async_copy(w3_hbm.at[:, pl.ds(FA, FF - FA)], w3b.at[:, pl.ds(FA, FF - FA)], sem.at[SB + 7]),
        pltpu.make_async_copy(w4_hbm.at[pl.ds(FA, FF - FA), :], w4b.at[pl.ds(FA, FF - FA), :], sem.at[SB + 8]))

    def wait_all(cps):
        for cp in cps:
            cp.wait()

    cp_sk.start()
    cp_dd.start()
    for grp in ([cp_g0(i) for i in range(4)] + [cp_g1(n) for n in range(N1)]
                + [cp_grp(c) for c in range(2, LG)]):
        for cp in grp:
            cp.start()
    for cp in (cp_q0, cp_w1, cp_w2) + cp_w34a + cp_w34b + tuple(cp_qb(j) for j in range(3, NB)):
        cp.start()

    zsm[0] = 0
    kbuf[0:16, :] = jnp.zeros((16, D), bf16)
    hbuf[0:8, :] = jnp.zeros((8, D), f32)
    hbuf[S + 8:S + 16, :] = jnp.zeros((8, D), f32)

    def _basis(pos, part, n):
        k = jnp.where(pos < CB // 2, 2 * pos, 2 * pos - (CB - 1))
        m = ((2 * k + 1) * n + part * CB) & (4 * CB - 1)
        r = m & (2 * CB - 1)
        neg = jnp.logical_xor(m >= 2 * CB, r > CB)
        th = jnp.minimum(r, 2 * CB - r).astype(f32) * (math.pi / (2 * CB))
        t2 = th * th
        z = 1.0 / math.factorial(12)
        for e in (10, 8, 6, 4, 2, 0):
            z = 1.0 / math.factorial(e) - t2 * z
        z = jnp.where(neg, -z, z)
        return z, jnp.where(pos < CB // 2, z, -z)

    def dft_init(t, carry):
        rf = lax.broadcasted_iota(i32, (32, CB), 0)
        zs = _basis(t * 16 + (rf & 15), rf >> 4, lax.broadcasted_iota(i32, (32, CB), 1))
        cg = lax.broadcasted_iota(i32, (16, 2 * CB), 1)
        gs = _basis(cg >> 1, cg & 1, t * 16 + lax.broadcasted_iota(i32, (16, 2 * CB), 0))
        for par in range(2):
            Fm[par, pl.ds(pl.multiple_of(t * 16, 16), 16), :] = pltpu.bitcast(zs[par].astype(bf16), u32)
            Gm[par, pl.ds(pl.multiple_of(t * 8, 8), 8), :] = pltpu.bitcast(
                (gs[par] * (1.0 / CB)).astype(bf16), u32)
        return carry

    lax.fori_loop(0, CB // 16, dft_init, 0)

    cp_sk.wait()
    cp_dd.wait()
    sk32 = skb[...].astype(f32)
    for t in range(4):
        skf[t] = jnp.broadcast_to(sk32[t:t + 1, :], (8, D))
    skf[4] = jnp.broadcast_to(ddb[...].astype(f32).reshape(1, D), (8, D))

    def zero_vec():
        return jnp.full((8, 128), zsm[0], i32).astype(u32)

    def bmul(x, row8):
        n = x.shape[0] // 8
        return (x.reshape(n, 8, 128) * row8[None]).reshape(x.shape)

    def dsl(start, size, align):
        return pl.ds(start if isinstance(start, int) else pl.multiple_of(start, align), size)

    def unil(z):
        return (jnp.concatenate([z[32 * g:32 * g + 16] for g in range(CB // 16)], axis=0),
                jnp.concatenate([z[32 * g + 16:32 * g + 32] for g in range(CB // 16)], axis=0))

    def fwdh1(c, par, i, o, pins=None, skip=True):
        Z = (ZA if par == 0 else ZB).at[dsl(H0 + i * 2 * BS, 2 * BS, 8), :]
        ls = dsl(c * 128, 128, 128)
        a = 2 * i + o
        hh = lax.dot_general(_pin_at(pltpu.bitcast(Fm[o], bf16), pins, zero_vec()), hkb[ls, dsl(a * CB, CB, CB)], (((1,), (1,)), ((), ())),
                             preferred_element_type=f32)
        cc, dd = unil(hh)
        if o == 0 and skip and (not isinstance(i, int) or i == 0):
            d8 = skf[4, :, ls] if isinstance(i, int) else jnp.where(i == 0, skf[4, :, ls], 0.0)
            cc = (cc.reshape(CB // 8, 8, 128) + d8[None]).reshape(CB, 128)
        b = o * BS
        Z[b:b + CB, :] = cc
        Z[b + CS:b + CS + CB, :] = dd - cc
        Z[b + 2 * CS:b + 2 * CS + CB, :] = cc + dd
        return cc + dd

    def fwdx1(c, par, i, o, pins, sk, slot=0):
        Z = (ZA if par == 0 else ZB).at[dsl(i * 2 * BS, 2 * BS, 8), :]
        ls = dsl(c * 128, 128, 128)
        ks_ = i % 2 if isinstance(i, int) else slot
        if o == 0:
            kf[ks_] = kbuf[dsl(i * 2 * CB, 2 * CB + 16, 16), ls].astype(f32)
        a = 2 * i + o
        b0 = 16 + o * CB
        ks = bmul(kf[ks_, b0:b0 + CB, :], sk[0])
        for t in range(1, 4):
            ks = ks + bmul(kf[ks_, b0 - t:b0 - t + CB, :], sk[t])
        kv = (ks * vbuf[dsl(a * CB, CB, CB), ls].astype(f32)).astype(bf16)
        xh = _mm(_pin_at(pltpu.bitcast(Fm[o], bf16), pins, zero_vec()), kv)
        xr, xm = unil(xh)
        b = o * BS
        Z[b:b + CB, :] = xr
        Z[b + CS:b + CS + CB, :] = xm
        Z[b + 2 * CS:b + 2 * CS + CB, :] = xr + xm
        return xr + xm

    def mac_gen(par, i0, ns):
        for u in range(ns):
            yield from mac_gen1(par, i0 + u)

    def mac_gen1(par, i):
        Z, Y = (ZA, YA) if par == 0 else (ZB, YB)
        Z = Z.at[dsl(i * 16, 2 * H0 - CB + 16, 16), :]
        X, H = 0, H0
        prev = [None, None]
        for a0 in range(0, NA, NO):
            for h in range(2):
                def ld(ref, a):
                    b = ref + a * BS + h * 8
                    return tuple(Z[b + k * CS:b + k * CS + 8, :] for k in range(3))
                K = [None] * NO
                hw = {}
                for ap in range(a0 + NO):
                    xa, xb, xs = ld(X, ap)
                    for o in range(NO):
                        dl = a0 + o - ap
                        if dl < 0:
                            continue
                        if dl not in hw:
                            hw[dl] = ld(H, dl)
                        hc, he, hf = hw[dl]
                        t = (hc * xs, xa * he, xb * hf)
                        K[o] = t if K[o] is None else tuple(u + w for u, w in zip(K[o], t))
                        inj = yield K[o][2]
                        if inj is not None:
                            K[o] = (K[o][0], K[o][1], K[o][2] + inj)
                for o in range(NO):
                    re, im = K[o][0] - K[o][2], K[o][0] + K[o][1]
                    out = (re, im) if prev[h] is None else (re - prev[h][1], im + prev[h][0])
                    prev[h] = (re, im)
                    Y[a0 + o, dsl(i * 16 + h * 8, 8, 8), :] = pltpu.pack_elementwise(
                        list(out), packed_dtype=bf16).astype(u32)

    def inv1(c, par, i, o, pins=None):
        Y = YA if par == 0 else YB
        a = 2 * i + o
        y = _mm(_pin_at(pltpu.bitcast(Gm[o], bf16), pins, zero_vec()), pltpu.bitcast(Y[a], bf16))
        yv = ybuf.at[dsl(a * (CB // 2), CB // 2, CB // 2), :]
        for g in range(CB // 16):
            yv[8 * g:8 * g + 8, dsl(c * 128, 128, 128)] = pltpu.pack_elementwise(
                [y[16 * g:16 * g + 8], y[16 * g + 8:16 * g + 16]], packed_dtype=bf16).astype(u32)
        return y

    NPM = NA * (NA + 1)

    def group(c, par, do_inv, do_fwd, i0=0, ns=NA // 2):
        PI, P0, DP, NP_, R0, DR, G0 = (int(x) for x in '-20,12,12,16,220,12,4'.split(','))
        names = 'h0,x0,h1,x1'.split(',')
        zero = zero_vec()
        sk = [skf[t, :, dsl((c + 1) * 128, 128, 128)] for t in range(4)] if do_fwd else None
        gen = mac_gen(par, i0, ns)
        rec = [next(gen)]
        inj = {}
        for u in range(ns):
            i = i0 + u
            base = u * NPM
            while len(rec) <= base + P0 + (NP_ - 1) * DP:
                rec.append(gen.send(inj.get(len(rec))))
            pins = {k: {} for k in ('i0', 'i1', 'h0', 'h1', 'x0', 'x1')}
            if base + PI >= 0:
                pins['i0'][(0, 0)] = [rec[base + PI]]
                pins['i1'][(0, 0)] = [rec[base + PI]]
            for n in range(NP_):
                r = ((n + 1) * 16) // NP_ - 1
                pins[names[n % len(names)]][(r, 0)] = [rec[base + P0 + n * DP]]
            if do_inv:
                ys = [inv1(c - 1, 1 - par, i, 0, pins['i0']), inv1(c - 1, 1 - par, i, 1, pins['i1'])]
                if not do_fwd:
                    inj[base + R0] = pltpu.bitcast(_tok([y[CB - 8:CB] for y in ys]) & zero, f32)
            if do_fwd:
                res = [fwdh1(c + 1, 1 - par, i, 0, pins['h0'], skip=(u == 0)),
                       fwdh1(c + 1, 1 - par, i, 1, pins['h1']),
                       fwdx1(c + 1, 1 - par, i, 0, pins['x0'], sk, slot=u % 2),
                       fwdx1(c + 1, 1 - par, i, 1, pins['x1'], sk, slot=u % 2)]
                for g in range(G0, CB // 16):
                    tk = _tok([z[16 * g + 8:16 * g + 16] for z in res]) & zero
                    inj[base + R0 + (g - G0) * DR] = pltpu.bitcast(tk, f32)
        try:
            while True:
                rec.append(gen.send(inj.get(len(rec))))
        except StopIteration:
            pass

    def conv():
        def pre(i, carry):
            wait_all(cp_g0(i))
            sk = [skf[t, :, 0:128] for t in range(4)]
            for u in range(2):
                for o in range(2):
                    fwdh1(0, 0, 2 * i + u, o, skip=(u == 0))
                for o in range(2):
                    fwdx1(0, 0, 2 * i + u, o, None, sk, slot=u)
            return carry
        lax.fori_loop(0, NA // 4, pre, 0)
        NS0 = int('2')

        def step0(t, carry):
            wait_all(cp_g1(t))
            group(0, 0, False, True, t * NS0, NS0)
            return carry
        lax.fori_loop(0, NA // 2 // NS0, step0, 0)

        def it(t, carry):
            wait_all(cp_grp(2 * t + 2))
            group(2 * t + 1, 1, True, True)
            wait_all(cp_grp(2 * t + 3))
            group(2 * t + 2, 0, True, True)
            return carry
        lax.fori_loop(0, (LG - 2) // 2, it, 0)
        group(LG - 1, 1, True, False)

    conv()

    def rows(j):
        return j * TM if isinstance(j, int) else pl.multiple_of(j * TM, TM)

    def s0_rows(r, nr, s0, ns, from_q=False):
        sl = slice(s0 * R, (s0 + ns) * R)
        xv = xbuf.at[dsl(r, nr, nr), :]
        uv = ubuf.at[dsl(r, nr, nr), :]
        x = qbuf.at[dsl(r, nr, nr), :][sl, :].astype(f32)
        if from_q is not True:
            x = jnp.where(from_q, x, xv[sl, :])
        r2 = r // 2 if isinstance(r, int) else lax.shift_right_logical(r, 1)
        yw = ybuf.at[dsl(r2, nr // 2, nr // 2), :][s0 * 8:(s0 + ns) * 8, :]
        yy = [pltpu.unpack_elementwise(yw, index=k, packed_dtype=bf16, unpacked_dtype=f32)
              for k in range(2)]
        y = jnp.concatenate([yy[k][s * 8:(s + 1) * 8] for s in range(ns) for k in range(2)], axis=0)
        q, t1 = _ln_t(x)
        x1 = x + q * y
        u, t2 = _ln_t(x1)
        xv[sl, :] = x1 + u
        uv[sl, :] = u
        z, t3 = _ln_t(u)
        return z.astype(bf16), t1 + t2 + t3 + [[z[:, D - 128:]]]

    def rhs_pins(steps, ksteps, rot=[0]):
        pins = {}
        for t, lst in enumerate(steps):
            n, kg = t // ksteps, t % ksteps
            for i, vals in enumerate(lst):
                m = rot[0] % 4
                rot[0] += 1
                rg = 7 if (i % 2 == 0 and len(lst) > 1) else 0
                pins.setdefault(((kg * 4 + m) * 8 + rg, n), []).extend(vals)
        return pins

    def at_steps(toks, first, last, nsteps):
        steps = [[] for _ in range(nsteps)]
        for k, t in enumerate(toks):
            steps[first + (k * (last - first)) // max(len(toks) - 1, 1)].append(t)
        return steps

    def m1(r, z1, steps=None):
        w = w1b[...]
        if steps is not None:
            w = _pin_at(w, rhs_pins(steps, 2), zero_vec())
        hbuf[pl.ds(r + 8, z1.shape[0]), :] = _gelu(_mm(z1, w))

    def m2_dot(j, steps=None):
        r = rows(j)
        c = D // 4
        hv = hbuf.at[pl.ds(r, TM + 16), :]
        hs_in = jnp.concatenate([
            hv[8 - 1:8 - 1 + TM, 0 * c:1 * c], hv[8 + 1:8 + 1 + TM, 1 * c:2 * c],
            hv[8 - 2:8 - 2 + TM, 2 * c:3 * c], hv[8 + 2:8 + 2 + TM, 3 * c:4 * c]],
            axis=-1).astype(bf16)
        w = w2b[...]
        if steps is not None:
            w = _pin_at(w, rhs_pins(steps, 2), zero_vec())
        return _mm(hs_in, w)

    def ln3(j, hs, nb=4):
        r = rows(j)
        xv = xbuf.at[pl.ds(r, TM), :]
        uv = ubuf.at[pl.ds(r, TM), :]
        toks = []
        for s in range(0, NS, nb):
            sl = slice(s * R, (s + nb) * R)
            x1p = uv[sl, :] + hs[sl, :]
            xv[sl, :] += hs[sl, :]
            z, t = _ln_t(x1p)
            z3buf[sl, :] = z.astype(bf16)
            toks += (t if None else []) + [[z[:, D - 128:]]]
        return toks

    def m34(j, c0, c1, steps=None, to_x=True, to_o=False):
        r = rows(j)
        z3 = z3buf[...]
        zero = zero_vec()
        steps = (steps() if callable(steps) else steps) or [[] for _ in range(16 * NC)]
        acc = None
        for c in range(c0, c1):
            w3 = _pin_at(w3b[:, c * TF:(c + 1) * TF], rhs_pins(steps[16 * c:16 * c + 8], 2), zero)
            a = _gelu(_mm(z3, w3)).astype(bf16)
            w4 = _pin_at(w4b[c * TF:(c + 1) * TF, :], rhs_pins(steps[16 * c + 8:16 * c + 16], 1), zero)
            p = _mm(a, w4)
            acc = p if acc is None else acc + p
        xn = xbuf[pl.ds(r, TM), :] + acc
        if to_x:
            xbuf[pl.ds(r, TM), :] = xn
        if to_o:
            obuf[pl.ds(r, TM), :] = xn.astype(bf16)

    def cat(zs):
        return jnp.concatenate([z for z, _ in zs], axis=0)

    def toks(zs):
        return [t for _, ts in zs for t in ts]

    def prologue(_, carry):
        cp_q0.wait()
        cp_w1.wait()
        cp_w2.wait()
        F1, L1_, NBT = (int(x) for x in '1,15,4'.split(','))
        hn = NS // 2

        HM = TM // 2

        def half(k):
            return [s0_rows(k * HM, HM, s, NBT, True) for s in range(0, hn, NBT)]

        inv1(LG - 1, 1, 0, 0)
        inv1(LG - 1, 1, 0, 1)
        z0 = half(0)
        z1buf[...] = cat(z0)
        st = at_steps(toks(z0), 2, NA - 1, NA)
        for a in range(2, NA):
            inv1(LG - 1, 1, a // 2, a % 2, {(0, 0): [v for t in st[a] for v in t]} if st[a] else None)

        def it(k, carry):
            zc = z1buf[...]
            zn = half(k + 1)
            m1(pl.multiple_of(k * HM, HM), zc, at_steps(toks(zn), F1, L1_, 16))
            z1buf[...] = cat(zn)
            return carry
        lax.fori_loop(0, 5, it, 0)
        hs = m2_dot(0)
        lt = ln3(0, hs, 2)
        m1(5 * HM, z1buf[...], at_steps(lt, 2, 14, 16))
        wait_all(cp_w34a)
        m34(0, 0, KR)
        return carry

    lax.fori_loop(0, zsm[0] + 1, prologue, 0)
    wait_all(cp_w34b)

    def mm4_steps(items, sa, sz, c0, c1):
        st = [[] for _ in range(16 * NC)]
        slots = [16 * c + 8 + k for c in range(c0, c1) for k in range(sa, 8, sz)]
        for k, t in enumerate(items):
            st[slots[(k * len(slots)) // len(items)]].append(t)
        return st

    def body(g, carry):
        @pl.when(g + 3 < NB)
        def _():
            cp_qb(g + 3).wait()
        j = lax.rem(g + 3, NB)
        SB_, SA, SZ = (int(x) for x in '1,1,2'.split(','))
        zs = [s0_rows(rows(j), TM, s, SB_, g + 3 < NB) for s in range(0, NS, SB_)]
        jg = lax.rem(g, NB)
        m34(jg, KR, NC, mm4_steps([ts[-1] for _, ts in zs], SA, SZ, KR, NC), to_o=True)
        j1 = lax.rem(g + 1, NB)
        hs = m2_dot(j1)
        lt = ln3(j1, hs, int('1'))
        LA, LB = (int(x) for x in '2,13'.split(','))
        m1(rows(j), cat(zs), at_steps(lt, LA, LB, 16) if LA >= 0 else None)
        m34(j1, 0, KR)

        @pl.when(g >= NB)
        def _():
            cp_o(jg).start()
        return carry

    lax.fori_loop(0, G - 3, body, 0)

    def body3(j, carry):
        hs = m2_dot(j + 1)
        m34(j, KR, NC, lambda: mm4_steps(ln3(j + 1, hs, 2), 3, 3, KR, KR + 4), to_x=False, to_o=True)
        m34(j + 1, 0, KR)
        cp_o(j).start()
        return carry

    lax.fori_loop(NB - 3, NB - 1, body3, 0)
    m34(NB - 1, KR, NC, to_x=False, to_o=True)
    cp_o(NB - 1).start()
    for j in range(NB):
        cp_o(j).wait()


@jax.jit
def pallas_interleave_layers__ssm_conv_h3__mixer_s_mlp__prompt_kernel(
    A_q, A_k, A_v, A_shift_k, A_ssm_k, A_ssm_D, B_x, B_w1, B_w2, B_w3, B_w4,
):
    del B_x
    vm = pltpu.VMEM
    scratch = [
        vm((D, D), bf16), vm((D, D), bf16), vm((D, FF), bf16), vm((FF, D), bf16),
        vm((S + 16, D), bf16), vm((S, D), bf16), vm((D, S), bf16), vm((S, D), bf16),
        vm((4, D), bf16), vm((D,), bf16),
        vm((2, CB, CB), u32), vm((2, CB // 2, 2 * CB), u32),
        vm((5, 8, D), f32),
        vm((2, 2 * CB + 16, 128), f32),
        vm((2 * H0, 128), f32), vm((2 * H0, 128), f32),
        vm((NA, CB, 128), u32), vm((NA, CB, 128), u32),
        vm((S // 2, D), u32), vm((S, D), f32), vm((S, D), f32),
        vm((S + 16, D), f32), vm((TM, D), bf16), vm((TM // 2, D), bf16),
        pltpu.SMEM((1,), i32),
        pltpu.SemaphoreType.DMA((3 * (6 + LG) + 11 + NB + 5,)),
    ]
    return pl.pallas_call(
        _kernel,
        out_shape=jax.ShapeDtypeStruct(A_q.shape, bf16),
        in_specs=[pl.BlockSpec(memory_space=pl.ANY)] * 10,
        out_specs=pl.BlockSpec(memory_space=pl.ANY),
        scratch_shapes=scratch,
        compiler_params=pltpu.CompilerParams(vmem_limit_bytes=100 * 1024 * 1024),
    )(A_q, A_k, A_v, A_shift_k.T, A_ssm_k, A_ssm_D, B_w1, B_w2, B_w3, B_w4)
```

```python
import math

import jax
import jax.numpy as jnp
from jax import lax
import jax.experimental.pallas as pl
import jax.experimental.pallas.tpu as pltpu


f32, bf16, u32, i32 = jnp.float32, jnp.bfloat16, jnp.uint32, jnp.int32

S, D, FF = 2048, 1024, 3584
TM = 256
NB = S // TM
G = 2 * NB
CB = 128
NA = S // CB
NO = 4
TF = 512
NC = FF // TF
R = 16
NS = TM // R
LG = D // 128
KR = int('1')
EPS = 1e-5
CS = CB + 8
BS = 3 * CS
H0 = NA * BS + 16
C0 = math.sqrt(2.0 / math.pi)
C1 = C0 * 0.044715


def _ln(x):
    m = jnp.mean(x, axis=-1, keepdims=True)
    xc = x - m
    v = jnp.mean(xc * xc, axis=-1, keepdims=True)
    return xc * lax.rsqrt(v + EPS)


def _ln_t(x):
    m = jnp.mean(x, axis=-1, keepdims=True)
    xc = x - m
    v = jnp.mean(xc * xc, axis=-1, keepdims=True)
    r = lax.rsqrt(v + EPS)
    n = x.shape[0]
    return xc * r, [[jnp.broadcast_to(m, (n, 128))], [jnp.broadcast_to(r, (n, 128))]]


def _gelu(x):
    hx = 0.5 * x
    return hx + hx * jnp.tanh(x * (C0 + C1 * (x * x)))


def _mm(a, b):
    return jnp.dot(a, b, preferred_element_type=f32)


def _tok(vals):
    t = None
    for v in vals:
        b = pltpu.bitcast(v, u32)
        for i in range(b.shape[0] // 8):
            for j in range(b.shape[1] // 128):
                p = b[i * 8:(i + 1) * 8, j * 128:(j + 1) * 128]
                t = p if t is None else t | p
    return t


def _pin(x, vals, zero):
    if not vals:
        return x
    top = pltpu.bitcast(pltpu.bitcast(x[0:16, 0:128], u32) | (_tok(vals) & zero), bf16)
    row0 = jnp.concatenate([top, x[0:16, 128:]], axis=1)
    return jnp.concatenate([row0, x[16:]], axis=0)


def _pin_at(x, pins, zero):
    if not pins:
        return x
    out, last = [], 0
    for k in sorted({k for k, _ in pins}):
        if k * 16 > last:
            out.append(x[last:k * 16])
        blk = x[k * 16:(k + 1) * 16]
        for (kk, n), vals in pins.items():
            if kk != k:
                continue
            top = pltpu.bitcast(pltpu.bitcast(blk[:, n * 128:(n + 1) * 128], u32) | (_tok(vals) & zero), bf16)
            parts = ([blk[:, :n * 128]] if n > 0 else []) + [top] + (
                [blk[:, (n + 1) * 128:]] if (n + 1) * 128 < blk.shape[1] else [])
            blk = jnp.concatenate(parts, axis=1) if len(parts) > 1 else top
        out.append(blk)
        last = (k + 1) * 16
    if last < x.shape[0]:
        out.append(x[last:])
    return jnp.concatenate(out, axis=0) if len(out) > 1 else out[0]


def _spread(items, n):
    return [items[(i * len(items)) // n:((i + 1) * len(items)) // n] for i in range(n)]


def _kernel(q_hbm, k_hbm, v_hbm, sk_hbm, hk_hbm, dd_hbm, w1_hbm, w2_hbm, w3_hbm, w4_hbm,
            o_hbm,
            w1b, w2b, w3b, w4b, kbuf, vbuf, hkb, qbuf, skb, ddb,
            Fm, Gm, skf, kf, ZA, ZB, YA, YB, ybuf, xbuf, ubuf, hbuf, z3buf, accb,
            zsm, sem):
    obuf = vbuf

    def cp_kvh(c, r0, nr, si):
        ch = pl.ds(c * 128, 128)
        return (
            pltpu.make_async_copy(k_hbm.at[0, pl.ds(r0, nr), ch], kbuf.at[pl.ds(16 + r0, nr), ch], sem.at[si]),
            pltpu.make_async_copy(v_hbm.at[0, pl.ds(r0, nr), ch], vbuf.at[pl.ds(r0, nr), ch], sem.at[si + 1]),
            pltpu.make_async_copy(hk_hbm.at[ch, pl.ds(r0, nr)], hkb.at[ch, pl.ds(r0, nr)], sem.at[si + 2]))

    N1 = int('4')

    def cp_g0(i):
        return cp_kvh(0, i * 2 * TM, 2 * TM, 3 * i)

    def cp_g1(n):
        return cp_kvh(1, n * (S // N1), S // N1, 3 * (4 + n))

    def cp_grp(c):
        return cp_kvh(c, 0, S, 3 * (6 + c))

    SB = 3 * (6 + LG)

    def cp_q(j0, nb, si):
        return pltpu.make_async_copy(q_hbm.at[0, pl.ds(j0 * TM, nb * TM), :],
                                     qbuf.at[pl.ds(j0 * TM, nb * TM), :], sem.at[si])

    def cp_o(j):
        return pltpu.make_async_copy(obuf.at[pl.ds(j * TM, TM), :],
                                     o_hbm.at[0, pl.ds(j * TM, TM), :], sem.at[SB + 11 + j])

    cp_sk = pltpu.make_async_copy(sk_hbm, skb, sem.at[SB])
    cp_dd = pltpu.make_async_copy(dd_hbm, ddb, sem.at[SB + 1])
    cp_q0 = cp_q(0, 3, SB + 2)

    def cp_qb(j):
        return cp_q(j, 1, SB + 11 + NB + j - 3)

    cp_w1 = pltpu.make_async_copy(w1_hbm, w1b, sem.at[SB + 3])
    cp_w2 = pltpu.make_async_copy(w2_hbm, w2b, sem.at[SB + 4])
    FA = KR * TF
    cp_w34a = (
        pltpu.make_async_copy(w3_hbm.at[:, pl.ds(0, FA)], w3b.at[:, pl.ds(0, FA)], sem.at[SB + 5]),
        pltpu.make_async_copy(w4_hbm.at[pl.ds(0, FA), :], w4b.at[pl.ds(0, FA), :], sem.at[SB + 6]))
    cp_w34b = (
        pltpu.make_async_copy(w3_hbm.at[:, pl.ds(FA, FF - FA)], w3b.at[:, pl.ds(FA, FF - FA)], sem.at[SB + 7]),
        pltpu.make_async_copy(w4_hbm.at[pl.ds(FA, FF - FA), :], w4b.at[pl.ds(FA, FF - FA), :], sem.at[SB + 8]))

    def wait_all(cps):
        for cp in cps:
            cp.wait()

    cp_sk.start()
    cp_dd.start()
    for grp in ([cp_g0(i) for i in range(4)] + [cp_g1(n) for n in range(N1)]
                + [cp_grp(c) for c in range(2, LG)]):
        for cp in grp:
            cp.start()
    for cp in (cp_q0, cp_w1, cp_w2) + cp_w34a + cp_w34b + tuple(cp_qb(j) for j in range(3, NB)):
        cp.start()

    zsm[0] = 0
    kbuf[0:16, :] = jnp.zeros((16, D), bf16)
    hbuf[0:8, :] = jnp.zeros((8, D), f32)
    hbuf[S + 8:S + 16, :] = jnp.zeros((8, D), f32)

    def _basis(pos, part, n):
        k = jnp.where(pos < CB // 2, 2 * pos, 2 * pos - (CB - 1))
        m = ((2 * k + 1) * n + part * CB) & (4 * CB - 1)
        r = m & (2 * CB - 1)
        neg = jnp.logical_xor(m >= 2 * CB, r > CB)
        th = jnp.minimum(r, 2 * CB - r).astype(f32) * (math.pi / (2 * CB))
        t2 = th * th
        z = 1.0 / math.factorial(12)
        for e in (10, 8, 6, 4, 2, 0):
            z = 1.0 / math.factorial(e) - t2 * z
        z = jnp.where(neg, -z, z)
        return z, jnp.where(pos < CB // 2, z, -z)

    def dft_init(t, carry):
        rf = lax.broadcasted_iota(i32, (32, CB), 0)
        zs = _basis(t * 16 + (rf & 15), rf >> 4, lax.broadcasted_iota(i32, (32, CB), 1))
        cg = lax.broadcasted_iota(i32, (16, 2 * CB), 1)
        gs = _basis(cg >> 1, cg & 1, t * 16 + lax.broadcasted_iota(i32, (16, 2 * CB), 0))
        for par in range(2):
            Fm[par, pl.ds(pl.multiple_of(t * 16, 16), 16), :] = pltpu.bitcast(zs[par].astype(bf16), u32)
            Gm[par, pl.ds(pl.multiple_of(t * 8, 8), 8), :] = pltpu.bitcast(
                (gs[par] * (1.0 / CB)).astype(bf16), u32)
        return carry

    lax.fori_loop(0, CB // 16, dft_init, 0)

    cp_sk.wait()
    cp_dd.wait()
    sk32 = skb[...].astype(f32)
    for t in range(4):
        skf[t] = jnp.broadcast_to(sk32[t:t + 1, :], (8, D))
    skf[4] = jnp.broadcast_to(ddb[...].astype(f32).reshape(1, D), (8, D))

    def zero_vec():
        return jnp.full((8, 128), zsm[0], i32).astype(u32)

    def bmul(x, row8):
        n = x.shape[0] // 8
        return (x.reshape(n, 8, 128) * row8[None]).reshape(x.shape)

    def dsl(start, size, align):
        return pl.ds(start if isinstance(start, int) else pl.multiple_of(start, align), size)

    def unil(z):
        return (jnp.concatenate([z[32 * g:32 * g + 16] for g in range(CB // 16)], axis=0),
                jnp.concatenate([z[32 * g + 16:32 * g + 32] for g in range(CB // 16)], axis=0))

    def fwdh1(c, par, i, o, pins=None, skip=True):
        Z = (ZA if par == 0 else ZB).at[dsl(H0 + i * 2 * BS, 2 * BS, 8), :]
        ls = dsl(c * 128, 128, 128)
        a = 2 * i + o
        hh = lax.dot_general(_pin_at(pltpu.bitcast(Fm[o], bf16), pins, zero_vec()), hkb[ls, dsl(a * CB, CB, CB)], (((1,), (1,)), ((), ())),
                             preferred_element_type=f32)
        cc, dd = unil(hh)
        if o == 0 and skip and (not isinstance(i, int) or i == 0):
            d8 = skf[4, :, ls] if isinstance(i, int) else jnp.where(i == 0, skf[4, :, ls], 0.0)
            cc = (cc.reshape(CB // 8, 8, 128) + d8[None]).reshape(CB, 128)
        b = o * BS
        Z[b:b + CB, :] = cc
        Z[b + CS:b + CS + CB, :] = dd - cc
        Z[b + 2 * CS:b + 2 * CS + CB, :] = cc + dd
        return cc + dd

    def fwdx1(c, par, i, o, pins, sk, slot=0):
        Z = (ZA if par == 0 else ZB).at[dsl(i * 2 * BS, 2 * BS, 8), :]
        ls = dsl(c * 128, 128, 128)
        ks_ = i % 2 if isinstance(i, int) else slot
        if o == 0:
            kf[ks_] = kbuf[dsl(i * 2 * CB, 2 * CB + 16, 16), ls].astype(f32)
        a = 2 * i + o
        b0 = 16 + o * CB
        ks = bmul(kf[ks_, b0:b0 + CB, :], sk[0])
        for t in range(1, 4):
            ks = ks + bmul(kf[ks_, b0 - t:b0 - t + CB, :], sk[t])
        kv = (ks * vbuf[dsl(a * CB, CB, CB), ls].astype(f32)).astype(bf16)
        xh = _mm(_pin_at(pltpu.bitcast(Fm[o], bf16), pins, zero_vec()), kv)
        xr, xm = unil(xh)
        b = o * BS
        Z[b:b + CB, :] = xr
        Z[b + CS:b + CS + CB, :] = xm
        Z[b + 2 * CS:b + 2 * CS + CB, :] = xr + xm
        return xr + xm

    def mac_gen(par, i0, ns):
        for u in range(ns):
            yield from mac_gen1(par, i0 + u)

    def mac_gen1(par, i):
        Z, Y = (ZA, YA) if par == 0 else (ZB, YB)
        Z = Z.at[dsl(i * 16, 2 * H0 - CB + 16, 16), :]
        X, H = 0, H0
        prev = [None, None]
        for a0 in range(0, NA, NO):
            for h in range(2):
                def ld(ref, a):
                    b = ref + a * BS + h * 8
                    return tuple(Z[b + k * CS:b + k * CS + 8, :] for k in range(3))
                K = [None] * NO
                hw = {}
                for ap in range(a0 + NO):
                    xa, xb, xs = ld(X, ap)
                    for o in range(NO):
                        dl = a0 + o - ap
                        if dl < 0:
                            continue
                        if dl not in hw:
                            hw[dl] = ld(H, dl)
                        hc, he, hf = hw[dl]
                        t = (hc * xs, xa * he, xb * hf)
                        K[o] = t if K[o] is None else tuple(u + w for u, w in zip(K[o], t))
                        inj = yield K[o][2]
                        if inj is not None:
                            K[o] = (K[o][0], K[o][1], K[o][2] + inj)
                for o in range(NO):
                    re, im = K[o][0] - K[o][2], K[o][0] + K[o][1]
                    out = (re, im) if prev[h] is None else (re - prev[h][1], im + prev[h][0])
                    prev[h] = (re, im)
                    Y[a0 + o, dsl(i * 16 + h * 8, 8, 8), :] = pltpu.pack_elementwise(
                        list(out), packed_dtype=bf16).astype(u32)

    def inv1(c, par, i, o, pins=None):
        Y = YA if par == 0 else YB
        a = 2 * i + o
        y = _mm(_pin_at(pltpu.bitcast(Gm[o], bf16), pins, zero_vec()), pltpu.bitcast(Y[a], bf16))
        yv = ybuf.at[dsl(a * (CB // 2), CB // 2, CB // 2), :]
        for g in range(CB // 16):
            yv[8 * g:8 * g + 8, dsl(c * 128, 128, 128)] = pltpu.pack_elementwise(
                [y[16 * g:16 * g + 8], y[16 * g + 8:16 * g + 16]], packed_dtype=bf16).astype(u32)
        return y

    NPM = NA * (NA + 1)

    def group(c, par, do_inv, do_fwd, i0=0, ns=NA // 2):
        PI, P0, DP, NP_, R0, DR, G0 = (int(x) for x in '-20,12,12,16,220,12,4'.split(','))
        names = 'h0,x0,h1,x1'.split(',')
        zero = zero_vec()
        sk = [skf[t, :, dsl((c + 1) * 128, 128, 128)] for t in range(4)] if do_fwd else None
        gen = mac_gen(par, i0, ns)
        rec = [next(gen)]
        inj = {}
        for u in range(ns):
            i = i0 + u
            base = u * NPM
            while len(rec) <= base + P0 + (NP_ - 1) * DP:
                rec.append(gen.send(inj.get(len(rec))))
            pins = {k: {} for k in ('i0', 'i1', 'h0', 'h1', 'x0', 'x1')}
            if base + PI >= 0:
                pins['i0'][(0, 0)] = [rec[base + PI]]
                pins['i1'][(0, 0)] = [rec[base + PI]]
            for n in range(NP_):
                r = ((n + 1) * 16) // NP_ - 1
                pins[names[n % len(names)]][(r, 0)] = [rec[base + P0 + n * DP]]
            if do_inv:
                ys = [inv1(c - 1, 1 - par, i, 0, pins['i0']), inv1(c - 1, 1 - par, i, 1, pins['i1'])]
                if not do_fwd:
                    inj[base + R0] = pltpu.bitcast(_tok([y[CB - 8:CB] for y in ys]) & zero, f32)
            if do_fwd:
                res = [fwdh1(c + 1, 1 - par, i, 0, pins['h0'], skip=(u == 0)),
                       fwdh1(c + 1, 1 - par, i, 1, pins['h1']),
                       fwdx1(c + 1, 1 - par, i, 0, pins['x0'], sk, slot=u % 2),
                       fwdx1(c + 1, 1 - par, i, 1, pins['x1'], sk, slot=u % 2)]
                for g in range(G0, CB // 16):
                    tk = _tok([z[16 * g + 8:16 * g + 16] for z in res]) & zero
                    inj[base + R0 + (g - G0) * DR] = pltpu.bitcast(tk, f32)
        try:
            while True:
                rec.append(gen.send(inj.get(len(rec))))
        except StopIteration:
            pass

    def conv():
        def pre(i, carry):
            wait_all(cp_g0(i))
            sk = [skf[t, :, 0:128] for t in range(4)]
            for u in range(2):
                for o in range(2):
                    fwdh1(0, 0, 2 * i + u, o, skip=(u == 0))
                for o in range(2):
                    fwdx1(0, 0, 2 * i + u, o, None, sk, slot=u)
            return carry
        lax.fori_loop(0, NA // 4, pre, 0)
        NS0 = NA // 2 // N1

        def step0(t, carry):
            wait_all(cp_g1(t))
            group(0, 0, False, True, t * NS0, NS0)
            return carry
        lax.fori_loop(0, N1, step0, 0)

        def it(t, carry):
            wait_all(cp_grp(2 * t + 2))
            group(2 * t + 1, 1, True, True)
            wait_all(cp_grp(2 * t + 3))
            group(2 * t + 2, 0, True, True)
            return carry
        lax.fori_loop(0, (LG - 2) // 2, it, 0)
        group(LG - 1, 1, True, False)

    conv()

    def rows(j):
        return j * TM if isinstance(j, int) else pl.multiple_of(j * TM, TM)

    def s0_rows(r, nr, s0, ns, from_q=False, after=None):
        sl = slice(s0 * R, (s0 + ns) * R)
        xv = xbuf.at[dsl(r, nr, nr), :]
        uv = ubuf.at[dsl(r, nr, nr), :]
        x = qbuf.at[dsl(r, nr, nr), :][sl, :].astype(f32)
        if from_q is not True:
            x = jnp.where(from_q, x, xv[sl, :])
        if after is not None:
            z8 = pltpu.bitcast(_tok([after]) & zero_vec(), f32)
            x0 = (x[:, 0:128].reshape(2 * ns, 8, 128) + z8[None]).reshape(ns * R, 128)
            x = jnp.concatenate([x0, x[:, 128:]], axis=1)
        r2 = r // 2 if isinstance(r, int) else lax.shift_right_logical(r, 1)
        yw = ybuf.at[dsl(r2, nr // 2, nr // 2), :][s0 * 8:(s0 + ns) * 8, :]
        yy = [pltpu.unpack_elementwise(yw, index=k, packed_dtype=bf16, unpacked_dtype=f32)
              for k in range(2)]
        y = jnp.concatenate([yy[k][s * 8:(s + 1) * 8] for s in range(ns) for k in range(2)], axis=0)
        q, t1 = _ln_t(x)
        x1 = x + q * y
        u, t2 = _ln_t(x1)
        xv[sl, :] = x1
        uv[sl, :] = u
        z, t3 = _ln_t(u)
        return z.astype(bf16), t1 + t2 + t3 + [[z[:, D - 128:]]]

    def rhs_pins(steps, ksteps, rot=[0]):
        pins = {}
        for t, lst in enumerate(steps):
            n, kg = t // ksteps, t % ksteps
            for i, vals in enumerate(lst):
                m = rot[0] % 4
                rot[0] += 1
                rg = 7 if (i % 2 == 0 and len(lst) > 1) else 0
                pins.setdefault(((kg * 4 + m) * 8 + rg, n), []).extend(vals)
        return pins

    def at_steps(toks, first, last, nsteps):
        steps = [[] for _ in range(nsteps)]
        for k, t in enumerate(toks):
            steps[first + (k * (last - first)) // max(len(toks) - 1, 1)].append(t)
        return steps

    def m1(r, z1, steps=None):
        w = w1b[...]
        if steps is not None:
            w = _pin_at(w, rhs_pins(steps, 2), zero_vec())
        h = _gelu(_mm(z1, w))
        hbuf[pl.ds(r + 8, z1.shape[0]), :] = h
        return h

    def m2_dot(j, steps=None):
        r = rows(j)
        c = D // 4
        hv = hbuf.at[pl.ds(r, TM + 16), :]
        hs_in = jnp.concatenate([
            hv[8 - 1:8 - 1 + TM, 0 * c:1 * c], hv[8 + 1:8 + 1 + TM, 1 * c:2 * c],
            hv[8 - 2:8 - 2 + TM, 2 * c:3 * c], hv[8 + 2:8 + 2 + TM, 3 * c:4 * c]],
            axis=-1).astype(bf16)
        w = w2b[...]
        if steps is not None:
            w = _pin_at(w, rhs_pins(steps, 2), zero_vec())
        return _mm(hs_in, w)

    def ln3(j, hs, nb=4):
        r = rows(j)
        xv = xbuf.at[pl.ds(r, TM), :]
        uv = ubuf.at[pl.ds(r, TM), :]
        toks, res = [], []
        for s in range(0, NS, nb):
            sl = slice(s * R, (s + nb) * R)
            x1p = uv[sl, :] + hs[sl, :]
            res.append(xv[sl, :] + x1p)
            z, t = _ln_t(x1p)
            z3buf[sl, :] = z.astype(bf16)
            toks += (t if None else []) + [[z[:, D - 128:]]]
        return jnp.concatenate(res, axis=0), toks

    def mlp(c0, c1, acc, steps=None):
        z3 = z3buf[...]
        zero = zero_vec()
        steps = (steps() if callable(steps) else steps) or [[] for _ in range(16 * NC)]
        for c in range(c0, c1):
            w3 = _pin_at(w3b[:, c * TF:(c + 1) * TF], rhs_pins(steps[16 * c:16 * c + 8], 2), zero)
            a = _gelu(_mm(z3, w3)).astype(bf16)
            w4 = _pin_at(w4b[c * TF:(c + 1) * TF, :], rhs_pins(steps[16 * c + 8:16 * c + 16], 1), zero)
            acc = acc + _mm(a, w4)
        return acc

    def m34b(j, steps=None, to_x=True):
        r = rows(j)
        xn = mlp(KR, NC, accb[...], steps)
        if to_x:
            xbuf[pl.ds(r, TM), :] = xn
        obuf[pl.ds(r, TM), :] = xn.astype(bf16)

    def cat(zs):
        return jnp.concatenate([z for z, _ in zs], axis=0)

    def toks(zs):
        sel = [int(x) for x in '0,1,2,3,4,5,6'.split(',')]
        return [ts[i] for _, ts in zs for i in sel]

    def mm4_steps(items, sa, sz, c0, c1):
        st = [[] for _ in range(16 * NC)]
        slots = [16 * c + 8 + k for c in range(c0, c1) for k in range(sa, 8, sz)]
        for k, t in enumerate(items):
            st[slots[(k * len(slots)) // len(items)]].append(t)
        return st

    def prologue(_, carry):
        cp_q0.wait()
        cp_w1.wait()
        cp_w2.wait()
        wait_all(cp_w34a)
        F1, L1_, NBT = (int(x) for x in '2,15,4'.split(','))
        hn = NS // 2

        HM = TM // 2

        def half(k, nbt=NBT, after=None):
            CH = int('-1')
            out = []
            for s in range(0, hn, nbt):
                out.append(s0_rows(k * HM, HM, s, nbt, True, after))
                if CH >= 0 and k > 0:
                    after = out[-1][1][CH][0][0:8]
            return out

        AF = [int(x) for x in '6,6,7,7'.split(',')]

        def mark(h, n):
            return None if n < 0 else h[0:8, n * 128:(n + 1) * 128]

        inv1(LG - 1, 1, 0, 0)
        inv1(LG - 1, 1, 0, 1)
        HB, HA, HZ = (int(x) for x in '8,-1,0'.split(','))
        z = [half(0, HB)]
        st = at_steps(toks(z[0]), HA, HZ, NA) if HA >= 0 else [[] for _ in range(NA)]
        for a in range(2, NA):
            inv1(LG - 1, 1, a // 2, a % 2, {(0, 0): [v for t in st[a] for v in t]} if st[a] else None)
        z.append(half(1))
        h = m1(0, cat(z[0]), at_steps(toks(z[1]), F1, L1_, 16))
        z.append(half(2, after=mark(h, AF[0])))
        h = m1(HM, cat(z[1]), at_steps(toks(z[2]), F1, L1_, 16))
        z.append(half(3, after=mark(h, AF[1])))
        t3 = toks(z[3])
        n3 = int('7')
        h = m1(2 * HM, cat(z[2]), at_steps(t3[:n3], F1, L1_, 16))
        z.append(half(4, after=mark(h, AF[2])))
        hs = m2_dot(0, at_steps(t3[n3:] + toks(z[4]), F1, L1_, 16))
        res, lt = ln3(0, hs, 2)
        m1(3 * HM, cat(z[3]), at_steps(lt[:len(lt) // 2], 2, 14, 16))
        h = m1(4 * HM, cat(z[4]), at_steps(lt[len(lt) // 2:], 1, 12, 16))
        z.append(half(5, after=mark(h, AF[3])))
        accb[...] = mlp(0, KR, res, mm4_steps(toks(z[5]), 0, 1, 0, KR))
        m1(5 * HM, cat(z[5]))
        return carry

    lax.fori_loop(0, zsm[0] + 1, prologue, 0)
    wait_all(cp_w34b)

    def body(g, carry):
        @pl.when(g + 3 < NB)
        def _():
            cp_qb(g + 3).wait()
        j = lax.rem(g + 3, NB)
        SB_, SA, SZ = (int(x) for x in '1,1,2'.split(','))
        zs = [s0_rows(rows(j), TM, s, SB_, g + 3 < NB) for s in range(0, NS, SB_)]
        jg = lax.rem(g, NB)
        m34b(jg, mm4_steps([ts[-1] for _, ts in zs], SA, SZ, KR, NC))
        j1 = lax.rem(g + 1, NB)
        hs = m2_dot(j1)
        res, lt = ln3(j1, hs, int('1'))
        LA, LB = (int(x) for x in '3,15'.split(','))
        m1(rows(j), cat(zs), at_steps(lt, LA, LB, 16) if LA >= 0 else None)
        accb[...] = mlp(0, KR, res)

        @pl.when(g >= NB)
        def _():
            cp_o(jg).start()
        return carry

    lax.fori_loop(0, G - 3, body, 0)

    def body3(j, carry):
        hs = m2_dot(j + 1)
        st = {}

        def side():
            st['res'], lt = ln3(j + 1, hs, 2)
            return mm4_steps(lt, 3, 3, KR, KR + 4)
        m34b(j, side, to_x=False)
        accb[...] = mlp(0, KR, st['res'])
        cp_o(j).start()
        return carry

    lax.fori_loop(NB - 3, NB - 1, body3, 0)
    m34b(NB - 1, to_x=False)
    cp_o(NB - 1).start()
    for j in range(NB):
        cp_o(j).wait()


@jax.jit
def pallas_interleave_layers__ssm_conv_h3__mixer_s_mlp__prompt_kernel(
    A_q, A_k, A_v, A_shift_k, A_ssm_k, A_ssm_D, B_x, B_w1, B_w2, B_w3, B_w4,
):
    del B_x
    vm = pltpu.VMEM
    scratch = [
        vm((D, D), bf16), vm((D, D), bf16), vm((D, FF), bf16), vm((FF, D), bf16),
        vm((S + 16, D), bf16), vm((S, D), bf16), vm((D, S), bf16), vm((S, D), bf16),
        vm((4, D), bf16), vm((D,), bf16),
        vm((2, CB, CB), u32), vm((2, CB // 2, 2 * CB), u32),
        vm((5, 8, D), f32),
        vm((2, 2 * CB + 16, 128), f32),
        vm((2 * H0, 128), f32), vm((2 * H0, 128), f32),
        vm((NA, CB, 128), u32), vm((NA, CB, 128), u32),
        vm((S // 2, D), u32), vm((S, D), f32), vm((S, D), f32),
        vm((S + 16, D), f32), vm((TM, D), bf16), vm((TM, D), f32),
        pltpu.SMEM((1,), i32),
        pltpu.SemaphoreType.DMA((3 * (6 + LG) + 11 + NB + 5,)),
    ]
    return pl.pallas_call(
        _kernel,
        out_shape=jax.ShapeDtypeStruct(A_q.shape, bf16),
        in_specs=[pl.BlockSpec(memory_space=pl.ANY)] * 10,
        out_specs=pl.BlockSpec(memory_space=pl.ANY),
        scratch_shapes=scratch,
        compiler_params=pltpu.CompilerParams(vmem_limit_bytes=100 * 1024 * 1024),
    )(A_q, A_k, A_v, A_shift_k.T, A_ssm_k, A_ssm_D, B_w1, B_w2, B_w3, B_w4)
```

```python
import math

import jax
import jax.numpy as jnp
from jax import lax
import jax.experimental.pallas as pl
import jax.experimental.pallas.tpu as pltpu


f32, bf16, u32, i32 = jnp.float32, jnp.bfloat16, jnp.uint32, jnp.int32

S, D, FF = 2048, 1024, 3584
TM = 256
NB = S // TM
G = 2 * NB
CB = 128
NA = S // CB
NO = 4
TF = 512
NC = FF // TF
R = 16
NS = TM // R
LG = D // 128
KR = int('1')
EPS = 1e-5
CS = CB + 8
BS = 3 * CS
H0 = NA * BS + 16
C0 = math.sqrt(2.0 / math.pi)
C1 = C0 * 0.044715


def _ln(x):
    m = jnp.mean(x, axis=-1, keepdims=True)
    xc = x - m
    v = jnp.mean(xc * xc, axis=-1, keepdims=True)
    return xc * lax.rsqrt(v + EPS)


def _ln_t(x):
    m = jnp.mean(x, axis=-1, keepdims=True)
    xc = x - m
    v = jnp.mean(xc * xc, axis=-1, keepdims=True)
    r = lax.rsqrt(v + EPS)
    n = x.shape[0]
    return xc * r, [[jnp.broadcast_to(m, (n, 128))], [jnp.broadcast_to(r, (n, 128))]]


def _gelu(x):
    hx = 0.5 * x
    return hx + hx * jnp.tanh(x * (C0 + C1 * (x * x)))


def _mm(a, b):
    return jnp.dot(a, b, preferred_element_type=f32)


def _tok(vals):
    t = None
    for v in vals:
        b = pltpu.bitcast(v, u32)
        for i in range(b.shape[0] // 8):
            for j in range(b.shape[1] // 128):
                p = b[i * 8:(i + 1) * 8, j * 128:(j + 1) * 128]
                t = p if t is None else t | p
    return t


def _pin(x, vals, zero):
    if not vals:
        return x
    top = pltpu.bitcast(pltpu.bitcast(x[0:16, 0:128], u32) | (_tok(vals) & zero), bf16)
    row0 = jnp.concatenate([top, x[0:16, 128:]], axis=1)
    return jnp.concatenate([row0, x[16:]], axis=0)


def _pin_at(x, pins, zero):
    if not pins:
        return x
    out, last = [], 0
    for k in sorted({k for k, _ in pins}):
        if k * 16 > last:
            out.append(x[last:k * 16])
        blk = x[k * 16:(k + 1) * 16]
        for (kk, n), vals in pins.items():
            if kk != k:
                continue
            top = pltpu.bitcast(pltpu.bitcast(blk[:, n * 128:(n + 1) * 128], u32) | (_tok(vals) & zero), bf16)
            parts = ([blk[:, :n * 128]] if n > 0 else []) + [top] + (
                [blk[:, (n + 1) * 128:]] if (n + 1) * 128 < blk.shape[1] else [])
            blk = jnp.concatenate(parts, axis=1) if len(parts) > 1 else top
        out.append(blk)
        last = (k + 1) * 16
    if last < x.shape[0]:
        out.append(x[last:])
    return jnp.concatenate(out, axis=0) if len(out) > 1 else out[0]


def _spread(items, n):
    return [items[(i * len(items)) // n:((i + 1) * len(items)) // n] for i in range(n)]


def _kernel(q_hbm, k_hbm, v_hbm, sk_hbm, hk_hbm, dd_hbm, w1_hbm, w2_hbm, w3_hbm, w4_hbm,
            o_hbm,
            w1b, w2b, w3b, w4b, kbuf, vbuf, hkb, qbuf, skb, ddb,
            Fm, Gm, skf, kf, ZA, ZB, YA, YB, ybuf, xbuf, ubuf, hbuf, z3buf, accb,
            zsm, sem):
    obuf = vbuf

    def cp_kvh(c, r0, nr, si):
        ch = pl.ds(c * 128, 128)
        return (
            pltpu.make_async_copy(k_hbm.at[0, pl.ds(r0, nr), ch], kbuf.at[pl.ds(16 + r0, nr), ch], sem.at[si]),
            pltpu.make_async_copy(v_hbm.at[0, pl.ds(r0, nr), ch], vbuf.at[pl.ds(r0, nr), ch], sem.at[si]),
            pltpu.make_async_copy(hk_hbm.at[ch, pl.ds(r0, nr)], hkb.at[ch, pl.ds(r0, nr)], sem.at[si]))

    N1 = int('2')

    def cp_g0(i):
        return cp_kvh(0, i * 2 * TM, 2 * TM, i)

    def cp_g1(n):
        return cp_kvh(1, n * (S // N1), S // N1, 4 + n)

    def cp_grp(c):
        return cp_kvh(c, 0, S, 2 + N1 + c)

    SB = 2 + N1 + LG

    def cp_q(j0, nb, si):
        return pltpu.make_async_copy(q_hbm.at[0, pl.ds(j0 * TM, nb * TM), :],
                                     qbuf.at[pl.ds(j0 * TM, nb * TM), :], sem.at[si])

    def cp_o(j, c0=0, nc=D):
        return pltpu.make_async_copy(obuf.at[pl.ds(j * TM, TM), pl.ds(c0, nc)],
                                     o_hbm.at[0, pl.ds(j * TM, TM), pl.ds(c0, nc)], sem.at[SB + 4])

    cp_sk = pltpu.make_async_copy(sk_hbm, skb, sem.at[SB])
    cp_dd = pltpu.make_async_copy(dd_hbm, ddb, sem.at[SB])
    cp_q0 = cp_q(0, 3, SB + 1)

    cp_q3 = cp_q(3, 1, SB + 2)
    cp_q4 = cp_q(4, NB - 4, SB + 3)

    cp_w1 = pltpu.make_async_copy(w1_hbm, w1b, sem.at[SB + 1])
    cp_w2 = pltpu.make_async_copy(w2_hbm, w2b, sem.at[SB + 1])
    FA = KR * TF
    cp_w34a = (
        pltpu.make_async_copy(w3_hbm.at[:, pl.ds(0, FA)], w3b.at[:, pl.ds(0, FA)], sem.at[SB + 1]),
        pltpu.make_async_copy(w4_hbm.at[pl.ds(0, FA), :], w4b.at[pl.ds(0, FA), :], sem.at[SB + 1]))
    cp_w34b = (
        pltpu.make_async_copy(w3_hbm.at[:, pl.ds(FA, FF - FA)], w3b.at[:, pl.ds(FA, FF - FA)], sem.at[SB + 2]),
        pltpu.make_async_copy(w4_hbm.at[pl.ds(FA, FF - FA), :], w4b.at[pl.ds(FA, FF - FA), :], sem.at[SB + 2]))

    def wait_all(cps):
        for cp in cps:
            cp.wait()

    cp_sk.start()
    cp_dd.start()
    for grp in ([cp_g0(i) for i in range(4)] + [cp_g1(n) for n in range(N1)]
                + [cp_grp(c) for c in range(2, LG)]):
        for cp in grp:
            cp.start()
    for cp in (cp_q0, cp_w1, cp_w2) + cp_w34a + cp_w34b + (cp_q3, cp_q4):
        cp.start()

    zsm[0] = 0
    kbuf[0:16, :] = jnp.zeros((16, D), bf16)
    hbuf[0:8, :] = jnp.zeros((8, D), f32)
    hbuf[S + 8:S + 16, :] = jnp.zeros((8, D), f32)

    def _basis(pos, part, n):
        k = jnp.where(pos < CB // 2, 2 * pos, 2 * pos - (CB - 1))
        m = ((2 * k + 1) * n + part * CB) & (4 * CB - 1)
        r = m & (2 * CB - 1)
        neg = jnp.logical_xor(m >= 2 * CB, r > CB)
        th = jnp.minimum(r, 2 * CB - r).astype(f32) * (math.pi / (2 * CB))
        t2 = th * th
        z = 1.0 / math.factorial(12)
        for e in (10, 8, 6, 4, 2, 0):
            z = 1.0 / math.factorial(e) - t2 * z
        z = jnp.where(neg, -z, z)
        return z, jnp.where(pos < CB // 2, z, -z)

    def dft_init(t, carry):
        rf = lax.broadcasted_iota(i32, (32, CB), 0)
        zs = _basis(t * 16 + (rf & 15), rf >> 4, lax.broadcasted_iota(i32, (32, CB), 1))
        cg = lax.broadcasted_iota(i32, (16, 2 * CB), 1)
        gs = _basis(cg >> 1, cg & 1, t * 16 + lax.broadcasted_iota(i32, (16, 2 * CB), 0))
        for par in range(2):
            Fm[par, pl.ds(pl.multiple_of(t * 16, 16), 16), :] = pltpu.bitcast(zs[par].astype(bf16), u32)
            Gm[par, pl.ds(pl.multiple_of(t * 8, 8), 8), :] = pltpu.bitcast(
                (gs[par] * (1.0 / CB)).astype(bf16), u32)
        return carry

    lax.fori_loop(0, CB // 16, dft_init, 0)

    cp_sk.wait()
    cp_dd.wait()
    sk32 = skb[...].astype(f32)
    for t in range(4):
        skf[t] = jnp.broadcast_to(sk32[t:t + 1, :], (8, D))
    skf[4] = jnp.broadcast_to(ddb[...].astype(f32).reshape(1, D), (8, D))

    def zero_vec():
        return jnp.full((8, 128), zsm[0], i32).astype(u32)

    def bmul(x, row8):
        n = x.shape[0] // 8
        return (x.reshape(n, 8, 128) * row8[None]).reshape(x.shape)

    def dsl(start, size, align):
        return pl.ds(start if isinstance(start, int) else pl.multiple_of(start, align), size)

    def unil(z):
        return (jnp.concatenate([z[32 * g:32 * g + 16] for g in range(CB // 16)], axis=0),
                jnp.concatenate([z[32 * g + 16:32 * g + 32] for g in range(CB // 16)], axis=0))

    def fwdh1(c, par, i, o, pins=None, skip=True):
        Z = (ZA if par == 0 else ZB).at[dsl(H0 + i * 2 * BS, 2 * BS, 8), :]
        ls = dsl(c * 128, 128, 128)
        a = 2 * i + o
        hh = lax.dot_general(_pin_at(pltpu.bitcast(Fm[o], bf16), pins, zero_vec()), hkb[ls, dsl(a * CB, CB, CB)], (((1,), (1,)), ((), ())),
                             preferred_element_type=f32)
        cc, dd = unil(hh)
        if o == 0 and skip and (not isinstance(i, int) or i == 0):
            d8 = skf[4, :, ls] if isinstance(i, int) else jnp.where(i == 0, skf[4, :, ls], 0.0)
            cc = (cc.reshape(CB // 8, 8, 128) + d8[None]).reshape(CB, 128)
        b = o * BS
        Z[b:b + CB, :] = cc
        Z[b + CS:b + CS + CB, :] = dd - cc
        Z[b + 2 * CS:b + 2 * CS + CB, :] = cc + dd
        return cc + dd

    def fwdx1(c, par, i, o, pins, sk, slot=0):
        Z = (ZA if par == 0 else ZB).at[dsl(i * 2 * BS, 2 * BS, 8), :]
        ls = dsl(c * 128, 128, 128)
        ks_ = i % 2 if isinstance(i, int) else slot
        if o == 0:
            kf[ks_] = kbuf[dsl(i * 2 * CB, 2 * CB + 16, 16), ls].astype(f32)
        a = 2 * i + o
        b0 = 16 + o * CB
        ks = bmul(kf[ks_, b0:b0 + CB, :], sk[0])
        for t in range(1, 4):
            ks = ks + bmul(kf[ks_, b0 - t:b0 - t + CB, :], sk[t])
        kv = (ks * vbuf[dsl(a * CB, CB, CB), ls].astype(f32)).astype(bf16)
        xh = _mm(_pin_at(pltpu.bitcast(Fm[o], bf16), pins, zero_vec()), kv)
        xr, xm = unil(xh)
        b = o * BS
        Z[b:b + CB, :] = xr
        Z[b + CS:b + CS + CB, :] = xm
        Z[b + 2 * CS:b + 2 * CS + CB, :] = xr + xm
        return xr + xm

    def mac_gen(par, i0, ns):
        for u in range(ns):
            yield from mac_gen1(par, i0 + u)

    def mac_gen1(par, i):
        Z, Y = (ZA, YA) if par == 0 else (ZB, YB)
        Z = Z.at[dsl(i * 16, 2 * H0 - CB + 16, 16), :]
        X, H = 0, H0
        prev = [None, None]
        for a0 in range(0, NA, NO):
            for h in range(2):
                def ld(ref, a):
                    b = ref + a * BS + h * 8
                    return tuple(Z[b + k * CS:b + k * CS + 8, :] for k in range(3))
                K = [None] * NO
                hw = {}
                for ap in range(a0 + NO):
                    xa, xb, xs = ld(X, ap)
                    for o in range(NO):
                        dl = a0 + o - ap
                        if dl < 0:
                            continue
                        if dl not in hw:
                            hw[dl] = ld(H, dl)
                        hc, he, hf = hw[dl]
                        t = (hc * xs, xa * he, xb * hf)
                        K[o] = t if K[o] is None else tuple(u + w for u, w in zip(K[o], t))
                        inj = yield K[o][2]
                        if inj is not None:
                            K[o] = (K[o][0], K[o][1], K[o][2] + inj)
                for o in range(NO):
                    re, im = K[o][0] - K[o][2], K[o][0] + K[o][1]
                    out = (re, im) if prev[h] is None else (re - prev[h][1], im + prev[h][0])
                    prev[h] = (re, im)
                    Y[a0 + o, dsl(i * 16 + h * 8, 8, 8), :] = pltpu.pack_elementwise(
                        list(out), packed_dtype=bf16).astype(u32)

    def inv1(c, par, i, o, pins=None):
        Y = YA if par == 0 else YB
        a = 2 * i + o
        y = _mm(_pin_at(pltpu.bitcast(Gm[o], bf16), pins, zero_vec()), pltpu.bitcast(Y[a], bf16))
        yv = ybuf.at[dsl(a * (CB // 2), CB // 2, CB // 2), :]
        for g in range(CB // 16):
            yv[8 * g:8 * g + 8, dsl(c * 128, 128, 128)] = pltpu.pack_elementwise(
                [y[16 * g:16 * g + 8], y[16 * g + 8:16 * g + 16]], packed_dtype=bf16).astype(u32)
        return y

    NPM = NA * (NA + 1)

    def group(c, par, do_inv, do_fwd, i0=0, ns=NA // 2):
        PI, P0, DP, NP_, R0, DR, G0 = (int(x) for x in '-20,12,12,16,220,12,4'.split(','))
        names = 'h0,x0,h1,x1'.split(',')
        zero = zero_vec()
        sk = [skf[t, :, dsl((c + 1) * 128, 128, 128)] for t in range(4)] if do_fwd else None
        gen = mac_gen(par, i0, ns)
        rec = [next(gen)]
        inj = {}
        for u in range(ns):
            i = i0 + u
            base = u * NPM
            while len(rec) <= base + P0 + (NP_ - 1) * DP:
                rec.append(gen.send(inj.get(len(rec))))
            pins = {k: {} for k in ('i0', 'i1', 'h0', 'h1', 'x0', 'x1')}
            if base + PI >= 0:
                pins['i0'][(0, 0)] = [rec[base + PI]]
                pins['i1'][(0, 0)] = [rec[base + PI]]
            for n in range(NP_):
                r = ((n + 1) * 16) // NP_ - 1
                pins[names[n % len(names)]][(r, 0)] = [rec[base + P0 + n * DP]]
            if do_inv:
                ys = [inv1(c - 1, 1 - par, i, 0, pins['i0']), inv1(c - 1, 1 - par, i, 1, pins['i1'])]
                if not do_fwd:
                    inj[base + R0] = pltpu.bitcast(_tok([y[CB - 8:CB] for y in ys]) & zero, f32)
            if do_fwd:
                res = [fwdh1(c + 1, 1 - par, i, 0, pins['h0'], skip=(u == 0)),
                       fwdh1(c + 1, 1 - par, i, 1, pins['h1']),
                       fwdx1(c + 1, 1 - par, i, 0, pins['x0'], sk, slot=u % 2),
                       fwdx1(c + 1, 1 - par, i, 1, pins['x1'], sk, slot=u % 2)]
                for g in range(G0, CB // 16):
                    tk = _tok([z[16 * g + 8:16 * g + 16] for z in res]) & zero
                    inj[base + R0 + (g - G0) * DR] = pltpu.bitcast(tk, f32)
        try:
            while True:
                rec.append(gen.send(inj.get(len(rec))))
        except StopIteration:
            pass

    def conv():
        def pre(i, carry):
            wait_all(cp_g0(i))
            sk = [skf[t, :, 0:128] for t in range(4)]
            for u in range(2):
                for o in range(2):
                    fwdh1(0, 0, 2 * i + u, o, skip=(u == 0))
                for o in range(2):
                    fwdx1(0, 0, 2 * i + u, o, None, sk, slot=u)
            return carry
        lax.fori_loop(0, NA // 4, pre, 0)
        NS0 = NA // 2 // N1

        def step0(t, carry):
            wait_all(cp_g1(t))
            group(0, 0, False, True, t * NS0, NS0)
            return carry
        lax.fori_loop(0, N1, step0, 0)

        def it(t, carry):
            wait_all(cp_grp(2 * t + 2))
            group(2 * t + 1, 1, True, True)
            wait_all(cp_grp(2 * t + 3))
            group(2 * t + 2, 0, True, True)
            return carry
        lax.fori_loop(0, (LG - 2) // 2, it, 0)
        group(LG - 1, 1, True, False)

    conv()

    def rows(j):
        return j * TM if isinstance(j, int) else pl.multiple_of(j * TM, TM)

    def s0_rows(r, nr, s0, ns, from_q=False, after=None):
        sl = slice(s0 * R, (s0 + ns) * R)
        xv = xbuf.at[dsl(r, nr, nr), :]
        uv = ubuf.at[dsl(r, nr, nr), :]
        x = qbuf.at[dsl(r, nr, nr), :][sl, :].astype(f32)
        if from_q is not True:
            x = jnp.where(from_q, x, xv[sl, :])
        if after is not None:
            z8 = pltpu.bitcast(_tok([after]) & zero_vec(), f32)
            x0 = (x[:, 0:128].reshape(2 * ns, 8, 128) + z8[None]).reshape(ns * R, 128)
            x = jnp.concatenate([x0, x[:, 128:]], axis=1)
        r2 = r // 2 if isinstance(r, int) else lax.shift_right_logical(r, 1)
        yw = ybuf.at[dsl(r2, nr // 2, nr // 2), :][s0 * 8:(s0 + ns) * 8, :]
        yy = [pltpu.unpack_elementwise(yw, index=k, packed_dtype=bf16, unpacked_dtype=f32)
              for k in range(2)]
        y = jnp.concatenate([yy[k][s * 8:(s + 1) * 8] for s in range(ns) for k in range(2)], axis=0)
        q, t1 = _ln_t(x)
        x1 = x + q * y
        u, t2 = _ln_t(x1)
        xv[sl, :] = x1
        uv[sl, :] = u
        z, t3 = _ln_t(u)
        return z.astype(bf16), t1 + t2 + t3 + [[z[:, D - 128:]]]

    def rhs_pins(steps, ksteps, rot=[0]):
        pins = {}
        for t, lst in enumerate(steps):
            n, kg = t // ksteps, t % ksteps
            for i, vals in enumerate(lst):
                m = rot[0] % 4
                rot[0] += 1
                rg = 7 if (i % 2 == 0 and len(lst) > 1) else 0
                pins.setdefault(((kg * 4 + m) * 8 + rg, n), []).extend(vals)
        return pins

    def at_steps(toks, first, last, nsteps):
        steps = [[] for _ in range(nsteps)]
        for k, t in enumerate(toks):
            steps[first + (k * (last - first)) // max(len(toks) - 1, 1)].append(t)
        return steps

    def m1(r, z1, steps=None):
        w = w1b[...]
        if steps is not None:
            w = _pin_at(w, rhs_pins(steps, 2), zero_vec())
        h = _gelu(_mm(z1, w))
        hbuf[pl.ds(r + 8, z1.shape[0]), :] = h
        return h

    def m2_dot(j, steps=None):
        r = rows(j)
        c = D // 4
        hv = hbuf.at[pl.ds(r, TM + 16), :]
        hs_in = jnp.concatenate([
            hv[8 - 1:8 - 1 + TM, 0 * c:1 * c], hv[8 + 1:8 + 1 + TM, 1 * c:2 * c],
            hv[8 - 2:8 - 2 + TM, 2 * c:3 * c], hv[8 + 2:8 + 2 + TM, 3 * c:4 * c]],
            axis=-1).astype(bf16)
        w = w2b[...]
        if steps is not None:
            w = _pin_at(w, rhs_pins(steps, 2), zero_vec())
        return _mm(hs_in, w)

    def delay(x, after):
        if after is None:
            return x
        z8 = pltpu.bitcast(_tok([after]) & zero_vec(), f32)
        x0 = (x[:, 0:128].reshape(x.shape[0] // 8, 8, 128) + z8[None]).reshape(x.shape[0], 128)
        return jnp.concatenate([x0, x[:, 128:]], axis=1)

    def ln3(j, hs, nb=4, lo=0, hi=NS, after=None):
        r = rows(j)
        xv = xbuf.at[pl.ds(r, TM), :]
        uv = ubuf.at[pl.ds(r, TM), :]
        toks, res = [], []
        for s in range(lo, hi, nb):
            sl = slice(s * R, (s + nb) * R)
            x1p = delay(uv[sl, :], after) + hs[sl, :]
            res.append(xv[sl, :] + x1p)
            z, t = _ln_t(x1p)
            z3buf[sl, :] = z.astype(bf16)
            toks += (t if None else []) + [[z[:, D - 128:]]]
        return jnp.concatenate(res, axis=0), toks

    def mlp(c0, c1, acc, steps=None, side=None):
        z3 = z3buf[...]
        zero = zero_vec()
        steps = (steps() if callable(steps) else steps) or [[] for _ in range(16 * NC)]
        for c in range(c0, c1):
            w3 = _pin_at(w3b[:, c * TF:(c + 1) * TF], rhs_pins(steps[16 * c:16 * c + 8], 2), zero)
            a = _gelu(_mm(z3, w3))
            if side is not None:
                side(c, a, steps)
            a = a.astype(bf16)
            w4 = _pin_at(w4b[c * TF:(c + 1) * TF, :], rhs_pins(steps[16 * c + 8:16 * c + 16], 1), zero)
            acc = acc + _mm(a, w4)
        return acc

    def m34b(j, steps=None, to_x=True, side=None):
        r = rows(j)
        xn = mlp(KR, NC, accb[...], steps, side)
        if to_x:
            xbuf[pl.ds(r, TM), :] = xn
        obuf[pl.ds(r, TM), :] = xn.astype(bf16)

    def cat(zs):
        return jnp.concatenate([z for z, _ in zs], axis=0)

    def toks(zs):
        sel = [int(x) for x in '0,1,2,3,4,5,6'.split(',')]
        return [ts[i] for _, ts in zs for i in sel]

    def mm4_steps(items, sa, sz, c0, c1):
        st = [[] for _ in range(16 * NC)]
        slots = [16 * c + 8 + k for c in range(c0, c1) for k in range(sa, 8, sz)]
        for k, t in enumerate(items):
            st[slots[(k * len(slots)) // len(items)]].append(t)
        return st

    def prologue(_, carry):
        cp_q0.wait()
        cp_w1.wait()
        cp_w2.wait()
        wait_all(cp_w34a)
        F1, L1_, NBT = (int(x) for x in '2,15,4'.split(','))
        hn = NS // 2

        HM = TM // 2

        def half(k, nbt=NBT, after=None):
            CH = int('-1')
            out = []
            for s in range(0, hn, nbt):
                out.append(s0_rows(k * HM, HM, s, nbt, True, after))
                if CH >= 0 and k > 0:
                    after = out[-1][1][CH][0][0:8]
            return out

        AF = [int(x) for x in '6,6,7,7'.split(',')]

        def mark(h, n):
            return None if n < 0 else h[0:8, n * 128:(n + 1) * 128]

        inv1(LG - 1, 1, 0, 0)
        inv1(LG - 1, 1, 0, 1)
        HB, HA, HZ = (int(x) for x in '8,-1,0'.split(','))
        z = [half(0, HB)]
        st = at_steps(toks(z[0]), HA, HZ, NA) if HA >= 0 else [[] for _ in range(NA)]
        for a in range(2, NA):
            inv1(LG - 1, 1, a // 2, a % 2, {(0, 0): [v for t in st[a] for v in t]} if st[a] else None)
        z.append(half(1))
        h = m1(0, cat(z[0]), at_steps(toks(z[1]), F1, L1_, 16))
        z.append(half(2, after=mark(h, AF[0])))
        h = m1(HM, cat(z[1]), at_steps(toks(z[2]), F1, L1_, 16))
        z.append(half(3, after=mark(h, AF[1])))
        t3 = toks(z[3])
        n3 = int('7')
        h = m1(2 * HM, cat(z[2]), at_steps(t3[:n3], F1, L1_, 16))
        z.append(half(4, after=mark(h, AF[2])))
        hs = m2_dot(0, at_steps(t3[n3:] + toks(z[4]), F1, L1_, 16))
        res, lt = ln3(0, hs, 2)
        m1(3 * HM, cat(z[3]), at_steps(lt[:len(lt) // 2], 2, 14, 16))
        h = m1(4 * HM, cat(z[4]), at_steps(lt[len(lt) // 2:], 1, 12, 16))
        z.append(half(5, after=mark(h, AF[3])))
        accb[...] = mlp(0, KR, res, mm4_steps(toks(z[5]), 0, 1, 0, KR))
        m1(5 * HM, cat(z[5]))
        return carry

    lax.fori_loop(0, zsm[0] + 1, prologue, 0)
    wait_all(cp_w34b + (cp_q3,))

    def body(g, carry):
        @pl.when(g == 1)
        def _():
            cp_q4.wait()
        j = lax.rem(g + 3, NB)
        jg = lax.rem(g, NB)
        if None:
            T3, ORD, D0, DD, DL = (int(x) for x in None.split(','))
            j1 = lax.rem(g + 1, NB)
            acc = mlp(KR, KR + T3, accb[...])
            hs = m2_dot(j1)
            rs, zs = [], []
            grp = _spread(list(range(NS)), NC - KR - T3)

            def side(c, a, steps):
                rel = a[0:8, 0:128]
                pos = 16 * c + 8 + D0
                for kind in (('l', 's') if ORD == 0 else ('s', 'l')):
                    for n, st_ in enumerate(grp[c - KR - T3]):
                        if kind == 'l':
                            r_, lt = ln3(j1, hs, 1, st_, st_ + 1, rel if n == 0 else None)
                            rs.append(r_)
                            if n == len(grp[c - KR - T3]) - 1:
                                steps[min(pos, 16 * NC - 1)].append(lt[-1])
                                pos += DL
                        else:
                            zs.append(s0_rows(rows(j), TM, st_, 1, g + 3 < NB, after=rel if n == 0 else None))
                            steps[min(pos, 16 * NC - 1)].append(zs[-1][1][-1])
                            pos += DD
            xn = mlp(KR + T3, NC, acc, None, side)
            xbuf[pl.ds(rows(jg), TM), :] = xn
            obuf[pl.ds(rows(jg), TM), :] = xn.astype(bf16)
            m1(rows(j), cat(zs))
            accb[...] = mlp(0, KR, jnp.concatenate(rs, axis=0))

            @pl.when(g >= NB)
            def _():
                cp_o(jg).start()
            return carry
        if '0,2,2':
            RT, D0, DD = (int(x) for x in '0,2,2'.split(','))
            zs = []
            grp = _spread(list(range(NS)), NC - KR)

            def side(c, a, steps):
                for n, st_ in enumerate(grp[c - KR]):
                    zs.append(s0_rows(rows(j), TM, st_, 1, g + 3 < NB,
                                      after=a[0:8, RT * 128:(RT + 1) * 128] if n == 0 else None))
                    steps[min(16 * c + 8 + D0 + n * DD, 16 * NC - 1)].append(zs[-1][1][-1])
            m34b(jg, side=side)
        else:
            SB_, SA, SZ = (int(x) for x in '1,1,2'.split(','))
            zs = [s0_rows(rows(j), TM, s, SB_, g + 3 < NB) for s in range(0, NS, SB_)]
            m34b(jg, mm4_steps([ts[-1] for _, ts in zs], SA, SZ, KR, NC))
        j1 = lax.rem(g + 1, NB)
        hs = m2_dot(j1)
        if None:
            NQ, LT, LD = (int(x) for x in None.split(','))
            wq = D // NQ
            z1 = cat(zs)
            rs, after, due = [], None, []
            for qd in range(NQ):
                r_, lt = ln3(j1, hs, 1, qd * NS // NQ, (qd + 1) * NS // NQ, after)
                rs.append(r_)
                nst = 16 // NQ
                w = _pin_at(w1b[:, qd * wq:(qd + 1) * wq],
                            rhs_pins(at_steps(due, LD, nst - 1, nst) if due else [], 2), zero_vec())
                due = lt
                h = _gelu(_mm(z1, w))
                hbuf[pl.ds(rows(j) + 8, TM), qd * wq:(qd + 1) * wq] = h
                after = h[0:8, LT * 128:(LT + 1) * 128]
            res = jnp.concatenate(rs, axis=0)
        else:
            res, lt = ln3(j1, hs, int('1'))
            LA, LB = (int(x) for x in '3,15'.split(','))
            m1(rows(j), cat(zs), at_steps(lt, LA, LB, 16) if LA >= 0 else None)
        accb[...] = mlp(0, KR, res)

        @pl.when(g >= NB)
        def _():
            cp_o(jg).start()
        return carry

    lax.fori_loop(0, G - 3, body, 0)

    def body3(j, carry):
        T3, NL, RT, D0, DD = (int(x) for x in '1,5,0,2,2'.split(','))
        acc = accb[...]
        if T3:
            acc = mlp(KR, KR + T3, acc)
        hs = m2_dot(j + 1)
        rs = []
        grp = _spread(list(range(NS)), NL) + [[]] * NC

        def side(c, a, steps):
            for n, st_ in enumerate(grp[c - KR - T3]):
                r_, lt = ln3(j + 1, hs, 1, st_, st_ + 1,
                             a[0:8, RT * 128:(RT + 1) * 128] if (n == 0 and RT >= 0) else None)
                rs.append(r_)
                steps[min(16 * c + 8 + D0 + n * DD, 16 * NC - 1)].append(lt[-1])
        obuf[pl.ds(rows(j), TM), :] = mlp(KR + T3, NC, acc, None, side).astype(bf16)
        accb[...] = mlp(0, KR, jnp.concatenate(rs, axis=0))
        cp_o(j).start()
        return carry

    lax.fori_loop(NB - 3, NB - 1, body3, 0)
    OC = [0] + [int(x) for x in '512,896'.split(',')] + [D]
    OS = tuple((OC[i], OC[i + 1] - OC[i]) for i in range(len(OC) - 1))
    acc = mlp(KR, NC - 1, accb[...])
    a = _gelu(_mm(z3buf[...], w3b[:, FF - TF:])).astype(bf16)
    for c0, nc in OS:
        obuf[S - TM:, c0:c0 + nc] = (acc[:, c0:c0 + nc] + _mm(a, w4b[FF - TF:, c0:c0 + nc])).astype(bf16)
        cp_o(NB - 1, c0, nc).start()
    for j in range(NB - 1):
        cp_o(j).wait()
    for c0, nc in OS:
        cp_o(NB - 1, c0, nc).wait()


@jax.jit
def pallas_interleave_layers__ssm_conv_h3__mixer_s_mlp__prompt_kernel(
    A_q, A_k, A_v, A_shift_k, A_ssm_k, A_ssm_D, B_x, B_w1, B_w2, B_w3, B_w4,
):
    del B_x
    vm = pltpu.VMEM
    scratch = [
        vm((D, D), bf16), vm((D, D), bf16), vm((D, FF), bf16), vm((FF, D), bf16),
        vm((S + 16, D), bf16), vm((S, D), bf16), vm((D, S), bf16), vm((S, D), bf16),
        vm((4, D), bf16), vm((D,), bf16),
        vm((2, CB, CB), u32), vm((2, CB // 2, 2 * CB), u32),
        vm((5, 8, D), f32),
        vm((2, 2 * CB + 16, 128), f32),
        vm((2 * H0, 128), f32), vm((2 * H0, 128), f32),
        vm((NA, CB, 128), u32), vm((NA, CB, 128), u32),
        vm((S // 2, D), u32), vm((S, D), f32), vm((S, D), f32),
        vm((S + 16, D), f32), vm((TM, D), bf16), vm((TM, D), f32),
        pltpu.SMEM((1,), i32),
        pltpu.SemaphoreType.DMA((2 + int('2') + LG + 5,)),
    ]
    return pl.pallas_call(
        _kernel,
        out_shape=jax.ShapeDtypeStruct(A_q.shape, bf16),
        in_specs=[pl.BlockSpec(memory_space=pl.ANY)] * 10,
        out_specs=pl.BlockSpec(memory_space=pl.ANY),
        scratch_shapes=scratch,
        compiler_params=pltpu.CompilerParams(vmem_limit_bytes=100 * 1024 * 1024),
    )(A_q, A_k, A_v, A_shift_k.T, A_ssm_k, A_ssm_D, B_w1, B_w2, B_w3, B_w4)
```

```python
import math

import jax
import jax.numpy as jnp
from jax import lax
import jax.experimental.pallas as pl
import jax.experimental.pallas.tpu as pltpu


f32, bf16, u32, i32 = jnp.float32, jnp.bfloat16, jnp.uint32, jnp.int32

S, D, FF = 2048, 1024, 3584
TM = 256
NB = S // TM
G = 2 * NB
CB = 128
NA = S // CB
NO = 4
TF = 512
NC = FF // TF
R = 16
NS = TM // R
LG = D // 128
KR = int('4')
EPS = 1e-5
CS = CB + 8
BS = 3 * CS
H0 = NA * BS + 16
C0 = math.sqrt(2.0 / math.pi)
C1 = C0 * 0.044715
SHIFTS = (1, 1, -1, -1, 2, 2, -2, -2)


def _ln(x):
    m = jnp.mean(x, axis=-1, keepdims=True)
    xc = x - m
    v = jnp.mean(xc * xc, axis=-1, keepdims=True)
    return xc * lax.rsqrt(v + EPS)


def _ln_t(x):
    m = jnp.mean(x, axis=-1, keepdims=True)
    xc = x - m
    v = jnp.mean(xc * xc, axis=-1, keepdims=True)
    r = lax.rsqrt(v + EPS)
    n = x.shape[0]
    return xc * r, [[jnp.broadcast_to(m, (n, 128))], [jnp.broadcast_to(r, (n, 128))]]


def _gelu(x):
    hx = 0.5 * x
    return hx + hx * jnp.tanh(x * (C0 + C1 * (x * x)))


def _mm(a, b):
    return jnp.dot(a, b, preferred_element_type=f32)


def _tok(vals):
    t = None
    for v in vals:
        b = pltpu.bitcast(v, u32)
        for i in range(b.shape[0] // 8):
            for j in range(b.shape[1] // 128):
                p = b[i * 8:(i + 1) * 8, j * 128:(j + 1) * 128]
                t = p if t is None else t | p
    return t


def _pin(x, vals, zero):
    if not vals:
        return x
    top = pltpu.bitcast(pltpu.bitcast(x[0:16, 0:128], u32) | (_tok(vals) & zero), bf16)
    row0 = jnp.concatenate([top, x[0:16, 128:]], axis=1)
    return jnp.concatenate([row0, x[16:]], axis=0)


def _pin_at(x, pins, zero):
    if not pins:
        return x
    out, last = [], 0
    for k in sorted({k for k, _ in pins}):
        if k * 16 > last:
            out.append(x[last:k * 16])
        blk = x[k * 16:(k + 1) * 16]
        for (kk, n), vals in pins.items():
            if kk != k:
                continue
            top = pltpu.bitcast(pltpu.bitcast(blk[:, n * 128:(n + 1) * 128], u32) | (_tok(vals) & zero), bf16)
            parts = ([blk[:, :n * 128]] if n > 0 else []) + [top] + (
                [blk[:, (n + 1) * 128:]] if (n + 1) * 128 < blk.shape[1] else [])
            blk = jnp.concatenate(parts, axis=1) if len(parts) > 1 else top
        out.append(blk)
        last = (k + 1) * 16
    if last < x.shape[0]:
        out.append(x[last:])
    return jnp.concatenate(out, axis=0) if len(out) > 1 else out[0]


def _spread(items, n):
    return [items[(i * len(items)) // n:((i + 1) * len(items)) // n] for i in range(n)]


def _kernel(q_hbm, k_hbm, v_hbm, sk_hbm, hk_hbm, dd_hbm, w1_hbm, w2_hbm, w3_hbm, w4_hbm,
            o_hbm,
            w1b, w2b, w3b, w4b, kbuf, vbuf, hkb, qbuf, skb, ddb,
            Fm, Gm, skf, kf, ZA, ZB, YA, YB, ybuf, xbuf, x1b, ub, hwin, hcar, z1buf, z3buf, accb,
            zsm, sem):
    obuf = vbuf

    def cp_kvh(c, r0, nr, si):
        ch = pl.ds(c * 128, 128)
        return (
            pltpu.make_async_copy(k_hbm.at[0, pl.ds(r0, nr), ch], kbuf.at[pl.ds(16 + r0, nr), ch], sem.at[si]),
            pltpu.make_async_copy(v_hbm.at[0, pl.ds(r0, nr), ch], vbuf.at[pl.ds(r0, nr), ch], sem.at[si]),
            pltpu.make_async_copy(hk_hbm.at[ch, pl.ds(r0, nr)], hkb.at[ch, pl.ds(r0, nr)], sem.at[si]))

    G1 = [int(x) for x in '0,3,8'.split(',')]
    N1 = len(G1) - 1

    def cp_g0(i):
        return cp_kvh(0, i * 2 * TM, 2 * TM, i)

    def cp_g1(n):
        return cp_kvh(1, G1[n] * TM, (G1[n + 1] - G1[n]) * TM, 4 + n)

    def cp_grp(c):
        return cp_kvh(c, 0, S, 2 + N1 + c)

    SB = 2 + N1 + LG

    def cp_q(j0, nb, si):
        return pltpu.make_async_copy(q_hbm.at[0, pl.ds(j0 * TM, nb * TM), :],
                                     qbuf.at[pl.ds(j0 * TM, nb * TM), :], sem.at[si])

    def cp_o(j, c0=0, nc=D):
        return pltpu.make_async_copy(obuf.at[pl.ds(j * TM, TM), pl.ds(c0, nc)],
                                     o_hbm.at[0, pl.ds(j * TM, TM), pl.ds(c0, nc)], sem.at[SB + 4])

    cp_sk = pltpu.make_async_copy(sk_hbm, skb, sem.at[SB])
    cp_dd = pltpu.make_async_copy(dd_hbm, ddb, sem.at[SB])
    cp_q0 = cp_q(0, 3, SB + 1)

    cp_q3 = cp_q(3, 1, SB + 2)
    cp_q4 = cp_q(4, NB - 4, SB + 3)

    cp_w1 = pltpu.make_async_copy(w1_hbm, w1b, sem.at[SB + 1])
    cp_w2 = pltpu.make_async_copy(w2_hbm, w2b, sem.at[SB + 1])
    FA = KR * TF
    cp_w34a = (
        pltpu.make_async_copy(w3_hbm.at[:, pl.ds(0, FA)], w3b.at[:, pl.ds(0, FA)], sem.at[SB + 5]),
        pltpu.make_async_copy(w4_hbm.at[pl.ds(0, FA), :], w4b.at[pl.ds(0, FA), :], sem.at[SB + 5]))
    cp_w34b = (
        pltpu.make_async_copy(w3_hbm.at[:, pl.ds(FA, FF - FA)], w3b.at[:, pl.ds(FA, FF - FA)], sem.at[SB + 2]),
        pltpu.make_async_copy(w4_hbm.at[pl.ds(FA, FF - FA), :], w4b.at[pl.ds(FA, FF - FA), :], sem.at[SB + 2]))

    def wait_all(cps):
        for cp in cps:
            cp.wait()

    cp_sk.start()
    cp_dd.start()
    for grp in ([cp_g0(i) for i in range(4)] + [cp_g1(n) for n in range(N1)]
                + [cp_grp(c) for c in range(2, LG)]):
        for cp in grp:
            cp.start()
    for cp in (cp_q0, cp_w1, cp_w2) + cp_w34a + cp_w34b + (cp_q3, cp_q4):
        cp.start()

    zsm[0] = 0
    kbuf[0:16, :] = jnp.zeros((16, D), bf16)

    def _basis(pos, part, n):
        k = jnp.where(pos < CB // 2, 2 * pos, 2 * pos - (CB - 1))
        m = ((2 * k + 1) * n + part * CB) & (4 * CB - 1)
        r = m & (2 * CB - 1)
        neg = jnp.logical_xor(m >= 2 * CB, r > CB)
        th = jnp.minimum(r, 2 * CB - r).astype(f32) * (math.pi / (2 * CB))
        t2 = th * th
        z = 1.0 / math.factorial(12)
        for e in (10, 8, 6, 4, 2, 0):
            z = 1.0 / math.factorial(e) - t2 * z
        z = jnp.where(neg, -z, z)
        return z, jnp.where(pos < CB // 2, z, -z)

    def dft_init(t, carry):
        rf = lax.broadcasted_iota(i32, (32, CB), 0)
        zs = _basis(t * 16 + (rf & 15), rf >> 4, lax.broadcasted_iota(i32, (32, CB), 1))
        cg = lax.broadcasted_iota(i32, (16, 2 * CB), 1)
        gs = _basis(cg >> 1, cg & 1, t * 16 + lax.broadcasted_iota(i32, (16, 2 * CB), 0))
        for par in range(2):
            Fm[par, pl.ds(pl.multiple_of(t * 16, 16), 16), :] = pltpu.bitcast(zs[par].astype(bf16), u32)
            Gm[par, pl.ds(pl.multiple_of(t * 8, 8), 8), :] = pltpu.bitcast(
                (gs[par] * (1.0 / CB)).astype(bf16), u32)
        return carry

    lax.fori_loop(0, CB // 16, dft_init, 0)

    cp_sk.wait()
    cp_dd.wait()
    sk32 = skb[...].astype(f32)
    for t in range(4):
        skf[t] = jnp.broadcast_to(sk32[t:t + 1, :], (8, D))
    skf[4] = jnp.broadcast_to(ddb[...].astype(f32).reshape(1, D), (8, D))

    def zero_vec():
        return jnp.full((8, 128), zsm[0], i32).astype(u32)

    def bmul(x, row8):
        n = x.shape[0] // 8
        return (x.reshape(n, 8, 128) * row8[None]).reshape(x.shape)

    def dsl(start, size, align):
        return pl.ds(start if isinstance(start, int) else pl.multiple_of(start, align), size)

    def unil(z):
        return (jnp.concatenate([z[32 * g:32 * g + 16] for g in range(CB // 16)], axis=0),
                jnp.concatenate([z[32 * g + 16:32 * g + 32] for g in range(CB // 16)], axis=0))

    def fwdh1(c, par, i, o, pins=None, skip=True):
        Z = (ZA if par == 0 else ZB).at[dsl(H0 + i * 2 * BS, 2 * BS, 8), :]
        ls = dsl(c * 128, 128, 128)
        a = 2 * i + o
        hh = lax.dot_general(_pin_at(pltpu.bitcast(Fm[o], bf16), pins, zero_vec()), hkb[ls, dsl(a * CB, CB, CB)], (((1,), (1,)), ((), ())),
                             preferred_element_type=f32)
        cc, dd = unil(hh)
        if o == 0 and skip and (not isinstance(i, int) or i == 0):
            d8 = skf[4, :, ls] if isinstance(i, int) else jnp.where(i == 0, skf[4, :, ls], 0.0)
            cc = (cc.reshape(CB // 8, 8, 128) + d8[None]).reshape(CB, 128)
        b = o * BS
        Z[b:b + CB, :] = cc
        Z[b + CS:b + CS + CB, :] = dd - cc
        Z[b + 2 * CS:b + 2 * CS + CB, :] = cc + dd
        return cc + dd

    def fwdx1(c, par, i, o, pins, sk, slot=0):
        Z = (ZA if par == 0 else ZB).at[dsl(i * 2 * BS, 2 * BS, 8), :]
        ls = dsl(c * 128, 128, 128)
        ks_ = i % 2 if isinstance(i, int) else slot
        if o == 0:
            kf[ks_] = kbuf[dsl(i * 2 * CB, 2 * CB + 16, 16), ls].astype(f32)
        a = 2 * i + o
        b0 = 16 + o * CB
        ks = bmul(kf[ks_, b0:b0 + CB, :], sk[0])
        for t in range(1, 4):
            ks = ks + bmul(kf[ks_, b0 - t:b0 - t + CB, :], sk[t])
        kv = (ks * vbuf[dsl(a * CB, CB, CB), ls].astype(f32)).astype(bf16)
        xh = _mm(_pin_at(pltpu.bitcast(Fm[o], bf16), pins, zero_vec()), kv)
        xr, xm = unil(xh)
        b = o * BS
        Z[b:b + CB, :] = xr
        Z[b + CS:b + CS + CB, :] = xm
        Z[b + 2 * CS:b + 2 * CS + CB, :] = xr + xm
        return xr + xm

    def mac_gen(par, i0, ns):
        for u in range(ns):
            yield from mac_gen1(par, i0 + u)

    def mac_gen1(par, i):
        Z, Y = (ZA, YA) if par == 0 else (ZB, YB)
        Z = Z.at[dsl(i * 16, 2 * H0 - CB + 16, 16), :]
        X, H = 0, H0
        prev = [None, None]
        for a0 in range(0, NA, NO):
            for h in range(2):
                def ld(ref, a):
                    b = ref + a * BS + h * 8
                    return tuple(Z[b + k * CS:b + k * CS + 8, :] for k in range(3))
                K = [None] * NO
                hw = {}
                for ap in range(a0 + NO):
                    xa, xb, xs = ld(X, ap)
                    for o in range(NO):
                        dl = a0 + o - ap
                        if dl < 0:
                            continue
                        if dl not in hw:
                            hw[dl] = ld(H, dl)
                        hc, he, hf = hw[dl]
                        t = (hc * xs, xa * he, xb * hf)
                        K[o] = t if K[o] is None else tuple(u + w for u, w in zip(K[o], t))
                        inj = yield K[o][2]
                        if inj is not None:
                            K[o] = (K[o][0], K[o][1], K[o][2] + inj)
                for o in range(NO):
                    re, im = K[o][0] - K[o][2], K[o][0] + K[o][1]
                    out = (re, im) if prev[h] is None else (re - prev[h][1], im + prev[h][0])
                    prev[h] = (re, im)
                    Y[a0 + o, dsl(i * 16 + h * 8, 8, 8), :] = pltpu.pack_elementwise(
                        list(out), packed_dtype=bf16).astype(u32)

    def inv1(c, par, i, o, pins=None):
        Y = YA if par == 0 else YB
        a = 2 * i + o
        y = _mm(_pin_at(pltpu.bitcast(Gm[o], bf16), pins, zero_vec()), pltpu.bitcast(Y[a], bf16))
        yv = ybuf.at[dsl(a * (CB // 2), CB // 2, CB // 2), :]
        for g in range(CB // 16):
            yv[8 * g:8 * g + 8, dsl(c * 128, 128, 128)] = pltpu.pack_elementwise(
                [y[16 * g:16 * g + 8], y[16 * g + 8:16 * g + 16]], packed_dtype=bf16).astype(u32)
        return y

    NPM = NA * (NA + 1)

    def group(c, par, do_inv, do_fwd, i0=0, ns=NA // 2):
        PI, P0, DP, NP_, R0, DR, G0 = (int(x) for x in '-20,12,12,16,220,12,4'.split(','))
        names = 'h0,x0,h1,x1'.split(',')
        zero = zero_vec()
        sk = [skf[t, :, dsl((c + 1) * 128, 128, 128)] for t in range(4)] if do_fwd else None
        gen = mac_gen(par, i0, ns)
        rec = [next(gen)]
        inj = {}
        for u in range(ns):
            i = i0 + u
            base = u * NPM
            while len(rec) <= base + P0 + (NP_ - 1) * DP:
                rec.append(gen.send(inj.get(len(rec))))
            pins = {k: {} for k in ('i0', 'i1', 'h0', 'h1', 'x0', 'x1')}
            if base + PI >= 0:
                pins['i0'][(0, 0)] = [rec[base + PI]]
                pins['i1'][(0, 0)] = [rec[base + PI]]
            for n in range(NP_):
                r = ((n + 1) * 16) // NP_ - 1
                pins[names[n % len(names)]][(r, 0)] = [rec[base + P0 + n * DP]]
            XP = int('-999')
            if base + XP >= 0:
                for nm in ('x0', 'x1'):
                    pins[nm].setdefault((0, 0), []).append(rec[base + XP])
            if do_inv:
                ys = [inv1(c - 1, 1 - par, i, 0, pins['i0']), inv1(c - 1, 1 - par, i, 1, pins['i1'])]
                if not do_fwd:
                    inj[base + R0] = pltpu.bitcast(_tok([y[CB - 8:CB] for y in ys]) & zero, f32)
            if do_fwd:
                res = [fwdh1(c + 1, 1 - par, i, 0, pins['h0'], skip=(u == 0)),
                       fwdh1(c + 1, 1 - par, i, 1, pins['h1']),
                       fwdx1(c + 1, 1 - par, i, 0, pins['x0'], sk, slot=u % 2),
                       fwdx1(c + 1, 1 - par, i, 1, pins['x1'], sk, slot=u % 2)]
                for g in range(G0, CB // 16):
                    tk = _tok([z[16 * g + 8:16 * g + 16] for z in res]) & zero
                    inj[base + R0 + (g - G0) * DR] = pltpu.bitcast(tk, f32)
        try:
            while True:
                rec.append(gen.send(inj.get(len(rec))))
        except StopIteration:
            pass

    def conv():
        def pre(i, carry):
            wait_all(cp_g0(i))
            sk = [skf[t, :, 0:128] for t in range(4)]
            for u in range(2):
                for o in range(2):
                    fwdh1(0, 0, 2 * i + u, o, skip=(u == 0))
                for o in range(2):
                    fwdx1(0, 0, 2 * i + u, o, None, sk, slot=u)
            return carry
        lax.fori_loop(0, NA // 4, pre, 0)
        for t in range(N1):
            wait_all(cp_g1(t))
            group(0, 0, False, True, G1[t], G1[t + 1] - G1[t])

        def it(t, carry):
            wait_all(cp_grp(2 * t + 2))
            group(2 * t + 1, 1, True, True)
            wait_all(cp_grp(2 * t + 3))
            group(2 * t + 2, 0, True, True)
            return carry
        lax.fori_loop(0, (LG - 2) // 2, it, 0)
        group(LG - 1, 1, True, False)

    conv()

    def rows(j):
        return j * TM if isinstance(j, int) else pl.multiple_of(j * TM, TM)

    def delay(x, after):
        if after is None:
            return x
        z8 = pltpu.bitcast(_tok([after]) & zero_vec(), f32)
        x0 = (x[:, 0:128].reshape(x.shape[0] // 8, 8, 128) + z8[None]).reshape(x.shape[0], 128)
        return jnp.concatenate([x0, x[:, 128:]], axis=1)

    def s0_rows(j, s0, ns, slot, from_q, after=None):
        r = rows(j)
        sl = slice(s0 * R, (s0 + ns) * R)
        x = qbuf.at[pl.ds(r, TM), :][sl, :].astype(f32)
        if from_q is not True:
            x = jnp.where(from_q, x, xbuf.at[pl.ds(r, TM), :][sl, :])
        x = delay(x, after)
        r2 = j * (TM // 2) if isinstance(j, int) else pl.multiple_of(j * (TM // 2), TM // 2)
        yw = ybuf.at[pl.ds(r2, TM // 2), :][s0 * 8:(s0 + ns) * 8, :]
        yy = [pltpu.unpack_elementwise(yw, index=k, packed_dtype=bf16, unpacked_dtype=f32)
              for k in range(2)]
        y = jnp.concatenate([yy[k][s * 8:(s + 1) * 8] for s in range(ns) for k in range(2)], axis=0)
        q, t1 = _ln_t(x)
        x1 = x + q * y
        u, t2 = _ln_t(x1)
        x1b[slot * R:(slot + ns) * R, :] = x1
        ub[slot * R:(slot + ns) * R, :] = u
        z, t3 = _ln_t(u)
        return z.astype(bf16), t1 + t2 + t3 + [[z[:, D - 128:]]]

    def rhs_pins(steps, ksteps, rot=[0]):
        pins = {}
        for t, lst in enumerate(steps):
            n, kg = t // ksteps, t % ksteps
            for i, vals in enumerate(lst):
                m = rot[0] % 4
                rot[0] += 1
                rg = 7 if (i % 2 == 0 and len(lst) > 1) else 0
                pins.setdefault(((kg * 4 + m) * 8 + rg, n), []).extend(vals)
        return pins

    def at_steps(toks, first, last, nsteps):
        steps = [[] for _ in range(nsteps)]
        for k, t in enumerate(toks):
            steps[first + (k * (last - first)) // max(len(toks) - 1, 1)].append(t)
        return steps

    def pinned(w, steps):
        return w if steps is None else _pin_at(w, rhs_pins(steps, 2), zero_vec())

    def put_h(row0, h):
        for l in range(LG):
            hwin[l, row0:row0 + h.shape[0], :] = h[:, l * 128:(l + 1) * 128]

    def m2_dot(r0, nr, steps=None):
        hs_in = jnp.concatenate(
            [hwin[l, 8 + r0 - SHIFTS[l]:8 + r0 - SHIFTS[l] + nr, :].astype(bf16) for l in range(LG)], axis=1)
        return _mm(hs_in, pinned(w2b[...], steps))

    def ln3(hs, lo, ns, after=None):
        sl = slice(lo * R, (lo + ns) * R)
        x1p = delay(ub[sl, :], after) + hs
        z, _ = _ln_t(x1p)
        z3buf[sl, :] = z.astype(bf16)
        return x1b[sl, :] + x1p, [z[:, D - 128:]]

    def mlp(c0, c1, acc, side=None, z3=None):
        z3 = z3buf[...] if z3 is None else z3
        zero = zero_vec()
        steps = [[] for _ in range(16 * NC)]
        for c in range(c0, c1):
            w3 = _pin_at(w3b[:, c * TF:(c + 1) * TF], rhs_pins(steps[16 * c:16 * c + 8], 2), zero)
            a = _gelu(_mm(z3, w3))
            if side is not None:
                side(c, a, steps)
            a = a.astype(bf16)
            w4 = _pin_at(w4b[c * TF:(c + 1) * TF, :], rhs_pins(steps[16 * c + 8:16 * c + 16], 1), zero)
            acc = acc + _mm(a, w4)
        return acc

    def s0_side(b, grp=None):
        RT, D0, DD, CH = (int(x) for x in '0,2,1,3'.split(','))
        grp = grp or _spread(list(range(NS)), KR)
        if isinstance(b, int):
            blk, fq = (b % NB, (b + 1) % NB), (b < NB, b + 1 < NB)
        else:
            blk, fq = (lax.rem(b, NB), lax.rem(b + 1, NB)), (b < NB, b + 1 < NB)

        def side(c, a, steps):
            if c == 0:
                x1b[0:R, :] = x1b[TM:TM + R, :]
                ub[0:R, :] = ub[TM:TM + R, :]
            after = a[0:8, RT * 128:(RT + 1) * 128]
            for n, s in enumerate(grp[c]):
                last = s == NS - 1
                z, t = s0_rows(blk[last], 0 if last else s + 1, 1, s + 1, fq[last], after)
                z1buf[s * R:(s + 1) * R, :] = z
                after = t[CH][0][0:8] if CH >= 0 else None
                steps[min(16 * c + 8 + D0 + n * DD, 16 * KR - 1)].append(t[-1])
        return side

    def toks(zs):
        return [t for _, ts in zs for t in ts]

    def cat(zs):
        return jnp.concatenate([z for z, _ in zs], axis=0)

    def prologue(_, carry):
        cp_q0.wait()
        cp_w1.wait()
        cp_w2.wait()
        F1, L1_ = (int(x) for x in '2,15'.split(','))
        HM = TM // 2
        for a in range(3):
            inv1(LG - 1, 1, a // 2, a % 2)
        za = [s0_rows(0, 0, 8, 0, True)]
        for a in range(3, NA):
            inv1(LG - 1, 1, a // 2, a % 2)
        zb = [s0_rows(0, 8, 4, 8, True), s0_rows(0, 12, 4, 12, True), s0_rows(1, 0, 1, 16, True)]
        for l in range(LG):
            hwin[l, 0:8, :] = jnp.zeros((8, 128), f32)
        put_h(8, _gelu(_mm(cat(za), pinned(w1b[...], at_steps(toks(zb[:2]) + [zb[2][1][-1]], F1, L1_, 16)))))
        h = _gelu(_mm(cat(zb), w1b[...]))
        put_h(8 + HM, h[0:HM + 8])
        hcar[...] = h[HM + R - 24:HM + R]
        accb[0:HM, :] = m2_dot(0, HM)
        return carry

    def prologue2(_, carry):
        HM = TM // 2
        hs0 = accb[0:HM, :]
        l0 = [ln3(hs0[n * 32:(n + 1) * 32], 2 * n, 2) for n in range(4)]
        hs1 = m2_dot(HM, HM, at_steps([t for _, t in l0], 3, 14, 16))
        if '1' == '0':
            wait_all(cp_w34a)
        l1 = [ln3(hs1[n * 32:(n + 1) * 32], 8 + 2 * n, 2) for n in range(4)]
        if '1' == '1':
            wait_all(cp_w34a)
        accb[...] = mlp(0, KR, jnp.concatenate([r for r, _ in l0 + l1], axis=0), s0_side(1))
        return carry

    prologue(0, 0)

    def mark(i, carry):
        zsm[1 + i] = i
        return carry
    lax.fori_loop(0, 2, mark, 0)
    prologue2(0, 0)
    wait_all(cp_w34b + (cp_q3,))

    def body(g, carry):
        @pl.when(g == 1)
        def _():
            cp_q4.wait()
        b = g + 1
        jb = lax.rem(b, NB)
        T3, RT, D0, DD = (int(x) for x in '2,0,0,1'.split(','))
        T0 = int('1')
        z3 = z3buf[...]
        acc = mlp(KR, KR + T0, accb[...], None, z3)
        top = hcar[...]
        put_h(0, jnp.where(jb == 0, 0.0, top[0:8]))
        put_h(8, top[8:24])
        h = _gelu(_mm(z1buf[...], w1b[...]))
        put_h(24, h[0:TM - R])
        put_h(8 + TM, jnp.where(jb == NB - 1, 0.0, h[TM - R:TM - 8]))
        hcar[...] = h[TM - 24:TM]
        acc = mlp(KR + T0, KR + T3, acc, None, z3)
        hs = m2_dot(0, TM)
        rs = []
        grp = _spread(list(range(NS)), NC - KR - T3)

        def side(c, a, steps):
            for n, s in enumerate(grp[c - KR - T3]):
                r_, t = ln3(hs[s * R:(s + 1) * R], s, 1,
                            a[0:8, RT * 128:(RT + 1) * 128] if (n == 0 and RT >= 0) else None)
                rs.append(r_)
                steps[min(16 * c + 8 + D0 + (n * DD) // 2, 16 * NC - 1)].append(t)
        xn = mlp(KR + T3, NC, acc, side, z3)
        jg = lax.rem(g, NB)
        xbuf[pl.ds(rows(jg), TM), :] = xn
        obuf[pl.ds(rows(jg), TM), :] = xn.astype(bf16)
        accb[...] = mlp(0, KR, jnp.concatenate(rs, axis=0), s0_side(g + 2))

        @pl.when(g >= NB)
        def _():
            cp_o(jg).start()
        return carry

    lax.fori_loop(0, G - 1, body, 0)

    OC = [0] + [int(x) for x in '512,896'.split(',')] + [D]
    OS = tuple((OC[i], OC[i + 1] - OC[i]) for i in range(len(OC) - 1))
    acc = mlp(KR, NC - 1, accb[...])
    a = _gelu(_mm(z3buf[...], w3b[:, FF - TF:])).astype(bf16)
    for c0, nc in OS:
        obuf[S - TM:, c0:c0 + nc] = (acc[:, c0:c0 + nc] + _mm(a, w4b[FF - TF:, c0:c0 + nc])).astype(bf16)
        cp_o(NB - 1, c0, nc).start()
    for j in range(NB - 1):
        cp_o(j).wait()
    for c0, nc in OS:
        cp_o(NB - 1, c0, nc).wait()


@jax.jit
def pallas_interleave_layers__ssm_conv_h3__mixer_s_mlp__prompt_kernel(
    A_q, A_k, A_v, A_shift_k, A_ssm_k, A_ssm_D, B_x, B_w1, B_w2, B_w3, B_w4,
):
    del B_x
    vm = pltpu.VMEM
    scratch = [
        vm((D, D), bf16), vm((D, D), bf16), vm((D, FF), bf16), vm((FF, D), bf16),
        vm((S + 16, D), bf16), vm((S, D), bf16), vm((D, S), bf16), vm((S, D), bf16),
        vm((4, D), bf16), vm((D,), bf16),
        vm((2, CB, CB), u32), vm((2, CB // 2, 2 * CB), u32),
        vm((5, 8, D), f32),
        vm((2, 2 * CB + 16, 128), f32),
        vm((2 * H0, 128), f32), vm((2 * H0, 128), f32),
        vm((NA, CB, 128), u32), vm((NA, CB, 128), u32),
        vm((S // 2, D), u32), vm((S, D), f32), vm((TM + R, D), f32), vm((TM + R, D), f32),
        vm((LG, TM + R, 128), f32), vm((24, D), f32),
        vm((TM, D), bf16), vm((TM, D), bf16), vm((TM, D), f32),
        pltpu.SMEM((4,), i32),
        pltpu.SemaphoreType.DMA((1 + len('0,3,8'.split(',')) + LG + 6,)),
    ]
    return pl.pallas_call(
        _kernel,
        out_shape=jax.ShapeDtypeStruct(A_q.shape, bf16),
        in_specs=[pl.BlockSpec(memory_space=pl.ANY)] * 10,
        out_specs=pl.BlockSpec(memory_space=pl.ANY),
        scratch_shapes=scratch,
        compiler_params=pltpu.CompilerParams(vmem_limit_bytes=100 * 1024 * 1024),
    )(A_q, A_k, A_v, A_shift_k.T, A_ssm_k, A_ssm_D, B_w1, B_w2, B_w3, B_w4)
```

```python
import math

import jax
import jax.numpy as jnp
from jax import lax
import jax.experimental.pallas as pl
import jax.experimental.pallas.tpu as pltpu


f32, bf16, u32, i32 = jnp.float32, jnp.bfloat16, jnp.uint32, jnp.int32

S, D, FF = 2048, 1024, 3584
TM = 256
NB = S // TM
G = 2 * NB
CB = 128
NA = S // CB
NO = 4
TF = 512
NC = FF // TF
R = 16
NS = TM // R
LG = D // 128
KR = int('4')
EPS = 1e-5
CS = CB + 8
BS = 3 * CS
H0 = NA * BS + 16
C0 = math.sqrt(2.0 / math.pi)
C1 = C0 * 0.044715
SHIFTS = (1, 1, -1, -1, 2, 2, -2, -2)


def _ln(x):
    m = jnp.mean(x, axis=-1, keepdims=True)
    xc = x - m
    v = jnp.mean(xc * xc, axis=-1, keepdims=True)
    return xc * lax.rsqrt(v + EPS)


def _ln_t(x):
    m = jnp.mean(x, axis=-1, keepdims=True)
    xc = x - m
    v = jnp.mean(xc * xc, axis=-1, keepdims=True)
    r = lax.rsqrt(v + EPS)
    n = x.shape[0]
    return xc * r, [[jnp.broadcast_to(m, (n, 128))], [jnp.broadcast_to(r, (n, 128))]]


def _gelu(x):
    hx = 0.5 * x
    return hx + hx * jnp.tanh(x * (C0 + C1 * (x * x)))


def _mm(a, b):
    return jnp.dot(a, b, preferred_element_type=f32)


def _tok(vals):
    t = None
    for v in vals:
        b = pltpu.bitcast(v, u32)
        for i in range(b.shape[0] // 8):
            for j in range(b.shape[1] // 128):
                p = b[i * 8:(i + 1) * 8, j * 128:(j + 1) * 128]
                t = p if t is None else t | p
    return t


def _pin(x, vals, zero):
    if not vals:
        return x
    top = pltpu.bitcast(pltpu.bitcast(x[0:16, 0:128], u32) | (_tok(vals) & zero), bf16)
    row0 = jnp.concatenate([top, x[0:16, 128:]], axis=1)
    return jnp.concatenate([row0, x[16:]], axis=0)


def _pin_at(x, pins, zero):
    if not pins:
        return x
    out, last = [], 0
    for k in sorted({k for k, _ in pins}):
        if k * 16 > last:
            out.append(x[last:k * 16])
        blk = x[k * 16:(k + 1) * 16]
        for (kk, n), vals in pins.items():
            if kk != k:
                continue
            top = pltpu.bitcast(pltpu.bitcast(blk[:, n * 128:(n + 1) * 128], u32) | (_tok(vals) & zero), bf16)
            parts = ([blk[:, :n * 128]] if n > 0 else []) + [top] + (
                [blk[:, (n + 1) * 128:]] if (n + 1) * 128 < blk.shape[1] else [])
            blk = jnp.concatenate(parts, axis=1) if len(parts) > 1 else top
        out.append(blk)
        last = (k + 1) * 16
    if last < x.shape[0]:
        out.append(x[last:])
    return jnp.concatenate(out, axis=0) if len(out) > 1 else out[0]


def _spread(items, n):
    return [items[(i * len(items)) // n:((i + 1) * len(items)) // n] for i in range(n)]


def _kernel(q_hbm, k_hbm, v_hbm, sk_hbm, hk_hbm, dd_hbm, w1_hbm, w2_hbm, w3_hbm, w4_hbm,
            o_hbm,
            w1b, w2b, w3b, w4b, kbuf, vbuf, hkb, qbuf, skb, ddb,
            Fm, Gm, skf, kf, ZA, ZB, YA, YB, ybuf, xbuf, x1b, ub, hwin, hcar, z1buf, z3buf, accb,
            zsm, sem):
    obuf = vbuf

    def cp_kvh(c, r0, nr, si):
        ch = pl.ds(c * 128, 128)
        return (
            pltpu.make_async_copy(k_hbm.at[0, pl.ds(r0, nr), ch], kbuf.at[pl.ds(16 + r0, nr), ch], sem.at[si]),
            pltpu.make_async_copy(v_hbm.at[0, pl.ds(r0, nr), ch], vbuf.at[pl.ds(r0, nr), ch], sem.at[si]),
            pltpu.make_async_copy(hk_hbm.at[ch, pl.ds(r0, nr)], hkb.at[ch, pl.ds(r0, nr)], sem.at[si]))

    G1 = [int(x) for x in '0,3,8'.split(',')]
    N1 = len(G1) - 1

    def cp_g0(i):
        return cp_kvh(0, i * 2 * TM, 2 * TM, i)

    def cp_gp(c, n):
        return cp_kvh(c, G1[n] * TM, (G1[n + 1] - G1[n]) * TM, 4 + (c - 1) * N1 + n)

    def cp_grp(c):
        return cp_kvh(c, 0, S, 1 + 2 * N1 + c)

    SB = 1 + 2 * N1 + LG

    def cp_q(r0, r1, si):
        return pltpu.make_async_copy(q_hbm.at[0, pl.ds(r0, r1 - r0), :],
                                     qbuf.at[pl.ds(r0, r1 - r0), :], sem.at[si])

    def cp_o(j, c0=0, nc=D):
        return pltpu.make_async_copy(obuf.at[pl.ds(j * TM, TM), pl.ds(c0, nc)],
                                     o_hbm.at[0, pl.ds(j * TM, TM), pl.ds(c0, nc)], sem.at[SB + 4])

    cp_sk = pltpu.make_async_copy(sk_hbm, skb, sem.at[SB])
    cp_dd = pltpu.make_async_copy(dd_hbm, ddb, sem.at[SB])
    cp_q0 = cp_q(0, 2 * TM + R, SB + 1)

    cp_q3 = cp_q(2 * TM + R, 3 * TM + R, SB + 2)
    cp_q4 = cp_q(3 * TM + R, S, SB + 3)

    cp_w1 = pltpu.make_async_copy(w1_hbm, w1b, sem.at[SB + 1])
    cp_w2 = pltpu.make_async_copy(w2_hbm, w2b, sem.at[SB + 1])
    def cp_w34(c0, c1, si):
        n = (c1 - c0) * TF
        return (pltpu.make_async_copy(w3_hbm.at[:, pl.ds(c0 * TF, n)], w3b.at[:, pl.ds(c0 * TF, n)], sem.at[si]),
                pltpu.make_async_copy(w4_hbm.at[pl.ds(c0 * TF, n), :], w4b.at[pl.ds(c0 * TF, n), :], sem.at[si]))

    WS = int('2')
    cp_w34a = cp_w34(0, WS, SB + 5)
    cp_w34m = cp_w34(WS, KR, SB + 6)
    cp_w34b = cp_w34(KR, NC, SB + 2)

    def wait_all(cps):
        for cp in cps:
            cp.wait()

    cp_sk.start()
    cp_dd.start()
    for grp in ([cp_g0(i) for i in range(4)] + [cp_gp(c, n) for c in (1, 2) for n in range(N1)]
                + [cp_grp(c) for c in range(3, LG)]):
        for cp in grp:
            cp.start()
    for cp in (cp_q0, cp_w1, cp_w2) + cp_w34a + cp_w34m + cp_w34b + (cp_q3, cp_q4):
        cp.start()

    zsm[0] = 0
    kbuf[0:16, :] = jnp.zeros((16, D), bf16)

    def _basis(pos, part, n):
        k = jnp.where(pos < CB // 2, 2 * pos, 2 * pos - (CB - 1))
        m = ((2 * k + 1) * n + part * CB) & (4 * CB - 1)
        r = m & (2 * CB - 1)
        neg = jnp.logical_xor(m >= 2 * CB, r > CB)
        th = jnp.minimum(r, 2 * CB - r).astype(f32) * (math.pi / (2 * CB))
        t2 = th * th
        z = 1.0 / math.factorial(12)
        for e in (10, 8, 6, 4, 2, 0):
            z = 1.0 / math.factorial(e) - t2 * z
        z = jnp.where(neg, -z, z)
        return z, jnp.where(pos < CB // 2, z, -z)

    def dft_init(t, carry):
        rf = lax.broadcasted_iota(i32, (32, CB), 0)
        zs = _basis(t * 16 + (rf & 15), rf >> 4, lax.broadcasted_iota(i32, (32, CB), 1))
        cg = lax.broadcasted_iota(i32, (16, 2 * CB), 1)
        gs = _basis(cg >> 1, cg & 1, t * 16 + lax.broadcasted_iota(i32, (16, 2 * CB), 0))
        for par in range(2):
            Fm[par, pl.ds(pl.multiple_of(t * 16, 16), 16), :] = pltpu.bitcast(zs[par].astype(bf16), u32)
            Gm[par, pl.ds(pl.multiple_of(t * 8, 8), 8), :] = pltpu.bitcast(
                (gs[par] * (1.0 / CB)).astype(bf16), u32)
        return carry

    lax.fori_loop(0, CB // 16, dft_init, 0)

    cp_sk.wait()
    cp_dd.wait()
    sk32 = skb[...].astype(f32)
    for t in range(4):
        skf[t] = jnp.broadcast_to(sk32[t:t + 1, :], (8, D))
    skf[4] = jnp.broadcast_to(ddb[...].astype(f32).reshape(1, D), (8, D))

    def zero_vec():
        return jnp.full((8, 128), zsm[0], i32).astype(u32)

    def bmul(x, row8):
        n = x.shape[0] // 8
        return (x.reshape(n, 8, 128) * row8[None]).reshape(x.shape)

    def dsl(start, size, align):
        return pl.ds(start if isinstance(start, int) else pl.multiple_of(start, align), size)

    def unil(z):
        return (jnp.concatenate([z[32 * g:32 * g + 16] for g in range(CB // 16)], axis=0),
                jnp.concatenate([z[32 * g + 16:32 * g + 32] for g in range(CB // 16)], axis=0))

    def fwdh1(c, par, i, o, pins=None, skip=True):
        Z = (ZA if par == 0 else ZB).at[dsl(H0 + i * 2 * BS, 2 * BS, 8), :]
        ls = dsl(c * 128, 128, 128)
        a = 2 * i + o
        hh = lax.dot_general(_pin_at(pltpu.bitcast(Fm[o], bf16), pins, zero_vec()), hkb[ls, dsl(a * CB, CB, CB)], (((1,), (1,)), ((), ())),
                             preferred_element_type=f32)
        cc, dd = unil(hh)
        if o == 0 and skip and (not isinstance(i, int) or i == 0):
            d8 = skf[4, :, ls] if isinstance(i, int) else jnp.where(i == 0, skf[4, :, ls], 0.0)
            cc = (cc.reshape(CB // 8, 8, 128) + d8[None]).reshape(CB, 128)
        b = o * BS
        Z[b:b + CB, :] = cc
        Z[b + CS:b + CS + CB, :] = dd - cc
        Z[b + 2 * CS:b + 2 * CS + CB, :] = cc + dd
        return cc + dd

    def fwdx1(c, par, i, o, pins, sk, slot=0):
        Z = (ZA if par == 0 else ZB).at[dsl(i * 2 * BS, 2 * BS, 8), :]
        ls = dsl(c * 128, 128, 128)
        ks_ = i % 2 if isinstance(i, int) else slot
        if o == 0:
            kf[ks_] = kbuf[dsl(i * 2 * CB, 2 * CB + 16, 16), ls].astype(f32)
        a = 2 * i + o
        b0 = 16 + o * CB
        ks = bmul(kf[ks_, b0:b0 + CB, :], sk[0])
        for t in range(1, 4):
            ks = ks + bmul(kf[ks_, b0 - t:b0 - t + CB, :], sk[t])
        kv = (ks * vbuf[dsl(a * CB, CB, CB), ls].astype(f32)).astype(bf16)
        xh = _mm(_pin_at(pltpu.bitcast(Fm[o], bf16), pins, zero_vec()), kv)
        xr, xm = unil(xh)
        b = o * BS
        Z[b:b + CB, :] = xr
        Z[b + CS:b + CS + CB, :] = xm
        Z[b + 2 * CS:b + 2 * CS + CB, :] = xr + xm
        return xr + xm

    def mac_part(par, i, h, a0, st, NO=NO):
        Z, Y = (ZA, YA) if par == 0 else (ZB, YB)
        Z = Z.at[dsl(i * 16, 2 * H0 - CB + 16, 16), :]

        def ld(base, a):
            b = base + a * BS + h * 8
            return tuple(Z[b + k * CS:b + k * CS + 8, :] for k in range(3))
        K = [None] * NO
        hw = {}
        for ap in range(a0 + NO):
            xa, xb, xs = ld(0, ap)
            for o in range(NO):
                dl = a0 + o - ap
                if dl < 0:
                    continue
                if dl not in hw:
                    hw[dl] = ld(H0, dl)
                hc, he, hf = hw[dl]
                t = (hc * xs, xa * he, xb * hf)
                K[o] = t if K[o] is None else tuple(u + w for u, w in zip(K[o], t))
                inj = yield K[o][2]
                if inj is not None:
                    K[o] = (K[o][0], K[o][1], K[o][2] + inj)
        st['w'] = []
        for o in range(NO):
            re, im = K[o][0] - K[o][2], K[o][0] + K[o][1]
            prev = st.get('y')
            out = (re, im) if prev is None else (re - prev[1], im + prev[0])
            st['y'] = (re, im)
            st['w'].append(pltpu.pack_elementwise(list(out), packed_dtype=bf16).astype(u32))
            Y[a0 + o, dsl(i * 16 + h * 8, 8, 8), :] = st['w'][-1]

    def mac_gen(par, i0, ns, parts, sts):
        for u in range(ns):
            for a0 in parts:
                for h in range(2):
                    yield from mac_part(par, i0 + u, h, a0, sts.setdefault((u, h), {}))

    def inv1(c, par, i, o, pins=None):
        Y = YA if par == 0 else YB
        a = 2 * i + o
        y = _mm(_pin_at(pltpu.bitcast(Gm[o], bf16), pins, zero_vec()), pltpu.bitcast(Y[a], bf16))
        yv = ybuf.at[dsl(a * (CB // 2), CB // 2, CB // 2), :]
        for g in range(CB // 16):
            yv[8 * g:8 * g + 8, dsl(c * 128, 128, 128)] = pltpu.pack_elementwise(
                [y[16 * g:16 * g + 8], y[16 * g + 8:16 * g + 16]], packed_dtype=bf16).astype(u32)
        return y

    def group(c, par, do_inv, do_fwd, i0=0, ns=NA // 2, parts=(0, 4, 8, 12), cfg=None, ninv=NA // 2):
        PI, P0, DP, NP_, R0, DR, G0 = cfg or tuple(int(x) for x in '-20,12,12,16,220,12,4'.split(','))
        NPM = sum(2 * (NO * a0 + 10) for a0 in parts)
        names = 'h0,x0,h1,x1'.split(',')
        zero = zero_vec()
        sk = [skf[t, :, dsl((c + 1) * 128, 128, 128)] for t in range(4)] if do_fwd else None
        sts = {}
        gen = mac_gen(par, i0, ns, parts, sts)
        rec = [next(gen)]
        inj = {}
        for u in range(ns):
            i = i0 + u
            base = u * NPM
            while len(rec) <= base + P0 + (NP_ - 1) * DP:
                rec.append(gen.send(inj.get(len(rec))))
            pins = {k: {} for k in ('i0', 'i1', 'h0', 'h1', 'x0', 'x1')}
            if base + PI >= 0:
                pins['i0'][(0, 0)] = [rec[base + PI]]
                pins['i1'][(0, 0)] = [rec[base + PI]]
            for n in range(NP_):
                r = ((n + 1) * 16) // NP_ - 1
                pins[names[n % len(names)]][(r, 0)] = [rec[base + P0 + n * DP]]
            XP = int('-999')
            if base + XP >= 0:
                for nm in ('x0', 'x1'):
                    pins[nm].setdefault((0, 0), []).append(rec[base + XP])
            if do_inv and i < ninv:
                ys = [inv1(c - 1, 1 - par, i, 0, pins['i0']), inv1(c - 1, 1 - par, i, 1, pins['i1'])]
                if not do_fwd:
                    inj[base + R0] = pltpu.bitcast(_tok([y[CB - 8:CB] for y in ys]) & zero, f32)
            if do_fwd:
                res = [fwdh1(c + 1, 1 - par, i, 0, pins['h0'], skip=(u == 0)),
                       fwdh1(c + 1, 1 - par, i, 1, pins['h1']),
                       fwdx1(c + 1, 1 - par, i, 0, pins['x0'], sk, slot=u % 2),
                       fwdx1(c + 1, 1 - par, i, 1, pins['x1'], sk, slot=u % 2)]
                for g in range(G0, CB // 16):
                    tk = _tok([z[16 * g + 8:16 * g + 16] for z in res]) & zero
                    inj[base + R0 + (g - G0) * DR] = pltpu.bitcast(tk, f32)
        try:
            while True:
                rec.append(gen.send(inj.get(len(rec))))
        except StopIteration:
            pass
        return sts

    late = {}
    NI7 = int('2')

    def conv():
        def pre(i, carry):
            wait_all(cp_g0(i))
            sk = [skf[t, :, 0:128] for t in range(4)]
            for u in range(2):
                for o in range(2):
                    fwdh1(0, 0, 2 * i + u, o, skip=(u == 0))
                for o in range(2):
                    fwdx1(0, 0, 2 * i + u, o, None, sk, slot=u)
            return carry
        lax.fori_loop(0, NA // 4, pre, 0)
        for c in range(2):
            for t in range(N1):
                wait_all(cp_gp(c + 1, t))
                group(c, c, c > 0, True, G1[t], G1[t + 1] - G1[t])

        def it(t, carry):
            wait_all(cp_grp(2 * t + 3))
            group(2 * t + 2, 0, True, True)
            wait_all(cp_grp(2 * t + 4))
            group(2 * t + 3, 1, True, True)
            return carry
        lax.fori_loop(0, 2, it, 0)
        wait_all(cp_grp(LG - 1))
        late[0] = group(LG - 2, 0, True, True, parts=(0, 4),
                        cfg=tuple(int(x) for x in '-30,-10,5,16,68,1,7'.split(',')))
        late[1] = group(LG - 1, 1, True, False, parts=(0, 4), ninv=NI7,
                        cfg=tuple(int(x) for x in '-10,0,0,1,40,0,0'.split(',')))

    conv()

    def rows(j):
        return j * TM if isinstance(j, int) else pl.multiple_of(j * TM, TM)

    def delay(x, after):
        if after is None:
            return x
        z8 = pltpu.bitcast(_tok([after]) & zero_vec(), f32)
        x0 = (x[:, 0:128].reshape(x.shape[0] // 8, 8, 128) + z8[None]).reshape(x.shape[0], 128)
        return jnp.concatenate([x0, x[:, 128:]], axis=1)

    def s0_rows(j, s0, ns, slot, from_q, after=None):
        r = rows(j)
        sl = slice(s0 * R, (s0 + ns) * R)
        x = qbuf.at[pl.ds(r, TM), :][sl, :].astype(f32)
        if from_q is not True:
            x = jnp.where(from_q, x, xbuf.at[pl.ds(r, TM), :][sl, :])
        x = delay(x, after)
        r2 = j * (TM // 2) if isinstance(j, int) else pl.multiple_of(j * (TM // 2), TM // 2)
        yw = ybuf.at[pl.ds(r2, TM // 2), :][s0 * 8:(s0 + ns) * 8, :]
        yy = [pltpu.unpack_elementwise(yw, index=k, packed_dtype=bf16, unpacked_dtype=f32)
              for k in range(2)]
        y = jnp.concatenate([yy[k][s * 8:(s + 1) * 8] for s in range(ns) for k in range(2)], axis=0)
        q, t1 = _ln_t(x)
        x1 = x + q * y
        u, t2 = _ln_t(x1)
        x1b[slot * R:(slot + ns) * R, :] = x1
        ub[slot * R:(slot + ns) * R, :] = u
        z, t3 = _ln_t(u)
        return z.astype(bf16), t1 + t2 + t3 + [[z[:, D - 128:]]]

    def rhs_pins(steps, ksteps, rot=[0]):
        pins = {}
        for t, lst in enumerate(steps):
            n, kg = t // ksteps, t % ksteps
            for i, vals in enumerate(lst):
                m = rot[0] % 4
                rot[0] += 1
                rg = 7 if (i % 2 == 0 and len(lst) > 1) else 0
                pins.setdefault(((kg * 4 + m) * 8 + rg, n), []).extend(vals)
        return pins

    def at_steps(toks, first, last, nsteps):
        steps = [[] for _ in range(nsteps)]
        for k, t in enumerate(toks):
            steps[first + (k * (last - first)) // max(len(toks) - 1, 1)].append(t)
        return steps

    def pinned(w, steps):
        return w if steps is None else _pin_at(w, rhs_pins(steps, 2), zero_vec())

    def put_h(row0, h):
        for l in range(LG):
            hwin[l, row0:row0 + h.shape[0], :] = h[:, l * 128:(l + 1) * 128]

    def m2_dot(r0, nr, steps=None):
        hs_in = jnp.concatenate(
            [hwin[l, 8 + r0 - SHIFTS[l]:8 + r0 - SHIFTS[l] + nr, :].astype(bf16) for l in range(LG)], axis=1)
        return _mm(hs_in, pinned(w2b[...], steps))

    def ln3(hs, lo, ns, after=None):
        sl = slice(lo * R, (lo + ns) * R)
        x1p = delay(ub[sl, :], after) + hs
        z, _ = _ln_t(x1p)
        z3buf[sl, :] = z.astype(bf16)
        return x1b[sl, :] + x1p, [z[:, D - 128:]]

    def mlp(c0, c1, acc, side=None, z3=None, pre=None):
        z3 = z3buf[...] if z3 is None else z3
        zero = zero_vec()
        steps = [[] for _ in range(16 * NC)]
        for c in range(c0, c1):
            if pre is not None:
                pre(c, steps)
            w3 = _pin_at(w3b[:, c * TF:(c + 1) * TF], rhs_pins(steps[16 * c:16 * c + 8], 2), zero)
            a = _gelu(_mm(z3, w3))
            if side is not None:
                side(c, a, steps)
            a = a.astype(bf16)
            w4 = _pin_at(w4b[c * TF:(c + 1) * TF, :], rhs_pins(steps[16 * c + 8:16 * c + 16], 1), zero)
            acc = acc + _mm(a, w4)
        return acc

    def s0_side(b, grp=None):
        RT, D0, DD, CH = (int(x) for x in '0,2,1,3'.split(','))
        grp = grp or _spread(list(range(NS)), KR)
        if isinstance(b, int):
            blk, fq = (b % NB, (b + 1) % NB), (b < NB, b + 1 < NB)
        else:
            blk, fq = (lax.rem(b, NB), lax.rem(b + 1, NB)), (b < NB, b + 1 < NB)

        def side(c, a, steps):
            if c == 0:
                x1b[0:R, :] = x1b[TM:TM + R, :]
                ub[0:R, :] = ub[TM:TM + R, :]
            after = a[0:8, RT * 128:(RT + 1) * 128]
            for n, s in enumerate(grp[c]):
                last = s == NS - 1
                z, t = s0_rows(blk[last], 0 if last else s + 1, 1, s + 1, fq[last], after)
                z1buf[s * R:(s + 1) * R, :] = z
                after = t[CH][0][0:8] if CH >= 0 else None
                steps[min(16 * c + 8 + D0 + n * DD, 16 * KR - 1)].append(t[-1])
        return side

    def toks(zs):
        return [t for _, ts in zs for t in ts]

    def cat(zs):
        return jnp.concatenate([z for z, _ in zs], axis=0)

    LNO = int('2')
    pend = [(par, u, h, a0) for u in range(NA // 2) for h in range(2)
            for a0 in range(8, NA, LNO) for par in range(2)]

    def late_piece():
        par, u, h, a0 = pend.pop(0)
        for _ in mac_part(par, u, h, a0, late[par][(u, h)], LNO):
            pass
        return list(late[par][(u, h)]['w'])

    NPA, NPB, NPC = (int(x) for x in '8,8,0'.split(','))

    def prologue(_, carry):
        cp_q0.wait()
        cp_w1.wait()
        cp_w2.wait()
        F1, L1_ = (int(x) for x in '2,15'.split(','))
        HM = TM // 2
        for a in range(3):
            inv1(LG - 1, 1, a // 2, a % 2)
        za = [s0_rows(0, 0, 8, 0, True)]
        for a in range(2 * NI7, NA // 2):
            inv1(LG - 2, 0, a // 2, a % 2)
        for a in range(3, NA // 2):
            inv1(LG - 1, 1, a // 2, a % 2)
        zb = [s0_rows(0, 8, 4, 8, True), s0_rows(0, 12, 4, 12, True), s0_rows(1, 0, 1, 16, True)]
        for l in range(LG):
            hwin[l, 0:8, :] = jnp.zeros((8, 128), f32)
        put_h(8, _gelu(_mm(cat(za), pinned(w1b[...], at_steps(toks(zb[:2]) + [zb[2][1][-1]], F1, L1_, 16)))))
        h = _gelu(_mm(cat(zb), pinned(w1b[...], at_steps([late_piece() for _ in range(NPA)], 1, 15, 16))))
        put_h(8 + HM, h[0:HM + 8])
        hcar[...] = h[HM + R - 24:HM + R]
        accb[0:HM, :] = m2_dot(0, HM, at_steps([late_piece() for _ in range(NPB)], 2, 15, 16))
        return carry

    def prologue2(_, carry):
        HM = TM // 2
        hs0 = accb[0:HM, :]
        l0 = [ln3(hs0[n * 32:(n + 1) * 32], 2 * n, 2) for n in range(4)]
        st1 = at_steps([t for _, t in l0], 3, 14, 16)
        st2 = at_steps([late_piece() for _ in range(NPC)], 5, 15, 16)
        hs1 = m2_dot(HM, HM, [x + y for x, y in zip(st1, st2)])
        if '1' == '0':
            wait_all(cp_w34a)
        l1 = [ln3(hs1[n * 32:(n + 1) * 32], 8 + 2 * n, 2) for n in range(4)]
        if '1' == '1':
            wait_all(cp_w34a)
        s0s = s0_side(1)
        LA, LZ, LRT = (int(x) for x in '1,63,-1'.split(','))
        W3, W4 = (int(x) for x in '1,1'.split(','))
        slots = [t for t in range(LA, LZ + 1) if t != 16 * WS for _ in range(W3 if t % 16 < 8 else W4)]
        due = [slots[(k * len(slots)) // len(pend)] for k in range(len(pend))]

        def run_late(lo, hi, steps):
            while pend and lo <= due[0] < hi:
                steps[due.pop(0)].append(late_piece())

        def side(c, a, steps):
            s0s(c, a, steps)
            run_late(16 * c + 8, 16 * c + 16, steps)

        def pre(c, steps):
            if c == WS:
                wait_all(cp_w34m)
            run_late(16 * c, 16 * c + 8, steps)
        accb[...] = mlp(0, KR, jnp.concatenate([r for r, _ in l0 + l1], axis=0), side,
                        pre=pre)
        for par in late:
            for a in range(NA // 2, NA):
                inv1(LG - 2 + par, par, a // 2, a % 2)
        return carry

    prologue(0, 0)

    def mark(i, carry):
        zsm[1 + i] = i
        return carry
    lax.fori_loop(0, 2, mark, 0)
    prologue2(0, 0)
    wait_all(cp_w34b + (cp_q3,))

    def body(g, carry):
        @pl.when(g == 1)
        def _():
            cp_q4.wait()
        b = g + 1
        jb = lax.rem(b, NB)
        T3, RT, D0, DD = (int(x) for x in '2,0,0,1'.split(','))
        T0 = int('1')
        z3 = z3buf[...]
        acc = mlp(KR, KR + T0, accb[...], None, z3)
        top = hcar[...]
        put_h(0, jnp.where(jb == 0, 0.0, top[0:8]))
        put_h(8, top[8:24])
        h = _gelu(_mm(z1buf[...], w1b[...]))
        put_h(24, h[0:TM - R])
        put_h(8 + TM, jnp.where(jb == NB - 1, 0.0, h[TM - R:TM - 8]))
        hcar[...] = h[TM - 24:TM]
        acc = mlp(KR + T0, KR + T3, acc, None, z3)
        hs = m2_dot(0, TM)
        rs = []
        grp = _spread(list(range(NS)), NC - KR - T3)

        def side(c, a, steps):
            for n, s in enumerate(grp[c - KR - T3]):
                r_, t = ln3(hs[s * R:(s + 1) * R], s, 1,
                            a[0:8, RT * 128:(RT + 1) * 128] if (n == 0 and RT >= 0) else None)
                rs.append(r_)
                steps[min(16 * c + 8 + D0 + (n * DD) // 2, 16 * NC - 1)].append(t)
        xn = mlp(KR + T3, NC, acc, side, z3)
        jg = lax.rem(g, NB)
        xbuf[pl.ds(rows(jg), TM), :] = xn
        obuf[pl.ds(rows(jg), TM), :] = xn.astype(bf16)
        accb[...] = mlp(0, KR, jnp.concatenate(rs, axis=0), s0_side(g + 2))

        @pl.when(g >= NB)
        def _():
            cp_o(jg).start()
        return carry

    lax.fori_loop(0, G - 1, body, 0)

    OC = [0] + [int(x) for x in '512,896'.split(',')] + [D]
    OS = tuple((OC[i], OC[i + 1] - OC[i]) for i in range(len(OC) - 1))
    acc = mlp(KR, NC - 1, accb[...])
    a = _gelu(_mm(z3buf[...], w3b[:, FF - TF:])).astype(bf16)
    for c0, nc in OS:
        obuf[S - TM:, c0:c0 + nc] = (acc[:, c0:c0 + nc] + _mm(a, w4b[FF - TF:, c0:c0 + nc])).astype(bf16)
        cp_o(NB - 1, c0, nc).start()
    for j in range(NB - 1):
        cp_o(j).wait()
    for c0, nc in OS:
        cp_o(NB - 1, c0, nc).wait()


@jax.jit
def pallas_interleave_layers__ssm_conv_h3__mixer_s_mlp__prompt_kernel(
    A_q, A_k, A_v, A_shift_k, A_ssm_k, A_ssm_D, B_x, B_w1, B_w2, B_w3, B_w4,
):
    del B_x
    vm = pltpu.VMEM
    scratch = [
        vm((D, D), bf16), vm((D, D), bf16), vm((D, FF), bf16), vm((FF, D), bf16),
        vm((S + 16, D), bf16), vm((S, D), bf16), vm((D, S), bf16), vm((S, D), bf16),
        vm((4, D), bf16), vm((D,), bf16),
        vm((2, CB, CB), u32), vm((2, CB // 2, 2 * CB), u32),
        vm((5, 8, D), f32),
        vm((2, 2 * CB + 16, 128), f32),
        vm((2 * H0, 128), f32), vm((2 * H0, 128), f32),
        vm((NA, CB, 128), u32), vm((NA, CB, 128), u32),
        vm((S // 2, D), u32), vm((S, D), f32), vm((TM + R, D), f32), vm((TM + R, D), f32),
        vm((LG, TM + R, 128), f32), vm((24, D), f32),
        vm((TM, D), bf16), vm((TM, D), bf16), vm((TM, D), f32),
        pltpu.SMEM((4,), i32),
        pltpu.SemaphoreType.DMA((2 * len('0,3,8'.split(',')) - 1 + LG + 7,)),
    ]
    return pl.pallas_call(
        _kernel,
        out_shape=jax.ShapeDtypeStruct(A_q.shape, bf16),
        in_specs=[pl.BlockSpec(memory_space=pl.ANY)] * 10,
        out_specs=pl.BlockSpec(memory_space=pl.ANY),
        scratch_shapes=scratch,
        compiler_params=pltpu.CompilerParams(vmem_limit_bytes=100 * 1024 * 1024),
    )(A_q, A_k, A_v, A_shift_k.T, A_ssm_k, A_ssm_D, B_w1, B_w2, B_w3, B_w4)
```

```python
import math

import jax
import jax.numpy as jnp
from jax import lax
import jax.experimental.pallas as pl
import jax.experimental.pallas.tpu as pltpu


f32, bf16, u32, i32 = jnp.float32, jnp.bfloat16, jnp.uint32, jnp.int32

S, D, FF = 2048, 1024, 3584
TM = 256
NB = S // TM
G = 2 * NB
CB = 128
NA = S // CB
NO = 4
TF = 512
NC = FF // TF
R = 16
NS = TM // R
LG = D // 128
KR = int('4')
EPS = 1e-5
CS = CB + 8
BS = 3 * CS
H0 = NA * BS + 16
C0 = math.sqrt(2.0 / math.pi)
C1 = C0 * 0.044715
SHIFTS = (1, 1, -1, -1, 2, 2, -2, -2)


def _ln(x):
    m = jnp.mean(x, axis=-1, keepdims=True)
    xc = x - m
    v = jnp.mean(xc * xc, axis=-1, keepdims=True)
    return xc * lax.rsqrt(v + EPS)


def _ln_t(x):
    m = jnp.mean(x, axis=-1, keepdims=True)
    xc = x - m
    v = jnp.mean(xc * xc, axis=-1, keepdims=True)
    r = lax.rsqrt(v + EPS)
    n = x.shape[0]
    return xc * r, [[jnp.broadcast_to(m, (n, 128))], [jnp.broadcast_to(r, (n, 128))]]


def _gelu(x):
    hx = 0.5 * x
    return hx + hx * jnp.tanh(x * (C0 + C1 * (x * x)))


def _mm(a, b):
    return jnp.dot(a, b, preferred_element_type=f32)


def _tok(vals):
    t = None
    for v in vals:
        b = pltpu.bitcast(v, u32)
        for i in range(b.shape[0] // 8):
            for j in range(b.shape[1] // 128):
                p = b[i * 8:(i + 1) * 8, j * 128:(j + 1) * 128]
                t = p if t is None else t | p
    return t


def _pin(x, vals, zero):
    if not vals:
        return x
    top = pltpu.bitcast(pltpu.bitcast(x[0:16, 0:128], u32) | (_tok(vals) & zero), bf16)
    row0 = jnp.concatenate([top, x[0:16, 128:]], axis=1)
    return jnp.concatenate([row0, x[16:]], axis=0)


def _pin_at(x, pins, zero):
    if not pins:
        return x
    out, last = [], 0
    for k in sorted({k for k, _ in pins}):
        if k * 16 > last:
            out.append(x[last:k * 16])
        blk = x[k * 16:(k + 1) * 16]
        for (kk, n), vals in pins.items():
            if kk != k:
                continue
            top = pltpu.bitcast(pltpu.bitcast(blk[:, n * 128:(n + 1) * 128], u32) | (_tok(vals) & zero), bf16)
            parts = ([blk[:, :n * 128]] if n > 0 else []) + [top] + (
                [blk[:, (n + 1) * 128:]] if (n + 1) * 128 < blk.shape[1] else [])
            blk = jnp.concatenate(parts, axis=1) if len(parts) > 1 else top
        out.append(blk)
        last = (k + 1) * 16
    if last < x.shape[0]:
        out.append(x[last:])
    return jnp.concatenate(out, axis=0) if len(out) > 1 else out[0]


def _spread(items, n):
    return [items[(i * len(items)) // n:((i + 1) * len(items)) // n] for i in range(n)]


def _kernel(q_hbm, k_hbm, v_hbm, sk_hbm, hk_hbm, dd_hbm, w1_hbm, w2_hbm, w3_hbm, w4_hbm,
            o_hbm,
            w1b, w2b, w3b, w4b, kbuf, vbuf, hkb, qbuf, skb, ddb,
            Fm, Gm, skf, kf, ZA, ZB, YA, YB, ybuf, xbuf, x1b, ub, hwin, hcar, z1buf, z3buf, accb,
            zsm, sem):
    obuf = vbuf

    def cp_kvh(c, r0, nr, si):
        ch = pl.ds(c * 128, 128)
        return (
            pltpu.make_async_copy(k_hbm.at[0, pl.ds(r0, nr), ch], kbuf.at[pl.ds(16 + r0, nr), ch], sem.at[si]),
            pltpu.make_async_copy(v_hbm.at[0, pl.ds(r0, nr), ch], vbuf.at[pl.ds(r0, nr), ch], sem.at[si]),
            pltpu.make_async_copy(hk_hbm.at[ch, pl.ds(r0, nr)], hkb.at[ch, pl.ds(r0, nr)], sem.at[si]))

    G1 = [int(x) for x in '0,3,8'.split(',')]
    N1 = len(G1) - 1

    def cp_g0(i):
        return cp_kvh(0, i * 2 * TM, 2 * TM, i)

    def cp_gp(c, n):
        return cp_kvh(c, G1[n] * TM, (G1[n + 1] - G1[n]) * TM, 4 + (c - 1) * N1 + n)

    def cp_grp(c):
        return cp_kvh(c, 0, S, 1 + 2 * N1 + c)

    SB = 1 + 2 * N1 + LG

    def cp_q(r0, r1, si):
        return pltpu.make_async_copy(q_hbm.at[0, pl.ds(r0, r1 - r0), :],
                                     qbuf.at[pl.ds(r0, r1 - r0), :], sem.at[si])

    def cp_o(j, c0=0, nc=D):
        return pltpu.make_async_copy(obuf.at[pl.ds(j * TM, TM), pl.ds(c0, nc)],
                                     o_hbm.at[0, pl.ds(j * TM, TM), pl.ds(c0, nc)], sem.at[SB + 4])

    cp_sk = pltpu.make_async_copy(sk_hbm, skb, sem.at[SB])
    cp_dd = pltpu.make_async_copy(dd_hbm, ddb, sem.at[SB])
    cp_q0 = cp_q(0, 2 * TM + R, SB + 1)

    cp_q3 = cp_q(2 * TM + R, 3 * TM + R, SB + 2)
    cp_q4 = cp_q(3 * TM + R, S, SB + 3)

    cp_w1 = pltpu.make_async_copy(w1_hbm, w1b, sem.at[SB + 1])
    cp_w2 = pltpu.make_async_copy(w2_hbm, w2b, sem.at[SB + 1])
    def cp_w34(c0, c1, si):
        n = (c1 - c0) * TF
        return (pltpu.make_async_copy(w3_hbm.at[:, pl.ds(c0 * TF, n)], w3b.at[:, pl.ds(c0 * TF, n)], sem.at[si]),
                pltpu.make_async_copy(w4_hbm.at[pl.ds(c0 * TF, n), :], w4b.at[pl.ds(c0 * TF, n), :], sem.at[si]))

    WS = int('2')
    cp_w34a = cp_w34(0, WS, SB + 5)
    cp_w34m = cp_w34(WS, KR, SB + 6)
    cp_w34b = cp_w34(KR, NC, SB + 2)

    def wait_all(cps):
        for cp in cps:
            cp.wait()

    cp_sk.start()
    cp_dd.start()
    for grp in ([cp_g0(i) for i in range(4)] + [cp_gp(c, n) for c in (1, 2) for n in range(N1)]
                + [cp_grp(c) for c in range(3, LG)]):
        for cp in grp:
            cp.start()
    for cp in (cp_q0, cp_w1, cp_w2) + cp_w34a + cp_w34m + cp_w34b + (cp_q3, cp_q4):
        cp.start()

    zsm[0] = 0
    kbuf[0:16, :] = jnp.zeros((16, D), bf16)

    def _basis(pos, part, n):
        k = jnp.where(pos < CB // 2, 2 * pos, 2 * pos - (CB - 1))
        m = ((2 * k + 1) * n + part * CB) & (4 * CB - 1)
        r = m & (2 * CB - 1)
        neg = jnp.logical_xor(m >= 2 * CB, r > CB)
        th = jnp.minimum(r, 2 * CB - r).astype(f32) * (math.pi / (2 * CB))
        t2 = th * th
        z = 1.0 / math.factorial(12)
        for e in (10, 8, 6, 4, 2, 0):
            z = 1.0 / math.factorial(e) - t2 * z
        z = jnp.where(neg, -z, z)
        return z, jnp.where(pos < CB // 2, z, -z)

    def dft_init(t, carry):
        rf = lax.broadcasted_iota(i32, (32, CB), 0)
        zs = _basis(t * 16 + (rf & 15), rf >> 4, lax.broadcasted_iota(i32, (32, CB), 1))
        cg = lax.broadcasted_iota(i32, (16, 2 * CB), 1)
        gs = _basis(cg >> 1, cg & 1, t * 16 + lax.broadcasted_iota(i32, (16, 2 * CB), 0))
        for par in range(2):
            Fm[par, pl.ds(pl.multiple_of(t * 16, 16), 16), :] = pltpu.bitcast(zs[par].astype(bf16), u32)
            Gm[par, pl.ds(pl.multiple_of(t * 8, 8), 8), :] = pltpu.bitcast(
                (gs[par] * (1.0 / CB)).astype(bf16), u32)
        return carry

    lax.fori_loop(0, CB // 16, dft_init, 0)

    cp_sk.wait()
    cp_dd.wait()
    sk32 = skb[...].astype(f32)
    for t in range(4):
        skf[t] = jnp.broadcast_to(sk32[t:t + 1, :], (8, D))
    skf[4] = jnp.broadcast_to(ddb[...].astype(f32).reshape(1, D), (8, D))

    def zero_vec():
        return jnp.full((8, 128), zsm[0], i32).astype(u32)

    def bmul(x, row8):
        n = x.shape[0] // 8
        return (x.reshape(n, 8, 128) * row8[None]).reshape(x.shape)

    def dsl(start, size, align):
        return pl.ds(start if isinstance(start, int) else pl.multiple_of(start, align), size)

    def unil(z):
        return (jnp.concatenate([z[32 * g:32 * g + 16] for g in range(CB // 16)], axis=0),
                jnp.concatenate([z[32 * g + 16:32 * g + 32] for g in range(CB // 16)], axis=0))

    def fwdh1(c, par, i, o, pins=None, skip=True):
        Z = (ZA if par == 0 else ZB).at[dsl(H0 + i * 2 * BS, 2 * BS, 8), :]
        ls = dsl(c * 128, 128, 128)
        a = 2 * i + o
        hh = lax.dot_general(_pin_at(pltpu.bitcast(Fm[o], bf16), pins, zero_vec()), hkb[ls, dsl(a * CB, CB, CB)], (((1,), (1,)), ((), ())),
                             preferred_element_type=f32)
        cc, dd = unil(hh)
        if o == 0 and skip and (not isinstance(i, int) or i == 0):
            d8 = skf[4, :, ls] if isinstance(i, int) else jnp.where(i == 0, skf[4, :, ls], 0.0)
            cc = (cc.reshape(CB // 8, 8, 128) + d8[None]).reshape(CB, 128)
        b = o * BS
        Z[b:b + CB, :] = cc
        Z[b + CS:b + CS + CB, :] = dd - cc
        Z[b + 2 * CS:b + 2 * CS + CB, :] = cc + dd
        return cc + dd

    def fwdx1(c, par, i, o, pins, sk, slot=0):
        Z = (ZA if par == 0 else ZB).at[dsl(i * 2 * BS, 2 * BS, 8), :]
        ls = dsl(c * 128, 128, 128)
        ks_ = i % 2 if isinstance(i, int) else slot
        if o == 0:
            kf[ks_] = kbuf[dsl(i * 2 * CB, 2 * CB + 16, 16), ls].astype(f32)
        a = 2 * i + o
        b0 = 16 + o * CB
        ks = bmul(kf[ks_, b0:b0 + CB, :], sk[0])
        for t in range(1, 4):
            ks = ks + bmul(kf[ks_, b0 - t:b0 - t + CB, :], sk[t])
        kv = (ks * vbuf[dsl(a * CB, CB, CB), ls].astype(f32)).astype(bf16)
        xh = _mm(_pin_at(pltpu.bitcast(Fm[o], bf16), pins, zero_vec()), kv)
        xr, xm = unil(xh)
        b = o * BS
        Z[b:b + CB, :] = xr
        Z[b + CS:b + CS + CB, :] = xm
        Z[b + 2 * CS:b + 2 * CS + CB, :] = xr + xm
        return xr + xm

    def mac_part(par, i, h, a0, st, NO=NO):
        Z, Y = (ZA, YA) if par == 0 else (ZB, YB)
        Z = Z.at[dsl(i * 16, 2 * H0 - CB + 16, 16), :]

        def ld(base, a):
            b = base + a * BS + h * 8
            return tuple(Z[b + k * CS:b + k * CS + 8, :] for k in range(3))
        K = [None] * NO
        hw = {}
        for ap in range(a0 + NO):
            xa, xb, xs = ld(0, ap)
            for o in range(NO):
                dl = a0 + o - ap
                if dl < 0:
                    continue
                if dl not in hw:
                    hw[dl] = ld(H0, dl)
                hc, he, hf = hw[dl]
                t = (hc * xs, xa * he, xb * hf)
                K[o] = t if K[o] is None else tuple(u + w for u, w in zip(K[o], t))
                inj = yield K[o][2]
                if inj is not None:
                    K[o] = (K[o][0], K[o][1], K[o][2] + inj)
        st['w'] = []
        for o in range(NO):
            re, im = K[o][0] - K[o][2], K[o][0] + K[o][1]
            prev = st.get('y')
            out = (re, im) if prev is None else (re - prev[1], im + prev[0])
            st['y'] = (re, im)
            st['w'].append(pltpu.pack_elementwise(list(out), packed_dtype=bf16).astype(u32))
            Y[a0 + o, dsl(i * 16 + h * 8, 8, 8), :] = st['w'][-1]

    def mac_gen(par, i0, ns, parts, sts):
        for u in range(ns):
            for a0 in parts:
                for h in range(2):
                    yield from mac_part(par, i0 + u, h, a0, sts.setdefault((u, h), {}))

    def inv1(c, par, i, o, pins=None):
        Y = YA if par == 0 else YB
        a = 2 * i + o
        y = _mm(_pin_at(pltpu.bitcast(Gm[o], bf16), pins, zero_vec()), pltpu.bitcast(Y[a], bf16))
        yv = ybuf.at[dsl(a * (CB // 2), CB // 2, CB // 2), :]
        for g in range(CB // 16):
            yv[8 * g:8 * g + 8, dsl(c * 128, 128, 128)] = pltpu.pack_elementwise(
                [y[16 * g:16 * g + 8], y[16 * g + 8:16 * g + 16]], packed_dtype=bf16).astype(u32)
        return y

    def group(c, par, do_inv, do_fwd, i0=0, ns=NA // 2, parts=(0, 4, 8, 12), cfg=None, ninv=NA // 2):
        PI, P0, DP, NP_, R0, DR, G0 = cfg or tuple(int(x) for x in '-20,12,12,16,220,12,4'.split(','))
        NPM = sum(2 * (NO * a0 + 10) for a0 in parts)
        names = 'h0,x0,h1,x1'.split(',')
        zero = zero_vec()
        sk = [skf[t, :, dsl((c + 1) * 128, 128, 128)] for t in range(4)] if do_fwd else None
        sts = {}
        gen = mac_gen(par, i0, ns, parts, sts)
        rec = [next(gen)]
        inj = {}
        for u in range(ns):
            i = i0 + u
            base = u * NPM
            while len(rec) <= base + P0 + (NP_ - 1) * DP:
                rec.append(gen.send(inj.get(len(rec))))
            pins = {k: {} for k in ('i0', 'i1', 'h0', 'h1', 'x0', 'x1')}
            if base + PI >= 0:
                pins['i0'][(0, 0)] = [rec[base + PI]]
                pins['i1'][(0, 0)] = [rec[base + PI]]
            for n in range(NP_):
                r = ((n + 1) * 16) // NP_ - 1
                pins[names[n % len(names)]][(r, 0)] = [rec[base + P0 + n * DP]]
            XP = int('-999')
            if base + XP >= 0:
                for nm in ('x0', 'x1'):
                    pins[nm].setdefault((0, 0), []).append(rec[base + XP])
            if do_inv and i < ninv:
                ys = [inv1(c - 1, 1 - par, i, 0, pins['i0']), inv1(c - 1, 1 - par, i, 1, pins['i1'])]
                if not do_fwd:
                    inj[base + R0] = pltpu.bitcast(_tok([y[CB - 8:CB] for y in ys]) & zero, f32)
            if do_fwd:
                res = [fwdh1(c + 1, 1 - par, i, 0, pins['h0'], skip=(u == 0)),
                       fwdh1(c + 1, 1 - par, i, 1, pins['h1']),
                       fwdx1(c + 1, 1 - par, i, 0, pins['x0'], sk, slot=u % 2),
                       fwdx1(c + 1, 1 - par, i, 1, pins['x1'], sk, slot=u % 2)]
                for g in range(G0, CB // 16):
                    tk = _tok([z[16 * g + 8:16 * g + 16] for z in res]) & zero
                    inj[base + R0 + (g - G0) * DR] = pltpu.bitcast(tk, f32)
        try:
            while True:
                rec.append(gen.send(inj.get(len(rec))))
        except StopIteration:
            pass
        return sts

    late = {}
    NI7 = int('2')

    def conv():
        def pre(i, carry):
            wait_all(cp_g0(i))
            sk = [skf[t, :, 0:128] for t in range(4)]
            for u in range(2):
                for o in range(2):
                    fwdh1(0, 0, 2 * i + u, o, skip=(u == 0))
                for o in range(2):
                    fwdx1(0, 0, 2 * i + u, o, None, sk, slot=u)
            return carry
        lax.fori_loop(0, NA // 4, pre, 0)
        for c in range(2):
            for t in range(N1):
                wait_all(cp_gp(c + 1, t))
                group(c, c, c > 0, True, G1[t], G1[t + 1] - G1[t])

        def it(t, carry):
            wait_all(cp_grp(2 * t + 3))
            group(2 * t + 2, 0, True, True)
            wait_all(cp_grp(2 * t + 4))
            group(2 * t + 3, 1, True, True)
            return carry
        lax.fori_loop(0, 2, it, 0)
        wait_all(cp_grp(LG - 1))
        late[0] = group(LG - 2, 0, True, True, parts=(0, 4),
                        cfg=tuple(int(x) for x in '-30,-10,5,16,68,1,7'.split(',')))
        late[1] = group(LG - 1, 1, True, False, parts=(0, 4), ninv=NI7,
                        cfg=tuple(int(x) for x in '-10,0,0,1,40,0,0'.split(',')))

    conv()

    def rows(j):
        return j * TM if isinstance(j, int) else pl.multiple_of(j * TM, TM)

    def delay(x, after):
        if after is None:
            return x
        z8 = pltpu.bitcast(_tok([after]) & zero_vec(), f32)
        x0 = (x[:, 0:128].reshape(x.shape[0] // 8, 8, 128) + z8[None]).reshape(x.shape[0], 128)
        return jnp.concatenate([x0, x[:, 128:]], axis=1)

    def s0_rows(j, s0, ns, slot, from_q, after=None):
        r = rows(j)
        sl = slice(s0 * R, (s0 + ns) * R)
        x = qbuf.at[pl.ds(r, TM), :][sl, :].astype(f32)
        if from_q is not True:
            x = jnp.where(from_q, x, xbuf.at[pl.ds(r, TM), :][sl, :])
        x = delay(x, after)
        r2 = j * (TM // 2) if isinstance(j, int) else pl.multiple_of(j * (TM // 2), TM // 2)
        yw = ybuf.at[pl.ds(r2, TM // 2), :][s0 * 8:(s0 + ns) * 8, :]
        yy = [pltpu.unpack_elementwise(yw, index=k, packed_dtype=bf16, unpacked_dtype=f32)
              for k in range(2)]
        y = jnp.concatenate([yy[k][s * 8:(s + 1) * 8] for s in range(ns) for k in range(2)], axis=0)
        HS = int('1')
        if HS >= 0 and ns == 1:
            zs, aft = [], None
            for hh in range(2):
                xh = delay(x[8 * hh:8 * hh + 8], aft)
                q, t1 = _ln_t(xh)
                x1 = xh + q * y[8 * hh:8 * hh + 8]
                u, t2 = _ln_t(x1)
                x1b[slot * R + 8 * hh:slot * R + 8 * hh + 8, :] = x1
                ub[slot * R + 8 * hh:slot * R + 8 * hh + 8, :] = u
                z, t3 = _ln_t(u)
                zs.append(z)
                ts = t1 + t2 + t3 + [[z[:, D - 128:]]]
                aft = ts[HS][0][0:8]
            return jnp.concatenate(zs, axis=0).astype(bf16), ts
        q, t1 = _ln_t(x)
        x1 = x + q * y
        u, t2 = _ln_t(x1)
        x1b[slot * R:(slot + ns) * R, :] = x1
        ub[slot * R:(slot + ns) * R, :] = u
        z, t3 = _ln_t(u)
        return z.astype(bf16), t1 + t2 + t3 + [[z[:, D - 128:]]]

    rot = [0]

    def rhs_pins(steps, ksteps):
        pins = {}
        for t, lst in enumerate(steps):
            n, kg = t // ksteps, t % ksteps
            for i, vals in enumerate(lst):
                m = rot[0] % 4
                rot[0] += 1
                rg = 7 if (i % 2 == 0 and len(lst) > 1) else int('0')
                pins.setdefault(((kg * 4 + m) * 8 + rg, n), []).extend(vals)
        return pins

    def at_steps(toks, first, last, nsteps):
        steps = [[] for _ in range(nsteps)]
        for k, t in enumerate(toks):
            steps[first + (k * (last - first)) // max(len(toks) - 1, 1)].append(t)
        return steps

    def pinned(w, steps):
        return w if steps is None else _pin_at(w, rhs_pins(steps, 2), zero_vec())

    def put_h(row0, h):
        for l in range(LG):
            hwin[l, row0:row0 + h.shape[0], :] = h[:, l * 128:(l + 1) * 128]

    def m2_dot(r0, nr, steps=None):
        hs_in = jnp.concatenate(
            [hwin[l, 8 + r0 - SHIFTS[l]:8 + r0 - SHIFTS[l] + nr, :].astype(bf16) for l in range(LG)], axis=1)
        return _mm(hs_in, pinned(w2b[...], steps))

    def ln3(hs, lo, ns, after=None):
        sl = slice(lo * R, (lo + ns) * R)
        x1p = delay(ub[sl, :], after) + hs
        z, t = _ln_t(x1p)
        z3buf[sl, :] = z.astype(bf16)
        ln3.stats = [t[0][0][0:8], t[1][0][0:8], z[0:8, D - 128:]]
        return x1b[sl, :] + x1p, [z[:, D - 128:]]

    def mlp(c0, c1, acc, side=None, z3=None, pre=None):
        z3 = z3buf[...] if z3 is None else z3
        zero = zero_vec()
        steps = [[] for _ in range(16 * NC)]
        for c in range(c0, c1):
            if pre is not None:
                pre(c, steps)
            w3 = _pin_at(w3b[:, c * TF:(c + 1) * TF], rhs_pins(steps[16 * c:16 * c + 8], 2), zero)
            a = _gelu(_mm(z3, w3))
            if side is not None:
                side(c, a, steps)
            a = a.astype(bf16)
            w4 = _pin_at(w4b[c * TF:(c + 1) * TF, :], rhs_pins(steps[16 * c + 8:16 * c + 16], 1), zero)
            acc = acc + _mm(a, w4)
        return acc

    def s0_side(b, grp=None):
        RT, D0, DD, CH = (int(x) for x in '0,2,2,1'.split(','))
        grp = grp or _spread(list(range(NS)), KR)
        if isinstance(b, int):
            blk, fq = (b % NB, (b + 1) % NB), (b < NB, b + 1 < NB)
        else:
            blk, fq = (lax.rem(b, NB), lax.rem(b + 1, NB)), (b < NB, b + 1 < NB)

        def side(c, a, steps):
            if c == 0:
                x1b[0:R, :] = x1b[TM:TM + R, :]
                ub[0:R, :] = ub[TM:TM + R, :]
            after = a[0:8, RT * 128:(RT + 1) * 128]
            for n, s in enumerate(grp[c]):
                last = s == NS - 1
                z, t = s0_rows(blk[last], 0 if last else s + 1, 1, s + 1, fq[last], after)
                z1buf[s * R:(s + 1) * R, :] = z
                after = t[CH][0][0:8] if CH >= 0 else None
                steps[min(16 * c + 8 + D0 + n * DD, 16 * KR - 1)].append(t[-1])
        return side

    def toks(zs):
        return [t for _, ts in zs for t in ts]

    def cat(zs):
        return jnp.concatenate([z for z, _ in zs], axis=0)

    LNO = int('2')
    pend = [(par, u, h, a0) for u in range(NA // 2) for h in range(2)
            for a0 in range(8, NA, LNO) for par in range(2)]

    def late_piece():
        par, u, h, a0 = pend.pop(0)
        for _ in mac_part(par, u, h, a0, late[par][(u, h)], LNO):
            pass
        return list(late[par][(u, h)]['w'])

    NPA, NPB, NPC = (int(x) for x in '8,8,0'.split(','))

    def prologue(_, carry):
        cp_q0.wait()
        cp_w1.wait()
        cp_w2.wait()
        F1, L1_ = (int(x) for x in '2,15'.split(','))
        HM = TM // 2
        for a in range(3):
            inv1(LG - 1, 1, a // 2, a % 2)
        za = [s0_rows(0, 0, 8, 0, True)]
        for a in range(2 * NI7, NA // 2):
            inv1(LG - 2, 0, a // 2, a % 2)
        for a in range(3, NA // 2):
            inv1(LG - 1, 1, a // 2, a % 2)
        zb = [s0_rows(0, 8, 4, 8, True), s0_rows(0, 12, 4, 12, True), s0_rows(1, 0, 1, 16, True)]
        for l in range(LG):
            hwin[l, 0:8, :] = jnp.zeros((8, 128), f32)
        put_h(8, _gelu(_mm(cat(za), pinned(w1b[...], at_steps(toks(zb[:2]) + [zb[2][1][-1]], F1, L1_, 16)))))
        h = _gelu(_mm(cat(zb), pinned(w1b[...], at_steps([late_piece() for _ in range(NPA)], 1, 15, 16))))
        put_h(8 + HM, h[0:HM + 8])
        hcar[...] = h[HM + R - 24:HM + R]
        accb[0:HM, :] = m2_dot(0, HM, at_steps([late_piece() for _ in range(NPB)], 2, 15, 16))
        return carry

    def prologue2(_, carry):
        HM = TM // 2
        hs0 = accb[0:HM, :]
        l0 = [ln3(hs0[n * 32:(n + 1) * 32], 2 * n, 2) for n in range(4)]
        st1 = at_steps([t for _, t in l0], 3, 14, 16)
        st2 = at_steps([late_piece() for _ in range(NPC)], 5, 15, 16)
        hs1 = m2_dot(HM, HM, [x + y for x, y in zip(st1, st2)])
        if '1' == '0':
            wait_all(cp_w34a)
        l1 = [ln3(hs1[n * 32:(n + 1) * 32], 8 + 2 * n, 2) for n in range(4)]
        if '1' == '1':
            wait_all(cp_w34a)
        s0s = s0_side(1)
        LA, LZ, LRT = (int(x) for x in '1,63,-1'.split(','))
        W3, W4 = (int(x) for x in '1,1'.split(','))
        slots = [t for t in range(LA, LZ + 1) if t != 16 * WS for _ in range(W3 if t % 16 < 8 else W4)]
        due = [slots[(k * len(slots)) // len(pend)] for k in range(len(pend))]

        def run_late(lo, hi, steps):
            while pend and lo <= due[0] < hi:
                steps[due.pop(0)].append(late_piece())

        def side(c, a, steps):
            s0s(c, a, steps)
            run_late(16 * c + 8, 16 * c + 16, steps)

        def pre(c, steps):
            if c == WS:
                wait_all(cp_w34m)
            run_late(16 * c, 16 * c + 8, steps)
        accb[...] = mlp(0, KR, jnp.concatenate([r for r, _ in l0 + l1], axis=0), side,
                        pre=pre)
        for par in late:
            for a in range(NA // 2, NA):
                inv1(LG - 2 + par, par, a // 2, a % 2)
        return carry

    prologue(0, 0)

    def mark(i, carry):
        zsm[1 + i] = i
        return carry
    lax.fori_loop(0, 2, mark, 0)
    prologue2(0, 0)
    wait_all(cp_w34b + (cp_q3,))

    def body(g, carry):
        @pl.when(g == 1)
        def _():
            cp_q4.wait()
        rot[0] = int('1')
        b = g + 1
        jb = lax.rem(b, NB)
        T3, RT, D0, DD = (int(x) for x in '2,0,0,1'.split(','))
        T0 = int('1')
        z3 = z3buf[...]
        acc = mlp(KR, KR + T0, accb[...], None, z3)
        top = hcar[...]
        put_h(0, jnp.where(jb == 0, 0.0, top[0:8]))
        put_h(8, top[8:24])
        h = _gelu(_mm(z1buf[...], w1b[...]))
        put_h(24, h[0:TM - R])
        put_h(8 + TM, jnp.where(jb == NB - 1, 0.0, h[TM - R:TM - 8]))
        hcar[...] = h[TM - 24:TM]
        acc = mlp(KR + T0, KR + T3, acc, None, z3)
        hs = m2_dot(0, TM)
        rs = []
        grp = _spread(list(range(NS)), NC - KR - T3)

        def side(c, a, steps):
            for n, s in enumerate(grp[c - KR - T3]):
                LC, LB = (int(x) for x in '-1,1'.split(','))
                if n == 0:
                    aft = a[0:8, RT * 128:(RT + 1) * 128] if RT >= 0 else None
                elif LC >= 0 and n % LB == 0:
                    aft = ln3.stats[LC]
                elif LC < 0:
                    aft = None
                side.aft = aft if (n == 0 or LC < 0 or n % LB == 0) else side.aft
                r_, t = ln3(hs[s * R:(s + 1) * R], s, 1, side.aft)
                rs.append(r_)
                steps[min(16 * c + 8 + D0 + (n * DD) // 2, 16 * NC - 1)].append(t)
        xn = mlp(KR + T3, NC, acc, side, z3)
        jg = lax.rem(g, NB)
        xbuf[pl.ds(rows(jg), TM), :] = xn
        obuf[pl.ds(rows(jg), TM), :] = xn.astype(bf16)
        accb[...] = mlp(0, KR, jnp.concatenate(rs, axis=0), s0_side(g + 2))

        @pl.when(g >= NB)
        def _():
            cp_o(jg).start()
        return carry

    lax.fori_loop(0, G - 1, body, 0)

    OC = [0] + [int(x) for x in '512,896'.split(',')] + [D]
    OS = tuple((OC[i], OC[i + 1] - OC[i]) for i in range(len(OC) - 1))
    acc = mlp(KR, NC - 1, accb[...])
    a = _gelu(_mm(z3buf[...], w3b[:, FF - TF:])).astype(bf16)
    for c0, nc in OS:
        obuf[S - TM:, c0:c0 + nc] = (acc[:, c0:c0 + nc] + _mm(a, w4b[FF - TF:, c0:c0 + nc])).astype(bf16)
        cp_o(NB - 1, c0, nc).start()
    for j in range(NB - 1):
        cp_o(j).wait()
    for c0, nc in OS:
        cp_o(NB - 1, c0, nc).wait()


@jax.jit
def pallas_interleave_layers__ssm_conv_h3__mixer_s_mlp__prompt_kernel(
    A_q, A_k, A_v, A_shift_k, A_ssm_k, A_ssm_D, B_x, B_w1, B_w2, B_w3, B_w4,
):
    del B_x
    vm = pltpu.VMEM
    scratch = [
        vm((D, D), bf16), vm((D, D), bf16), vm((D, FF), bf16), vm((FF, D), bf16),
        vm((S + 16, D), bf16), vm((S, D), bf16), vm((D, S), bf16), vm((S, D), bf16),
        vm((4, D), bf16), vm((D,), bf16),
        vm((2, CB, CB), u32), vm((2, CB // 2, 2 * CB), u32),
        vm((5, 8, D), f32),
        vm((2, 2 * CB + 16, 128), f32),
        vm((2 * H0, 128), f32), vm((2 * H0, 128), f32),
        vm((NA, CB, 128), u32), vm((NA, CB, 128), u32),
        vm((S // 2, D), u32), vm((S, D), f32), vm((TM + R, D), f32), vm((TM + R, D), f32),
        vm((LG, TM + R, 128), f32), vm((24, D), f32),
        vm((TM, D), bf16), vm((TM, D), bf16), vm((TM, D), f32),
        pltpu.SMEM((4,), i32),
        pltpu.SemaphoreType.DMA((2 * len('0,3,8'.split(',')) - 1 + LG + 7,)),
    ]
    return pl.pallas_call(
        _kernel,
        out_shape=jax.ShapeDtypeStruct(A_q.shape, bf16),
        in_specs=[pl.BlockSpec(memory_space=pl.ANY)] * 10,
        out_specs=pl.BlockSpec(memory_space=pl.ANY),
        scratch_shapes=scratch,
        compiler_params=pltpu.CompilerParams(vmem_limit_bytes=100 * 1024 * 1024),
    )(A_q, A_k, A_v, A_shift_k.T, A_ssm_k, A_ssm_D, B_w1, B_w2, B_w3, B_w4)
```

```python
import math

import jax
import jax.numpy as jnp
from jax import lax
import jax.experimental.pallas as pl
import jax.experimental.pallas.tpu as pltpu


f32, bf16, u32, i32 = jnp.float32, jnp.bfloat16, jnp.uint32, jnp.int32

S, D, FF = 2048, 1024, 3584
TM = 256
NB = S // TM
G = 2 * NB
CB = 128
NA = S // CB
NO = 4
TF = 512
NC = FF // TF
R = 16
NS = TM // R
LG = D // 128
KR = int('4')
ND = int('4')
EPS = 1e-5
CS = CB + 8
BS = 3 * CS
H0 = NA * BS + 16
C0 = math.sqrt(2.0 / math.pi)
C1 = C0 * 0.044715
SHIFTS = (1, 1, -1, -1, 2, 2, -2, -2)


def _ln(x):
    m = jnp.mean(x, axis=-1, keepdims=True)
    xc = x - m
    v = jnp.mean(xc * xc, axis=-1, keepdims=True)
    return xc * lax.rsqrt(v + EPS)


def _ln_t(x):
    m = jnp.mean(x, axis=-1, keepdims=True)
    xc = x - m
    v = jnp.mean(xc * xc, axis=-1, keepdims=True)
    r = lax.rsqrt(v + EPS)
    n = x.shape[0]
    return xc * r, [[jnp.broadcast_to(m, (n, 128))], [jnp.broadcast_to(r, (n, 128))]]


def _gelu(x):
    hx = 0.5 * x
    return hx + hx * jnp.tanh(x * (C0 + C1 * (x * x)))


def _mm(a, b):
    return jnp.dot(a, b, preferred_element_type=f32)


def _tok(vals):
    t = None
    for v in vals:
        b = pltpu.bitcast(v, u32)
        for i in range(b.shape[0] // 8):
            for j in range(b.shape[1] // 128):
                p = b[i * 8:(i + 1) * 8, j * 128:(j + 1) * 128]
                t = p if t is None else t | p
    return t


def _pin(x, vals, zero):
    if not vals:
        return x
    top = pltpu.bitcast(pltpu.bitcast(x[0:16, 0:128], u32) | (_tok(vals) & zero), bf16)
    row0 = jnp.concatenate([top, x[0:16, 128:]], axis=1)
    return jnp.concatenate([row0, x[16:]], axis=0)


def _pin_at(x, pins, zero):
    if not pins:
        return x
    out, last = [], 0
    for k in sorted({k for k, _ in pins}):
        if k * 16 > last:
            out.append(x[last:k * 16])
        blk = x[k * 16:(k + 1) * 16]
        for (kk, n), vals in pins.items():
            if kk != k:
                continue
            top = pltpu.bitcast(pltpu.bitcast(blk[:, n * 128:(n + 1) * 128], u32) | (_tok(vals) & zero), bf16)
            parts = ([blk[:, :n * 128]] if n > 0 else []) + [top] + (
                [blk[:, (n + 1) * 128:]] if (n + 1) * 128 < blk.shape[1] else [])
            blk = jnp.concatenate(parts, axis=1) if len(parts) > 1 else top
        out.append(blk)
        last = (k + 1) * 16
    if last < x.shape[0]:
        out.append(x[last:])
    return jnp.concatenate(out, axis=0) if len(out) > 1 else out[0]


def _spread(items, n):
    return [items[(i * len(items)) // n:((i + 1) * len(items)) // n] for i in range(n)]


def _kernel(q_hbm, k_hbm, v_hbm, sk_hbm, hk_hbm, dd_hbm, w1_hbm, w2_hbm, w3_hbm, w4_hbm,
            o_hbm,
            w1b, w2b, w3b, w4b, kbuf, vbuf, hkb, qbuf, skb, ddb,
            Fm, Gm, skf, kf, ZS, YS, ybuf, xbuf, x1b, ub, hwin, hcar, z3buf, accb,
            zsm, sem):
    obuf = vbuf

    def cp_kvh(c, r0, nr, si):
        ch = pl.ds(c * 128, 128)
        return (
            pltpu.make_async_copy(k_hbm.at[0, pl.ds(r0, nr), ch], kbuf.at[pl.ds(16 + r0, nr), ch], sem.at[si]),
            pltpu.make_async_copy(v_hbm.at[0, pl.ds(r0, nr), ch], vbuf.at[pl.ds(r0, nr), ch], sem.at[si]),
            pltpu.make_async_copy(hk_hbm.at[ch, pl.ds(r0, nr)], hkb.at[ch, pl.ds(r0, nr)], sem.at[si]))

    G1 = [int(x) for x in '0,3,8'.split(',')]
    N1 = len(G1) - 1

    def cp_g0(i):
        return cp_kvh(0, i * 2 * TM, 2 * TM, i)

    def cp_gp(c, n):
        return cp_kvh(c, G1[n] * TM, (G1[n + 1] - G1[n]) * TM, 4 + (c - 1) * N1 + n)

    def cp_grp(c):
        return cp_kvh(c, 0, S, 1 + 2 * N1 + c)

    SB = 1 + 2 * N1 + LG

    def cp_q(r0, r1, si):
        return pltpu.make_async_copy(q_hbm.at[0, pl.ds(r0, r1 - r0), :],
                                     qbuf.at[pl.ds(r0, r1 - r0), :], sem.at[si])

    def cp_o(j, c0=0, nc=D):
        return pltpu.make_async_copy(obuf.at[pl.ds(j * TM, TM), pl.ds(c0, nc)],
                                     o_hbm.at[0, pl.ds(j * TM, TM), pl.ds(c0, nc)], sem.at[SB + 4])

    cp_sk = pltpu.make_async_copy(sk_hbm, skb, sem.at[SB])
    cp_dd = pltpu.make_async_copy(dd_hbm, ddb, sem.at[SB])
    cp_q0 = cp_q(0, 2 * TM + R, SB + 1)

    cp_q3 = cp_q(2 * TM + R, 3 * TM + R, SB + 7)
    cp_q4 = cp_q(3 * TM + R, S, SB + 3)

    cp_w1 = pltpu.make_async_copy(w1_hbm, w1b, sem.at[SB + 1])
    cp_w2 = pltpu.make_async_copy(w2_hbm, w2b, sem.at[SB + 8])
    def cp_w34(c0, c1, si):
        n = (c1 - c0) * TF
        return (pltpu.make_async_copy(w3_hbm.at[:, pl.ds(c0 * TF, n)], w3b.at[:, pl.ds(c0 * TF, n)], sem.at[si]),
                pltpu.make_async_copy(w4_hbm.at[pl.ds(c0 * TF, n), :], w4b.at[pl.ds(c0 * TF, n), :], sem.at[si]))

    WS = int('2')
    cp_w34a = cp_w34(0, WS, SB + 5)
    cp_w34m = cp_w34(WS, KR, SB + 6)
    cp_w34b = cp_w34(KR, KR + 1, SB + 2)
    cp_w34c = cp_w34(KR + 1, NC, SB + 9)

    def wait_all(cps):
        for cp in cps:
            cp.wait()

    cp_sk.start()
    cp_dd.start()
    for grp in ([cp_g0(i) for i in range(4)] + [cp_gp(c, n) for c in (1, 2) for n in range(N1)]
                + [cp_grp(c) for c in range(3, LG)]):
        for cp in grp:
            cp.start()
    for cp in (cp_q0, cp_w1, cp_w2) + cp_w34a + cp_w34m + cp_w34b + cp_w34c + (cp_q3, cp_q4):
        cp.start()

    zsm[0] = 0
    kbuf[0:16, :] = jnp.zeros((16, D), bf16)

    def _basis(pos, part, n):
        k = jnp.where(pos < CB // 2, 2 * pos, 2 * pos - (CB - 1))
        m = ((2 * k + 1) * n + part * CB) & (4 * CB - 1)
        r = m & (2 * CB - 1)
        neg = jnp.logical_xor(m >= 2 * CB, r > CB)
        th = jnp.minimum(r, 2 * CB - r).astype(f32) * (math.pi / (2 * CB))
        t2 = th * th
        z = 1.0 / math.factorial(12)
        for e in (10, 8, 6, 4, 2, 0):
            z = 1.0 / math.factorial(e) - t2 * z
        z = jnp.where(neg, -z, z)
        return z, jnp.where(pos < CB // 2, z, -z)

    def dft_init(t, carry):
        rf = lax.broadcasted_iota(i32, (32, CB), 0)
        zs = _basis(t * 16 + (rf & 15), rf >> 4, lax.broadcasted_iota(i32, (32, CB), 1))
        cg = lax.broadcasted_iota(i32, (16, 2 * CB), 1)
        gs = _basis(cg >> 1, cg & 1, t * 16 + lax.broadcasted_iota(i32, (16, 2 * CB), 0))
        for par in range(2):
            Fm[par, pl.ds(pl.multiple_of(t * 16, 16), 16), :] = pltpu.bitcast(zs[par].astype(bf16), u32)
            Gm[par, pl.ds(pl.multiple_of(t * 8, 8), 8), :] = pltpu.bitcast(
                (gs[par] * (1.0 / CB)).astype(bf16), u32)
        return carry

    lax.fori_loop(0, CB // 16, dft_init, 0)

    cp_sk.wait()
    cp_dd.wait()
    sk32 = skb[...].astype(f32)
    for t in range(4):
        skf[t] = jnp.broadcast_to(sk32[t:t + 1, :], (8, D))
    skf[4] = jnp.broadcast_to(ddb[...].astype(f32).reshape(1, D), (8, D))

    SET = [(c + LG - ND) % 2 for c in range(LG - ND + 2)] + list(range(2, ND))

    def zero_vec():
        return jnp.full((8, 128), zsm[0], i32).astype(u32)

    def bmul(x, row8):
        n = x.shape[0] // 8
        return (x.reshape(n, 8, 128) * row8[None]).reshape(x.shape)

    def dsl(start, size, align):
        return pl.ds(start if isinstance(start, int) else pl.multiple_of(start, align), size)

    def unil(z):
        return (jnp.concatenate([z[32 * g:32 * g + 16] for g in range(CB // 16)], axis=0),
                jnp.concatenate([z[32 * g + 16:32 * g + 32] for g in range(CB // 16)], axis=0))

    def fwdh1(c, par, i, o, pins=None, skip=True):
        Z = ZS[par].at[dsl(H0 + i * 2 * BS, 2 * BS, 8), :]
        ls = dsl(c * 128, 128, 128)
        a = 2 * i + o
        hh = lax.dot_general(_pin_at(pltpu.bitcast(Fm[o], bf16), pins, zero_vec()), hkb[ls, dsl(a * CB, CB, CB)], (((1,), (1,)), ((), ())),
                             preferred_element_type=f32)
        cc, dd = unil(hh)
        if o == 0 and skip and (not isinstance(i, int) or i == 0):
            d8 = skf[4, :, ls] if isinstance(i, int) else jnp.where(i == 0, skf[4, :, ls], 0.0)
            cc = (cc.reshape(CB // 8, 8, 128) + d8[None]).reshape(CB, 128)
        b = o * BS
        Z[b:b + CB, :] = cc
        Z[b + CS:b + CS + CB, :] = dd - cc
        Z[b + 2 * CS:b + 2 * CS + CB, :] = cc + dd
        return cc + dd

    def fwdx1(c, par, i, o, pins, sk, slot=0):
        Z = ZS[par].at[dsl(i * 2 * BS, 2 * BS, 8), :]
        ls = dsl(c * 128, 128, 128)
        ks_ = i % 2 if isinstance(i, int) else slot
        if o == 0:
            kf[ks_] = kbuf[dsl(i * 2 * CB, 2 * CB + 16, 16), ls].astype(f32)
        a = 2 * i + o
        b0 = 16 + o * CB
        ks = bmul(kf[ks_, b0:b0 + CB, :], sk[0])
        for t in range(1, 4):
            ks = ks + bmul(kf[ks_, b0 - t:b0 - t + CB, :], sk[t])
        kv = (ks * vbuf[dsl(a * CB, CB, CB), ls].astype(f32)).astype(bf16)
        xh = _mm(_pin_at(pltpu.bitcast(Fm[o], bf16), pins, zero_vec()), kv)
        xr, xm = unil(xh)
        b = o * BS
        Z[b:b + CB, :] = xr
        Z[b + CS:b + CS + CB, :] = xm
        Z[b + 2 * CS:b + 2 * CS + CB, :] = xr + xm
        return xr + xm

    def mac_part(par, i, h, a0, st, NO=NO):
        Z, Y = ZS[par], YS[par]
        Z = Z.at[dsl(i * 16, 2 * H0 - CB + 16, 16), :]

        def ld(base, a):
            b = base + a * BS + h * 8
            return tuple(Z[b + k * CS:b + k * CS + 8, :] for k in range(3))
        K = [None] * NO
        hw = {}
        for ap in range(a0 + NO):
            xa, xb, xs = ld(0, ap)
            for o in range(NO):
                dl = a0 + o - ap
                if dl < 0:
                    continue
                if dl not in hw:
                    hw[dl] = ld(H0, dl)
                hc, he, hf = hw[dl]
                t = (hc * xs, xa * he, xb * hf)
                K[o] = t if K[o] is None else tuple(u + w for u, w in zip(K[o], t))
                inj = yield K[o][2]
                if inj is not None:
                    K[o] = (K[o][0], K[o][1], K[o][2] + inj)
        st['w'] = []
        for o in range(NO):
            re, im = K[o][0] - K[o][2], K[o][0] + K[o][1]
            prev = st.get('y')
            out = (re, im) if prev is None else (re - prev[1], im + prev[0])
            st['y'] = (re, im)
            st['w'].append(pltpu.pack_elementwise(list(out), packed_dtype=bf16).astype(u32))
            Y[a0 + o, dsl(i * 16 + h * 8, 8, 8), :] = st['w'][-1]

    def mac_gen(par, i0, ns, parts, sts):
        for u in range(ns):
            for a0 in parts:
                for h in range(2):
                    yield from mac_part(par, i0 + u, h, a0, sts.setdefault((u, h), {}))

    def inv1(c, par, i, o, pins=None):
        Y = YS[par]
        a = 2 * i + o
        y = _mm(_pin_at(pltpu.bitcast(Gm[o], bf16), pins, zero_vec()), pltpu.bitcast(Y[a], bf16))
        yv = ybuf.at[dsl(a * (CB // 2), CB // 2, CB // 2), :]
        for g in range(CB // 16):
            yv[8 * g:8 * g + 8, dsl(c * 128, 128, 128)] = pltpu.pack_elementwise(
                [y[16 * g:16 * g + 8], y[16 * g + 8:16 * g + 16]], packed_dtype=bf16).astype(u32)
        return y

    def group(c, sets, do_inv, do_fwd, i0=0, ns=NA // 2, parts=(0, 4, 8, 12), cfg=None, ninv=NA // 2):
        PI, P0, DP, NP_, R0, DR, G0 = cfg or tuple(int(x) for x in '-20,12,12,16,220,12,4'.split(','))
        NPM = sum(2 * (NO * a0 + 10) for a0 in parts)
        names = 'h0,x0,h1,x1'.split(',')
        zero = zero_vec()
        sk = [skf[t, :, dsl((c + 1) * 128, 128, 128)] for t in range(4)] if do_fwd else None
        sts = {}
        pprev, par, pnext = sets
        gen = mac_gen(par, i0, ns, parts, sts)
        rec = [next(gen)]
        inj = {}
        for u in range(ns):
            i = i0 + u
            base = u * NPM
            while len(rec) <= base + P0 + (NP_ - 1) * DP:
                rec.append(gen.send(inj.get(len(rec))))
            pins = {k: {} for k in ('i0', 'i1', 'h0', 'h1', 'x0', 'x1')}
            if base + PI >= 0:
                pins['i0'][(0, 0)] = [rec[base + PI]]
                pins['i1'][(0, 0)] = [rec[base + PI]]
            for n in range(NP_):
                r = ((n + 1) * 16) // NP_ - 1
                pins[names[n % len(names)]][(r, 0)] = [rec[base + P0 + n * DP]]
            XP = int('-999')
            if base + XP >= 0:
                for nm in ('x0', 'x1'):
                    pins[nm].setdefault((0, 0), []).append(rec[base + XP])
            if do_inv and i < ninv:
                ys = [inv1(c - 1, pprev, i, 0, pins['i0']), inv1(c - 1, pprev, i, 1, pins['i1'])]
                if not do_fwd:
                    inj[base + R0] = pltpu.bitcast(_tok([y[CB - 8:CB] for y in ys]) & zero, f32)
            if do_fwd:
                res = [fwdh1(c + 1, pnext, i, 0, pins['h0'], skip=(u == 0)),
                       fwdh1(c + 1, pnext, i, 1, pins['h1']),
                       fwdx1(c + 1, pnext, i, 0, pins['x0'], sk, slot=u % 2),
                       fwdx1(c + 1, pnext, i, 1, pins['x1'], sk, slot=u % 2)]
                for g in range(G0, CB // 16):
                    tk = _tok([z[16 * g + 8:16 * g + 16] for z in res]) & zero
                    inj[base + R0 + (g - G0) * DR] = pltpu.bitcast(tk, f32)
        try:
            while True:
                rec.append(gen.send(inj.get(len(rec))))
        except StopIteration:
            pass
        return sts

    late = {}
    NI7 = int('2')

    def conv():
        def pre(i, carry):
            wait_all(cp_g0(i))
            sk = [skf[t, :, 0:128] for t in range(4)]
            for u in range(2):
                for o in range(2):
                    fwdh1(0, SET[0], 2 * i + u, o, skip=(u == 0))
                for o in range(2):
                    fwdx1(0, SET[0], 2 * i + u, o, None, sk, slot=u)
            return carry
        lax.fori_loop(0, NA // 4, pre, 0)
        def sets(c):
            return (SET[c - 1], SET[c], SET[c + 1] if c + 1 < LG else None)

        for c in range(2):
            for t in range(N1):
                wait_all(cp_gp(c + 1, t))
                group(c, sets(c), c > 0, True, G1[t], G1[t + 1] - G1[t])
        CUT = int('4')
        for c in range(2, LG - ND):
            if c == CUT:
                lax.fori_loop(0, 2, mark, 0)
            wait_all(cp_grp(c + 1))
            group(c, sets(c), True, True)
        for c in range(LG - ND, LG - 1):
            if c == CUT:
                lax.fori_loop(0, 2, mark, 0)
            wait_all(cp_grp(c + 1))
            late[c] = group(c, sets(c), True, True, parts=(0, 4), ninv=NA // (2 if c == LG - ND else 4),
                            cfg=tuple(int(x) for x in '-30,-10,5,16,68,1,7'.split(',')))
        late[LG - 1] = group(LG - 1, sets(LG - 1), True, False, parts=(0, 4), ninv=NI7,
                             cfg=tuple(int(x) for x in '-10,0,0,1,40,0,0'.split(',')))

    def mark(i, carry):
        zsm[1 + i] = i
        return carry

    conv()

    def rows(j):
        return j * TM if isinstance(j, int) else pl.multiple_of(j * TM, TM)

    def delay(x, after):
        if after is None:
            return x
        z8 = pltpu.bitcast(_tok([after]) & zero_vec(), f32)
        x0 = (x[:, 0:128].reshape(x.shape[0] // 8, 8, 128) + z8[None]).reshape(x.shape[0], 128)
        return jnp.concatenate([x0, x[:, 128:]], axis=1)

    def s0_rows(j, s0, ns, slot, from_q, after=None):
        r = rows(j)
        sl = slice(s0 * R, (s0 + ns) * R)
        x = qbuf.at[pl.ds(r, TM), :][sl, :].astype(f32)
        if from_q is not True:
            x = jnp.where(from_q, x, xbuf.at[pl.ds(r, TM), :][sl, :])
        x = delay(x, after)
        r2 = j * (TM // 2) if isinstance(j, int) else pl.multiple_of(j * (TM // 2), TM // 2)
        yw = ybuf.at[pl.ds(r2, TM // 2), :][s0 * 8:(s0 + ns) * 8, :]
        yy = [pltpu.unpack_elementwise(yw, index=k, packed_dtype=bf16, unpacked_dtype=f32)
              for k in range(2)]
        y = jnp.concatenate([yy[k][s * 8:(s + 1) * 8] for s in range(ns) for k in range(2)], axis=0)
        HS = int('1')
        if HS >= 0 and ns == 1:
            zs, aft = [], None
            for hh in range(2):
                xh = delay(x[8 * hh:8 * hh + 8], aft)
                q, t1 = _ln_t(xh)
                x1 = xh + q * y[8 * hh:8 * hh + 8]
                u, t2 = _ln_t(x1)
                x1b[slot * R + 8 * hh:slot * R + 8 * hh + 8, :] = x1
                ub[slot * R + 8 * hh:slot * R + 8 * hh + 8, :] = u
                z, t3 = _ln_t(u)
                zs.append(z)
                ts = t1 + t2 + t3 + [[z[:, D - 128:]]]
                aft = ts[HS][0][0:8]
            return jnp.concatenate(zs, axis=0).astype(bf16), ts
        q, t1 = _ln_t(x)
        x1 = x + q * y
        u, t2 = _ln_t(x1)
        x1b[slot * R:(slot + ns) * R, :] = x1
        ub[slot * R:(slot + ns) * R, :] = u
        z, t3 = _ln_t(u)
        return z.astype(bf16), t1 + t2 + t3 + [[z[:, D - 128:]]]

    rot = [0]

    def rhs_pins(steps, ksteps):
        pins = {}
        for t, lst in enumerate(steps):
            n, kg = t // ksteps, t % ksteps
            for i, vals in enumerate(lst):
                m = rot[0] % 4
                rot[0] += 1
                rg = 7 if (i % 2 == 0 and len(lst) > 1) else int('0')
                pins.setdefault(((kg * 4 + m) * 8 + rg, n), []).extend(vals)
        return pins

    def at_steps(toks, first, last, nsteps):
        steps = [[] for _ in range(nsteps)]
        for k, t in enumerate(toks):
            steps[first + (k * (last - first)) // max(len(toks) - 1, 1)].append(t)
        return steps

    def pinned(w, steps):
        return w if steps is None else _pin_at(w, rhs_pins(steps, 2), zero_vec())

    def put_h(row0, h):
        for l in range(LG):
            hwin[l, row0:row0 + h.shape[0], :] = h[:, l * 128:(l + 1) * 128]

    def m2_dot(r0, nr, steps=None):
        hs_in = jnp.concatenate(
            [hwin[l, 8 + r0 - SHIFTS[l]:8 + r0 - SHIFTS[l] + nr, :].astype(bf16) for l in range(LG)], axis=1)
        return _mm(hs_in, pinned(w2b[...], steps))

    def ln3(hs, lo, ns, after=None):
        sl = slice(lo * R, (lo + ns) * R)
        x1p = delay(ub[sl, :], after) + hs
        z, t = _ln_t(x1p)
        z3buf[sl, :] = z.astype(bf16)
        ln3.stats = [t[0][0][0:8], t[1][0][0:8], z[0:8, D - 128:]]
        return x1b[sl, :] + x1p, [z[:, D - 128:]]

    def mlp(c0, c1, acc, side=None, z3=None, pre=None):
        z3 = z3buf[...] if z3 is None else z3
        zero = zero_vec()
        steps = [[] for _ in range(16 * NC)]
        for c in range(c0, c1):
            if pre is not None:
                pre(c, steps)
            w3 = _pin_at(w3b[:, c * TF:(c + 1) * TF], rhs_pins(steps[16 * c:16 * c + 8], 2), zero)
            a = _gelu(_mm(z3, w3))
            if side is not None:
                side(c, a, steps)
            a = a.astype(bf16)
            w4 = _pin_at(w4b[c * TF:(c + 1) * TF, :], rhs_pins(steps[16 * c + 8:16 * c + 16], 1), zero)
            acc = acc + _mm(a, w4)
        return acc

    def s0_side(b, grp=None):
        RT, D0, DD, CH = (int(x) for x in '0,2,2,1'.split(','))
        DL = int('-1')
        grp = (grp or _spread(list(range(NS)), KR)) + [[]] * NC
        if isinstance(b, int):
            blk, fq = (b % NB, (b + 1) % NB), (b < NB, b + 1 < NB)
        else:
            blk, fq = (lax.rem(b, NB), lax.rem(b + 1, NB)), (b < NB, b + 1 < NB)

        def side(c, a, steps):
            if c == 0:
                x1b[0:R, :] = x1b[TM:TM + R, :]
                ub[0:R, :] = ub[TM:TM + R, :]
            after = a[0:8, RT * 128:(RT + 1) * 128]
            for n, s in enumerate(grp[c]):
                last = s == NS - 1
                z, t = s0_rows(blk[last], 0 if last else s + 1, 1, s + 1, fq[last], after)
                side.zs.append(z)
                after = t[CH][0][0:8] if CH >= 0 else None
                steps[min(16 * c + 8 + D0 + n * DD, 16 * KR + DL)].append(t[-1])
        side.zs = []
        return side

    def toks(zs):
        return [t for _, ts in zs for t in ts]

    def cat(zs):
        return jnp.concatenate([z for z, _ in zs], axis=0)

    LNO = int('2')
    pend = [(par, u, h, a0) for u in range(NA // 2) for h in range(2)
            for a0 in range(8, NA, LNO) for par in range(LG - ND, LG)]

    def late_piece():
        par, u, h, a0 = pend.pop(0)
        for _ in mac_part(SET[par], u, h, a0, late[par][(u, h)], LNO):
            pass
        return list(late[par][(u, h)]['w'])

    NPA, NPB, NPC = (int(x) for x in '8,8,0'.split(','))

    def prologue(_, carry):
        cp_q0.wait()
        cp_w1.wait()
        F1, L1_ = (int(x) for x in '2,15'.split(','))
        HM = TM // 2
        for a in range(3):
            inv1(LG - 1, SET[LG - 1], a // 2, a % 2)
        za = [s0_rows(0, 0, 8, 0, True)]
        for a in range(2 * NI7, NA // 2):
            inv1(LG - 2, SET[LG - 2], a // 2, a % 2)
        for a in range(3, NA // 2):
            inv1(LG - 1, SET[LG - 1], a // 2, a % 2)
        zb = [s0_rows(0, 8, 4, 8, True), s0_rows(0, 12, 4, 12, True), s0_rows(1, 0, 1, 16, True)]
        for l in range(LG):
            hwin[l, 0:8, :] = jnp.zeros((8, 128), f32)
        put_h(8, _gelu(_mm(cat(za), pinned(w1b[...], at_steps(toks(zb[:2]) + [zb[2][1][-1]], F1, L1_, 16)))))
        h = _gelu(_mm(cat(zb), pinned(w1b[...], at_steps([late_piece() for _ in range(NPA)], 1, 15, 16))))
        put_h(8 + HM, h[0:HM + 8])
        hcar[...] = h[HM + R - 24:HM + R]
        return carry

    def prologue2(_, carry):
        HM = TM // 2
        cp_w2.wait()
        hs0 = m2_dot(0, HM, at_steps([late_piece() for _ in range(NPB)], 2, 15, 16))
        l0 = [ln3(hs0[n * 32:(n + 1) * 32], 2 * n, 2) for n in range(4)]
        st1 = at_steps([t for _, t in l0], 3, 14, 16)
        st2 = at_steps([late_piece() for _ in range(NPC)], 5, 15, 16)
        hs1 = m2_dot(HM, HM, [x + y for x, y in zip(st1, st2)])
        if '1' == '0':
            wait_all(cp_w34a)
        l1 = [ln3(hs1[n * 32:(n + 1) * 32], 8 + 2 * n, 2) for n in range(4)]
        if '1' == '1':
            wait_all(cp_w34a)
        st['s0'] = s0_side(1)
        LA, LZ = (int(x) for x in '1,126'.split(','))
        skip = (16 * WS, 16 * KR, 16 * (KR + 2))
        WA, WB, WM = (int(x) for x in '1,1,1'.split(','))

        def wt(t):
            if t < 16 * KR:
                return WA if t % 16 < 8 else WB
            return WM
        slots = [t for t in range(LA, LZ + 1) if t not in skip for _ in range(wt(t))]
        st['due'] = [slots[(k * len(slots)) // len(pend)] for k in range(len(pend))]

        def side(c, a, steps):
            st['s0'](c, a, steps)
            run_late(16 * c + 8, 16 * c + 16, steps)

        def pre(c, steps):
            if c == WS:
                wait_all(cp_w34m)
            run_late(16 * c, 16 * c + 8, steps)
        st['z3'] = z3buf[...]
        st['acc'] = mlp(0, KR, jnp.concatenate([r for r, _ in l0 + l1], axis=0), side, st['z3'], pre)
        return carry

    st = {}

    def run_late(lo, hi, steps, off=0):
        while pend and lo <= st['due'][0] < hi:
            steps[st['due'].pop(0) - off].append(late_piece())

    def late_steps(lo):
        steps = [[] for _ in range(16)]
        run_late(lo, lo + 16, steps, lo)
        return steps

    def second_half(b, acc, z3, z1, first):
        RT, D0, DD = (int(x) for x in '0,0,1'.split(','))
        jb = b % NB if first else lax.rem(b, NB)
        if first:
            def mk(off):
                return (lambda c, a, steps: run_late(16 * c + 8 + off, 16 * c + 16 + off, steps, off),
                        lambda c, steps: run_late(16 * c + off, 16 * c + 8 + off, steps, off))
        else:
            def mk(off):
                return None, None
        sd, pr = mk(0)
        acc = mlp(KR, KR + 1, acc, sd, z3, pr)
        top = hcar[...]
        put_h(0, top[0:8] if first else jnp.where(jb == 0, 0.0, top[0:8]))
        put_h(8, top[8:24])
        h = _gelu(_mm(z1, pinned(w1b[...], late_steps(16 * (KR + 1)) if first else None)))
        put_h(24, h[0:TM - R])
        put_h(8 + TM, h[TM - R:TM - 8] if first else jnp.where(jb == NB - 1, 0.0, h[TM - R:TM - 8]))
        hcar[...] = h[TM - 24:TM]
        if first:
            wait_all(cp_w34c)
        sd, pr = mk(16)
        acc = mlp(KR + 1, KR + 2, acc, sd, z3, pr)
        hs = m2_dot(0, TM, late_steps(16 * (KR + 3)) if first else None)
        if first:
            for par in late:
                for a in range(NA // 2, NA):
                    inv1(par, SET[par], a // 2, a % 2)
        rs = []

        def side(c, a, steps):
            for n in range(NS):
                r_, t = ln3(hs[n * R:(n + 1) * R], n, 1,
                            a[0:8, RT * 128:(RT + 1) * 128] if (n == 0 and RT >= 0) else None)
                rs.append(r_)
                steps[min(16 * c + 8 + D0 + (n * DD) // 2, 16 * NC - 1)].append(t)
        xn = mlp(KR + 2, NC, acc, side, z3)
        jg = (b - 1) % NB if first else lax.rem(b - 1, NB)
        xbuf[pl.ds(rows(jg), TM), :] = xn
        if not first:
            obuf[pl.ds(rows(jg), TM), :] = xn.astype(bf16)
        accb[...] = jnp.concatenate(rs, axis=0)

    prologue(0, 0)
    lax.fori_loop(0, 2, mark, 0)
    prologue2(0, 0)
    lax.fori_loop(0, 2, mark, 0)
    wait_all(cp_w34b)
    second_half(1, st['acc'], st['z3'], jnp.concatenate(st['s0'].zs, axis=0), True)
    cp_q3.wait()

    def body(b, carry):
        @pl.when(b == 2)
        def _():
            cp_q4.wait()
        rot[0] = int('2')
        z3 = z3buf[...]
        sd = s0_side(b + 1)
        acc = mlp(0, KR, accb[...], sd, z3)
        second_half(b + 1, acc, z3, jnp.concatenate(sd.zs, axis=0), False)

        @pl.when(b >= NB)
        def _():
            cp_o(b - NB).start()
        return carry

    lax.fori_loop(1, G - 1, body, 0)

    OC = [0] + [int(x) for x in '512,896'.split(',')] + [D]
    OS = tuple((OC[i], OC[i + 1] - OC[i]) for i in range(len(OC) - 1))
    accb[...] = mlp(0, KR, accb[...])
    lax.fori_loop(0, 2, mark, 0)
    acc = mlp(KR, NC - 1, accb[...])
    a = _gelu(_mm(z3buf[...], w3b[:, FF - TF:])).astype(bf16)
    for c0, nc in OS:
        obuf[S - TM:, c0:c0 + nc] = (acc[:, c0:c0 + nc] + _mm(a, w4b[FF - TF:, c0:c0 + nc])).astype(bf16)
        cp_o(NB - 1, c0, nc).start()
    for j in range(NB - 1):
        cp_o(j).wait()
    for c0, nc in OS:
        cp_o(NB - 1, c0, nc).wait()


@jax.jit
def pallas_interleave_layers__ssm_conv_h3__mixer_s_mlp__prompt_kernel(
    A_q, A_k, A_v, A_shift_k, A_ssm_k, A_ssm_D, B_x, B_w1, B_w2, B_w3, B_w4,
):
    del B_x
    vm = pltpu.VMEM
    scratch = [
        vm((D, D), bf16), vm((D, D), bf16), vm((D, FF), bf16), vm((FF, D), bf16),
        vm((S + 16, D), bf16), vm((S, D), bf16), vm((D, S), bf16), vm((S, D), bf16),
        vm((4, D), bf16), vm((D,), bf16),
        vm((2, CB, CB), u32), vm((2, CB // 2, 2 * CB), u32),
        vm((5, 8, D), f32),
        vm((2, 2 * CB + 16, 128), f32),
        [vm((2 * H0, 128), f32)] * ND, [vm((NA, CB, 128), u32)] * ND,
        vm((S // 2, D), u32), vm((S, D), f32), vm((TM + R, D), f32), vm((TM + R, D), f32),
        vm((LG, TM + R, 128), f32), vm((24, D), f32),
        vm((TM, D), bf16), vm((TM, D), f32),
        pltpu.SMEM((4,), i32),
        pltpu.SemaphoreType.DMA((2 * len('0,3,8'.split(',')) - 1 + LG + 10,)),
    ]
    return pl.pallas_call(
        _kernel,
        out_shape=jax.ShapeDtypeStruct(A_q.shape, bf16),
        in_specs=[pl.BlockSpec(memory_space=pl.ANY)] * 10,
        out_specs=pl.BlockSpec(memory_space=pl.ANY),
        scratch_shapes=scratch,
        compiler_params=pltpu.CompilerParams(vmem_limit_bytes=116 * 1024 * 1024),
    )(A_q, A_k, A_v, A_shift_k.T, A_ssm_k, A_ssm_D, B_w1, B_w2, B_w3, B_w4)
```

```python
import math

import jax
import jax.numpy as jnp
from jax import lax
import jax.experimental.pallas as pl
import jax.experimental.pallas.tpu as pltpu


f32, bf16, u32, i32 = jnp.float32, jnp.bfloat16, jnp.uint32, jnp.int32

S, D, FF = 2048, 1024, 3584
TM = 256
NB = S // TM
G = 2 * NB
CB = 128
NA = S // CB
NO = 4
TF = 512
NC = FF // TF
R = 16
NS = TM // R
LG = D // 128
KR = int('4')
ND = int('4')
G1 = [int(x) for x in '0,2,5,8'.split(',')]
G2 = [int(x) for x in '0,3,8'.split(',')]
NP12 = len(G1) + len(G2) - 2
EPS = 1e-5
CS = CB + 8
BS = 3 * CS
H0 = NA * BS + 16
C0 = math.sqrt(2.0 / math.pi)
C1 = C0 * 0.044715
SHIFTS = (1, 1, -1, -1, 2, 2, -2, -2)


def _ln(x):
    m = jnp.mean(x, axis=-1, keepdims=True)
    xc = x - m
    v = jnp.mean(xc * xc, axis=-1, keepdims=True)
    return xc * lax.rsqrt(v + EPS)


def _ln_t(x):
    m = jnp.mean(x, axis=-1, keepdims=True)
    xc = x - m
    v = jnp.mean(xc * xc, axis=-1, keepdims=True)
    r = lax.rsqrt(v + EPS)
    n = x.shape[0]
    return xc * r, [[jnp.broadcast_to(m, (n, 128))], [jnp.broadcast_to(r, (n, 128))]]


def _gelu(x):
    hx = 0.5 * x
    return hx + hx * jnp.tanh(x * (C0 + C1 * (x * x)))


def _mm(a, b):
    return jnp.dot(a, b, preferred_element_type=f32)


def _tok(vals):
    t = None
    for v in vals:
        b = pltpu.bitcast(v, u32)
        for i in range(b.shape[0] // 8):
            for j in range(b.shape[1] // 128):
                p = b[i * 8:(i + 1) * 8, j * 128:(j + 1) * 128]
                t = p if t is None else t | p
    return t


def _pin(x, vals, zero):
    if not vals:
        return x
    top = pltpu.bitcast(pltpu.bitcast(x[0:16, 0:128], u32) | (_tok(vals) & zero), bf16)
    row0 = jnp.concatenate([top, x[0:16, 128:]], axis=1)
    return jnp.concatenate([row0, x[16:]], axis=0)


def _pin_at(x, pins, zero):
    if not pins:
        return x
    out, last = [], 0
    for k in sorted({k for k, _ in pins}):
        if k * 16 > last:
            out.append(x[last:k * 16])
        blk = x[k * 16:(k + 1) * 16]
        for (kk, n), vals in pins.items():
            if kk != k:
                continue
            top = pltpu.bitcast(pltpu.bitcast(blk[:, n * 128:(n + 1) * 128], u32) | (_tok(vals) & zero), bf16)
            parts = ([blk[:, :n * 128]] if n > 0 else []) + [top] + (
                [blk[:, (n + 1) * 128:]] if (n + 1) * 128 < blk.shape[1] else [])
            blk = jnp.concatenate(parts, axis=1) if len(parts) > 1 else top
        out.append(blk)
        last = (k + 1) * 16
    if last < x.shape[0]:
        out.append(x[last:])
    return jnp.concatenate(out, axis=0) if len(out) > 1 else out[0]


def _spread(items, n):
    return [items[(i * len(items)) // n:((i + 1) * len(items)) // n] for i in range(n)]


def _kernel(q_hbm, k_hbm, v_hbm, sk_hbm, hk_hbm, dd_hbm, w1_hbm, w2_hbm, w3_hbm, w4_hbm,
            o_hbm,
            w1b, w2b, w3b, w4b, kbuf, vbuf, hkb, qbuf, skb, ddb,
            Fm, Gm, skf, kf, ZS, YS, ybuf, xbuf, x1b, ub, hwin, hcar, z3buf, accb,
            zsm, sem):
    obuf = vbuf

    def cp_kvh(c, r0, nr, si):
        ch = pl.ds(c * 128, 128)
        return (
            pltpu.make_async_copy(k_hbm.at[0, pl.ds(r0, nr), ch], kbuf.at[pl.ds(16 + r0, nr), ch], sem.at[si]),
            pltpu.make_async_copy(v_hbm.at[0, pl.ds(r0, nr), ch], vbuf.at[pl.ds(r0, nr), ch], sem.at[si]),
            pltpu.make_async_copy(hk_hbm.at[ch, pl.ds(r0, nr)], hkb.at[ch, pl.ds(r0, nr)], sem.at[si]))

    GP = {1: G1, 2: G2}

    def cp_g0(i):
        return cp_kvh(0, i * 2 * TM, 2 * TM, i)

    def cp_gp(c, n):
        return cp_kvh(c, GP[c][n] * TM, (GP[c][n + 1] - GP[c][n]) * TM, 4 + (c - 1) * (len(G1) - 1) + n)

    def cp_grp(c):
        return cp_kvh(c, 0, S, 1 + NP12 + c)

    SB = 1 + NP12 + LG

    def cp_q(r0, r1, si):
        return pltpu.make_async_copy(q_hbm.at[0, pl.ds(r0, r1 - r0), :],
                                     qbuf.at[pl.ds(r0, r1 - r0), :], sem.at[si])

    def cp_o(j, c0=0, nc=D):
        return pltpu.make_async_copy(obuf.at[pl.ds(j * TM, TM), pl.ds(c0, nc)],
                                     o_hbm.at[0, pl.ds(j * TM, TM), pl.ds(c0, nc)], sem.at[SB + 4])

    cp_sk = pltpu.make_async_copy(sk_hbm, skb, sem.at[SB])
    cp_dd = pltpu.make_async_copy(dd_hbm, ddb, sem.at[SB])
    cp_q0 = cp_q(0, 2 * TM + R, SB + 1)

    cp_q3 = cp_q(2 * TM + R, 3 * TM + R, SB + 7)
    cp_q4 = cp_q(3 * TM + R, S, SB + 3)

    cp_w1 = pltpu.make_async_copy(w1_hbm, w1b, sem.at[SB + 1])
    cp_w2 = pltpu.make_async_copy(w2_hbm, w2b, sem.at[SB + 8])
    def cp_w34(c0, c1, si):
        n = (c1 - c0) * TF
        return (pltpu.make_async_copy(w3_hbm.at[:, pl.ds(c0 * TF, n)], w3b.at[:, pl.ds(c0 * TF, n)], sem.at[si]),
                pltpu.make_async_copy(w4_hbm.at[pl.ds(c0 * TF, n), :], w4b.at[pl.ds(c0 * TF, n), :], sem.at[si]))

    WS = int('2')
    cp_w34a = cp_w34(0, WS, SB + 5)
    WB = int('3')
    cp_w34m = cp_w34(WS, WB, SB + 6)
    cp_w34b = cp_w34(WB, KR + 1, SB + 2)
    cp_w34c = cp_w34(KR + 1, NC, SB + 9)

    def wait_all(cps):
        for cp in cps:
            cp.wait()

    cp_sk.start()
    cp_dd.start()
    for grp in ([cp_g0(i) for i in range(4)] + [cp_gp(c, n) for c in (1, 2) for n in range(len(GP[c]) - 1)]
                + [cp_grp(c) for c in range(3, LG)]):
        for cp in grp:
            cp.start()
    for cp in (cp_q0, cp_w1, cp_w2) + cp_w34a + cp_w34m + cp_w34b + cp_w34c + (cp_q3, cp_q4):
        cp.start()

    zsm[0] = 0
    kbuf[0:16, :] = jnp.zeros((16, D), bf16)

    def _basis(pos, part, n):
        k = jnp.where(pos < CB // 2, 2 * pos, 2 * pos - (CB - 1))
        m = ((2 * k + 1) * n + part * CB) & (4 * CB - 1)
        r = m & (2 * CB - 1)
        neg = jnp.logical_xor(m >= 2 * CB, r > CB)
        th = jnp.minimum(r, 2 * CB - r).astype(f32) * (math.pi / (2 * CB))
        t2 = th * th
        z = 1.0 / math.factorial(12)
        for e in (10, 8, 6, 4, 2, 0):
            z = 1.0 / math.factorial(e) - t2 * z
        z = jnp.where(neg, -z, z)
        return z, jnp.where(pos < CB // 2, z, -z)

    def dft_init(t, carry):
        rf = lax.broadcasted_iota(i32, (32, CB), 0)
        zs = _basis(t * 16 + (rf & 15), rf >> 4, lax.broadcasted_iota(i32, (32, CB), 1))
        cg = lax.broadcasted_iota(i32, (16, 2 * CB), 1)
        gs = _basis(cg >> 1, cg & 1, t * 16 + lax.broadcasted_iota(i32, (16, 2 * CB), 0))
        for par in range(2):
            Fm[par, pl.ds(pl.multiple_of(t * 16, 16), 16), :] = pltpu.bitcast(zs[par].astype(bf16), u32)
            Gm[par, pl.ds(pl.multiple_of(t * 8, 8), 8), :] = pltpu.bitcast(
                (gs[par] * (1.0 / CB)).astype(bf16), u32)
        return carry

    lax.fori_loop(0, CB // 16, dft_init, 0)

    cp_sk.wait()
    cp_dd.wait()
    sk32 = skb[...].astype(f32)
    for t in range(4):
        skf[t] = jnp.broadcast_to(sk32[t:t + 1, :], (8, D))
    skf[4] = jnp.broadcast_to(ddb[...].astype(f32).reshape(1, D), (8, D))

    SET = [(c + LG - ND) % 2 for c in range(LG - ND + 2)] + list(range(2, ND))

    def zero_vec():
        return jnp.full((8, 128), zsm[0], i32).astype(u32)

    def bmul(x, row8):
        n = x.shape[0] // 8
        return (x.reshape(n, 8, 128) * row8[None]).reshape(x.shape)

    def dsl(start, size, align):
        return pl.ds(start if isinstance(start, int) else pl.multiple_of(start, align), size)

    def unil(z):
        return (jnp.concatenate([z[32 * g:32 * g + 16] for g in range(CB // 16)], axis=0),
                jnp.concatenate([z[32 * g + 16:32 * g + 32] for g in range(CB // 16)], axis=0))

    def fwdh1(c, par, i, o, pins=None, skip=True):
        Z = ZS[par].at[dsl(H0 + i * 2 * BS, 2 * BS, 8), :]
        ls = dsl(c * 128, 128, 128)
        a = 2 * i + o
        hh = lax.dot_general(_pin_at(pltpu.bitcast(Fm[o], bf16), pins, zero_vec()), hkb[ls, dsl(a * CB, CB, CB)], (((1,), (1,)), ((), ())),
                             preferred_element_type=f32)
        cc, dd = unil(hh)
        if o == 0 and skip and (not isinstance(i, int) or i == 0):
            d8 = skf[4, :, ls] if isinstance(i, int) else jnp.where(i == 0, skf[4, :, ls], 0.0)
            cc = (cc.reshape(CB // 8, 8, 128) + d8[None]).reshape(CB, 128)
        b = o * BS
        Z[b:b + CB, :] = cc
        Z[b + CS:b + CS + CB, :] = dd - cc
        Z[b + 2 * CS:b + 2 * CS + CB, :] = cc + dd
        return cc + dd

    def fwdx1(c, par, i, o, pins, sk, slot=0):
        Z = ZS[par].at[dsl(i * 2 * BS, 2 * BS, 8), :]
        ls = dsl(c * 128, 128, 128)
        ks_ = i % 2 if isinstance(i, int) else slot
        if o == 0:
            kf[ks_] = kbuf[dsl(i * 2 * CB, 2 * CB + 16, 16), ls].astype(f32)
        a = 2 * i + o
        b0 = 16 + o * CB
        ks = bmul(kf[ks_, b0:b0 + CB, :], sk[0])
        for t in range(1, 4):
            ks = ks + bmul(kf[ks_, b0 - t:b0 - t + CB, :], sk[t])
        kv = (ks * vbuf[dsl(a * CB, CB, CB), ls].astype(f32)).astype(bf16)
        xh = _mm(_pin_at(pltpu.bitcast(Fm[o], bf16), pins, zero_vec()), kv)
        xr, xm = unil(xh)
        b = o * BS
        Z[b:b + CB, :] = xr
        Z[b + CS:b + CS + CB, :] = xm
        Z[b + 2 * CS:b + 2 * CS + CB, :] = xr + xm
        return xr + xm

    def mac_part(par, i, h, a0, st, NO=NO):
        Z, Y = ZS[par], YS[par]
        Z = Z.at[dsl(i * 16, 2 * H0 - CB + 16, 16), :]

        def ld(base, a):
            b = base + a * BS + h * 8
            return tuple(Z[b + k * CS:b + k * CS + 8, :] for k in range(3))
        K = [None] * NO
        hw = {}
        for ap in range(a0 + NO):
            xa, xb, xs = ld(0, ap)
            for o in range(NO):
                dl = a0 + o - ap
                if dl < 0:
                    continue
                if dl not in hw:
                    hw[dl] = ld(H0, dl)
                hc, he, hf = hw[dl]
                t = (hc * xs, xa * he, xb * hf)
                K[o] = t if K[o] is None else tuple(u + w for u, w in zip(K[o], t))
                inj = yield K[o][2]
                if inj is not None:
                    K[o] = (K[o][0], K[o][1], K[o][2] + inj)
        st['w'] = []
        for o in range(NO):
            re, im = K[o][0] - K[o][2], K[o][0] + K[o][1]
            prev = st.get('y')
            out = (re, im) if prev is None else (re - prev[1], im + prev[0])
            st['y'] = (re, im)
            st['w'].append(pltpu.pack_elementwise(list(out), packed_dtype=bf16).astype(u32))
            Y[a0 + o, dsl(i * 16 + h * 8, 8, 8), :] = st['w'][-1]

    def mac_gen(par, i0, ns, parts, sts):
        for u in range(ns):
            for a0 in parts:
                for h in range(2):
                    yield from mac_part(par, i0 + u, h, a0, sts.setdefault((u, h), {}))

    def inv1(c, par, i, o, pins=None):
        Y = YS[par]
        a = 2 * i + o
        y = _mm(_pin_at(pltpu.bitcast(Gm[o], bf16), pins, zero_vec()), pltpu.bitcast(Y[a], bf16))
        yv = ybuf.at[dsl(a * (CB // 2), CB // 2, CB // 2), :]
        for g in range(CB // 16):
            yv[8 * g:8 * g + 8, dsl(c * 128, 128, 128)] = pltpu.pack_elementwise(
                [y[16 * g:16 * g + 8], y[16 * g + 8:16 * g + 16]], packed_dtype=bf16).astype(u32)
        return y

    def group(c, sets, do_inv, do_fwd, i0=0, ns=NA // 2, parts=(0, 4, 8, 12), cfg=None, ninv=NA // 2):
        PI, P0, DP, NP_, R0, DR, G0 = cfg or tuple(int(x) for x in '-20,12,12,16,220,12,4'.split(','))
        NPM = sum(2 * (NO * a0 + 10) for a0 in parts)
        names = 'h0,x0,h1,x1'.split(',')
        zero = zero_vec()
        sk = [skf[t, :, dsl((c + 1) * 128, 128, 128)] for t in range(4)] if do_fwd else None
        sts = {}
        pprev, par, pnext = sets
        gen = mac_gen(par, i0, ns, parts, sts)
        rec = [next(gen)]
        inj = {}
        for u in range(ns):
            i = i0 + u
            base = u * NPM
            while len(rec) <= base + P0 + (NP_ - 1) * DP:
                rec.append(gen.send(inj.get(len(rec))))
            pins = {k: {} for k in ('i0', 'i1', 'h0', 'h1', 'x0', 'x1')}
            if base + PI >= 0:
                pins['i0'][(0, 0)] = [rec[base + PI]]
                pins['i1'][(0, 0)] = [rec[base + PI]]
            for n in range(NP_):
                r = ((n + 1) * 16) // NP_ - 1
                pins[names[n % len(names)]][(r, 0)] = [rec[base + P0 + n * DP]]
            XP = int('-999')
            if base + XP >= 0:
                for nm in ('x0', 'x1'):
                    pins[nm].setdefault((0, 0), []).append(rec[base + XP])
            if do_inv and i < ninv:
                ys = [inv1(c - 1, pprev, i, 0, pins['i0']), inv1(c - 1, pprev, i, 1, pins['i1'])]
                if not do_fwd:
                    inj[base + R0] = pltpu.bitcast(_tok([y[CB - 8:CB] for y in ys]) & zero, f32)
            if do_fwd:
                res = [fwdh1(c + 1, pnext, i, 0, pins['h0'], skip=(u == 0)),
                       fwdh1(c + 1, pnext, i, 1, pins['h1']),
                       fwdx1(c + 1, pnext, i, 0, pins['x0'], sk, slot=u % 2),
                       fwdx1(c + 1, pnext, i, 1, pins['x1'], sk, slot=u % 2)]
                for g in range(G0, CB // 16):
                    tk = _tok([z[16 * g + 8:16 * g + 16] for z in res]) & zero
                    inj[base + R0 + (g - G0) * DR] = pltpu.bitcast(tk, f32)
        try:
            while True:
                rec.append(gen.send(inj.get(len(rec))))
        except StopIteration:
            pass
        return sts

    late = {}
    NI7 = int('2')

    def conv():
        def pre(i, carry):
            wait_all(cp_g0(i))
            sk = [skf[t, :, 0:128] for t in range(4)]
            for u in range(2):
                for o in range(2):
                    fwdh1(0, SET[0], 2 * i + u, o, skip=(u == 0))
                for o in range(2):
                    fwdx1(0, SET[0], 2 * i + u, o, None, sk, slot=u)
            return carry
        lax.fori_loop(0, NA // 4, pre, 0)
        def sets(c):
            return (SET[c - 1], SET[c], SET[c + 1] if c + 1 < LG else None)

        for c in range(2):
            for t in range(len(GP[c + 1]) - 1):
                wait_all(cp_gp(c + 1, t))
                group(c, sets(c), c > 0, True, GP[c + 1][t], GP[c + 1][t + 1] - GP[c + 1][t])
        CUT = int('4')
        for c in range(2, LG - ND):
            if c == CUT:
                lax.fori_loop(0, 2, mark, 0)
            wait_all(cp_grp(c + 1))
            group(c, sets(c), True, True)
        for c in range(LG - ND, LG - 1):
            if c == CUT:
                lax.fori_loop(0, 2, mark, 0)
            wait_all(cp_grp(c + 1))
            late[c] = group(c, sets(c), True, True, parts=(0, 4), ninv=NA // (2 if c == LG - ND else 4),
                            cfg=tuple(int(x) for x in '-30,-6,5,16,68,1,5'.split(',')))
        late[LG - 1] = group(LG - 1, sets(LG - 1), True, False, parts=(0, 4), ninv=NI7,
                             cfg=tuple(int(x) for x in '-10,0,0,1,40,0,0'.split(',')))

    def mark(i, carry):
        zsm[1 + i] = i
        return carry

    conv()

    def rows(j):
        return j * TM if isinstance(j, int) else pl.multiple_of(j * TM, TM)

    def delay(x, after):
        if after is None:
            return x
        z8 = pltpu.bitcast(_tok([after]) & zero_vec(), f32)
        x0 = (x[:, 0:128].reshape(x.shape[0] // 8, 8, 128) + z8[None]).reshape(x.shape[0], 128)
        return jnp.concatenate([x0, x[:, 128:]], axis=1)

    def s0_rows(j, s0, ns, slot, from_q, after=None):
        r = rows(j)
        sl = slice(s0 * R, (s0 + ns) * R)
        x = qbuf.at[pl.ds(r, TM), :][sl, :].astype(f32)
        if from_q is not True:
            x = jnp.where(from_q, x, xbuf.at[pl.ds(r, TM), :][sl, :])
        x = delay(x, after)
        r2 = j * (TM // 2) if isinstance(j, int) else pl.multiple_of(j * (TM // 2), TM // 2)
        yw = ybuf.at[pl.ds(r2, TM // 2), :][s0 * 8:(s0 + ns) * 8, :]
        yy = [pltpu.unpack_elementwise(yw, index=k, packed_dtype=bf16, unpacked_dtype=f32)
              for k in range(2)]
        y = jnp.concatenate([yy[k][s * 8:(s + 1) * 8] for s in range(ns) for k in range(2)], axis=0)
        HS = int('1')
        if HS >= 0 and ns == 1:
            zs, aft = [], None
            for hh in range(2):
                xh = delay(x[8 * hh:8 * hh + 8], aft)
                q, t1 = _ln_t(xh)
                x1 = xh + q * y[8 * hh:8 * hh + 8]
                u, t2 = _ln_t(x1)
                x1b[slot * R + 8 * hh:slot * R + 8 * hh + 8, :] = x1
                ub[slot * R + 8 * hh:slot * R + 8 * hh + 8, :] = u
                z, t3 = _ln_t(u)
                zs.append(z)
                ts = t1 + t2 + t3 + [[z[:, D - 128:]]]
                aft = ts[HS][0][0:8]
            return jnp.concatenate(zs, axis=0).astype(bf16), ts
        q, t1 = _ln_t(x)
        x1 = x + q * y
        u, t2 = _ln_t(x1)
        x1b[slot * R:(slot + ns) * R, :] = x1
        ub[slot * R:(slot + ns) * R, :] = u
        z, t3 = _ln_t(u)
        return z.astype(bf16), t1 + t2 + t3 + [[z[:, D - 128:]]]

    rot = [0]

    def rhs_pins(steps, ksteps):
        pins = {}
        for t, lst in enumerate(steps):
            n, kg = t // ksteps, t % ksteps
            for i, vals in enumerate(lst):
                m = rot[0] % 4
                rot[0] += 1
                rg = 7 if (i % 2 == 0 and len(lst) > 1) else int('0')
                pins.setdefault(((kg * 4 + m) * 8 + rg, n), []).extend(vals)
        return pins

    def at_steps(toks, first, last, nsteps):
        steps = [[] for _ in range(nsteps)]
        for k, t in enumerate(toks):
            steps[first + (k * (last - first)) // max(len(toks) - 1, 1)].append(t)
        return steps

    def pinned(w, steps):
        return w if steps is None else _pin_at(w, rhs_pins(steps, 2), zero_vec())

    def put_h(row0, h):
        for l in range(LG):
            hwin[l, row0:row0 + h.shape[0], :] = h[:, l * 128:(l + 1) * 128]

    def m2_dot(r0, nr, steps=None):
        hs_in = jnp.concatenate(
            [hwin[l, 8 + r0 - SHIFTS[l]:8 + r0 - SHIFTS[l] + nr, :].astype(bf16) for l in range(LG)], axis=1)
        return _mm(hs_in, pinned(w2b[...], steps))

    def ln3(hs, lo, ns, after=None):
        sl = slice(lo * R, (lo + ns) * R)
        x1p = delay(ub[sl, :], after) + hs
        z, t = _ln_t(x1p)
        z3buf[sl, :] = z.astype(bf16)
        ln3.stats = [t[0][0][0:8], t[1][0][0:8], z[0:8, D - 128:]]
        return x1b[sl, :] + x1p, [z[:, D - 128:]]

    def mlp(c0, c1, acc, side=None, z3=None, pre=None):
        z3 = z3buf[...] if z3 is None else z3
        zero = zero_vec()
        steps = [[] for _ in range(16 * NC)]
        for c in range(c0, c1):
            if pre is not None:
                pre(c, steps)
            w3 = _pin_at(w3b[:, c * TF:(c + 1) * TF], rhs_pins(steps[16 * c:16 * c + 8], 2), zero)
            a = _gelu(_mm(z3, w3))
            if side is not None:
                side(c, a, steps)
            a = a.astype(bf16)
            w4 = _pin_at(w4b[c * TF:(c + 1) * TF, :], rhs_pins(steps[16 * c + 8:16 * c + 16], 1), zero)
            acc = acc + _mm(a, w4)
        return acc

    def s0_side(b, grp=None, bars=()):
        RT, D0, DD, CH = (int(x) for x in '0,2,2,1'.split(','))
        DL = int('-1')
        grp = (grp or _spread(list(range(NS)), KR)) + [[]] * NC
        if isinstance(b, int):
            blk, fq = (b % NB, (b + 1) % NB), (b < NB, b + 1 < NB)
        else:
            blk, fq = (lax.rem(b, NB), lax.rem(b + 1, NB)), (b < NB, b + 1 < NB)

        def side(c, a, steps):
            if c == 0:
                x1b[0:R, :] = x1b[TM:TM + R, :]
                ub[0:R, :] = ub[TM:TM + R, :]
            after = a[0:8, RT * 128:(RT + 1) * 128]
            for n, s in enumerate(grp[c]):
                last = s == NS - 1
                z, t = s0_rows(blk[last], 0 if last else s + 1, 1, s + 1, fq[last], after)
                side.zs.append(z)
                after = t[CH][0][0:8] if CH >= 0 else None
                steps[min(16 * c + 8 + D0 + n * DD, 16 * (c + 1) - 1 if c + 1 in bars else 16 * KR + DL)].append(t[-1])
        side.zs = []
        return side

    def toks(zs):
        return [t for _, ts in zs for t in ts]

    def cat(zs):
        return jnp.concatenate([z for z, _ in zs], axis=0)

    LNO = int('2')
    pend = [(par, u, h, a0) for u in range(NA // 2) for h in range(2)
            for a0 in range(8, NA, LNO) for par in range(LG - ND, LG)]

    def late_piece():
        par, u, h, a0 = pend.pop(0)
        for _ in mac_part(SET[par], u, h, a0, late[par][(u, h)], LNO):
            pass
        return list(late[par][(u, h)]['w'])

    NPA, NPB, NPC = (int(x) for x in '8,8,0'.split(','))

    def prologue(_, carry):
        cp_q0.wait()
        cp_w1.wait()
        F1, L1_ = (int(x) for x in '2,15'.split(','))
        HM = TM // 2
        for a in range(3):
            inv1(LG - 1, SET[LG - 1], a // 2, a % 2)
        za = [s0_rows(0, 0, 8, 0, True)]
        for a in range(2 * NI7, NA // 2):
            inv1(LG - 2, SET[LG - 2], a // 2, a % 2)
        for a in range(3, NA // 2):
            inv1(LG - 1, SET[LG - 1], a // 2, a % 2)
        zb = [s0_rows(0, 8, 4, 8, True), s0_rows(0, 12, 4, 12, True), s0_rows(1, 0, 1, 16, True)]
        for l in range(LG):
            hwin[l, 0:8, :] = jnp.zeros((8, 128), f32)
        put_h(8, _gelu(_mm(cat(za), pinned(w1b[...], at_steps(toks(zb[:2]) + [zb[2][1][-1]], F1, L1_, 16)))))
        h = _gelu(_mm(cat(zb), pinned(w1b[...], at_steps([late_piece() for _ in range(NPA)], 1, 15, 16))))
        put_h(8 + HM, h[0:HM + 8])
        hcar[...] = h[HM + R - 24:HM + R]
        return carry

    def prologue2(_, carry):
        HM = TM // 2
        cp_w2.wait()
        hs0 = m2_dot(0, HM, at_steps([late_piece() for _ in range(NPB)], 2, 15, 16))
        l0 = [ln3(hs0[n * 32:(n + 1) * 32], 2 * n, 2) for n in range(4)]
        st1 = at_steps([t for _, t in l0], 3, 14, 16)
        st2 = at_steps([late_piece() for _ in range(NPC)], 5, 15, 16)
        hs1 = m2_dot(HM, HM, [x + y for x, y in zip(st1, st2)])
        if '1' == '0':
            wait_all(cp_w34a)
        l1 = [ln3(hs1[n * 32:(n + 1) * 32], 8 + 2 * n, 2) for n in range(4)]
        if '1' == '1':
            wait_all(cp_w34a)
        st['s0'] = s0_side(1, bars=(WS, WB))
        LA, LZ = (int(x) for x in '1,126'.split(','))
        skip = (16 * WS, 16 * WB, 16 * (KR + 2))
        WA, WC, WM = (int(x) for x in '1,1,1'.split(','))

        def wt(t):
            if t < 16 * KR:
                return WA if t % 16 < 8 else WC
            return WM
        slots = [t for t in range(LA, LZ + 1) if t not in skip for _ in range(wt(t))]
        st['due'] = [slots[(k * len(slots)) // len(pend)] for k in range(len(pend))]

        def side(c, a, steps):
            st['s0'](c, a, steps)
            run_late(16 * c + 8, 16 * c + 16, steps)

        def pre(c, steps):
            if c == WS:
                wait_all(cp_w34m)
            if c == WB:
                lax.fori_loop(0, 2, mark, 0)
                wait_all(cp_w34b)
            run_late(16 * c, 16 * c + 8, steps)
        st['z3'] = z3buf[...]
        st['acc'] = mlp(0, KR, jnp.concatenate([r for r, _ in l0 + l1], axis=0), side, st['z3'], pre)
        return carry

    st = {}

    def run_late(lo, hi, steps, off=0):
        while pend and lo <= st['due'][0] < hi:
            steps[st['due'].pop(0) - off].append(late_piece())

    def late_steps(lo):
        steps = [[] for _ in range(16)]
        run_late(lo, lo + 16, steps, lo)
        return steps

    def second_half(b, acc, z3, z1, first):
        RT, D0, DD = (int(x) for x in '0,0,1'.split(','))
        jb = b % NB if first else lax.rem(b, NB)
        if first:
            def mk(off):
                return (lambda c, a, steps: run_late(16 * c + 8 + off, 16 * c + 16 + off, steps, off),
                        lambda c, steps: run_late(16 * c + off, 16 * c + 8 + off, steps, off))
        else:
            def mk(off):
                return None, None
        sd, pr = mk(0)
        acc = mlp(KR, KR + 1, acc, sd, z3, pr)
        top = hcar[...]
        put_h(0, top[0:8] if first else jnp.where(jb == 0, 0.0, top[0:8]))
        put_h(8, top[8:24])
        h = _gelu(_mm(z1, pinned(w1b[...], late_steps(16 * (KR + 1)) if first else None)))
        put_h(24, h[0:TM - R])
        put_h(8 + TM, h[TM - R:TM - 8] if first else jnp.where(jb == NB - 1, 0.0, h[TM - R:TM - 8]))
        hcar[...] = h[TM - 24:TM]
        if first:
            wait_all(cp_w34c)
        sd, pr = mk(16)
        acc = mlp(KR + 1, KR + 2, acc, sd, z3, pr)
        hs = m2_dot(0, TM, late_steps(16 * (KR + 3)) if first else None)
        if first:
            for par in late:
                for a in range(NA // 2, NA):
                    inv1(par, SET[par], a // 2, a % 2)
        rs = []

        def side(c, a, steps):
            for n in range(NS):
                r_, t = ln3(hs[n * R:(n + 1) * R], n, 1,
                            a[0:8, RT * 128:(RT + 1) * 128] if (n == 0 and RT >= 0) else None)
                rs.append(r_)
                steps[min(16 * c + 8 + D0 + (n * DD) // 2, 16 * NC - 1)].append(t)
        xn = mlp(KR + 2, NC, acc, side, z3)
        jg = (b - 1) % NB if first else lax.rem(b - 1, NB)
        xbuf[pl.ds(rows(jg), TM), :] = xn
        if not first:
            obuf[pl.ds(rows(jg), TM), :] = xn.astype(bf16)
        accb[...] = jnp.concatenate(rs, axis=0)

    prologue(0, 0)
    lax.fori_loop(0, 2, mark, 0)
    prologue2(0, 0)
    if WB == KR:
        lax.fori_loop(0, 2, mark, 0)
        wait_all(cp_w34b)
    second_half(1, st['acc'], st['z3'], jnp.concatenate(st['s0'].zs, axis=0), True)
    cp_q3.wait()

    def body(b, carry):
        @pl.when(b == 2)
        def _():
            cp_q4.wait()
        rot[0] = int('2')
        z3 = z3buf[...]
        sd = s0_side(b + 1)
        acc = mlp(0, KR, accb[...], sd, z3)
        second_half(b + 1, acc, z3, jnp.concatenate(sd.zs, axis=0), False)

        @pl.when(b >= NB)
        def _():
            cp_o(b - NB).start()
        return carry

    lax.fori_loop(1, G - 1, body, 0)

    OC = [0] + [int(x) for x in '512,896'.split(',')] + [D]
    OS = tuple((OC[i], OC[i + 1] - OC[i]) for i in range(len(OC) - 1))
    FS = int('0')
    if FS:
        accb[...] = mlp(0, FS, accb[...])
        lax.fori_loop(0, 2, mark, 0)
    acc = mlp(FS, NC - 1, accb[...])
    a = _gelu(_mm(z3buf[...], w3b[:, FF - TF:])).astype(bf16)
    for c0, nc in OS:
        obuf[S - TM:, c0:c0 + nc] = (acc[:, c0:c0 + nc] + _mm(a, w4b[FF - TF:, c0:c0 + nc])).astype(bf16)
        cp_o(NB - 1, c0, nc).start()
    for j in range(NB - 1):
        cp_o(j).wait()
    for c0, nc in OS:
        cp_o(NB - 1, c0, nc).wait()


@jax.jit
def pallas_interleave_layers__ssm_conv_h3__mixer_s_mlp__prompt_kernel(
    A_q, A_k, A_v, A_shift_k, A_ssm_k, A_ssm_D, B_x, B_w1, B_w2, B_w3, B_w4,
):
    del B_x
    vm = pltpu.VMEM
    scratch = [
        vm((D, D), bf16), vm((D, D), bf16), vm((D, FF), bf16), vm((FF, D), bf16),
        vm((S + 16, D), bf16), vm((S, D), bf16), vm((D, S), bf16), vm((S, D), bf16),
        vm((4, D), bf16), vm((D,), bf16),
        vm((2, CB, CB), u32), vm((2, CB // 2, 2 * CB), u32),
        vm((5, 8, D), f32),
        vm((2, 2 * CB + 16, 128), f32),
        [vm((2 * H0, 128), f32)] * ND, [vm((NA, CB, 128), u32)] * ND,
        vm((S // 2, D), u32), vm((S, D), f32), vm((TM + R, D), f32), vm((TM + R, D), f32),
        vm((LG, TM + R, 128), f32), vm((24, D), f32),
        vm((TM, D), bf16), vm((TM, D), f32),
        pltpu.SMEM((4,), i32),
        pltpu.SemaphoreType.DMA((1 + NP12 + LG + 10,)),
    ]
    return pl.pallas_call(
        _kernel,
        out_shape=jax.ShapeDtypeStruct(A_q.shape, bf16),
        in_specs=[pl.BlockSpec(memory_space=pl.ANY)] * 10,
        out_specs=pl.BlockSpec(memory_space=pl.ANY),
        scratch_shapes=scratch,
        compiler_params=pltpu.CompilerParams(vmem_limit_bytes=116 * 1024 * 1024),
    )(A_q, A_k, A_v, A_shift_k.T, A_ssm_k, A_ssm_D, B_w1, B_w2, B_w3, B_w4)
```

```python
import math

import jax
import jax.numpy as jnp
from jax import lax
import jax.experimental.pallas as pl
import jax.experimental.pallas.tpu as pltpu


f32, bf16, u32, i32 = jnp.float32, jnp.bfloat16, jnp.uint32, jnp.int32

S, D, FF = 2048, 1024, 3584
TM = 256
NB = S // TM
G = 2 * NB
CB = 128
NA = S // CB
NO = 4
TF = 512
NC = FF // TF
R = 16
NS = TM // R
LG = D // 128
KR = 4
ND = 4
G1 = [0, 2, 5, 8]
G2 = [0, 3, 8]
NP12 = len(G1) + len(G2) - 2
EPS = 1e-5
CS = CB + 8
BS = 3 * CS
H0 = NA * BS + 16
C0 = math.sqrt(2.0 / math.pi)
C1 = C0 * 0.044715
SHIFTS = (1, 1, -1, -1, 2, 2, -2, -2)


def _ln_t(x):
    m = jnp.mean(x, axis=-1, keepdims=True)
    xc = x - m
    v = jnp.mean(xc * xc, axis=-1, keepdims=True)
    r = lax.rsqrt(v + EPS)
    n = x.shape[0]
    return xc * r, [[jnp.broadcast_to(m, (n, 128))], [jnp.broadcast_to(r, (n, 128))]]


def _gelu(x):
    hx = 0.5 * x
    return hx + hx * jnp.tanh(x * (C0 + C1 * (x * x)))


def _mm(a, b):
    return jnp.dot(a, b, preferred_element_type=f32)


def _tok(vals):
    t = None
    for v in vals:
        b = pltpu.bitcast(v, u32)
        for i in range(b.shape[0] // 8):
            for j in range(b.shape[1] // 128):
                p = b[i * 8:(i + 1) * 8, j * 128:(j + 1) * 128]
                t = p if t is None else t | p
    return t


def _pin_at(x, pins, zero):
    if not pins:
        return x
    out, last = [], 0
    for k in sorted({k for k, _ in pins}):
        if k * 16 > last:
            out.append(x[last:k * 16])
        blk = x[k * 16:(k + 1) * 16]
        for (kk, n), vals in pins.items():
            if kk != k:
                continue
            top = pltpu.bitcast(pltpu.bitcast(blk[:, n * 128:(n + 1) * 128], u32) | (_tok(vals) & zero), bf16)
            parts = ([blk[:, :n * 128]] if n > 0 else []) + [top] + (
                [blk[:, (n + 1) * 128:]] if (n + 1) * 128 < blk.shape[1] else [])
            blk = jnp.concatenate(parts, axis=1) if len(parts) > 1 else top
        out.append(blk)
        last = (k + 1) * 16
    if last < x.shape[0]:
        out.append(x[last:])
    return jnp.concatenate(out, axis=0) if len(out) > 1 else out[0]


def _spread(items, n):
    return [items[(i * len(items)) // n:((i + 1) * len(items)) // n] for i in range(n)]


def _kernel(q_hbm, k_hbm, v_hbm, sk_hbm, hk_hbm, dd_hbm, w1_hbm, w2_hbm, w3_hbm, w4_hbm,
            o_hbm,
            w1b, w2b, w3b, w4b, kbuf, vbuf, hkb, qbuf, skb, ddb,
            Fm, Gm, skf, kf, ZS, YS, ybuf, xbuf, x1b, ub, hwin, hcar, z3buf, accb,
            zsm, sem):
    obuf = vbuf

    def cp_kvh(c, r0, nr, si):
        ch = pl.ds(c * 128, 128)
        return (
            pltpu.make_async_copy(k_hbm.at[0, pl.ds(r0, nr), ch], kbuf.at[pl.ds(16 + r0, nr), ch], sem.at[si]),
            pltpu.make_async_copy(v_hbm.at[0, pl.ds(r0, nr), ch], vbuf.at[pl.ds(r0, nr), ch], sem.at[si]),
            pltpu.make_async_copy(hk_hbm.at[ch, pl.ds(r0, nr)], hkb.at[ch, pl.ds(r0, nr)], sem.at[si]))

    GP = {1: G1, 2: G2}

    def cp_g0(i):
        return cp_kvh(0, i * 2 * TM, 2 * TM, i)

    def cp_gp(c, n):
        return cp_kvh(c, GP[c][n] * TM, (GP[c][n + 1] - GP[c][n]) * TM, 4 + (c - 1) * (len(G1) - 1) + n)

    def cp_grp(c):
        return cp_kvh(c, 0, S, 1 + NP12 + c)

    SB = 1 + NP12 + LG

    def cp_q(r0, r1, si):
        return pltpu.make_async_copy(q_hbm.at[0, pl.ds(r0, r1 - r0), :],
                                     qbuf.at[pl.ds(r0, r1 - r0), :], sem.at[si])

    def cp_o(j, c0=0, nc=D):
        return pltpu.make_async_copy(obuf.at[pl.ds(j * TM, TM), pl.ds(c0, nc)],
                                     o_hbm.at[0, pl.ds(j * TM, TM), pl.ds(c0, nc)], sem.at[SB + 4])

    cp_sk = pltpu.make_async_copy(sk_hbm, skb, sem.at[SB])
    cp_dd = pltpu.make_async_copy(dd_hbm, ddb, sem.at[SB])
    cp_q0 = cp_q(0, 2 * TM + R, SB + 1)

    cp_q3 = cp_q(2 * TM + R, 3 * TM + R, SB + 7)
    cp_q4 = cp_q(3 * TM + R, S, SB + 3)

    cp_w1 = pltpu.make_async_copy(w1_hbm, w1b, sem.at[SB + 1])
    cp_w2 = pltpu.make_async_copy(w2_hbm, w2b, sem.at[SB + 8])
    def cp_w34(c0, c1, si):
        n = (c1 - c0) * TF
        return (pltpu.make_async_copy(w3_hbm.at[:, pl.ds(c0 * TF, n)], w3b.at[:, pl.ds(c0 * TF, n)], sem.at[si]),
                pltpu.make_async_copy(w4_hbm.at[pl.ds(c0 * TF, n), :], w4b.at[pl.ds(c0 * TF, n), :], sem.at[si]))

    WS = 2
    cp_w34a = cp_w34(0, WS, SB + 5)
    WB = 3
    cp_w34m = cp_w34(WS, WB, SB + 6)
    cp_w34b = cp_w34(WB, KR + 1, SB + 2)
    cp_w34c = cp_w34(KR + 1, NC, SB + 9)

    def wait_all(cps):
        for cp in cps:
            cp.wait()

    cp_sk.start()
    cp_dd.start()
    for grp in ([cp_g0(i) for i in range(4)] + [cp_gp(c, n) for c in (1, 2) for n in range(len(GP[c]) - 1)]
                + [cp_grp(c) for c in range(3, LG)]):
        for cp in grp:
            cp.start()
    for cp in (cp_q0, cp_w1, cp_w2) + cp_w34a + cp_w34m + cp_w34b + cp_w34c + (cp_q3, cp_q4):
        cp.start()

    zsm[0] = 0
    kbuf[0:16, :] = jnp.zeros((16, D), bf16)

    def _basis(pos, part, n):
        k = jnp.where(pos < CB // 2, 2 * pos, 2 * pos - (CB - 1))
        m = ((2 * k + 1) * n + part * CB) & (4 * CB - 1)
        r = m & (2 * CB - 1)
        neg = jnp.logical_xor(m >= 2 * CB, r > CB)
        th = jnp.minimum(r, 2 * CB - r).astype(f32) * (math.pi / (2 * CB))
        t2 = th * th
        z = 1.0 / math.factorial(12)
        for e in (10, 8, 6, 4, 2, 0):
            z = 1.0 / math.factorial(e) - t2 * z
        z = jnp.where(neg, -z, z)
        return z, jnp.where(pos < CB // 2, z, -z)

    def dft_init(t, carry):
        rf = lax.broadcasted_iota(i32, (32, CB), 0)
        zs = _basis(t * 16 + (rf & 15), rf >> 4, lax.broadcasted_iota(i32, (32, CB), 1))
        cg = lax.broadcasted_iota(i32, (16, 2 * CB), 1)
        gs = _basis(cg >> 1, cg & 1, t * 16 + lax.broadcasted_iota(i32, (16, 2 * CB), 0))
        for par in range(2):
            Fm[par, pl.ds(pl.multiple_of(t * 16, 16), 16), :] = pltpu.bitcast(zs[par].astype(bf16), u32)
            Gm[par, pl.ds(pl.multiple_of(t * 8, 8), 8), :] = pltpu.bitcast(
                (gs[par] * (1.0 / CB)).astype(bf16), u32)
        return carry

    lax.fori_loop(0, CB // 16, dft_init, 0)

    cp_sk.wait()
    cp_dd.wait()
    sk32 = skb[...].astype(f32)
    for t in range(4):
        skf[t] = jnp.broadcast_to(sk32[t:t + 1, :], (8, D))
    skf[4] = jnp.broadcast_to(ddb[...].astype(f32).reshape(1, D), (8, D))

    SET = [(c + LG - ND) % 2 for c in range(LG - ND + 2)] + list(range(2, ND))

    def zero_vec():
        return jnp.full((8, 128), zsm[0], i32).astype(u32)

    def bmul(x, row8):
        n = x.shape[0] // 8
        return (x.reshape(n, 8, 128) * row8[None]).reshape(x.shape)

    def dsl(start, size, align):
        return pl.ds(start if isinstance(start, int) else pl.multiple_of(start, align), size)

    def unil(z):
        return (jnp.concatenate([z[32 * g:32 * g + 16] for g in range(CB // 16)], axis=0),
                jnp.concatenate([z[32 * g + 16:32 * g + 32] for g in range(CB // 16)], axis=0))

    def fwdh1(c, par, i, o, pins=None, skip=True):
        Z = ZS[par].at[dsl(H0 + i * 2 * BS, 2 * BS, 8), :]
        ls = dsl(c * 128, 128, 128)
        a = 2 * i + o
        hh = lax.dot_general(_pin_at(pltpu.bitcast(Fm[o], bf16), pins, zero_vec()), hkb[ls, dsl(a * CB, CB, CB)], (((1,), (1,)), ((), ())),
                             preferred_element_type=f32)
        cc, dd = unil(hh)
        if o == 0 and skip and (not isinstance(i, int) or i == 0):
            d8 = skf[4, :, ls] if isinstance(i, int) else jnp.where(i == 0, skf[4, :, ls], 0.0)
            cc = (cc.reshape(CB // 8, 8, 128) + d8[None]).reshape(CB, 128)
        b = o * BS
        Z[b:b + CB, :] = cc
        Z[b + CS:b + CS + CB, :] = dd - cc
        Z[b + 2 * CS:b + 2 * CS + CB, :] = cc + dd
        return cc + dd

    def fwdx1(c, par, i, o, pins, sk, slot=0):
        Z = ZS[par].at[dsl(i * 2 * BS, 2 * BS, 8), :]
        ls = dsl(c * 128, 128, 128)
        ks_ = i % 2 if isinstance(i, int) else slot
        if o == 0:
            kf[ks_] = kbuf[dsl(i * 2 * CB, 2 * CB + 16, 16), ls].astype(f32)
        a = 2 * i + o
        b0 = 16 + o * CB
        ks = bmul(kf[ks_, b0:b0 + CB, :], sk[0])
        for t in range(1, 4):
            ks = ks + bmul(kf[ks_, b0 - t:b0 - t + CB, :], sk[t])
        kv = (ks * vbuf[dsl(a * CB, CB, CB), ls].astype(f32)).astype(bf16)
        xh = _mm(_pin_at(pltpu.bitcast(Fm[o], bf16), pins, zero_vec()), kv)
        xr, xm = unil(xh)
        b = o * BS
        Z[b:b + CB, :] = xr
        Z[b + CS:b + CS + CB, :] = xm
        Z[b + 2 * CS:b + 2 * CS + CB, :] = xr + xm
        return xr + xm

    def mac_part(par, i, h, a0, st, NO=NO):
        Z, Y = ZS[par], YS[par]
        Z = Z.at[dsl(i * 16, 2 * H0 - CB + 16, 16), :]

        def ld(base, a):
            b = base + a * BS + h * 8
            return tuple(Z[b + k * CS:b + k * CS + 8, :] for k in range(3))
        K = [None] * NO
        hw = {}
        for ap in range(a0 + NO):
            xa, xb, xs = ld(0, ap)
            for o in range(NO):
                dl = a0 + o - ap
                if dl < 0:
                    continue
                if dl not in hw:
                    hw[dl] = ld(H0, dl)
                hc, he, hf = hw[dl]
                t = (hc * xs, xa * he, xb * hf)
                K[o] = t if K[o] is None else tuple(u + w for u, w in zip(K[o], t))
                inj = yield K[o][2]
                if inj is not None:
                    K[o] = (K[o][0], K[o][1], K[o][2] + inj)
        st['w'] = []
        for o in range(NO):
            re, im = K[o][0] - K[o][2], K[o][0] + K[o][1]
            prev = st.get('y')
            out = (re, im) if prev is None else (re - prev[1], im + prev[0])
            st['y'] = (re, im)
            st['w'].append(pltpu.pack_elementwise(list(out), packed_dtype=bf16).astype(u32))
            Y[a0 + o, dsl(i * 16 + h * 8, 8, 8), :] = st['w'][-1]

    def mac_gen(par, i0, ns, parts, sts):
        for u in range(ns):
            for a0 in parts:
                for h in range(2):
                    yield from mac_part(par, i0 + u, h, a0, sts.setdefault((u, h), {}))

    def inv1(c, par, i, o, pins=None):
        Y = YS[par]
        a = 2 * i + o
        y = _mm(_pin_at(pltpu.bitcast(Gm[o], bf16), pins, zero_vec()), pltpu.bitcast(Y[a], bf16))
        yv = ybuf.at[dsl(a * (CB // 2), CB // 2, CB // 2), :]
        for g in range(CB // 16):
            yv[8 * g:8 * g + 8, dsl(c * 128, 128, 128)] = pltpu.pack_elementwise(
                [y[16 * g:16 * g + 8], y[16 * g + 8:16 * g + 16]], packed_dtype=bf16).astype(u32)
        return y

    def group(c, sets, do_inv, do_fwd, i0=0, ns=NA // 2, parts=(0, 4, 8, 12), cfg=None, ninv=NA // 2):
        PI, P0, DP, NP_, R0, DR, G0 = cfg or (-20, 12, 12, 16, 220, 12, 4)
        NPM = sum(2 * (NO * a0 + 10) for a0 in parts)
        names = ('h0', 'x0', 'h1', 'x1')
        zero = zero_vec()
        sk = [skf[t, :, dsl((c + 1) * 128, 128, 128)] for t in range(4)] if do_fwd else None
        sts = {}
        pprev, par, pnext = sets
        gen = mac_gen(par, i0, ns, parts, sts)
        rec = [next(gen)]
        inj = {}
        for u in range(ns):
            i = i0 + u
            base = u * NPM
            while len(rec) <= base + P0 + (NP_ - 1) * DP:
                rec.append(gen.send(inj.get(len(rec))))
            pins = {k: {} for k in ('i0', 'i1', 'h0', 'h1', 'x0', 'x1')}
            if base + PI >= 0:
                pins['i0'][(0, 0)] = [rec[base + PI]]
                pins['i1'][(0, 0)] = [rec[base + PI]]
            for n in range(NP_):
                r = ((n + 1) * 16) // NP_ - 1
                pins[names[n % len(names)]][(r, 0)] = [rec[base + P0 + n * DP]]
            if do_inv and i < ninv:
                ys = [inv1(c - 1, pprev, i, 0, pins['i0']), inv1(c - 1, pprev, i, 1, pins['i1'])]
                if not do_fwd:
                    inj[base + R0] = pltpu.bitcast(_tok([y[CB - 8:CB] for y in ys]) & zero, f32)
            if do_fwd:
                res = [fwdh1(c + 1, pnext, i, 0, pins['h0'], skip=(u == 0)),
                       fwdh1(c + 1, pnext, i, 1, pins['h1']),
                       fwdx1(c + 1, pnext, i, 0, pins['x0'], sk, slot=u % 2),
                       fwdx1(c + 1, pnext, i, 1, pins['x1'], sk, slot=u % 2)]
                for g in range(G0, CB // 16):
                    tk = _tok([z[16 * g + 8:16 * g + 16] for z in res]) & zero
                    inj[base + R0 + (g - G0) * DR] = pltpu.bitcast(tk, f32)
        try:
            while True:
                rec.append(gen.send(inj.get(len(rec))))
        except StopIteration:
            pass
        return sts

    late = {}
    NI7 = 2

    def conv():
        def pre(i, carry):
            wait_all(cp_g0(i))
            sk = [skf[t, :, 0:128] for t in range(4)]
            for u in range(2):
                for o in range(2):
                    fwdh1(0, SET[0], 2 * i + u, o, skip=(u == 0))
                for o in range(2):
                    fwdx1(0, SET[0], 2 * i + u, o, None, sk, slot=u)
            return carry
        lax.fori_loop(0, NA // 4, pre, 0)

        def sets(c):
            return (SET[c - 1], SET[c], SET[c + 1] if c + 1 < LG else None)

        for c in range(2):
            for t in range(len(GP[c + 1]) - 1):
                wait_all(cp_gp(c + 1, t))
                group(c, sets(c), c > 0, True, GP[c + 1][t], GP[c + 1][t + 1] - GP[c + 1][t])
        for c in range(2, LG - ND):
            wait_all(cp_grp(c + 1))
            group(c, sets(c), True, True)
        for c in range(LG - ND, LG - 1):
            wait_all(cp_grp(c + 1))
            late[c] = group(c, sets(c), True, True, parts=(0, 4), ninv=NA // (2 if c == LG - ND else 4),
                            cfg=(-30, -6, 5, 16, 68, 1, 5))
        late[LG - 1] = group(LG - 1, sets(LG - 1), True, False, parts=(0, 4), ninv=NI7,
                             cfg=(-10, 0, 0, 1, 40, 0, 0))

    def mark(i, carry):
        zsm[1 + i] = i
        return carry

    conv()

    def rows(j):
        return j * TM if isinstance(j, int) else pl.multiple_of(j * TM, TM)

    def delay(x, after):
        if after is None:
            return x
        z8 = pltpu.bitcast(_tok([after]) & zero_vec(), f32)
        x0 = (x[:, 0:128].reshape(x.shape[0] // 8, 8, 128) + z8[None]).reshape(x.shape[0], 128)
        return jnp.concatenate([x0, x[:, 128:]], axis=1)

    def s0_rows(j, s0, ns, slot, from_q, after=None):
        r = rows(j)
        sl = slice(s0 * R, (s0 + ns) * R)
        x = qbuf.at[pl.ds(r, TM), :][sl, :].astype(f32)
        if from_q is not True:
            x = jnp.where(from_q, x, xbuf.at[pl.ds(r, TM), :][sl, :])
        x = delay(x, after)
        r2 = j * (TM // 2) if isinstance(j, int) else pl.multiple_of(j * (TM // 2), TM // 2)
        yw = ybuf.at[pl.ds(r2, TM // 2), :][s0 * 8:(s0 + ns) * 8, :]
        yy = [pltpu.unpack_elementwise(yw, index=k, packed_dtype=bf16, unpacked_dtype=f32)
              for k in range(2)]
        y = jnp.concatenate([yy[k][s * 8:(s + 1) * 8] for s in range(ns) for k in range(2)], axis=0)
        if ns == 1:
            zs, aft = [], None
            for hh in range(2):
                xh = delay(x[8 * hh:8 * hh + 8], aft)
                q, t1 = _ln_t(xh)
                x1 = xh + q * y[8 * hh:8 * hh + 8]
                u, t2 = _ln_t(x1)
                x1b[slot * R + 8 * hh:slot * R + 8 * hh + 8, :] = x1
                ub[slot * R + 8 * hh:slot * R + 8 * hh + 8, :] = u
                z, t3 = _ln_t(u)
                zs.append(z)
                ts = t1 + t2 + t3 + [[z[:, D - 128:]]]
                aft = ts[1][0][0:8]
            return jnp.concatenate(zs, axis=0).astype(bf16), ts
        q, t1 = _ln_t(x)
        x1 = x + q * y
        u, t2 = _ln_t(x1)
        x1b[slot * R:(slot + ns) * R, :] = x1
        ub[slot * R:(slot + ns) * R, :] = u
        z, t3 = _ln_t(u)
        return z.astype(bf16), t1 + t2 + t3 + [[z[:, D - 128:]]]

    rot = [0]

    def rhs_pins(steps, ksteps):
        pins = {}
        for t, lst in enumerate(steps):
            n, kg = t // ksteps, t % ksteps
            for i, vals in enumerate(lst):
                m = rot[0] % 4
                rot[0] += 1
                rg = 7 if (i % 2 == 0 and len(lst) > 1) else 0
                pins.setdefault(((kg * 4 + m) * 8 + rg, n), []).extend(vals)
        return pins

    def at_steps(toks, first, last, nsteps):
        steps = [[] for _ in range(nsteps)]
        for k, t in enumerate(toks):
            steps[first + (k * (last - first)) // max(len(toks) - 1, 1)].append(t)
        return steps

    def pinned(w, steps):
        return w if steps is None else _pin_at(w, rhs_pins(steps, 2), zero_vec())

    def put_h(row0, h):
        for l in range(LG):
            hwin[l, row0:row0 + h.shape[0], :] = h[:, l * 128:(l + 1) * 128]

    def m2_dot(r0, nr, steps=None):
        hs_in = jnp.concatenate(
            [hwin[l, 8 + r0 - SHIFTS[l]:8 + r0 - SHIFTS[l] + nr, :].astype(bf16) for l in range(LG)], axis=1)
        return _mm(hs_in, pinned(w2b[...], steps))

    def ln3(hs, lo, ns, after=None):
        sl = slice(lo * R, (lo + ns) * R)
        x1p = delay(ub[sl, :], after) + hs
        z, t = _ln_t(x1p)
        z3buf[sl, :] = z.astype(bf16)
        return x1b[sl, :] + x1p, [z[:, D - 128:]]

    def mlp(c0, c1, acc, side=None, z3=None, pre=None):
        z3 = z3buf[...] if z3 is None else z3
        zero = zero_vec()
        steps = [[] for _ in range(16 * NC)]
        for c in range(c0, c1):
            if pre is not None:
                pre(c, steps)
            w3 = _pin_at(w3b[:, c * TF:(c + 1) * TF], rhs_pins(steps[16 * c:16 * c + 8], 2), zero)
            a = _gelu(_mm(z3, w3))
            if side is not None:
                side(c, a, steps)
            a = a.astype(bf16)
            w4 = _pin_at(w4b[c * TF:(c + 1) * TF, :], rhs_pins(steps[16 * c + 8:16 * c + 16], 1), zero)
            acc = acc + _mm(a, w4)
        return acc

    def s0_side(b, grp=None, bars=()):
        RT, D0, DD, CH = (0, 2, 2, 1)
        DL = -1
        grp = (grp or _spread(list(range(NS)), KR)) + [[]] * NC
        if isinstance(b, int):
            blk, fq = (b % NB, (b + 1) % NB), (b < NB, b + 1 < NB)
        else:
            blk, fq = (lax.rem(b, NB), lax.rem(b + 1, NB)), (b < NB, b + 1 < NB)

        def side(c, a, steps):
            if c == 0:
                x1b[0:R, :] = x1b[TM:TM + R, :]
                ub[0:R, :] = ub[TM:TM + R, :]
            after = a[0:8, RT * 128:(RT + 1) * 128]
            for n, s in enumerate(grp[c]):
                last = s == NS - 1
                z, t = s0_rows(blk[last], 0 if last else s + 1, 1, s + 1, fq[last], after)
                side.zs.append(z)
                after = t[CH][0][0:8] if CH >= 0 else None
                steps[min(16 * c + 8 + D0 + n * DD, 16 * (c + 1) - 1 if c + 1 in bars else 16 * KR + DL)].append(t[-1])
        side.zs = []
        return side

    def toks(zs):
        return [t for _, ts in zs for t in ts]

    def cat(zs):
        return jnp.concatenate([z for z, _ in zs], axis=0)

    LNO = 2
    pend = [(par, u, h, a0) for u in range(NA // 2) for h in range(2)
            for a0 in range(8, NA, LNO) for par in range(LG - ND, LG)]

    def late_piece():
        par, u, h, a0 = pend.pop(0)
        for _ in mac_part(SET[par], u, h, a0, late[par][(u, h)], LNO):
            pass
        return list(late[par][(u, h)]['w'])

    NPA, NPB = 8, 8

    def prologue():
        cp_q0.wait()
        cp_w1.wait()
        F1, L1_ = (2, 15)
        HM = TM // 2
        for a in range(3):
            inv1(LG - 1, SET[LG - 1], a // 2, a % 2)
        za = [s0_rows(0, 0, 8, 0, True)]
        for a in range(2 * NI7, NA // 2):
            inv1(LG - 2, SET[LG - 2], a // 2, a % 2)
        for a in range(3, NA // 2):
            inv1(LG - 1, SET[LG - 1], a // 2, a % 2)
        zb = [s0_rows(0, 8, 4, 8, True), s0_rows(0, 12, 4, 12, True), s0_rows(1, 0, 1, 16, True)]
        for l in range(LG):
            hwin[l, 0:8, :] = jnp.zeros((8, 128), f32)
        put_h(8, _gelu(_mm(cat(za), pinned(w1b[...], at_steps(toks(zb[:2]) + [zb[2][1][-1]], F1, L1_, 16)))))
        h = _gelu(_mm(cat(zb), pinned(w1b[...], at_steps([late_piece() for _ in range(NPA)], 1, 15, 16))))
        put_h(8 + HM, h[0:HM + 8])
        hcar[...] = h[HM + R - 24:HM + R]

    def prologue2():
        HM = TM // 2
        cp_w2.wait()
        hs0 = m2_dot(0, HM, at_steps([late_piece() for _ in range(NPB)], 2, 15, 16))
        l0 = [ln3(hs0[n * 32:(n + 1) * 32], 2 * n, 2) for n in range(4)]
        hs1 = m2_dot(HM, HM, at_steps([t for _, t in l0], 3, 14, 16))
        l1 = [ln3(hs1[n * 32:(n + 1) * 32], 8 + 2 * n, 2) for n in range(4)]
        wait_all(cp_w34a)
        st['s0'] = s0_side(1, bars=(WS, WB))
        LA, LZ = (1, 126)
        skip = (16 * WS, 16 * WB, 16 * (KR + 2))
        slots = [t for t in range(LA, LZ + 1) if t not in skip]
        st['due'] = [slots[(k * len(slots)) // len(pend)] for k in range(len(pend))]

        def side(c, a, steps):
            st['s0'](c, a, steps)
            run_late(16 * c + 8, 16 * c + 16, steps)

        def pre(c, steps):
            if c == WS:
                wait_all(cp_w34m)
            if c == WB:
                lax.fori_loop(0, 2, mark, 0)
                wait_all(cp_w34b)
            run_late(16 * c, 16 * c + 8, steps)
        st['z3'] = z3buf[...]
        st['acc'] = mlp(0, KR, jnp.concatenate([r for r, _ in l0 + l1], axis=0), side, st['z3'], pre)

    st = {}

    def run_late(lo, hi, steps, off=0):
        while pend and lo <= st['due'][0] < hi:
            steps[st['due'].pop(0) - off].append(late_piece())

    def late_steps(lo):
        steps = [[] for _ in range(16)]
        run_late(lo, lo + 16, steps, lo)
        return steps

    def second_half(b, acc, z3, z1, first):
        RT, D0, DD = (0, 0, 1)
        jb = b % NB if first else lax.rem(b, NB)
        if first:
            def mk(off):
                return (lambda c, a, steps: run_late(16 * c + 8 + off, 16 * c + 16 + off, steps, off),
                        lambda c, steps: run_late(16 * c + off, 16 * c + 8 + off, steps, off))
        else:
            def mk(off):
                return None, None
        sd, pr = mk(0)
        acc = mlp(KR, KR + 1, acc, sd, z3, pr)
        top = hcar[...]
        put_h(0, top[0:8] if first else jnp.where(jb == 0, 0.0, top[0:8]))
        put_h(8, top[8:24])
        h = _gelu(_mm(z1, pinned(w1b[...], late_steps(16 * (KR + 1)) if first else None)))
        put_h(24, h[0:TM - R])
        put_h(8 + TM, h[TM - R:TM - 8] if first else jnp.where(jb == NB - 1, 0.0, h[TM - R:TM - 8]))
        hcar[...] = h[TM - 24:TM]
        if first:
            wait_all(cp_w34c)
        sd, pr = mk(16)
        acc = mlp(KR + 1, KR + 2, acc, sd, z3, pr)
        hs = m2_dot(0, TM, late_steps(16 * (KR + 3)) if first else None)
        if first:
            for par in late:
                for a in range(NA // 2, NA):
                    inv1(par, SET[par], a // 2, a % 2)
        rs = []

        def side(c, a, steps):
            for n in range(NS):
                r_, t = ln3(hs[n * R:(n + 1) * R], n, 1,
                            a[0:8, RT * 128:(RT + 1) * 128] if (n == 0 and RT >= 0) else None)
                rs.append(r_)
                steps[min(16 * c + 8 + D0 + (n * DD) // 2, 16 * NC - 1)].append(t)
        xn = mlp(KR + 2, NC, acc, side, z3)
        jg = (b - 1) % NB if first else lax.rem(b - 1, NB)
        xbuf[pl.ds(rows(jg), TM), :] = xn
        if not first:
            obuf[pl.ds(rows(jg), TM), :] = xn.astype(bf16)
        accb[...] = jnp.concatenate(rs, axis=0)

    prologue()
    lax.fori_loop(0, 2, mark, 0)
    prologue2()
    second_half(1, st['acc'], st['z3'], jnp.concatenate(st['s0'].zs, axis=0), True)
    cp_q3.wait()

    def body(b, carry):
        @pl.when(b == 2)
        def _():
            cp_q4.wait()
        rot[0] = 2
        z3 = z3buf[...]
        sd = s0_side(b + 1)
        acc = mlp(0, KR, accb[...], sd, z3)
        second_half(b + 1, acc, z3, jnp.concatenate(sd.zs, axis=0), False)

        @pl.when(b >= NB)
        def _():
            cp_o(b - NB).start()
        return carry

    lax.fori_loop(1, G - 1, body, 0)

    OC = [0] + [512, 896] + [D]
    OS = tuple((OC[i], OC[i + 1] - OC[i]) for i in range(len(OC) - 1))
    acc = mlp(0, NC - 1, accb[...])
    a = _gelu(_mm(z3buf[...], w3b[:, FF - TF:])).astype(bf16)
    for c0, nc in OS:
        obuf[S - TM:, c0:c0 + nc] = (acc[:, c0:c0 + nc] + _mm(a, w4b[FF - TF:, c0:c0 + nc])).astype(bf16)
        cp_o(NB - 1, c0, nc).start()
    for j in range(NB - 1):
        cp_o(j).wait()
    for c0, nc in OS:
        cp_o(NB - 1, c0, nc).wait()


@jax.jit
def pallas_interleave_layers__ssm_conv_h3__mixer_s_mlp__prompt_kernel(
    A_q: jax.Array,
    A_k: jax.Array,
    A_v: jax.Array,
    A_shift_k: jax.Array,
    A_ssm_k: jax.Array,
    A_ssm_D: jax.Array,
    B_x: jax.Array,
    B_w1: jax.Array,
    B_w2: jax.Array,
    B_w3: jax.Array,
    B_w4: jax.Array,
):
    del B_x
    vm = pltpu.VMEM
    scratch = [
        vm((D, D), bf16), vm((D, D), bf16), vm((D, FF), bf16), vm((FF, D), bf16),
        vm((S + 16, D), bf16), vm((S, D), bf16), vm((D, S), bf16), vm((S, D), bf16),
        vm((4, D), bf16), vm((D,), bf16),
        vm((2, CB, CB), u32), vm((2, CB // 2, 2 * CB), u32),
        vm((5, 8, D), f32),
        vm((2, 2 * CB + 16, 128), f32),
        [vm((2 * H0, 128), f32)] * ND, [vm((NA, CB, 128), u32)] * ND,
        vm((S // 2, D), u32), vm((S, D), f32), vm((TM + R, D), f32), vm((TM + R, D), f32),
        vm((LG, TM + R, 128), f32), vm((24, D), f32),
        vm((TM, D), bf16), vm((TM, D), f32),
        pltpu.SMEM((4,), i32),
        pltpu.SemaphoreType.DMA((1 + NP12 + LG + 10,)),
    ]
    return pl.pallas_call(
        _kernel,
        out_shape=jax.ShapeDtypeStruct(A_q.shape, bf16),
        in_specs=[pl.BlockSpec(memory_space=pl.ANY)] * 10,
        out_specs=pl.BlockSpec(memory_space=pl.ANY),
        scratch_shapes=scratch,
        compiler_params=pltpu.CompilerParams(vmem_limit_bytes=116 * 1024 * 1024),
    )(A_q, A_k, A_v, A_shift_k.T, A_ssm_k, A_ssm_D, B_w1, B_w2, B_w3, B_w4)
```

```python
import math

import jax
import jax.numpy as jnp
from jax import lax
import jax.experimental.pallas as pl
import jax.experimental.pallas.tpu as pltpu


f32, bf16, u32, i32 = jnp.float32, jnp.bfloat16, jnp.uint32, jnp.int32

S, D, FF = 2048, 1024, 3584
TM = 256
NB = S // TM
G = 2 * NB
CB = 128
NA = S // CB
NO = 4
TF = 512
NC = FF // TF
R = 16
NS = TM // R
LG = D // 128
KR = 4
ND = 4
G1 = [0, 2, 5, 8]
G2 = [0, 3, 8]
NP12 = len(G1) + len(G2) - 2
EPS = 1e-5
CS = CB + 8
BS = 3 * CS
H0 = NA * BS + 16
C0 = math.sqrt(2.0 / math.pi)
C1 = C0 * 0.044715
SHIFTS = (1, 1, -1, -1, 2, 2, -2, -2)


def _ln_t(x):
    m = jnp.mean(x, axis=-1, keepdims=True)
    xc = x - m
    v = jnp.mean(xc * xc, axis=-1, keepdims=True)
    r = lax.rsqrt(v + EPS)
    n = x.shape[0]
    return xc * r, [[jnp.broadcast_to(m, (n, 128))], [jnp.broadcast_to(r, (n, 128))]]


def _gelu(x):
    hx = 0.5 * x
    return hx + hx * jnp.tanh(x * (C0 + C1 * (x * x)))


def _mm(a, b):
    return jnp.dot(a, b, preferred_element_type=f32)


def _tok(vals):
    t = None
    for v in vals:
        b = pltpu.bitcast(v, u32)
        for i in range(b.shape[0] // 8):
            for j in range(b.shape[1] // 128):
                p = b[i * 8:(i + 1) * 8, j * 128:(j + 1) * 128]
                t = p if t is None else t | p
    return t


def _pin_at(x, pins, zero):
    if not pins:
        return x
    out, last = [], 0
    for k in sorted({k for k, _ in pins}):
        if k * 16 > last:
            out.append(x[last:k * 16])
        blk = x[k * 16:(k + 1) * 16]
        for (kk, n), vals in pins.items():
            if kk != k:
                continue
            top = pltpu.bitcast(pltpu.bitcast(blk[:, n * 128:(n + 1) * 128], u32) | (_tok(vals) & zero), bf16)
            parts = ([blk[:, :n * 128]] if n > 0 else []) + [top] + (
                [blk[:, (n + 1) * 128:]] if (n + 1) * 128 < blk.shape[1] else [])
            blk = jnp.concatenate(parts, axis=1) if len(parts) > 1 else top
        out.append(blk)
        last = (k + 1) * 16
    if last < x.shape[0]:
        out.append(x[last:])
    return jnp.concatenate(out, axis=0) if len(out) > 1 else out[0]


def _spread(items, n):
    return [items[(i * len(items)) // n:((i + 1) * len(items)) // n] for i in range(n)]


def _kernel(q_hbm, k_hbm, v_hbm, sk_hbm, hk_hbm, dd_hbm, w1_hbm, w2_hbm, w3_hbm, w4_hbm,
            o_hbm,
            w1b, w2b, w3b, w4b, kbuf, vbuf, hkb, qbuf, skb, ddb,
            Fm, Gm, skf, kf, ZS, YS, ybuf, xbuf, x1b, ub, hwin, hcar, z3buf, accb,
            zsm, sem):
    obuf = vbuf

    def cp_kvh(c, r0, nr, si):
        ch = pl.ds(c * 128, 128)
        return (
            pltpu.make_async_copy(k_hbm.at[0, pl.ds(r0, nr), ch], kbuf.at[pl.ds(16 + r0, nr), ch], sem.at[si]),
            pltpu.make_async_copy(v_hbm.at[0, pl.ds(r0, nr), ch], vbuf.at[pl.ds(r0, nr), ch], sem.at[si]),
            pltpu.make_async_copy(hk_hbm.at[ch, pl.ds(r0, nr)], hkb.at[ch, pl.ds(r0, nr)], sem.at[si]))

    GP = {1: G1, 2: G2}

    def cp_g0(i):
        return cp_kvh(0, i * 2 * TM, 2 * TM, i)

    def cp_gp(c, n):
        return cp_kvh(c, GP[c][n] * TM, (GP[c][n + 1] - GP[c][n]) * TM, 4 + (c - 1) * (len(G1) - 1) + n)

    def cp_grp(c):
        return cp_kvh(c, 0, S, 1 + NP12 + c)

    SB = 1 + NP12 + LG

    def cp_q(r0, r1, si):
        return pltpu.make_async_copy(q_hbm.at[0, pl.ds(r0, r1 - r0), :],
                                     qbuf.at[pl.ds(r0, r1 - r0), :], sem.at[si])

    def cp_o(j, c0=0, nc=D):
        return pltpu.make_async_copy(obuf.at[pl.ds(j * TM, TM), pl.ds(c0, nc)],
                                     o_hbm.at[0, pl.ds(j * TM, TM), pl.ds(c0, nc)], sem.at[SB + 4])

    cp_sk = pltpu.make_async_copy(sk_hbm, skb, sem.at[SB])
    cp_dd = pltpu.make_async_copy(dd_hbm, ddb, sem.at[SB])
    cp_q0 = cp_q(0, 2 * TM + R, SB + 1)

    cp_q1 = cp_q(2 * TM + R, S, SB + 3)

    cp_w1 = pltpu.make_async_copy(w1_hbm, w1b, sem.at[SB + 1])
    cp_w2 = pltpu.make_async_copy(w2_hbm, w2b, sem.at[SB + 8])
    def cp_w34(c0, c1, si):
        n = (c1 - c0) * TF
        return (pltpu.make_async_copy(w3_hbm.at[:, pl.ds(c0 * TF, n)], w3b.at[:, pl.ds(c0 * TF, n)], sem.at[si]),
                pltpu.make_async_copy(w4_hbm.at[pl.ds(c0 * TF, n), :], w4b.at[pl.ds(c0 * TF, n), :], sem.at[si]))

    WS = 2
    cp_w34a = cp_w34(0, WS, SB + 5)
    WB = 3
    cp_w34m = cp_w34(WS, WB, SB + 6)
    cp_w34b = cp_w34(WB, KR + 1, SB + 2)
    cp_w34c = cp_w34(KR + 1, NC, SB + 7)

    def wait_all(cps):
        for cp in cps:
            cp.wait()

    cp_sk.start()
    cp_dd.start()
    for grp in ([cp_g0(i) for i in range(4)] + [cp_gp(c, n) for c in (1, 2) for n in range(len(GP[c]) - 1)]
                + [cp_grp(c) for c in range(3, LG)]):
        for cp in grp:
            cp.start()
    for cp in (cp_q0, cp_w1, cp_w2) + cp_w34a + cp_w34m + cp_w34b + cp_w34c + (cp_q1,):
        cp.start()

    zsm[0] = 0
    kbuf[0:16, :] = jnp.zeros((16, D), bf16)

    def _basis(pos, part, n):
        k = jnp.where(pos < CB // 2, 2 * pos, 2 * pos - (CB - 1))
        m = ((2 * k + 1) * n + part * CB) & (4 * CB - 1)
        r = m & (2 * CB - 1)
        neg = jnp.logical_xor(m >= 2 * CB, r > CB)
        th = jnp.minimum(r, 2 * CB - r).astype(f32) * (math.pi / (2 * CB))
        t2 = th * th
        z = 1.0 / math.factorial(12)
        for e in (10, 8, 6, 4, 2, 0):
            z = 1.0 / math.factorial(e) - t2 * z
        z = jnp.where(neg, -z, z)
        return z, jnp.where(pos < CB // 2, z, -z)

    def dft_init(t, carry):
        rf = lax.broadcasted_iota(i32, (32, CB), 0)
        zs = _basis(t * 16 + (rf & 15), rf >> 4, lax.broadcasted_iota(i32, (32, CB), 1))
        cg = lax.broadcasted_iota(i32, (16, 2 * CB), 1)
        gs = _basis(cg >> 1, cg & 1, t * 16 + lax.broadcasted_iota(i32, (16, 2 * CB), 0))
        for par in range(2):
            Fm[par, pl.ds(pl.multiple_of(t * 16, 16), 16), :] = pltpu.bitcast(zs[par].astype(bf16), u32)
            Gm[par, pl.ds(pl.multiple_of(t * 8, 8), 8), :] = pltpu.bitcast(
                (gs[par] * (1.0 / CB)).astype(bf16), u32)
        return carry

    lax.fori_loop(0, CB // 16, dft_init, 0)

    cp_sk.wait()
    cp_dd.wait()
    sk32 = skb[...].astype(f32)
    for t in range(4):
        skf[t] = jnp.broadcast_to(sk32[t:t + 1, :], (8, D))
    skf[4] = jnp.broadcast_to(ddb[...].astype(f32).reshape(1, D), (8, D))

    SET = [(c + LG - ND) % 2 for c in range(LG - ND + 2)] + list(range(2, ND))

    def zero_vec():
        return jnp.full((8, 128), zsm[0], i32).astype(u32)

    def bmul(x, row8):
        n = x.shape[0] // 8
        return (x.reshape(n, 8, 128) * row8[None]).reshape(x.shape)

    def dsl(start, size, align):
        return pl.ds(start if isinstance(start, int) else pl.multiple_of(start, align), size)

    def unil(z):
        return (jnp.concatenate([z[32 * g:32 * g + 16] for g in range(CB // 16)], axis=0),
                jnp.concatenate([z[32 * g + 16:32 * g + 32] for g in range(CB // 16)], axis=0))

    def fwdh1(c, par, i, o, pins=None, skip=True):
        Z = ZS[par].at[dsl(H0 + i * 2 * BS, 2 * BS, 8), :]
        ls = dsl(c * 128, 128, 128)
        a = 2 * i + o
        hh = lax.dot_general(_pin_at(pltpu.bitcast(Fm[o], bf16), pins, zero_vec()), hkb[ls, dsl(a * CB, CB, CB)], (((1,), (1,)), ((), ())),
                             preferred_element_type=f32)
        cc, dd = unil(hh)
        if o == 0 and skip and (not isinstance(i, int) or i == 0):
            d8 = skf[4, :, ls] if isinstance(i, int) else jnp.where(i == 0, skf[4, :, ls], 0.0)
            cc = (cc.reshape(CB // 8, 8, 128) + d8[None]).reshape(CB, 128)
        b = o * BS
        Z[b:b + CB, :] = cc
        Z[b + CS:b + CS + CB, :] = dd - cc
        Z[b + 2 * CS:b + 2 * CS + CB, :] = cc + dd
        return cc + dd

    def fwdx1(c, par, i, o, pins, sk, slot=0):
        Z = ZS[par].at[dsl(i * 2 * BS, 2 * BS, 8), :]
        ls = dsl(c * 128, 128, 128)
        ks_ = i % 2 if isinstance(i, int) else slot
        if o == 0:
            kf[ks_] = kbuf[dsl(i * 2 * CB, 2 * CB + 16, 16), ls].astype(f32)
        a = 2 * i + o
        b0 = 16 + o * CB
        ks = bmul(kf[ks_, b0:b0 + CB, :], sk[0])
        for t in range(1, 4):
            ks = ks + bmul(kf[ks_, b0 - t:b0 - t + CB, :], sk[t])
        kv = (ks * vbuf[dsl(a * CB, CB, CB), ls].astype(f32)).astype(bf16)
        xh = _mm(_pin_at(pltpu.bitcast(Fm[o], bf16), pins, zero_vec()), kv)
        xr, xm = unil(xh)
        b = o * BS
        Z[b:b + CB, :] = xr
        Z[b + CS:b + CS + CB, :] = xm
        Z[b + 2 * CS:b + 2 * CS + CB, :] = xr + xm
        return xr + xm

    def mac_part(par, i, h, a0, st, NO=NO):
        Z, Y = ZS[par], YS[par]
        Z = Z.at[dsl(i * 16, 2 * H0 - CB + 16, 16), :]

        def ld(base, a):
            b = base + a * BS + h * 8
            return tuple(Z[b + k * CS:b + k * CS + 8, :] for k in range(3))
        K = [None] * NO
        hw = {}
        for ap in range(a0 + NO):
            xa, xb, xs = ld(0, ap)
            for o in range(NO):
                dl = a0 + o - ap
                if dl < 0:
                    continue
                if dl not in hw:
                    hw[dl] = ld(H0, dl)
                hc, he, hf = hw[dl]
                t = (hc * xs, xa * he, xb * hf)
                K[o] = t if K[o] is None else tuple(u + w for u, w in zip(K[o], t))
                inj = yield K[o][2]
                if inj is not None:
                    K[o] = (K[o][0], K[o][1], K[o][2] + inj)
        st['w'] = []
        for o in range(NO):
            re, im = K[o][0] - K[o][2], K[o][0] + K[o][1]
            prev = st.get('y')
            out = (re, im) if prev is None else (re - prev[1], im + prev[0])
            st['y'] = (re, im)
            st['w'].append(pltpu.pack_elementwise(list(out), packed_dtype=bf16).astype(u32))
            Y[a0 + o, dsl(i * 16 + h * 8, 8, 8), :] = st['w'][-1]

    def mac_gen(par, i0, ns, parts, sts):
        for u in range(ns):
            for a0 in parts:
                for h in range(2):
                    yield from mac_part(par, i0 + u, h, a0, sts.setdefault((u, h), {}))

    def inv1(c, par, i, o, pins=None):
        Y = YS[par]
        a = 2 * i + o
        y = _mm(_pin_at(pltpu.bitcast(Gm[o], bf16), pins, zero_vec()), pltpu.bitcast(Y[a], bf16))
        yv = ybuf.at[dsl(a * (CB // 2), CB // 2, CB // 2), :]
        for g in range(CB // 16):
            yv[8 * g:8 * g + 8, dsl(c * 128, 128, 128)] = pltpu.pack_elementwise(
                [y[16 * g:16 * g + 8], y[16 * g + 8:16 * g + 16]], packed_dtype=bf16).astype(u32)
        return y

    def group(c, sets, do_inv, do_fwd, i0=0, ns=NA // 2, parts=(0, 4, 8, 12), cfg=None, ninv=NA // 2):
        PI, P0, DP, NP_, R0, DR, G0 = cfg or (-20, 12, 12, 16, 220, 12, 4)
        NPM = sum(2 * (NO * a0 + 10) for a0 in parts)
        names = ('h0', 'x0', 'h1', 'x1')
        zero = zero_vec()
        sk = [skf[t, :, dsl((c + 1) * 128, 128, 128)] for t in range(4)] if do_fwd else None
        sts = {}
        pprev, par, pnext = sets
        gen = mac_gen(par, i0, ns, parts, sts)
        rec = [next(gen)]
        inj = {}
        for u in range(ns):
            i = i0 + u
            base = u * NPM
            while len(rec) <= base + P0 + (NP_ - 1) * DP:
                rec.append(gen.send(inj.get(len(rec))))
            pins = {k: {} for k in ('i0', 'i1', 'h0', 'h1', 'x0', 'x1')}
            if base + PI >= 0:
                pins['i0'][(0, 0)] = [rec[base + PI]]
                pins['i1'][(0, 0)] = [rec[base + PI]]
            for n in range(NP_):
                r = ((n + 1) * 16) // NP_ - 1
                pins[names[n % len(names)]][(r, 0)] = [rec[base + P0 + n * DP]]
            if do_inv and i < ninv:
                ys = [inv1(c - 1, pprev, i, 0, pins['i0']), inv1(c - 1, pprev, i, 1, pins['i1'])]
                if not do_fwd:
                    inj[base + R0] = pltpu.bitcast(_tok([y[CB - 8:CB] for y in ys]) & zero, f32)
            if do_fwd:
                res = [fwdh1(c + 1, pnext, i, 0, pins['h0'], skip=(u == 0)),
                       fwdh1(c + 1, pnext, i, 1, pins['h1']),
                       fwdx1(c + 1, pnext, i, 0, pins['x0'], sk, slot=u % 2),
                       fwdx1(c + 1, pnext, i, 1, pins['x1'], sk, slot=u % 2)]
                for g in range(G0, CB // 16):
                    tk = _tok([z[16 * g + 8:16 * g + 16] for z in res]) & zero
                    inj[base + R0 + (g - G0) * DR] = pltpu.bitcast(tk, f32)
        try:
            while True:
                rec.append(gen.send(inj.get(len(rec))))
        except StopIteration:
            pass
        return sts

    late = {}
    NI7 = 2

    def conv():
        def pre(i, carry):
            wait_all(cp_g0(i))
            sk = [skf[t, :, 0:128] for t in range(4)]
            for u in range(2):
                for o in range(2):
                    fwdh1(0, SET[0], 2 * i + u, o, skip=(u == 0))
                for o in range(2):
                    fwdx1(0, SET[0], 2 * i + u, o, None, sk, slot=u)
            return carry
        lax.fori_loop(0, NA // 4, pre, 0)

        def sets(c):
            return (SET[c - 1], SET[c], SET[c + 1] if c + 1 < LG else None)

        for c in range(2):
            for t in range(len(GP[c + 1]) - 1):
                wait_all(cp_gp(c + 1, t))
                group(c, sets(c), c > 0, True, GP[c + 1][t], GP[c + 1][t + 1] - GP[c + 1][t])
        for c in range(2, LG - ND):
            wait_all(cp_grp(c + 1))
            group(c, sets(c), True, True)
        for c in range(LG - ND, LG - 1):
            wait_all(cp_grp(c + 1))
            late[c] = group(c, sets(c), True, True, parts=(0, 4), ninv=NA // (2 if c == LG - ND else 4),
                            cfg=(-30, -6, 5, 16, 68, 1, 5))
        late[LG - 1] = group(LG - 1, sets(LG - 1), True, False, parts=(0, 4), ninv=NI7,
                             cfg=(-10, 0, 0, 1, 40, 0, 0))

    def mark(i, carry):
        zsm[1 + i] = i
        return carry

    conv()

    def rows(j):
        return j * TM if isinstance(j, int) else pl.multiple_of(j * TM, TM)

    def delay(x, after):
        if after is None:
            return x
        z8 = pltpu.bitcast(_tok([after]) & zero_vec(), f32)
        x0 = (x[:, 0:128].reshape(x.shape[0] // 8, 8, 128) + z8[None]).reshape(x.shape[0], 128)
        return jnp.concatenate([x0, x[:, 128:]], axis=1)

    def s0_rows(j, s0, ns, slot, from_q, after=None):
        r = rows(j)
        sl = slice(s0 * R, (s0 + ns) * R)
        if isinstance(j, int):
            x = qbuf[r + s0 * R:r + (s0 + ns) * R, :].astype(f32)
        else:
            x = qbuf.at[pl.ds(r, TM), :][sl, :].astype(f32)
        if from_q is not True:
            x = jnp.where(from_q, x, xbuf.at[pl.ds(r, TM), :][sl, :])
        x = delay(x, after)
        r2 = j * (TM // 2) if isinstance(j, int) else pl.multiple_of(j * (TM // 2), TM // 2)
        yw = ybuf.at[pl.ds(r2, TM // 2), :][s0 * 8:(s0 + ns) * 8, :]
        yy = [pltpu.unpack_elementwise(yw, index=k, packed_dtype=bf16, unpacked_dtype=f32)
              for k in range(2)]
        y = jnp.concatenate([yy[k][s * 8:(s + 1) * 8] for s in range(ns) for k in range(2)], axis=0)
        if ns == 1:
            zs, aft = [], None
            for hh in range(2):
                xh = delay(x[8 * hh:8 * hh + 8], aft)
                q, t1 = _ln_t(xh)
                x1 = xh + q * y[8 * hh:8 * hh + 8]
                u, t2 = _ln_t(x1)
                x1b[slot * R + 8 * hh:slot * R + 8 * hh + 8, :] = x1
                ub[slot * R + 8 * hh:slot * R + 8 * hh + 8, :] = u
                z, t3 = _ln_t(u)
                zs.append(z)
                ts = t1 + t2 + t3 + [[z[:, D - 128:]]]
                aft = ts[1][0][0:8]
            return jnp.concatenate(zs, axis=0).astype(bf16), ts
        q, t1 = _ln_t(x)
        x1 = x + q * y
        u, t2 = _ln_t(x1)
        x1b[slot * R:(slot + ns) * R, :] = x1
        ub[slot * R:(slot + ns) * R, :] = u
        z, t3 = _ln_t(u)
        return z.astype(bf16), t1 + t2 + t3 + [[z[:, D - 128:]]]

    rot = [0]

    def rhs_pins(steps, ksteps):
        pins = {}
        for t, lst in enumerate(steps):
            n, kg = t // ksteps, t % ksteps
            for i, vals in enumerate(lst):
                m = rot[0] % 4
                rot[0] += 1
                rg = 7 if (i % 2 == 0 and len(lst) > 1) else 0
                pins.setdefault(((kg * 4 + m) * 8 + rg, n), []).extend(vals)
        return pins

    def at_steps(toks, first, last, nsteps):
        steps = [[] for _ in range(nsteps)]
        for k, t in enumerate(toks):
            steps[first + (k * (last - first)) // max(len(toks) - 1, 1)].append(t)
        return steps

    def pinned(w, steps):
        return w if steps is None else _pin_at(w, rhs_pins(steps, 2), zero_vec())

    def put_h(row0, h):
        for l in range(LG):
            hwin[l, row0:row0 + h.shape[0], :] = h[:, l * 128:(l + 1) * 128]

    def m2_dot(r0, nr, steps=None):
        hs_in = jnp.concatenate(
            [hwin[l, 8 + r0 - SHIFTS[l]:8 + r0 - SHIFTS[l] + nr, :].astype(bf16) for l in range(LG)], axis=1)
        return _mm(hs_in, pinned(w2b[...], steps))

    def ln3(hs, lo, ns, after=None):
        sl = slice(lo * R, (lo + ns) * R)
        x1p = delay(ub[sl, :], after) + hs
        z, t = _ln_t(x1p)
        z3buf[sl, :] = z.astype(bf16)
        return x1b[sl, :] + x1p, [z[:, D - 128:]]

    def mlp(c0, c1, acc, side=None, z3=None, pre=None):
        z3 = z3buf[...] if z3 is None else z3
        zero = zero_vec()
        steps = [[] for _ in range(16 * NC)]
        for c in range(c0, c1):
            if pre is not None:
                pre(c, steps)
            w3 = _pin_at(w3b[:, c * TF:(c + 1) * TF], rhs_pins(steps[16 * c:16 * c + 8], 2), zero)
            a = _gelu(_mm(z3, w3))
            if side is not None:
                side(c, a, steps)
            a = a.astype(bf16)
            w4 = _pin_at(w4b[c * TF:(c + 1) * TF, :], rhs_pins(steps[16 * c + 8:16 * c + 16], 1), zero)
            acc = acc + _mm(a, w4)
        return acc

    def s0_side(b, grp=None, bars=()):
        RT, D0, DD, CH = (0, 2, 2, 1)
        DL = -1
        grp = (grp or _spread(list(range(NS)), KR)) + [[]] * NC
        if isinstance(b, int):
            blk, fq = (b % NB, (b + 1) % NB), (b < NB, b + 1 < NB)
        else:
            blk, fq = (lax.rem(b, NB), lax.rem(b + 1, NB)), (b < NB, b + 1 < NB)

        def side(c, a, steps):
            if c == 0:
                x1b[0:R, :] = x1b[TM:TM + R, :]
                ub[0:R, :] = ub[TM:TM + R, :]
            after = a[0:8, RT * 128:(RT + 1) * 128]
            for n, s in enumerate(grp[c]):
                last = s == NS - 1
                z, t = s0_rows(blk[last], 0 if last else s + 1, 1, s + 1, fq[last], after)
                side.zs.append(z)
                after = t[CH][0][0:8] if CH >= 0 else None
                steps[min(16 * c + 8 + D0 + n * DD, 16 * (c + 1) - 1 if c + 1 in bars else 16 * KR + DL)].append(t[-1])
        side.zs = []
        return side

    def toks(zs):
        return [t for _, ts in zs for t in ts]

    def cat(zs):
        return jnp.concatenate([z for z, _ in zs], axis=0)

    LNO = 2
    pend = [(par, u, h, a0) for u in range(NA // 2) for h in range(2)
            for a0 in range(8, NA, LNO) for par in range(LG - ND, LG)]

    def late_piece():
        par, u, h, a0 = pend.pop(0)
        for _ in mac_part(SET[par], u, h, a0, late[par][(u, h)], LNO):
            pass
        return list(late[par][(u, h)]['w'])

    NPA, NPB = 8, 8

    def prologue():
        cp_q0.wait()
        cp_w1.wait()
        F1, L1_ = (2, 15)
        HM = TM // 2
        for a in range(3):
            inv1(LG - 1, SET[LG - 1], a // 2, a % 2)
        za = [s0_rows(0, 0, 8, 0, True)]
        for a in range(2 * NI7, NA // 2):
            inv1(LG - 2, SET[LG - 2], a // 2, a % 2)
        for a in range(3, NA // 2):
            inv1(LG - 1, SET[LG - 1], a // 2, a % 2)
        zb = [s0_rows(0, 8, 4, 8, True), s0_rows(0, 12, 4, 12, True), s0_rows(1, 0, 1, 16, True)]
        for l in range(LG):
            hwin[l, 0:8, :] = jnp.zeros((8, 128), f32)
        put_h(8, _gelu(_mm(cat(za), pinned(w1b[...], at_steps(toks(zb[:2]) + [zb[2][1][-1]], F1, L1_, 16)))))
        h = _gelu(_mm(cat(zb), pinned(w1b[...], at_steps([late_piece() for _ in range(NPA)], 1, 15, 16))))
        put_h(8 + HM, h[0:HM + 8])
        hcar[...] = h[HM + R - 24:HM + R]

    def prologue2():
        HM = TM // 2
        cp_w2.wait()
        hs0 = m2_dot(0, HM, at_steps([late_piece() for _ in range(NPB)], 2, 15, 16))
        l0 = [ln3(hs0[n * 32:(n + 1) * 32], 2 * n, 2) for n in range(4)]
        hs1 = m2_dot(HM, HM, at_steps([t for _, t in l0], 3, 14, 16))
        l1 = [ln3(hs1[n * 32:(n + 1) * 32], 8 + 2 * n, 2) for n in range(4)]
        wait_all(cp_w34a)
        st['s0'] = s0_side(1, bars=(WS, WB))
        LA, LZ = (1, 126)
        skip = (16 * WS, 16 * WB, 16 * (KR + 2))
        slots = [t for t in range(LA, LZ + 1) if t not in skip]
        st['due'] = [slots[(k * len(slots)) // len(pend)] for k in range(len(pend))]

        def side(c, a, steps):
            st['s0'](c, a, steps)
            run_late(16 * c + 8, 16 * c + 16, steps)

        def pre(c, steps):
            if c == WS:
                wait_all(cp_w34m)
            if c == WB:
                lax.fori_loop(0, 2, mark, 0)
                wait_all(cp_w34b)
            run_late(16 * c, 16 * c + 8, steps)
        st['z3'] = z3buf[...]
        st['acc'] = mlp(0, KR, jnp.concatenate([r for r, _ in l0 + l1], axis=0), side, st['z3'], pre)

    st = {}

    def run_late(lo, hi, steps, off=0):
        while pend and lo <= st['due'][0] < hi:
            steps[st['due'].pop(0) - off].append(late_piece())

    def late_steps(lo):
        steps = [[] for _ in range(16)]
        run_late(lo, lo + 16, steps, lo)
        return steps

    def second_half(b, acc, z3, z1, first):
        RT, D0, DD = (0, 0, 1)
        jb = b % NB if first else lax.rem(b, NB)
        if first:
            def mk(off):
                return (lambda c, a, steps: run_late(16 * c + 8 + off, 16 * c + 16 + off, steps, off),
                        lambda c, steps: run_late(16 * c + off, 16 * c + 8 + off, steps, off))
        else:
            def mk(off):
                return None, None
        sd, pr = mk(0)
        acc = mlp(KR, KR + 1, acc, sd, z3, pr)
        top = hcar[...]
        put_h(0, top[0:8] if first else jnp.where(jb == 0, 0.0, top[0:8]))
        put_h(8, top[8:24])
        h = _gelu(_mm(z1, pinned(w1b[...], late_steps(16 * (KR + 1)) if first else None)))
        put_h(24, h[0:TM - R])
        put_h(8 + TM, h[TM - R:TM - 8] if first else jnp.where(jb == NB - 1, 0.0, h[TM - R:TM - 8]))
        hcar[...] = h[TM - 24:TM]
        if first:
            wait_all(cp_w34c)
        sd, pr = mk(16)
        acc = mlp(KR + 1, KR + 2, acc, sd, z3, pr)
        hs = m2_dot(0, TM, late_steps(16 * (KR + 3)) if first else None)
        if first:
            for par in late:
                for a in range(NA // 2, NA):
                    inv1(par, SET[par], a // 2, a % 2)
        rs = []

        def side(c, a, steps):
            for n in range(NS):
                r_, t = ln3(hs[n * R:(n + 1) * R], n, 1,
                            a[0:8, RT * 128:(RT + 1) * 128] if (n == 0 and RT >= 0) else None)
                rs.append(r_)
                steps[min(16 * c + 8 + D0 + (n * DD) // 2, 16 * NC - 1)].append(t)
        xn = mlp(KR + 2, NC, acc, side, z3)
        jg = (b - 1) % NB if first else lax.rem(b - 1, NB)
        xbuf[pl.ds(rows(jg), TM), :] = xn
        if not first:
            obuf[pl.ds(rows(jg), TM), :] = xn.astype(bf16)
        accb[...] = jnp.concatenate(rs, axis=0)

    prologue()
    lax.fori_loop(0, 2, mark, 0)
    prologue2()
    second_half(1, st['acc'], st['z3'], jnp.concatenate(st['s0'].zs, axis=0), True)
    cp_q1.wait()

    def body(b, carry):
        rot[0] = 2
        z3 = z3buf[...]
        sd = s0_side(b + 1)
        acc = mlp(0, KR, accb[...], sd, z3)
        second_half(b + 1, acc, z3, jnp.concatenate(sd.zs, axis=0), False)

        @pl.when(b >= NB)
        def _():
            cp_o(b - NB).start()
        return carry

    lax.fori_loop(1, G - 1, body, 0)

    OC = [0] + [512, 896] + [D]
    OS = tuple((OC[i], OC[i + 1] - OC[i]) for i in range(len(OC) - 1))
    acc = mlp(0, NC - 1, accb[...])
    a = _gelu(_mm(z3buf[...], w3b[:, FF - TF:])).astype(bf16)
    for c0, nc in OS:
        obuf[S - TM:, c0:c0 + nc] = (acc[:, c0:c0 + nc] + _mm(a, w4b[FF - TF:, c0:c0 + nc])).astype(bf16)
        cp_o(NB - 1, c0, nc).start()
    for j in range(NB - 1):
        cp_o(j).wait()
    for c0, nc in OS:
        cp_o(NB - 1, c0, nc).wait()


@jax.jit
def pallas_interleave_layers__ssm_conv_h3__mixer_s_mlp__prompt_kernel(
    A_q: jax.Array,
    A_k: jax.Array,
    A_v: jax.Array,
    A_shift_k: jax.Array,
    A_ssm_k: jax.Array,
    A_ssm_D: jax.Array,
    B_x: jax.Array,
    B_w1: jax.Array,
    B_w2: jax.Array,
    B_w3: jax.Array,
    B_w4: jax.Array,
):
    del B_x
    vm = pltpu.VMEM
    scratch = [
        vm((D, D), bf16), vm((D, D), bf16), vm((D, FF), bf16), vm((FF, D), bf16),
        vm((S + 16, D), bf16), vm((S, D), bf16), vm((D, S), bf16), vm((S, D), bf16),
        vm((4, D), bf16), vm((D,), bf16),
        vm((2, CB, CB), u32), vm((2, CB // 2, 2 * CB), u32),
        vm((5, 8, D), f32),
        vm((2, 2 * CB + 16, 128), f32),
        [vm((2 * H0, 128), f32)] * ND, [vm((NA, CB, 128), u32)] * ND,
        vm((S // 2, D), u32), vm((S, D), f32), vm((TM + R, D), f32), vm((TM + R, D), f32),
        vm((LG, TM + R, 128), f32), vm((24, D), f32),
        vm((TM, D), bf16), vm((TM, D), f32),
        pltpu.SMEM((4,), i32),
        pltpu.SemaphoreType.DMA((1 + NP12 + LG + 9,)),
    ]
    return pl.pallas_call(
        _kernel,
        out_shape=jax.ShapeDtypeStruct(A_q.shape, bf16),
        in_specs=[pl.BlockSpec(memory_space=pl.ANY)] * 10,
        out_specs=pl.BlockSpec(memory_space=pl.ANY),
        scratch_shapes=scratch,
        compiler_params=pltpu.CompilerParams(vmem_limit_bytes=116 * 1024 * 1024),
    )(A_q, A_k, A_v, A_shift_k.T, A_ssm_k, A_ssm_D, B_w1, B_w2, B_w3, B_w4)
```

```python
import math

import jax
import jax.numpy as jnp
from jax import lax
import jax.experimental.pallas as pl
import jax.experimental.pallas.tpu as pltpu


f32, bf16, u32, i32 = jnp.float32, jnp.bfloat16, jnp.uint32, jnp.int32

S, D, FF = 2048, 1024, 3584
TM = 256
NB = S // TM
G = 2 * NB
CB = 128
NA = S // CB
NO = 4
TF = 512
NC = FF // TF
R = 16
NS = TM // R
LG = D // 128
KR = 4
ND = 4
G1 = [0, 2, 5, 8]
G2 = [0, 3, 8]
NP12 = len(G1) + len(G2) - 2
EPS = 1e-5
BS = 3 * CB + 8
H0 = NA * BS + 16
C0 = math.sqrt(2.0 / math.pi)
C1 = C0 * 0.044715
SHIFTS = (1, 1, -1, -1, 2, 2, -2, -2)


def _ln_t(x):
    m = jnp.mean(x, axis=-1, keepdims=True)
    xc = x - m
    v = jnp.mean(xc * xc, axis=-1, keepdims=True)
    r = lax.rsqrt(v + EPS)
    n = x.shape[0]
    return xc * r, [[jnp.broadcast_to(m, (n, 128))], [jnp.broadcast_to(r, (n, 128))]]


def _gelu(x):
    hx = 0.5 * x
    return hx + hx * jnp.tanh(x * (C0 + C1 * (x * x)))


def _mm(a, b):
    return jnp.dot(a, b, preferred_element_type=f32)


def _tok(vals):
    t = None
    for v in vals:
        b = v if v.dtype == u32 else pltpu.bitcast(v, u32)
        if b.shape == (8, 128):
            t = b if t is None else t | b
            continue
        for i in range(b.shape[0] // 8):
            for j in range(b.shape[1] // 128):
                p = b[i * 8:(i + 1) * 8, j * 128:(j + 1) * 128]
                t = p if t is None else t | p
    return t


def _pin_at(x, pins, zero):
    if not pins:
        return x
    out, last = [], 0
    for k in sorted({k for k, _ in pins}):
        if k * 16 > last:
            out.append(x[last:k * 16])
        blk = x[k * 16:(k + 1) * 16]
        for (kk, n), vals in pins.items():
            if kk != k:
                continue
            top = pltpu.bitcast(pltpu.bitcast(blk[:, n * 128:(n + 1) * 128], u32) | (_tok(vals) & zero), bf16)
            parts = ([blk[:, :n * 128]] if n > 0 else []) + [top] + (
                [blk[:, (n + 1) * 128:]] if (n + 1) * 128 < blk.shape[1] else [])
            blk = jnp.concatenate(parts, axis=1) if len(parts) > 1 else top
        out.append(blk)
        last = (k + 1) * 16
    if last < x.shape[0]:
        out.append(x[last:])
    return jnp.concatenate(out, axis=0) if len(out) > 1 else out[0]


def _spread(items, n):
    return [items[(i * len(items)) // n:((i + 1) * len(items)) // n] for i in range(n)]


def _kernel(q_hbm, k_hbm, v_hbm, sk_hbm, hk_hbm, dd_hbm, w1_hbm, w2_hbm, w3_hbm, w4_hbm,
            o_hbm,
            w1b, w2b, w3b, w4b, kbuf, vbuf, hkb, qbuf, skb, ddb,
            Fm, Gm, skf, kf, ZS, YS, ybuf, xbuf, x1b, ub, hwin, hcar, z3buf, accb,
            zsm, sem):
    obuf = vbuf

    def cp_kvh(c, r0, nr, si):
        ch = pl.ds(c * 128, 128)
        return (
            pltpu.make_async_copy(k_hbm.at[0, pl.ds(r0, nr), ch], kbuf.at[pl.ds(16 + r0, nr), ch], sem.at[si]),
            pltpu.make_async_copy(v_hbm.at[0, pl.ds(r0, nr), ch], vbuf.at[pl.ds(r0, nr), ch], sem.at[si]),
            pltpu.make_async_copy(hk_hbm.at[ch, pl.ds(r0, nr)], hkb.at[ch, pl.ds(r0, nr)], sem.at[si]))

    GP = {1: G1, 2: G2}

    def cp_g0(i):
        return cp_kvh(0, i * 2 * TM, 2 * TM, i)

    def cp_gp(c, n):
        return cp_kvh(c, GP[c][n] * TM, (GP[c][n + 1] - GP[c][n]) * TM, 4 + (c - 1) * (len(G1) - 1) + n)

    def cp_grp(c):
        return cp_kvh(c, 0, S, 1 + NP12 + c)

    SB = 1 + NP12 + LG

    def cp_q(r0, r1, si):
        return pltpu.make_async_copy(q_hbm.at[0, pl.ds(r0, r1 - r0), :],
                                     qbuf.at[pl.ds(r0, r1 - r0), :], sem.at[si])

    def cp_o(j, c0=0, nc=D):
        return pltpu.make_async_copy(obuf.at[pl.ds(j * TM, TM), pl.ds(c0, nc)],
                                     o_hbm.at[0, pl.ds(j * TM, TM), pl.ds(c0, nc)], sem.at[SB + 4])

    cp_sk = pltpu.make_async_copy(sk_hbm, skb, sem.at[SB])
    cp_dd = pltpu.make_async_copy(dd_hbm, ddb, sem.at[SB])
    cp_q0 = cp_q(0, 2 * TM + R, SB + 1)

    cp_q1 = cp_q(2 * TM + R, S, SB + 3)

    cp_w1 = pltpu.make_async_copy(w1_hbm, w1b, sem.at[SB + 1])
    cp_w2 = pltpu.make_async_copy(w2_hbm, w2b, sem.at[SB + 8])
    def cp_w34(c0, c1, si):
        n = (c1 - c0) * TF
        return (pltpu.make_async_copy(w3_hbm.at[:, pl.ds(c0 * TF, n)], w3b.at[:, pl.ds(c0 * TF, n)], sem.at[si]),
                pltpu.make_async_copy(w4_hbm.at[pl.ds(c0 * TF, n), :], w4b.at[pl.ds(c0 * TF, n), :], sem.at[si]))

    WS = 2
    cp_w34a = cp_w34(0, WS, SB + 5)
    WB = 3
    cp_w34m = cp_w34(WS, WB, SB + 6)
    cp_w34b = cp_w34(WB, KR + 1, SB + 2)
    cp_w34c = cp_w34(KR + 1, NC, SB + 7)

    def wait_all(cps):
        for cp in cps:
            cp.wait()

    cp_sk.start()
    cp_dd.start()
    for grp in ([cp_g0(i) for i in range(4)] + [cp_gp(c, n) for c in (1, 2) for n in range(len(GP[c]) - 1)]
                + [cp_grp(c) for c in range(3, LG)]):
        for cp in grp:
            cp.start()
    for cp in (cp_q0, cp_w1, cp_w2) + cp_w34a + cp_w34m + cp_w34b + cp_w34c + (cp_q1,):
        cp.start()

    zsm[0] = 0
    kbuf[0:16, :] = jnp.zeros((16, D), bf16)

    def _basis(pos, part, n):
        k = jnp.where(pos < CB // 2, 2 * pos, 2 * pos - (CB - 1))
        m = ((2 * k + 1) * n + part * CB) & (4 * CB - 1)
        r = m & (2 * CB - 1)
        neg = jnp.logical_xor(m >= 2 * CB, r > CB)
        th = jnp.minimum(r, 2 * CB - r).astype(f32) * (math.pi / (2 * CB))
        t2 = th * th
        z = 1.0 / math.factorial(12)
        for e in (10, 8, 6, 4, 2, 0):
            z = 1.0 / math.factorial(e) - t2 * z
        z = jnp.where(neg, -z, z)
        return z, jnp.where(pos < CB // 2, z, -z)

    def dft_init(t, carry):
        rf = lax.broadcasted_iota(i32, (32, CB), 0)
        zs = _basis(t * 16 + (rf & 15), rf >> 4, lax.broadcasted_iota(i32, (32, CB), 1))
        cg = lax.broadcasted_iota(i32, (16, 2 * CB), 1)
        gs = _basis(cg >> 1, cg & 1, t * 16 + lax.broadcasted_iota(i32, (16, 2 * CB), 0))
        for par in range(2):
            Fm[par, pl.ds(pl.multiple_of(t * 16, 16), 16), :] = pltpu.bitcast(zs[par].astype(bf16), u32)
            Gm[par, pl.ds(pl.multiple_of(t * 8, 8), 8), :] = pltpu.bitcast(
                (gs[par] * (1.0 / CB)).astype(bf16), u32)
        return carry

    lax.fori_loop(0, CB // 16, dft_init, 0)

    cp_sk.wait()
    cp_dd.wait()
    sk32 = skb[...].astype(f32)
    for t in range(4):
        skf[t] = jnp.broadcast_to(sk32[t:t + 1, :], (8, D))
    skf[4] = jnp.broadcast_to(ddb[...].astype(f32).reshape(1, D), (8, D))

    SET = [(c + LG - ND) % 2 for c in range(LG - ND + 2)] + list(range(2, ND))

    def zero_vec():
        return jnp.full((8, 128), zsm[0], i32).astype(u32)

    def bmul(x, row8):
        n = x.shape[0] // 8
        return (x.reshape(n, 8, 128) * row8[None]).reshape(x.shape)

    def dsl(start, size, align):
        return pl.ds(start if isinstance(start, int) else pl.multiple_of(start, align), size)

    def unil(z):
        z = z.reshape(CB // 16, 32, 128)
        return z[:, 0:16].reshape(CB, 128), z[:, 16:32].reshape(CB, 128)

    def il3(*comps):
        return jnp.concatenate([z.reshape(CB // 8, 8, 128) for z in comps], axis=1).reshape(3 * CB, 128)

    def fwdh1(c, par, i, o, pins=None, skip=True):
        Z = ZS[par].at[dsl(H0 + i * 2 * BS, 2 * BS, 8), :]
        ls = dsl(c * 128, 128, 128)
        a = 2 * i + o
        hh = lax.dot_general(_pin_at(pltpu.bitcast(Fm[o], bf16), pins, zero_vec()), hkb[ls, dsl(a * CB, CB, CB)], (((1,), (1,)), ((), ())),
                             preferred_element_type=f32)
        cc, dd = unil(hh)
        if o == 0 and skip and (not isinstance(i, int) or i == 0):
            d8 = skf[4, :, ls] if isinstance(i, int) else jnp.where(i == 0, skf[4, :, ls], 0.0)
            cc = (cc.reshape(CB // 8, 8, 128) + d8[None]).reshape(CB, 128)
        ff = cc + dd
        Z[o * BS:o * BS + 3 * CB, :] = il3(cc, dd - cc, ff)
        return ff

    def fwdx1(c, par, i, o, pins, sk, slot=0):
        Z = ZS[par].at[dsl(i * 2 * BS, 2 * BS, 8), :]
        ls = dsl(c * 128, 128, 128)
        ks_ = i % 2 if isinstance(i, int) else slot
        if o == 0:
            kf[ks_] = kbuf[dsl(i * 2 * CB, 2 * CB + 16, 16), ls].astype(f32)
        a = 2 * i + o
        b0 = 16 + o * CB
        ks = bmul(kf[ks_, b0:b0 + CB, :], sk[0])
        for t in range(1, 4):
            ks = ks + bmul(kf[ks_, b0 - t:b0 - t + CB, :], sk[t])
        kv = (ks * vbuf[dsl(a * CB, CB, CB), ls].astype(f32)).astype(bf16)
        xh = _mm(_pin_at(pltpu.bitcast(Fm[o], bf16), pins, zero_vec()), kv)
        xr, xm = unil(xh)
        xs = xr + xm
        Z[o * BS:o * BS + 3 * CB, :] = il3(xs, xr, xm)
        return xs

    def mac_part(par, i, h, a0, st, NO=NO):
        Z, Y = ZS[par], YS[par]
        p0 = (2 * i + h) * 24

        def ld(base, a):
            return Z[base + a * BS + p0:base + a * BS + p0 + 24, :]
        K = [None] * NO
        hw = {}
        for ap in range(a0 + NO):
            x = ld(0, ap)
            for o in range(NO):
                dl = a0 + o - ap
                if dl < 0:
                    continue
                if dl not in hw:
                    hw[dl] = ld(H0, dl)
                t = hw[dl] * x
                K[o] = t if K[o] is None else K[o] + t
                inj = yield K[o]
                if inj is not None:
                    K[o] = jnp.concatenate([K[o][0:16], K[o][16:24] + inj], axis=0)
        st['w'] = []
        for o in range(NO):
            k1 = K[o][0:8]
            re, im = k1 - K[o][16:24], k1 + K[o][8:16]
            prev = st.get('y')
            out = (re, im) if prev is None else (re - prev[1], im + prev[0])
            st['y'] = (re, im)
            st['w'].append(pltpu.pack_elementwise(list(out), packed_dtype=bf16).astype(u32))
            Y[a0 + o, dsl(i * 16 + h * 8, 8, 8), :] = st['w'][-1]

    def mac_gen(par, i0, ns, parts, sts):
        for u in range(ns):
            for a0 in parts:
                for h in range(2):
                    yield from mac_part(par, i0 + u, h, a0, sts.setdefault((u, h), {}))

    def inv1(c, par, i, o, pins=None):
        Y = YS[par]
        a = 2 * i + o
        y = _mm(_pin_at(pltpu.bitcast(Gm[o], bf16), pins, zero_vec()), pltpu.bitcast(Y[a], bf16))
        y3 = y.reshape(CB // 16, 16, 128)
        ybuf[a * (CB // 2):(a + 1) * (CB // 2), c * 128:(c + 1) * 128] = pltpu.pack_elementwise(
            [y3[:, 0:8].reshape(CB // 2, 128), y3[:, 8:16].reshape(CB // 2, 128)], packed_dtype=bf16).astype(u32)
        return y

    def group(c, sets, do_inv, do_fwd, i0=0, ns=NA // 2, parts=(0, 4, 8, 12), cfg=None, ninv=NA // 2):
        PI, P0, DP, NP_, R0, DR, G0 = cfg or (-20, 12, 12, 16, 220, 12, 4)
        NPM = sum(2 * (NO * a0 + 10) for a0 in parts)
        names = ('h0', 'x0', 'h1', 'x1')
        zero = zero_vec()
        sk = [skf[t, :, dsl((c + 1) * 128, 128, 128)] for t in range(4)] if do_fwd else None
        sts = {}
        pprev, par, pnext = sets
        gen = mac_gen(par, i0, ns, parts, sts)
        rec = [next(gen)]
        inj = {}
        for u in range(ns):
            i = i0 + u
            base = u * NPM
            while len(rec) <= base + P0 + (NP_ - 1) * DP:
                rec.append(gen.send(inj.get(len(rec))))
            pins = {k: {} for k in ('i0', 'i1', 'h0', 'h1', 'x0', 'x1')}
            if base + PI >= 0:
                pins['i0'][(0, 0)] = [rec[base + PI][16:24]]
                pins['i1'][(0, 0)] = pins['i0'][(0, 0)]
            for n in range(NP_):
                r = ((n + 1) * 16) // NP_ - 1
                pins[names[n % len(names)]][(r, 0)] = [rec[base + P0 + n * DP][16:24]]
            if do_inv and i < ninv:
                ys = [inv1(c - 1, pprev, i, 0, pins['i0']), inv1(c - 1, pprev, i, 1, pins['i1'])]
                if not do_fwd:
                    inj[base + R0] = pltpu.bitcast(_tok([y[CB - 8:CB] for y in ys]) & zero, f32)
            if do_fwd:
                res = [fwdh1(c + 1, pnext, i, 0, pins['h0'], skip=(u == 0)),
                       fwdh1(c + 1, pnext, i, 1, pins['h1']),
                       fwdx1(c + 1, pnext, i, 0, pins['x0'], sk, slot=u % 2),
                       fwdx1(c + 1, pnext, i, 1, pins['x1'], sk, slot=u % 2)]
                for g in range(G0, CB // 16):
                    tk = _tok([z[16 * g + 8:16 * g + 16] for z in res]) & zero
                    inj[base + R0 + (g - G0) * DR] = pltpu.bitcast(tk, f32)
        try:
            while True:
                rec.append(gen.send(inj.get(len(rec))))
        except StopIteration:
            pass
        return sts

    late = {}
    NI7 = 2

    def conv():
        def pre(i, carry):
            wait_all(cp_g0(i))
            sk = [skf[t, :, 0:128] for t in range(4)]
            for u in range(2):
                for o in range(2):
                    fwdh1(0, SET[0], 2 * i + u, o, skip=(u == 0))
                for o in range(2):
                    fwdx1(0, SET[0], 2 * i + u, o, None, sk, slot=u)
            return carry
        lax.fori_loop(0, NA // 4, pre, 0)

        def sets(c):
            return (SET[c - 1], SET[c], SET[c + 1] if c + 1 < LG else None)

        for c in range(2):
            for t in range(len(GP[c + 1]) - 1):
                wait_all(cp_gp(c + 1, t))
                group(c, sets(c), c > 0, True, GP[c + 1][t], GP[c + 1][t + 1] - GP[c + 1][t])
        for c in range(2, LG - ND):
            wait_all(cp_grp(c + 1))
            group(c, sets(c), True, True)
        for c in range(LG - ND, LG - 1):
            wait_all(cp_grp(c + 1))
            late[c] = group(c, sets(c), True, True, parts=(0, 4), ninv=NA // (2 if c == LG - ND else 4),
                            cfg=(-30, -6, 5, 16, 68, 1, 5))
        late[LG - 1] = group(LG - 1, sets(LG - 1), True, False, parts=(0, 4), ninv=NI7,
                             cfg=(-10, 0, 0, 1, 40, 0, 0))

    def mark(i, carry):
        zsm[1 + i] = i
        return carry

    conv()

    def rows(j):
        return j * TM if isinstance(j, int) else pl.multiple_of(j * TM, TM)

    def delay(x, after):
        if after is None:
            return x
        z8 = pltpu.bitcast(_tok([after]) & zero_vec(), f32)
        x0 = (x[:, 0:128].reshape(x.shape[0] // 8, 8, 128) + z8[None]).reshape(x.shape[0], 128)
        return jnp.concatenate([x0, x[:, 128:]], axis=1)

    def s0_rows(j, s0, ns, slot, from_q, after=None):
        r = rows(j)
        sl = slice(s0 * R, (s0 + ns) * R)
        if isinstance(j, int):
            x = qbuf[r + s0 * R:r + (s0 + ns) * R, :].astype(f32)
        else:
            x = qbuf.at[pl.ds(r, TM), :][sl, :].astype(f32)
        if from_q is not True:
            x = jnp.where(from_q, x, xbuf.at[pl.ds(r, TM), :][sl, :])
        x = delay(x, after)
        r2 = j * (TM // 2) if isinstance(j, int) else pl.multiple_of(j * (TM // 2), TM // 2)
        yw = ybuf.at[pl.ds(r2, TM // 2), :][s0 * 8:(s0 + ns) * 8, :]
        yy = [pltpu.unpack_elementwise(yw, index=k, packed_dtype=bf16, unpacked_dtype=f32)
              for k in range(2)]
        y = jnp.concatenate([yy[k][s * 8:(s + 1) * 8] for s in range(ns) for k in range(2)], axis=0)
        if ns == 1:
            zs, aft = [], None
            for hh in range(2):
                xh = delay(x[8 * hh:8 * hh + 8], aft)
                q, t1 = _ln_t(xh)
                x1 = xh + q * y[8 * hh:8 * hh + 8]
                u, t2 = _ln_t(x1)
                x1b[slot * R + 8 * hh:slot * R + 8 * hh + 8, :] = x1
                ub[slot * R + 8 * hh:slot * R + 8 * hh + 8, :] = u
                z, t3 = _ln_t(u)
                zs.append(z)
                ts = t1 + t2 + t3 + [[z[:, D - 128:]]]
                aft = ts[1][0][0:8]
            return jnp.concatenate(zs, axis=0).astype(bf16), ts
        q, t1 = _ln_t(x)
        x1 = x + q * y
        u, t2 = _ln_t(x1)
        x1b[slot * R:(slot + ns) * R, :] = x1
        ub[slot * R:(slot + ns) * R, :] = u
        z, t3 = _ln_t(u)
        return z.astype(bf16), t1 + t2 + t3 + [[z[:, D - 128:]]]

    rot = [0]

    def rhs_pins(steps, ksteps):
        pins = {}
        for t, lst in enumerate(steps):
            n, kg = t // ksteps, t % ksteps
            for i, vals in enumerate(lst):
                m = rot[0] % 4
                rot[0] += 1
                rg = 7 if (i % 2 == 0 and len(lst) > 1) else 0
                pins.setdefault(((kg * 4 + m) * 8 + rg, n), []).extend(vals)
        return pins

    def at_steps(toks, first, last, nsteps):
        steps = [[] for _ in range(nsteps)]
        for k, t in enumerate(toks):
            steps[first + (k * (last - first)) // max(len(toks) - 1, 1)].append(t)
        return steps

    def pinned(w, steps):
        return w if steps is None else _pin_at(w, rhs_pins(steps, 2), zero_vec())

    def put_h(row0, h):
        for l in range(LG):
            hwin[l, row0:row0 + h.shape[0], :] = h[:, l * 128:(l + 1) * 128]

    def m2_dot(r0, nr, steps=None):
        hs_in = jnp.concatenate(
            [hwin[l, 8 + r0 - SHIFTS[l]:8 + r0 - SHIFTS[l] + nr, :].astype(bf16) for l in range(LG)], axis=1)
        return _mm(hs_in, pinned(w2b[...], steps))

    def ln3(hs, lo, ns, after=None):
        sl = slice(lo * R, (lo + ns) * R)
        x1p = delay(ub[sl, :], after) + hs
        z, t = _ln_t(x1p)
        z3buf[sl, :] = z.astype(bf16)
        return x1b[sl, :] + x1p, [z[:, D - 128:]]

    def mlp(c0, c1, acc, side=None, z3=None, pre=None):
        z3 = z3buf[...] if z3 is None else z3
        zero = zero_vec()
        steps = [[] for _ in range(16 * NC)]
        for c in range(c0, c1):
            if pre is not None:
                pre(c, steps)
            w3 = _pin_at(w3b[:, c * TF:(c + 1) * TF], rhs_pins(steps[16 * c:16 * c + 8], 2), zero)
            a = _gelu(_mm(z3, w3))
            if side is not None:
                side(c, a, steps)
            a = a.astype(bf16)
            w4 = _pin_at(w4b[c * TF:(c + 1) * TF, :], rhs_pins(steps[16 * c + 8:16 * c + 16], 1), zero)
            acc = acc + _mm(a, w4)
        return acc

    def s0_side(b, bars=()):
        RT, D0, DD, CH = (0, 2, 2, 1)
        grp = _spread(list(range(NS)), KR) + [[]] * NC
        if isinstance(b, int):
            blk, fq = (b % NB, (b + 1) % NB), (b < NB, b + 1 < NB)
        else:
            blk, fq = (lax.rem(b, NB), lax.rem(b + 1, NB)), (b < NB, b + 1 < NB)

        def side(c, a, steps):
            if c == 0:
                x1b[0:R, :] = x1b[TM:TM + R, :]
                ub[0:R, :] = ub[TM:TM + R, :]
            after = a[0:8, RT * 128:(RT + 1) * 128]
            for n, s in enumerate(grp[c]):
                last = s == NS - 1
                z, t = s0_rows(blk[last], 0 if last else s + 1, 1, s + 1, fq[last], after)
                side.zs.append(z)
                after = t[CH][0][0:8] if CH >= 0 else None
                steps[min(16 * c + 8 + D0 + n * DD, 16 * (c + 1 if c + 1 in bars else KR) - 1)].append(t[-1])
        side.zs = []
        return side

    def toks(zs):
        return [t for _, ts in zs for t in ts]

    def cat(zs):
        return jnp.concatenate([z for z, _ in zs], axis=0)

    LNO = 2
    pend = [(par, u, h, a0) for u in range(NA // 2) for h in range(2)
            for a0 in range(8, NA, LNO) for par in range(LG - ND, LG)]

    def late_piece():
        par, u, h, a0 = pend.pop(0)
        for _ in mac_part(SET[par], u, h, a0, late[par][(u, h)], LNO):
            pass
        return list(late[par][(u, h)]['w'])

    NPA, NPB = 8, 8

    def prologue():
        cp_q0.wait()
        cp_w1.wait()
        F1, L1_ = (2, 15)
        HM = TM // 2
        for a in range(3):
            inv1(LG - 1, SET[LG - 1], a // 2, a % 2)
        za = [s0_rows(0, 0, 8, 0, True)]
        for a in range(2 * NI7, NA // 2):
            inv1(LG - 2, SET[LG - 2], a // 2, a % 2)
        for a in range(3, NA // 2):
            inv1(LG - 1, SET[LG - 1], a // 2, a % 2)
        zb = [s0_rows(0, 8, 4, 8, True), s0_rows(0, 12, 4, 12, True), s0_rows(1, 0, 1, 16, True)]
        for l in range(LG):
            hwin[l, 0:8, :] = jnp.zeros((8, 128), f32)
        put_h(8, _gelu(_mm(cat(za), pinned(w1b[...], at_steps(toks(zb[:2]) + [zb[2][1][-1]], F1, L1_, 16)))))
        h = _gelu(_mm(cat(zb), pinned(w1b[...], at_steps([late_piece() for _ in range(NPA)], 1, 15, 16))))
        put_h(8 + HM, h[0:HM + 8])
        hcar[...] = h[HM + R - 24:HM + R]

    def prologue2():
        HM = TM // 2
        cp_w2.wait()
        hs0 = m2_dot(0, HM, at_steps([late_piece() for _ in range(NPB)], 2, 15, 16))
        l0 = [ln3(hs0[n * 32:(n + 1) * 32], 2 * n, 2) for n in range(4)]
        hs1 = m2_dot(HM, HM, at_steps([t for _, t in l0], 3, 14, 16))
        l1 = [ln3(hs1[n * 32:(n + 1) * 32], 8 + 2 * n, 2) for n in range(4)]
        wait_all(cp_w34a)
        st['s0'] = s0_side(1, bars=(WS, WB))
        LA, LZ = (1, 126)
        skip = (16 * WS, 16 * WB, 16 * (KR + 2))
        slots = [t for t in range(LA, LZ + 1) if t not in skip]
        st['due'] = [slots[(k * len(slots)) // len(pend)] for k in range(len(pend))]

        def side(c, a, steps):
            st['s0'](c, a, steps)
            run_late(16 * c + 8, 16 * c + 16, steps)

        def pre(c, steps):
            if c == WS:
                wait_all(cp_w34m)
            if c == WB:
                lax.fori_loop(0, 2, mark, 0)
                wait_all(cp_w34b)
            run_late(16 * c, 16 * c + 8, steps)
        st['z3'] = z3buf[...]
        st['acc'] = mlp(0, KR, jnp.concatenate([r for r, _ in l0 + l1], axis=0), side, st['z3'], pre)

    st = {}

    def run_late(lo, hi, steps, off=0):
        while pend and lo <= st['due'][0] < hi:
            steps[st['due'].pop(0) - off].append(late_piece())

    def late_steps(lo):
        steps = [[] for _ in range(16)]
        run_late(lo, lo + 16, steps, lo)
        return steps

    def second_half(b, acc, z3, z1, first):
        RT, D0, DD = (0, 0, 1)
        jb = b % NB if first else lax.rem(b, NB)
        if first:
            def mk(off):
                return (lambda c, a, steps: run_late(16 * c + 8 + off, 16 * c + 16 + off, steps, off),
                        lambda c, steps: run_late(16 * c + off, 16 * c + 8 + off, steps, off))
        else:
            def mk(off):
                return None, None
        sd, pr = mk(0)
        acc = mlp(KR, KR + 1, acc, sd, z3, pr)
        top = hcar[...]
        put_h(0, top[0:8] if first else jnp.where(jb == 0, 0.0, top[0:8]))
        put_h(8, top[8:24])
        h = _gelu(_mm(z1, pinned(w1b[...], late_steps(16 * (KR + 1)) if first else None)))
        put_h(24, h[0:TM - R])
        put_h(8 + TM, h[TM - R:TM - 8] if first else jnp.where(jb == NB - 1, 0.0, h[TM - R:TM - 8]))
        hcar[...] = h[TM - 24:TM]
        if first:
            wait_all(cp_w34c)
        sd, pr = mk(16)
        acc = mlp(KR + 1, KR + 2, acc, sd, z3, pr)
        hs = m2_dot(0, TM, late_steps(16 * (KR + 3)) if first else None)
        if first:
            for par in late:
                for a in range(NA // 2, NA):
                    inv1(par, SET[par], a // 2, a % 2)
        rs = []

        def side(c, a, steps):
            for n in range(NS):
                r_, t = ln3(hs[n * R:(n + 1) * R], n, 1,
                            a[0:8, RT * 128:(RT + 1) * 128] if (n == 0 and RT >= 0) else None)
                rs.append(r_)
                steps[min(16 * c + 8 + D0 + (n * DD) // 2, 16 * NC - 1)].append(t)
        xn = mlp(KR + 2, NC, acc, side, z3)
        jg = (b - 1) % NB if first else lax.rem(b - 1, NB)
        xbuf[pl.ds(rows(jg), TM), :] = xn
        if not first:
            obuf[pl.ds(rows(jg), TM), :] = xn.astype(bf16)
        accb[...] = jnp.concatenate(rs, axis=0)

    prologue()
    lax.fori_loop(0, 2, mark, 0)
    prologue2()
    second_half(1, st['acc'], st['z3'], jnp.concatenate(st['s0'].zs, axis=0), True)
    cp_q1.wait()

    def body(b, carry):
        rot[0] = 2
        z3 = z3buf[...]
        sd = s0_side(b + 1)
        acc = mlp(0, KR, accb[...], sd, z3)
        second_half(b + 1, acc, z3, jnp.concatenate(sd.zs, axis=0), False)

        @pl.when(b >= NB)
        def _():
            cp_o(b - NB).start()
        return carry

    lax.fori_loop(1, G - 1, body, 0)

    OC = [0] + [512, 896] + [D]
    OS = tuple((OC[i], OC[i + 1] - OC[i]) for i in range(len(OC) - 1))
    acc = mlp(0, NC - 1, accb[...])
    a = _gelu(_mm(z3buf[...], w3b[:, FF - TF:])).astype(bf16)
    for c0, nc in OS:
        obuf[S - TM:, c0:c0 + nc] = (acc[:, c0:c0 + nc] + _mm(a, w4b[FF - TF:, c0:c0 + nc])).astype(bf16)
        cp_o(NB - 1, c0, nc).start()
    for j in range(NB - 1):
        cp_o(j).wait()
    for c0, nc in OS:
        cp_o(NB - 1, c0, nc).wait()


@jax.jit
def pallas_interleave_layers__ssm_conv_h3__mixer_s_mlp__prompt_kernel(
    A_q: jax.Array,
    A_k: jax.Array,
    A_v: jax.Array,
    A_shift_k: jax.Array,
    A_ssm_k: jax.Array,
    A_ssm_D: jax.Array,
    B_x: jax.Array,
    B_w1: jax.Array,
    B_w2: jax.Array,
    B_w3: jax.Array,
    B_w4: jax.Array,
):
    del B_x
    vm = pltpu.VMEM
    scratch = [
        vm((D, D), bf16), vm((D, D), bf16), vm((D, FF), bf16), vm((FF, D), bf16),
        vm((S + 16, D), bf16), vm((S, D), bf16), vm((D, S), bf16), vm((S, D), bf16),
        vm((4, D), bf16), vm((D,), bf16),
        vm((2, CB, CB), u32), vm((2, CB // 2, 2 * CB), u32),
        vm((5, 8, D), f32),
        vm((2, 2 * CB + 16, 128), f32),
        [vm((2 * H0, 128), f32)] * ND, [vm((NA, CB, 128), u32)] * ND,
        vm((S // 2, D), u32), vm((S, D), f32), vm((TM + R, D), f32), vm((TM + R, D), f32),
        vm((LG, TM + R, 128), f32), vm((24, D), f32),
        vm((TM, D), bf16), vm((TM, D), f32),
        pltpu.SMEM((4,), i32),
        pltpu.SemaphoreType.DMA((1 + NP12 + LG + 9,)),
    ]
    return pl.pallas_call(
        _kernel,
        out_shape=jax.ShapeDtypeStruct(A_q.shape, bf16),
        in_specs=[pl.BlockSpec(memory_space=pl.ANY)] * 10,
        out_specs=pl.BlockSpec(memory_space=pl.ANY),
        scratch_shapes=scratch,
        compiler_params=pltpu.CompilerParams(vmem_limit_bytes=116 * 1024 * 1024),
    )(A_q, A_k, A_v, A_shift_k.T, A_ssm_k, A_ssm_D, B_w1, B_w2, B_w3, B_w4)
```

```python
import math

import jax
import jax.numpy as jnp
from jax import lax
import jax.experimental.pallas as pl
import jax.experimental.pallas.tpu as pltpu


f32, bf16, u32, i32 = jnp.float32, jnp.bfloat16, jnp.uint32, jnp.int32

S, D, FF = 2048, 1024, 3584
TM = 256
NB = S // TM
G = 2 * NB
CB = 128
NA = S // CB
NO = 4
TF = 512
NC = FF // TF
R = 16
NS = TM // R
LG = D // 128
KR = 4
ND = 4
G1 = [0, 2, 5, 8]
G2 = [0, 3, 8]
NP12 = len(G1) + len(G2) - 2
EPS = 1e-5
BS = 3 * CB + 8
H0 = NA * BS + 16
C0 = math.sqrt(2.0 / math.pi)
C1 = C0 * 0.044715
SHIFTS = (1, 1, -1, -1, 2, 2, -2, -2)


def _ln_t(x):
    m = jnp.mean(x, axis=-1, keepdims=True)
    xc = x - m
    v = jnp.mean(xc * xc, axis=-1, keepdims=True)
    r = lax.rsqrt(v + EPS)
    n = x.shape[0]
    return xc * r, [[jnp.broadcast_to(m, (n, 128))], [jnp.broadcast_to(r, (n, 128))]]


def _gelu(x):
    hx = 0.5 * x
    return hx + hx * jnp.tanh(x * (C0 + C1 * (x * x)))


def _mm(a, b):
    return jnp.dot(a, b, preferred_element_type=f32)


def _tok(vals):
    t = None
    for v in vals:
        b = v if v.dtype == u32 else pltpu.bitcast(v, u32)
        if b.shape == (8, 128):
            t = b if t is None else t | b
            continue
        for i in range(b.shape[0] // 8):
            for j in range(b.shape[1] // 128):
                p = b[i * 8:(i + 1) * 8, j * 128:(j + 1) * 128]
                t = p if t is None else t | p
    return t


def _pin_at(x, pins, zero):
    if not pins:
        return x
    out, last = [], 0
    for k in sorted({k for k, _ in pins}):
        if k * 16 > last:
            out.append(x[last:k * 16])
        blk = x[k * 16:(k + 1) * 16]
        for (kk, n), vals in pins.items():
            if kk != k:
                continue
            top = pltpu.bitcast(pltpu.bitcast(blk[:, n * 128:(n + 1) * 128], u32) | (_tok(vals) & zero), bf16)
            parts = ([blk[:, :n * 128]] if n > 0 else []) + [top] + (
                [blk[:, (n + 1) * 128:]] if (n + 1) * 128 < blk.shape[1] else [])
            blk = jnp.concatenate(parts, axis=1) if len(parts) > 1 else top
        out.append(blk)
        last = (k + 1) * 16
    if last < x.shape[0]:
        out.append(x[last:])
    return jnp.concatenate(out, axis=0) if len(out) > 1 else out[0]


def _spread(items, n):
    return [items[(i * len(items)) // n:((i + 1) * len(items)) // n] for i in range(n)]


def _kernel(q_hbm, k_hbm, v_hbm, sk_hbm, hk_hbm, dd_hbm, w1_hbm, w2_hbm, w3_hbm, w4_hbm,
            o_hbm,
            w1b, w2b, w3b, w4b, kbuf, vbuf, hkb, qbuf, skb, ddb,
            Fm, Gm, skf, kf, ZS, YS, ybuf, xbuf, x1b, ub, hwin, hcar, z3buf, accb,
            zsm, sem):
    obuf = vbuf

    def cp_kvh(c, r0, nr, si):
        ch = pl.ds(c * 128, 128)
        return (
            pltpu.make_async_copy(k_hbm.at[0, pl.ds(r0, nr), ch], kbuf.at[pl.ds(16 + r0, nr), ch], sem.at[si]),
            pltpu.make_async_copy(v_hbm.at[0, pl.ds(r0, nr), ch], vbuf.at[pl.ds(r0, nr), ch], sem.at[si]),
            pltpu.make_async_copy(hk_hbm.at[ch, pl.ds(r0, nr)], hkb.at[ch, pl.ds(r0, nr)], sem.at[si]))

    GP = {1: G1, 2: G2}

    def cp_g0(i):
        return cp_kvh(0, i * 2 * TM, 2 * TM, i)

    def cp_gp(c, n):
        return cp_kvh(c, GP[c][n] * TM, (GP[c][n + 1] - GP[c][n]) * TM, 4 + (c - 1) * (len(G1) - 1) + n)

    def cp_grp(c):
        return cp_kvh(c, 0, S, 1 + NP12 + c)

    SB = 1 + NP12 + LG

    def cp_q(r0, r1, si):
        return pltpu.make_async_copy(q_hbm.at[0, pl.ds(r0, r1 - r0), :],
                                     qbuf.at[pl.ds(r0, r1 - r0), :], sem.at[si])

    def cp_o(j, c0=0, nc=D):
        return pltpu.make_async_copy(obuf.at[pl.ds(j * TM, TM), pl.ds(c0, nc)],
                                     o_hbm.at[0, pl.ds(j * TM, TM), pl.ds(c0, nc)], sem.at[SB + 4])

    cp_sk = pltpu.make_async_copy(sk_hbm, skb, sem.at[SB])
    cp_dd = pltpu.make_async_copy(dd_hbm, ddb, sem.at[SB])
    cp_q0 = cp_q(0, 2 * TM + R, SB + 1)

    cp_q1 = cp_q(2 * TM + R, S, SB + 3)

    cp_w1 = pltpu.make_async_copy(w1_hbm, w1b, sem.at[SB + 1])
    cp_w2 = pltpu.make_async_copy(w2_hbm, w2b, sem.at[SB + 8])
    def cp_w34(c0, c1, si):
        n = (c1 - c0) * TF
        return (pltpu.make_async_copy(w3_hbm.at[:, pl.ds(c0 * TF, n)], w3b.at[:, pl.ds(c0 * TF, n)], sem.at[si]),
                pltpu.make_async_copy(w4_hbm.at[pl.ds(c0 * TF, n), :], w4b.at[pl.ds(c0 * TF, n), :], sem.at[si]))

    WS = 2
    cp_w34a = cp_w34(0, WS, SB + 5)
    WB = 3
    cp_w34m = cp_w34(WS, WB, SB + 6)
    cp_w34b = cp_w34(WB, KR + 1, SB + 2)
    cp_w34c = cp_w34(KR + 1, NC, SB + 7)

    def wait_all(cps):
        for cp in cps:
            cp.wait()

    cp_sk.start()
    cp_dd.start()
    for grp in ([cp_g0(i) for i in range(4)] + [cp_gp(c, n) for c in (1, 2) for n in range(len(GP[c]) - 1)]
                + [cp_grp(c) for c in range(3, LG)]):
        for cp in grp:
            cp.start()
    for cp in (cp_q0, cp_w1, cp_w2) + cp_w34a + cp_w34m + cp_w34b + cp_w34c + (cp_q1,):
        cp.start()

    zsm[0] = 0
    kbuf[0:16, :] = jnp.zeros((16, D), bf16)

    def _basis(pos, part, n):
        k = jnp.where(pos < CB // 2, 2 * pos, 2 * pos - (CB - 1))
        m = ((2 * k + 1) * n + part * CB) & (4 * CB - 1)
        r = m & (2 * CB - 1)
        neg = jnp.logical_xor(m >= 2 * CB, r > CB)
        th = jnp.minimum(r, 2 * CB - r).astype(f32) * (math.pi / (2 * CB))
        t2 = th * th
        z = 1.0 / math.factorial(12)
        for e in (10, 8, 6, 4, 2, 0):
            z = 1.0 / math.factorial(e) - t2 * z
        z = jnp.where(neg, -z, z)
        return z, jnp.where(pos < CB // 2, z, -z)

    def dft_init(t, carry):
        rf = lax.broadcasted_iota(i32, (32, CB), 0)
        zs = _basis(t * 16 + (rf & 15), rf >> 4, lax.broadcasted_iota(i32, (32, CB), 1))
        cg = lax.broadcasted_iota(i32, (16, 2 * CB), 1)
        gs = _basis(cg >> 1, cg & 1, t * 16 + lax.broadcasted_iota(i32, (16, 2 * CB), 0))
        for par in range(2):
            Fm[par, pl.ds(pl.multiple_of(t * 16, 16), 16), :] = pltpu.bitcast(zs[par].astype(bf16), u32)
            Gm[par, pl.ds(pl.multiple_of(t * 8, 8), 8), :] = pltpu.bitcast(
                (gs[par] * (1.0 / CB)).astype(bf16), u32)
        return carry

    lax.fori_loop(0, CB // 16, dft_init, 0)

    cp_sk.wait()
    cp_dd.wait()
    sk32 = skb[...].astype(f32)
    for t in range(4):
        skf[t] = jnp.broadcast_to(sk32[t:t + 1, :], (8, D))
    skf[4] = jnp.broadcast_to(ddb[...].astype(f32).reshape(1, D), (8, D))

    SET = [(c + LG - ND) % 2 for c in range(LG - ND + 2)] + list(range(2, ND))

    def zero_vec():
        return jnp.full((8, 128), zsm[0], i32).astype(u32)

    def bmul(x, row8):
        n = x.shape[0] // 8
        return (x.reshape(n, 8, 128) * row8[None]).reshape(x.shape)

    def dsl(start, size, align):
        return pl.ds(start if isinstance(start, int) else pl.multiple_of(start, align), size)

    def unil(z):
        z = z.reshape(CB // 16, 32, 128)
        return z[:, 0:16].reshape(CB, 128), z[:, 16:32].reshape(CB, 128)

    def il3(*comps):
        return jnp.concatenate([z.reshape(CB // 8, 8, 128) for z in comps], axis=1).reshape(3 * CB, 128)

    def fwdh1(c, par, i, o, pins=None, skip=True):
        Z = ZS[par].at[dsl(H0 + i * 2 * BS, 2 * BS, 8), :]
        ls = dsl(c * 128, 128, 128)
        a = 2 * i + o
        hh = lax.dot_general(_pin_at(pltpu.bitcast(Fm[o], bf16), pins, zero_vec()), hkb[ls, dsl(a * CB, CB, CB)], (((1,), (1,)), ((), ())),
                             preferred_element_type=f32)
        cc, dd = unil(hh)
        if o == 0 and skip and (not isinstance(i, int) or i == 0):
            d8 = skf[4, :, ls] if isinstance(i, int) else jnp.where(i == 0, skf[4, :, ls], 0.0)
            cc = (cc.reshape(CB // 8, 8, 128) + d8[None]).reshape(CB, 128)
        ff = cc + dd
        Z[o * BS:o * BS + 3 * CB, :] = il3(cc, dd - cc, ff)
        return ff

    def fwdx1(c, par, i, o, pins, sk, slot=0):
        Z = ZS[par].at[dsl(i * 2 * BS, 2 * BS, 8), :]
        ls = dsl(c * 128, 128, 128)
        ks_ = i % 2 if isinstance(i, int) else slot
        if o == 0:
            kf[ks_] = kbuf[dsl(i * 2 * CB, 2 * CB + 16, 16), ls].astype(f32)
        a = 2 * i + o
        b0 = 16 + o * CB
        ks = bmul(kf[ks_, b0:b0 + CB, :], sk[0])
        for t in range(1, 4):
            ks = ks + bmul(kf[ks_, b0 - t:b0 - t + CB, :], sk[t])
        kv = (ks * vbuf[dsl(a * CB, CB, CB), ls].astype(f32)).astype(bf16)
        xh = _mm(_pin_at(pltpu.bitcast(Fm[o], bf16), pins, zero_vec()), kv)
        xr, xm = unil(xh)
        xs = xr + xm
        Z[o * BS:o * BS + 3 * CB, :] = il3(xs, xr, xm)
        return xs

    def mac_part(par, i, h, a0, st, NO=NO):
        Z, Y = ZS[par], YS[par]
        p0 = (2 * i + h) * 24

        def ld(base, a):
            return Z[base + a * BS + p0:base + a * BS + p0 + 24, :]
        K = [None] * NO
        hw = {}
        for ap in range(a0 + NO):
            x = ld(0, ap)
            for o in range(NO):
                dl = a0 + o - ap
                if dl < 0:
                    continue
                if dl not in hw:
                    hw[dl] = ld(H0, dl)
                t = hw[dl] * x
                K[o] = t if K[o] is None else K[o] + t
                inj = yield K[o]
                if inj is not None:
                    K[o] = jnp.concatenate([K[o][0:16], K[o][16:24] + inj], axis=0)
        st['w'] = []
        for o in range(NO):
            k1 = K[o][0:8]
            re, im = k1 - K[o][16:24], k1 + K[o][8:16]
            prev = st.get('y')
            out = (re, im) if prev is None else (re - prev[1], im + prev[0])
            st['y'] = (re, im)
            st['w'].append(pltpu.pack_elementwise(list(out), packed_dtype=bf16).astype(u32))
            Y[a0 + o, dsl(i * 16 + h * 8, 8, 8), :] = st['w'][-1]

    def mac_gen(par, i0, ns, parts, sts):
        for u in range(ns):
            for a0 in parts:
                for h in range(2):
                    yield from mac_part(par, i0 + u, h, a0, sts.setdefault((u, h), {}))

    def inv1(c, par, i, o, pins=None):
        Y = YS[par]
        a = 2 * i + o
        y = _mm(_pin_at(pltpu.bitcast(Gm[o], bf16), pins, zero_vec()), pltpu.bitcast(Y[a], bf16))
        y3 = y.reshape(CB // 16, 16, 128)
        ybuf[a * (CB // 2):(a + 1) * (CB // 2), c * 128:(c + 1) * 128] = pltpu.pack_elementwise(
            [y3[:, 0:8].reshape(CB // 2, 128), y3[:, 8:16].reshape(CB // 2, 128)], packed_dtype=bf16).astype(u32)
        return y

    def group(c, sets, do_inv, do_fwd, i0=0, ns=NA // 2, parts=(0, 4, 8, 12), cfg=None, ninv=NA // 2):
        PI, P0, DP, NP_, R0, DR, G0 = cfg or (-20, 12, 12, 16, 220, 12, 4)
        NPM = sum(2 * (NO * a0 + 10) for a0 in parts)
        names = ('h0', 'x0', 'h1', 'x1')
        zero = zero_vec()
        sk = [skf[t, :, dsl((c + 1) * 128, 128, 128)] for t in range(4)] if do_fwd else None
        sts = {}
        pprev, par, pnext = sets
        gen = mac_gen(par, i0, ns, parts, sts)
        rec = [next(gen)]
        inj = {}
        for u in range(ns):
            i = i0 + u
            base = u * NPM
            while len(rec) <= base + P0 + (NP_ - 1) * DP:
                rec.append(gen.send(inj.get(len(rec))))
            pins = {k: {} for k in ('i0', 'i1', 'h0', 'h1', 'x0', 'x1')}
            if base + PI >= 0:
                pins['i0'][(0, 0)] = [rec[base + PI][16:24]]
                pins['i1'][(0, 0)] = pins['i0'][(0, 0)]
            for n in range(NP_):
                r = ((n + 1) * 16) // NP_ - 1
                pins[names[n % len(names)]][(r, 0)] = [rec[base + P0 + n * DP][16:24]]
            if do_inv and i < ninv:
                ys = [inv1(c - 1, pprev, i, 0, pins['i0']), inv1(c - 1, pprev, i, 1, pins['i1'])]
                if not do_fwd:
                    inj[base + R0] = pltpu.bitcast(_tok([y[CB - 8:CB] for y in ys]) & zero, f32)
            if do_fwd:
                res = [fwdh1(c + 1, pnext, i, 0, pins['h0'], skip=(u == 0)),
                       fwdh1(c + 1, pnext, i, 1, pins['h1']),
                       fwdx1(c + 1, pnext, i, 0, pins['x0'], sk, slot=u % 2),
                       fwdx1(c + 1, pnext, i, 1, pins['x1'], sk, slot=u % 2)]
                for g in range(G0, CB // 16):
                    tk = _tok([z[16 * g + 8:16 * g + 16] for z in res]) & zero
                    inj[base + R0 + (g - G0) * DR] = pltpu.bitcast(tk, f32)
        try:
            while True:
                rec.append(gen.send(inj.get(len(rec))))
        except StopIteration:
            pass
        return sts

    late = {}
    NI7 = 2
    NIE = 2

    def conv():
        def pre(i, carry):
            wait_all(cp_g0(i))
            sk = [skf[t, :, 0:128] for t in range(4)]
            for u in range(2):
                for o in range(2):
                    fwdh1(0, SET[0], 2 * i + u, o, skip=(u == 0))
                for o in range(2):
                    fwdx1(0, SET[0], 2 * i + u, o, None, sk, slot=u)
            return carry
        lax.fori_loop(0, NA // 4, pre, 0)

        def sets(c):
            return (SET[c - 1], SET[c], SET[c + 1] if c + 1 < LG else None)

        for c in range(2):
            for t in range(len(GP[c + 1]) - 1):
                wait_all(cp_gp(c + 1, t))
                group(c, sets(c), c > 0, True, GP[c + 1][t], GP[c + 1][t + 1] - GP[c + 1][t])
        for c in range(2, LG - ND):
            wait_all(cp_grp(c + 1))
            group(c, sets(c), True, True)
        for c in range(LG - ND, LG - 1):
            wait_all(cp_grp(c + 1))
            late[c] = group(c, sets(c), True, True, parts=(0, 4), ninv=NA // 2 if c == LG - ND else NIE,
                            cfg=(-30, -6, 5, 16, 68, 1, 5))
        late[LG - 1] = group(LG - 1, sets(LG - 1), True, False, parts=(0, 4), ninv=NI7,
                             cfg=(-10, 0, 0, 1, 40, 0, 0))

    def mark(i, carry):
        zsm[1 + i] = i
        return carry

    conv()

    def rows(j):
        return j * TM if isinstance(j, int) else pl.multiple_of(j * TM, TM)

    def delay(x, after):
        if after is None:
            return x
        z8 = pltpu.bitcast(_tok([after]) & zero_vec(), f32)
        x0 = (x[:, 0:128].reshape(x.shape[0] // 8, 8, 128) + z8[None]).reshape(x.shape[0], 128)
        return jnp.concatenate([x0, x[:, 128:]], axis=1)

    def s0_rows(j, s0, ns, slot, from_q, after=None):
        r = rows(j)
        sl = slice(s0 * R, (s0 + ns) * R)
        if isinstance(j, int):
            x = qbuf[r + s0 * R:r + (s0 + ns) * R, :].astype(f32)
        else:
            x = qbuf.at[pl.ds(r, TM), :][sl, :].astype(f32)
        if from_q is not True:
            x = jnp.where(from_q, x, xbuf.at[pl.ds(r, TM), :][sl, :])
        x = delay(x, after)
        r2 = j * (TM // 2) if isinstance(j, int) else pl.multiple_of(j * (TM // 2), TM // 2)
        yw = ybuf.at[pl.ds(r2, TM // 2), :][s0 * 8:(s0 + ns) * 8, :]
        yy = [pltpu.unpack_elementwise(yw, index=k, packed_dtype=bf16, unpacked_dtype=f32)
              for k in range(2)]
        y = jnp.concatenate([yy[k][s * 8:(s + 1) * 8] for s in range(ns) for k in range(2)], axis=0)
        if ns == 1:
            zs, aft = [], None
            for hh in range(2):
                xh = delay(x[8 * hh:8 * hh + 8], aft)
                q, t1 = _ln_t(xh)
                x1 = xh + q * y[8 * hh:8 * hh + 8]
                u, t2 = _ln_t(x1)
                x1b[slot * R + 8 * hh:slot * R + 8 * hh + 8, :] = x1
                ub[slot * R + 8 * hh:slot * R + 8 * hh + 8, :] = u
                z, t3 = _ln_t(u)
                zs.append(z)
                ts = t1 + t2 + t3 + [[z[:, D - 128:]]]
                aft = ts[1][0][0:8]
            return jnp.concatenate(zs, axis=0).astype(bf16), ts
        q, t1 = _ln_t(x)
        x1 = x + q * y
        u, t2 = _ln_t(x1)
        x1b[slot * R:(slot + ns) * R, :] = x1
        ub[slot * R:(slot + ns) * R, :] = u
        z, t3 = _ln_t(u)
        return z.astype(bf16), t1 + t2 + t3 + [[z[:, D - 128:]]]

    rot = [0]

    def rhs_pins(steps, ksteps):
        pins = {}
        for t, lst in enumerate(steps):
            n, kg = t // ksteps, t % ksteps
            for i, vals in enumerate(lst):
                m = rot[0] % 4
                rot[0] += 1
                rg = 7 if (i % 2 == 0 and len(lst) > 1) else 0
                pins.setdefault(((kg * 4 + m) * 8 + rg, n), []).extend(vals)
        return pins

    def at_steps(toks, first, last, nsteps):
        steps = [[] for _ in range(nsteps)]
        for k, t in enumerate(toks):
            steps[first + (k * (last - first)) // max(len(toks) - 1, 1)].append(t)
        return steps

    def pinned(w, steps):
        return w if steps is None else _pin_at(w, rhs_pins(steps, 2), zero_vec())

    def put_h(row0, h):
        for l in range(LG):
            hwin[l, row0:row0 + h.shape[0], :] = h[:, l * 128:(l + 1) * 128]

    def m2_dot(r0, nr, steps=None):
        hs_in = jnp.concatenate(
            [hwin[l, 8 + r0 - SHIFTS[l]:8 + r0 - SHIFTS[l] + nr, :].astype(bf16) for l in range(LG)], axis=1)
        return _mm(hs_in, pinned(w2b[...], steps))

    def ln3(hs, lo, ns, after=None):
        sl = slice(lo * R, (lo + ns) * R)
        x1p = delay(ub[sl, :], after) + hs
        z, t = _ln_t(x1p)
        z3buf[sl, :] = z.astype(bf16)
        return x1b[sl, :] + x1p, [z[:, D - 128:]]

    def mlp(c0, c1, acc, side=None, z3=None, pre=None):
        z3 = z3buf[...] if z3 is None else z3
        zero = zero_vec()
        steps = [[] for _ in range(16 * NC)]
        for c in range(c0, c1):
            if pre is not None:
                pre(c, steps)
            w3 = _pin_at(w3b[:, c * TF:(c + 1) * TF], rhs_pins(steps[16 * c:16 * c + 8], 2), zero)
            a = _gelu(_mm(z3, w3))
            if side is not None:
                side(c, a, steps)
            a = a.astype(bf16)
            w4 = _pin_at(w4b[c * TF:(c + 1) * TF, :], rhs_pins(steps[16 * c + 8:16 * c + 16], 1), zero)
            acc = acc + _mm(a, w4)
        return acc

    def s0_side(b, bars=()):
        RT, D0, DD, CH = (0, 2, 2, 1)
        grp = _spread(list(range(NS)), KR) + [[]] * NC
        if isinstance(b, int):
            blk, fq = (b % NB, (b + 1) % NB), (b < NB, b + 1 < NB)
        else:
            blk, fq = (lax.rem(b, NB), lax.rem(b + 1, NB)), (b < NB, b + 1 < NB)

        def side(c, a, steps):
            if c == 0:
                x1b[0:R, :] = x1b[TM:TM + R, :]
                ub[0:R, :] = ub[TM:TM + R, :]
            after = a[0:8, RT * 128:(RT + 1) * 128]
            for n, s in enumerate(grp[c]):
                last = s == NS - 1
                z, t = s0_rows(blk[last], 0 if last else s + 1, 1, s + 1, fq[last], after)
                side.zs.append(z)
                after = t[CH][0][0:8] if CH >= 0 else None
                steps[min(16 * c + 8 + D0 + n * DD, 16 * (c + 1 if c + 1 in bars else KR) - 1)].append(t[-1])
        side.zs = []
        return side

    def toks(zs):
        return [t for _, ts in zs for t in ts]

    def cat(zs):
        return jnp.concatenate([z for z, _ in zs], axis=0)

    LNO = 2
    pend = [(par, u, h, a0) for u in range(NA // 2) for h in range(2)
            for a0 in range(8, NA, LNO) for par in range(LG - ND, LG)]

    def late_piece():
        par, u, h, a0 = pend.pop(0)
        for _ in mac_part(SET[par], u, h, a0, late[par][(u, h)], LNO):
            pass
        return list(late[par][(u, h)]['w'])

    NPA, NPB = 8, 8

    def prologue():
        cp_q0.wait()
        cp_w1.wait()
        F1, L1_ = (1, 14)
        HM = TM // 2
        for a in range(3):
            inv1(LG - 1, SET[LG - 1], a // 2, a % 2)
        za = [s0_rows(0, 0, 8, 0, True)]
        for c in range(LG - ND, LG - 2):
            for a in range(2 * NIE, NA // 2):
                inv1(c, SET[c], a // 2, a % 2)
        for a in range(2 * NI7, NA // 2):
            inv1(LG - 2, SET[LG - 2], a // 2, a % 2)
        for a in range(3, NA // 2):
            inv1(LG - 1, SET[LG - 1], a // 2, a % 2)
        zb = [s0_rows(0, 8, 4, 8, True), s0_rows(0, 12, 4, 12, True), s0_rows(1, 0, 1, 16, True)]
        for l in range(LG):
            hwin[l, 0:8, :] = jnp.zeros((8, 128), f32)
        put_h(8, _gelu(_mm(cat(za), pinned(w1b[...], at_steps(toks(zb[:-1]) + [zb[-1][1][-1]], F1, L1_, 16)))))
        h = _gelu(_mm(cat(zb), pinned(w1b[...], at_steps([late_piece() for _ in range(NPA)], 1, 15, 16))))
        put_h(8 + HM, h[0:HM + 8])
        hcar[...] = h[HM + R - 24:HM + R]

    def prologue2():
        HM = TM // 2
        cp_w2.wait()
        hs0 = m2_dot(0, HM, at_steps([late_piece() for _ in range(NPB)], 2, 15, 16))
        l0 = [ln3(hs0[n * 32:(n + 1) * 32], 2 * n, 2) for n in range(4)]
        hs1 = m2_dot(HM, HM, at_steps([t for _, t in l0], 3, 14, 16))
        l1 = [ln3(hs1[n * 32:(n + 1) * 32], 8 + 2 * n, 2) for n in range(4)]
        wait_all(cp_w34a)
        st['s0'] = s0_side(1, bars=(WS, WB))
        LA, LZ = (1, 126)
        skip = (16 * WS, 16 * WB, 16 * (KR + 2))
        slots = [t for t in range(LA, LZ + 1) if t not in skip]
        st['due'] = [slots[(k * len(slots)) // len(pend)] for k in range(len(pend))]

        def side(c, a, steps):
            st['s0'](c, a, steps)
            run_late(16 * c + 8, 16 * c + 16, steps)

        def pre(c, steps):
            if c == WS:
                wait_all(cp_w34m)
            if c == WB:
                lax.fori_loop(0, 2, mark, 0)
                wait_all(cp_w34b)
            run_late(16 * c, 16 * c + 8, steps)
        st['z3'] = z3buf[...]
        st['acc'] = mlp(0, KR, jnp.concatenate([r for r, _ in l0 + l1], axis=0), side, st['z3'], pre)

    st = {}

    def run_late(lo, hi, steps, off=0):
        while pend and lo <= st['due'][0] < hi:
            steps[st['due'].pop(0) - off].append(late_piece())

    def late_steps(lo):
        steps = [[] for _ in range(16)]
        run_late(lo, lo + 16, steps, lo)
        return steps

    def second_half(b, acc, z3, z1, first):
        RT, D0, DD = (0, 0, 1)
        jb = b % NB if first else lax.rem(b, NB)
        if first:
            def mk(off):
                return (lambda c, a, steps: run_late(16 * c + 8 + off, 16 * c + 16 + off, steps, off),
                        lambda c, steps: run_late(16 * c + off, 16 * c + 8 + off, steps, off))
        else:
            def mk(off):
                return None, None
        sd, pr = mk(0)
        acc = mlp(KR, KR + 1, acc, sd, z3, pr)
        top = hcar[...]
        put_h(0, top[0:8] if first else jnp.where(jb == 0, 0.0, top[0:8]))
        put_h(8, top[8:24])
        h = _gelu(_mm(z1, pinned(w1b[...], late_steps(16 * (KR + 1)) if first else None)))
        put_h(24, h[0:TM - R])
        put_h(8 + TM, h[TM - R:TM - 8] if first else jnp.where(jb == NB - 1, 0.0, h[TM - R:TM - 8]))
        hcar[...] = h[TM - 24:TM]
        if first:
            wait_all(cp_w34c)
        sd, pr = mk(16)
        acc = mlp(KR + 1, KR + 2, acc, sd, z3, pr)
        hs = m2_dot(0, TM, late_steps(16 * (KR + 3)) if first else None)
        if first:
            for par in late:
                for a in range(NA // 2, NA):
                    inv1(par, SET[par], a // 2, a % 2)
        rs = []

        def side(c, a, steps):
            for n in range(NS):
                r_, t = ln3(hs[n * R:(n + 1) * R], n, 1,
                            a[0:8, RT * 128:(RT + 1) * 128] if (n == 0 and RT >= 0) else None)
                rs.append(r_)
                steps[min(16 * c + 8 + D0 + (n * DD) // 2, 16 * NC - 1)].append(t)
        xn = mlp(KR + 2, NC, acc, side, z3)
        jg = (b - 1) % NB if first else lax.rem(b - 1, NB)
        xbuf[pl.ds(rows(jg), TM), :] = xn
        if not first:
            obuf[pl.ds(rows(jg), TM), :] = xn.astype(bf16)
        accb[...] = jnp.concatenate(rs, axis=0)

    prologue()
    lax.fori_loop(0, 2, mark, 0)
    prologue2()
    second_half(1, st['acc'], st['z3'], jnp.concatenate(st['s0'].zs, axis=0), True)
    cp_q1.wait()

    def body(b, carry):
        rot[0] = 2
        z3 = z3buf[...]
        sd = s0_side(b + 1)
        acc = mlp(0, KR, accb[...], sd, z3)
        second_half(b + 1, acc, z3, jnp.concatenate(sd.zs, axis=0), False)

        @pl.when(b >= NB)
        def _():
            cp_o(b - NB).start()
        return carry

    lax.fori_loop(1, G - 1, body, 0)

    OC = [0] + [512, 896] + [D]
    OS = tuple((OC[i], OC[i + 1] - OC[i]) for i in range(len(OC) - 1))
    acc = mlp(0, NC - 1, accb[...])
    a = _gelu(_mm(z3buf[...], w3b[:, FF - TF:])).astype(bf16)
    for c0, nc in OS:
        obuf[S - TM:, c0:c0 + nc] = (acc[:, c0:c0 + nc] + _mm(a, w4b[FF - TF:, c0:c0 + nc])).astype(bf16)
        cp_o(NB - 1, c0, nc).start()
    for j in range(NB - 1):
        cp_o(j).wait()
    for c0, nc in OS:
        cp_o(NB - 1, c0, nc).wait()


@jax.jit
def pallas_interleave_layers__ssm_conv_h3__mixer_s_mlp__prompt_kernel(
    A_q: jax.Array,
    A_k: jax.Array,
    A_v: jax.Array,
    A_shift_k: jax.Array,
    A_ssm_k: jax.Array,
    A_ssm_D: jax.Array,
    B_x: jax.Array,
    B_w1: jax.Array,
    B_w2: jax.Array,
    B_w3: jax.Array,
    B_w4: jax.Array,
):
    del B_x
    vm = pltpu.VMEM
    scratch = [
        vm((D, D), bf16), vm((D, D), bf16), vm((D, FF), bf16), vm((FF, D), bf16),
        vm((S + 16, D), bf16), vm((S, D), bf16), vm((D, S), bf16), vm((S, D), bf16),
        vm((4, D), bf16), vm((D,), bf16),
        vm((2, CB, CB), u32), vm((2, CB // 2, 2 * CB), u32),
        vm((5, 8, D), f32),
        vm((2, 2 * CB + 16, 128), f32),
        [vm((2 * H0, 128), f32)] * ND, [vm((NA, CB, 128), u32)] * ND,
        vm((S // 2, D), u32), vm((S, D), f32), vm((TM + R, D), f32), vm((TM + R, D), f32),
        vm((LG, TM + R, 128), f32), vm((24, D), f32),
        vm((TM, D), bf16), vm((TM, D), f32),
        pltpu.SMEM((4,), i32),
        pltpu.SemaphoreType.DMA((1 + NP12 + LG + 9,)),
    ]
    return pl.pallas_call(
        _kernel,
        out_shape=jax.ShapeDtypeStruct(A_q.shape, bf16),
        in_specs=[pl.BlockSpec(memory_space=pl.ANY)] * 10,
        out_specs=pl.BlockSpec(memory_space=pl.ANY),
        scratch_shapes=scratch,
        compiler_params=pltpu.CompilerParams(vmem_limit_bytes=116 * 1024 * 1024),
    )(A_q, A_k, A_v, A_shift_k.T, A_ssm_k, A_ssm_D, B_w1, B_w2, B_w3, B_w4)
```
